```python
import jax
import jax.numpy as jnp

def _softmax(x, axis=-1):
    return jax.nn.softmax(x, axis=axis)

def _gelu(x):
    return jax.nn.gelu(x, approximate=True)

def _silu(x):
    return jax.nn.silu(x)

def _sigmoid(x):
    return jax.nn.sigmoid(x)

def _layernorm(x, axis=-1, eps=1e-05):
    m = jnp.mean(x, axis=axis, keepdims=True)
    v = jnp.var(x, axis=axis, keepdims=True)
    return (x - m) / jnp.sqrt(v + eps)

def _scatter_add(tgt, idx, src, axis=0):
    return tgt.at[idx].add(src)

def _segment_sum(src, seg, n):
    return jax.ops.segment_sum(src, seg, n)

class _Rng:

    def __init__(self, key):
        self._k = key

    def _next(self):
        self._k, sub = jax.random.split(self._k)
        return sub

    def normal(self, shape):
        return jax.random.normal(self._next(), shape, dtype=jnp.bfloat16)

    def randint(self, lo, hi, shape):
        return jax.random.randint(self._next(), shape, lo, hi, dtype=jnp.int32)

    def uniform(self, shape, lo=0.0, hi=1.0):
        return jax.random.uniform(self._next(), shape, jnp.bfloat16, lo, hi)

    def permutation(self, n):
        return jax.random.permutation(self._next(), n)
kernel_name = 'interleave_layers__memory_aug_recurrent_mem_tr__glu_gated_swiglu__prompt'

def setup_inputs():
    _rng = _Rng(jax.random.key(int.from_bytes(__import__("os").urandom(4), "little")))
    _w = lambda a: (lambda t: t.astype(jnp.bfloat16) if jnp.issubdtype(t.dtype, jnp.floating) else t)(jnp.asarray(a))

    def _A_setup():
        B, S, Dm = (1, 2048, 576)
        H, Dh = (32, 128)
        M, seg = (8, 32)
        seg = min(seg, S)
        S = S // seg * seg
        return {'x': _w((lambda *s: _rng.normal(s) * 0.05)(B, S, Dm)), 'mem0': _w((lambda *s: _rng.normal(s) * 0.05)(B, M, Dm)), 'Wq': _w((lambda *s: _rng.normal(s) * 0.05)(Dm, H, Dh) * Dm ** (-0.5)), 'Wk': _w((lambda *s: _rng.normal(s) * 0.05)(Dm, H, Dh) * Dm ** (-0.5)), 'Wv': _w((lambda *s: _rng.normal(s) * 0.05)(Dm, H, Dh) * Dm ** (-0.5)), 'Wo': _w((lambda *s: _rng.normal(s) * 0.05)(H, Dh, Dm) * (H * Dh) ** (-0.5)), 'seg_len': seg}
    _A_in = _A_setup()

    def _B_setup():
        B, S, D, F = (1, 2048, 576, 4608)
        return {'x': _w((lambda *s: _rng.normal(s) * 0.05)(B, S, D)), 'w1': _w((lambda *s: _rng.normal(s) * 0.05)(D, F) * (2.0 / D) ** 0.5), 'w3': _w((lambda *s: _rng.normal(s) * 0.05)(D, F) * (2.0 / D) ** 0.5), 'w2': _w((lambda *s: _rng.normal(s) * 0.05)(F, D) * (2.0 / F) ** 0.5)}
    _B_in = _B_setup()
    return {'A_x': _A_in['x'], 'A_mem0': _A_in['mem0'], 'A_Wq': _A_in['Wq'], 'A_Wk': _A_in['Wk'], 'A_Wv': _A_in['Wv'], 'A_Wo': _A_in['Wo'], 'A_seg_len': _A_in['seg_len'], 'B_x': _B_in['x'], 'B_w1': _B_in['w1'], 'B_w3': _B_in['w3'], 'B_w2': _B_in['w2']}

def reference(A_x, A_mem0, A_Wq, A_Wk, A_Wv, A_Wo, A_seg_len, B_x, B_w1, B_w3, B_w2):

    def _A_ref(x, mem0, Wq, Wk, Wv, Wo, seg_len):
        B, S, Dm = x.shape
        H, Dh = (Wq.shape[1], Wq.shape[2])
        M = mem0.shape[1]
        scale = Dh ** (-0.5)
        n_seg = S // seg_len
        L = M + seg_len
        idx = jnp.arange(L)
        mask = (idx[:, None] < M) | (idx[:, None] >= idx[None, :])
        mem = mem0
        outs = []
        for s in range(n_seg):
            xs = x[:, s * seg_len:(s + 1) * seg_len, :].copy()
            h = jnp.concatenate([mem, xs], axis=1)
            q = jnp.einsum('btd,dhe->bhte', h, Wq)
            k = jnp.einsum('btd,dhe->bhte', h, Wk)
            v = jnp.einsum('btd,dhe->bhte', h, Wv)
            scores = jnp.einsum('bhqe,bhke->bhqk', q, k) * scale
            scores = jnp.where(mask[None, None], scores, -1000000000.0)
            p = _softmax(scores, axis=-1)
            o = jnp.einsum('bhqk,bhke->bhqe', p, v)
            o = jnp.einsum('bhte,hed->btd', o, Wo)
            mem = o[:, :M, :].copy()
            outs.append(o[:, M:, :])
        return jnp.concatenate(outs, axis=1)

    def _B_ref(x, w1, w3, w2):
        gate = jnp.einsum('bsd,df->bsf', x, w1)
        up = jnp.einsum('bsd,df->bsf', x, w3)
        h = _silu(gate) * up
        out = jnp.einsum('bsf,fd->bsd', h, w2)
        return out
    x = A_x
    x = x + _A_ref(_layernorm(x, axis=-1), A_mem0, A_Wq, A_Wk, A_Wv, A_Wo, A_seg_len)
    x = x + _B_ref(_layernorm(x, axis=-1), B_w1, B_w3, B_w2)
    x = x + _A_ref(_layernorm(x, axis=-1), A_mem0, A_Wq, A_Wk, A_Wv, A_Wo, A_seg_len)
    x = x + _B_ref(_layernorm(x, axis=-1), B_w1, B_w3, B_w2)
    return x
```

```python
import functools
import math
from typing import NamedTuple

import jax
import jax.numpy as jnp
import jax.experimental.pallas as pl
import jax.experimental.pallas.tpu as pltpu

_EPS = 1e-05
_MASKED = -1000000000.0
_LOG2E = math.log2(math.e)
_LANES = 128
_HALF = _LANES // 2
_TAIL = 4
_MXUS = 4
_LAG = 4
_ORDER_EVEN = "Q0 N K0 V0 S0 Q1 A0 K1 O0 V1 S1 G0 A1 Q2 O1 K2 V2 S2 G1 A2 Q3 O2 K3 V3 S3 G2 A3 G3 O3 D0 G4"
_ORDER_ODD = "Q0 K0 V0 S0 G5 A0 Q1 O0 K1 V1 S1 G6 A1 Q2 O1 K2 G7 V2 S2 G8 A2 Q3 O2 K3 D1 V3 D4 S3 D2 A3 D3 F O3"
_ORDER_SINGLE = "Q0 K0 V0 S0 Q1 K1 A0 V1 S1 Q2 K2 A1 V2 S2 Q3 K3 A2 V3 S3 O0 O1 A3 O2 O3"
_ORDER_DOUBLE = _ORDER_SINGLE
_ORDER_FFN = "N G0 G1 G2 D0 G3 G4 D1 G5 G6 G8 D2 G7 D4 D3 F"


class _Pass(NamedTuple):
    low: tuple
    high: tuple
    w_low: tuple
    w_high: tuple
    wide: tuple


def _scheme():
    x, y = 0, 1
    a = lambda d: d
    b = lambda d: 4 + d
    rest = lambda d: [e for e in range(4) if e != d]
    neg = lambda terms: tuple((-s, *t) for s, *t in terms)

    def whole(narrow, weight, wide):
        return _Pass(narrow, narrow, weight, weight, wide)

    def m1(d, e):
        return whole(((1, x, d), (1, y, e)), ((1, b(e), d), (1, a(d), e)),
                     ((1, y, a(d)), (1, x, b(e))))

    def m2(d, e):
        return whole(((1, y, min(d, e)), (1, y, max(d, e))), ((1, b(e), d),),
                     ((1, y, b(e)), (-1, y, a(d))))

    def m5(d, e):
        return whole(((1, x, min(d, e)), (1, x, max(d, e))), ((1, a(d), e),),
                     ((1, x, a(d)), (-1, x, b(e))))

    def m3(d):
        return whole(((1, x, d),), ((1, a(d), d), *((-1, a(d), e) for e in rest(d))),
                     ((1, x, a(d)), (1, y, a(d))))

    def m4(d):
        return whole(((1, y, d),), ((1, b(d), d), *((-1, b(d), e) for e in rest(d))),
                     ((1, y, b(d)), (1, x, b(d))))

    def m6(d):
        return whole(((1, y, d), (-1, x, d)), ((1, a(d), d), *((1, b(e), d) for e in rest(d))),
                     ((1, y, a(d)),))

    def m7(d):
        return whole(((1, y, d), (-1, x, d)), ((-1, b(d), d), *((-1, a(e), d) for e in rest(d))),
                     ((1, x, b(d)),))

    def with_tails(p, p_rows, p_cols, q, q_rows, q_cols):
        tail = lambda cols: tuple((1, c, _TAIL) for c in cols)
        return [
            _Pass(p.low, p.high, q.w_low, p.w_high, p.wide + q.wide),
            _Pass(p.low, ((1, p_rows, _TAIL),), p.w_low + neg(q.w_low), tail(p_cols), p.wide),
            _Pass(((1, q_rows, _TAIL),), q.high, tail(q_cols), q.w_high + neg(p.w_high), q.wide)]

    def near(d, e):
        return [*with_tails(m5(d, e), x, [a(d)], m5(e, d), x, [a(e)]), m3(d),
                *with_tails(m2(d, e), y, [b(e)], m2(e, d), y, [b(d)]), m3(e),
                *with_tails(m6(d), y, [a(d), b(e)], m7(d), x, [b(d), a(e)]), m1(d, e),
                *with_tails(m7(e), x, [b(e), a(d)], m6(e), y, [a(e), b(d)]), m1(e, d)]

    edge = lambda d, e: [m5(d, e), m1(d, e), m2(d, e)]
    return (*near(0, 1), *edge(0, 2), *edge(0, 3), *edge(1, 2), *edge(1, 3),
            *edge(2, 0), *edge(3, 0), m4(0), *edge(2, 1), *edge(3, 1), m4(1),
            m4(2), m4(3), *near(2, 3))


_PASSES = _scheme()
_OPERANDS = tuple(dict.fromkeys((p.low, p.high) for p in _PASSES))


def _selected(single, columns=8):
    for i, p in enumerate(_PASSES):
        if single:
            p = p._replace(wide=tuple((s, 0, c) for s, r, c in p.wide if r == c // 4 and c < columns),
                           low=tuple((s, 0, d) for s, _, d in p.low),
                           high=tuple((s, 0, d) for s, _, d in p.high))
        if p.wide:
            yield i, p


def _signed_sum(terms):
    terms = sorted(terms, key=lambda t: -t[0])
    total = terms[0][1] if terms[0][0] > 0 else -terms[0][1]
    for sign, value in terms[1:]:
        total = total + value if sign > 0 else total - value
    return total


def _accumulate(sums, key, sign, value):
    if key not in sums:
        sums[key] = (sign, value)
    elif sums[key][0] == sign:
        sums[key] = (sign, sums[key][1] + value)
    else:
        sums[key] = (1, value - sums[key][1] if sign > 0 else sums[key][1] - value)


def _low_lanes(rows):
    return jax.lax.broadcasted_iota(jnp.int32, (rows, _LANES), 1) < _HALF


def _blocks(x):
    return [x[:, d * _LANES:(d + 1) * _LANES] for d in range(_TAIL + 1)]


def _operands(row_blocks, keys):
    blocks = [_blocks(x) for x in row_blocks]
    low_lanes = _low_lanes(row_blocks[0].shape[0])
    total = functools.cache(lambda terms: _signed_sum([(s, blocks[r][d]) for s, r, d in terms]))
    return {(low, high): total(low) if low == high else jnp.where(low_lanes, total(low), total(high))
            for low, high in keys}


def _dot(a, words):
    return jnp.dot(a, pltpu.bitcast(words, jnp.bfloat16), preferred_element_type=jnp.float32)


def _expand(operand, tile, out, single=False):
    sums, shared = {}, []
    for n, (i, p) in enumerate(_selected(single)):
        product = _dot(operand((p.low, p.high)), tile(i))
        if i + 1 < len(_PASSES) and _PASSES[i + 1].high[0][2] == _TAIL:
            shared = [product, product]
        else:
            if shared:
                product = product + shared.pop()
            for s, r, c in p.wide:
                _accumulate(sums, (r, c), s, product)
        if n % _MXUS == _MXUS - 1:
            yield
    for key, (sign, value) in sums.items():
        assert sign > 0
        out[key] = value


def _contract(inputs, tile, sums, dtype, single=False, columns=8):
    total = functools.cache(lambda terms: _signed_sum([(s, inputs[r, c]) for s, r, c in terms]))
    low_lanes = _low_lanes(inputs[0, 0].shape[0])
    chosen = list(_selected(single, columns))
    held = []
    for n, (i, p) in enumerate(chosen):
        if i + 1 < len(_PASSES) and _PASSES[i + 1].high[0][2] == _TAIL:
            lhs = total(chosen[n + 1][1].wide) + total(chosen[n + 2][1].wide)
        else:
            lhs = total(p.wide)
        product = _dot(lhs.astype(dtype), tile(i))
        if held or (i + 1 < len(_PASSES) and _PASSES[i + 1].high[0][2] == _TAIL):
            held.append((p, product))
            if len(held) == 3:
                (p0, both), (p1, first), (p2, second) = held
                held = []
                product = both + jnp.where(low_lanes, first, second)
                for s, r, d in p0.low:
                    _accumulate(sums, (r, d), s, product)
                _accumulate(sums, (p1.high[0][1], _TAIL, 1), 1, first)
                _accumulate(sums, (p2.low[0][1], _TAIL, 0), 1, second)
        else:
            for s, r, d in p.low:
                _accumulate(sums, (r, d), s, product)
        if n % _MXUS == _MXUS - 1:
            yield


def _contracted(sums, r):
    assert all(sign > 0 for sign, _ in sums.values())
    low, high = sums[r, _TAIL, 0][1], sums[r, _TAIL, 1][1]
    tail = jnp.where(_low_lanes(low.shape[0]), low, high)
    tail = tail + pltpu.roll(tail, _HALF, 1)
    return jnp.concatenate([sums[r, d][1] for d in range(_TAIL)] + [tail], axis=1)


def _layernorm(x):
    low_lanes = _low_lanes(x.shape[0])
    width = _TAIL * _LANES + _HALF

    def mean(v):
        *full, tail = _blocks(v)
        return jnp.sum(sum(full) + jnp.where(low_lanes, tail, 0.0), axis=-1, keepdims=True) / width

    d = x - mean(x)
    return d * jax.lax.rsqrt(mean(d * d) + _EPS)


def _attention_masks(n_layers, n_mem, seg):
    rows = n_mem + seg
    i = jax.lax.broadcasted_iota(jnp.int32, (n_layers * rows, n_layers * rows), 0)
    j = jax.lax.broadcasted_iota(jnp.int32, (n_layers * rows, n_layers * rows), 1)
    if n_layers == 1:
        return (i < n_mem) | (i >= j), _MASKED * _LOG2E
    same = (i >= rows) == (j >= rows)
    visible = (i < n_mem) | ((i >= rows) & (i < rows + n_mem)) | (i >= j)
    fill = jnp.where(same, _MASKED * _LOG2E, -jnp.inf).astype(jnp.float32)
    return same & visible, fill


def _attention_tasks(operand, w_ref, n_layers, n_mem, seg, result):
    single = n_layers == 1
    rows = n_mem + seg
    visible, fill = _attention_masks(n_layers, n_mem, seg)
    scale = _LANES ** -0.5 * _LOG2E
    qkv, probs, heads, sums = {}, {}, {}, {}

    def stacked(g, which, h):
        return jnp.concatenate([qkv[g, which][r, h] for r in range(n_layers)], axis=0)

    def project(g, which):
        qkv[g, which] = {}
        yield from _expand(operand, lambda i: w_ref[3 * g + which, i], qkv[g, which], single)

    def scores(g):
        for first in range(0, 8, _MXUS):
            raw = [jax.lax.dot_general(stacked(g, 0, h), stacked(g, 1, h).astype(jnp.bfloat16),
                                       (((1,), (1,)), ((), ())), preferred_element_type=jnp.float32)
                   for h in range(first, first + _MXUS)]
            for h, s in enumerate(raw, first):
                s = jnp.where(visible, s * scale, fill)
                p = jnp.exp2(s - jnp.max(s, axis=-1, keepdims=True))
                probs[g, h] = p, 1.0 / jnp.sum(p, axis=-1, keepdims=True)
            yield

    def values(g):
        heads[g] = {}
        for h in range(8):
            p, inv = probs[g, h]
            o = jnp.dot(p, stacked(g, 2, h).astype(jnp.bfloat16),
                        preferred_element_type=jnp.float32) * inv
            for r in range(n_layers):
                heads[g][r, h] = o[r * rows:(r + 1) * rows]
            if h % _MXUS == _MXUS - 1:
                yield

    def output(g):
        yield from _contract(heads[g], lambda i: w_ref[12 + g, i], sums, jnp.float32, single)
        if g == 3:
            result([_contracted(sums, r) for r in range(n_layers)])

    tasks = {}
    for g in range(4):
        tasks.update({f"Q{g}": project(g, 0), f"K{g}": project(g, 1), f"V{g}": project(g, 2),
                      f"S{g}": scores(g), f"A{g}": values(g), f"O{g}": output(g)})
    return tasks


def _ffn_tasks(row_blocks, w_ref, result, first_unit=16):
    operands, hidden, sums, rest = {}, {}, {}, {}

    def prepare():
        normed = [_layernorm(x) for x in row_blocks]
        operands.update({k: v.astype(jnp.bfloat16) for k, v in _operands(normed, _OPERANDS).items()})
        yield

    def gated(u):
        both = {}
        yield from _expand(operands.__getitem__, lambda i: w_ref[first_unit + u, i], both)
        for r in range(2):
            for c in range(4):
                gate = both[r, c]
                hidden[r, 4 * u + c] = gate * jax.nn.sigmoid(gate) * both[r, 4 + c]

    def down(u):
        tile = lambda i: w_ref[first_unit + 9 + u, i]
        if u < 4:
            inputs = {(r, c): hidden[r, 8 * u + c] for r in range(2) for c in range(8)}
            yield from _contract(inputs, tile, sums, jnp.bfloat16)
        else:
            inputs = {(0, c): jnp.concatenate([hidden[r, 8 * u + c] for r in range(2)], axis=0)
                      for c in range(4)}
            yield from _contract(inputs, tile, rest, jnp.bfloat16, single=True, columns=4)

    def finish():
        for (_, *key), (sign, value) in rest.items():
            rows = value.shape[0] // 2
            for r in range(2):
                _accumulate(sums, (r, *key), sign, value[r * rows:(r + 1) * rows])
        result([_contracted(sums, r) for r in range(2)])
        yield

    tasks = {"N": prepare(), "F": finish()}
    tasks.update({f"G{u}": gated(u) for u in range(9)})
    tasks.update({f"D{u}": down(u) for u in range(5)})
    return tasks


def _emit(order, tasks):
    for item in order.split():
        name, _, count = item.partition(":")
        running = [tasks[n] for n in name.split("+")]
        done = object()
        rounds = 0
        while running and (not count or rounds < int(count)):
            running = [t for t in running if next(t, done) is not done]
            rounds += 1


def _lay_out(source, store, transposed, columns=8):
    def half(terms, offset):
        return _signed_sum([(s, source(c, d * _LANES + (0 if d == _TAIL else offset)))
                            for s, c, d in terms])

    for i, p in _selected(columns < 8, columns):
        tile = jnp.concatenate([half(p.w_low, 0), half(p.w_high, _HALF)], axis=0)
        tile = tile.astype(jnp.bfloat16)
        store(i, pltpu.bitcast(tile.T if transposed else tile, jnp.uint32))


def _kernel(xt_hbm, mem0_hbm, wq_hbm, wk_hbm, wv_hbm, wot_hbm, w1_hbm, w3_hbm, w2t_hbm,
            outt_hbm, mem0_ref, io_ref, res_ref, lhs_ref, w_ref, qkv_stage, wo_stage, up_stage,
            down_stage, qkv_sem, weight_sem, io_sem, *, seg):
    d_model, n_tok = xt_hbm.shape
    n_mem = mem0_ref.shape[0]
    n_seg = n_tok // seg
    n_io = n_tok // _LANES

    def block(r, n=1):
        return pl.ds(pl.multiple_of(r * seg, seg), n * seg)

    def transpose_in(i):
        x = io_ref[i].astype(jnp.float32)
        x = jnp.concatenate([x, x[_TAIL * _LANES:]], axis=0)
        res_ref[pl.ds(pl.multiple_of(i * _LANES, _LANES), _LANES), :] = x.T

    def transpose_out(i, x):
        io_ref[i] = x.T[:d_model].astype(io_ref.dtype)

    def store_operands(slot, rows, row_blocks):
        operands = _operands(row_blocks, _OPERANDS)
        for i, key in enumerate(_OPERANDS):
            lhs_ref[slot, i, rows, :] = operands[key]

    mem_rows, seg_rows = slice(0, n_mem), slice(n_mem, n_mem + seg)

    def single_step(r, mem, order=_ORDER_SINGLE, ffn=None):
        x = res_ref[block(r), :]
        keys = dict.fromkeys((p.low, p.high) for _, p in _selected(True))
        operands = _operands([jnp.concatenate([mem, _layernorm(x)], axis=0)], keys)
        outs = []
        _emit(order, {**(ffn or {}),
                      **_attention_tasks(operands.__getitem__, w_ref, 1, n_mem, seg, outs.extend)})
        res_ref[block(r), :] = x + outs[0][seg_rows]
        return outs[0][mem_rows]

    def double_tasks(slot, outs):
        def done(results):
            outs.extend(results)
            store_operands(1 - slot, mem_rows, [o[mem_rows] for o in results])

        return _attention_tasks(lambda key: lhs_ref[slot, _OPERANDS.index(key)], w_ref, 2,
                                n_mem, seg, done)

    def double_step(b, _):
        xs = [res_ref[block(b + _LAG, 2), :], res_ref[block(b, 2), :]]
        store_operands(1 - b, seg_rows, [_layernorm(x[seg:]) for x in xs])
        outs = []
        _emit(_ORDER_DOUBLE, double_tasks(b, outs))
        res_ref[block(b + _LAG), :] = xs[0][:seg] + outs[0][seg_rows]
        res_ref[block(b), :] = xs[1][:seg] + outs[1][seg_rows]

    def two_steps(j, _):
        b = 2 * j
        xs = [res_ref[block(b + _LAG, 2), :], res_ref[block(b, 2), :]]
        ffn_in = [res_ref[block(b + 2, 2), :], res_ref[block(b - 2, 2), :]]
        following = res_ref[block(jnp.minimum(b + _LAG + 2, n_seg - 1)), :]
        tile = jnp.maximum(j - 3, 0) // 2
        transpose_out(tile, res_ref[pl.ds(pl.multiple_of(tile * _LANES, _LANES), _LANES), :])
        ffn_out, even, odd = [], [], []

        def ffn_done(ys):
            ffn_out.extend(x + y for x, y in zip(ffn_in, ys))
            store_operands(0, seg_rows, [_layernorm(following), _layernorm(ffn_out[0][:seg])])

        ffn = _ffn_tasks(ffn_in, w_ref, ffn_done)
        store_operands(1, seg_rows, [_layernorm(x[seg:]) for x in xs])
        _emit(_ORDER_EVEN, {**ffn, **double_tasks(0, even)})
        _emit(_ORDER_ODD, {**ffn, **double_tasks(1, odd)})
        res_ref[block(b + 2, 2), :], res_ref[block(b - 2, 2), :] = ffn_out
        for r, x, first, second in zip((b + _LAG, b), xs, even, odd):
            res_ref[block(r, 2), :] = x + jnp.concatenate([first[seg_rows], second[seg_rows]], axis=0)
        return odd[1][mem_rows]

    def ffn_alone(first):
        xs = [res_ref[block(first, 2), :], res_ref[block(first + 2, 2), :]]
        ys = []
        _emit(_ORDER_FFN, _ffn_tasks(xs, w_ref, ys.extend))
        return jnp.concatenate([x + y for x, y in zip(xs, ys)], axis=0)

    def qkv_copies(g):
        return [pltpu.make_async_copy(w.bitcast(jnp.uint32).at[:, 4 * g + p, :],
                                      qkv_stage.at[3 * g + i, p], qkv_sem.at[4 * (3 * g + i) + p])
                for i, w in enumerate((wq_hbm, wk_hbm, wv_hbm)) for p in range(4)]

    def x_copy(i):
        return pltpu.make_async_copy(xt_hbm.at[:, pl.ds(i * _LANES, _LANES)], io_ref.at[i],
                                     io_sem.at[i])

    def out_copy(i):
        return pltpu.make_async_copy(io_ref.at[i], outt_hbm.at[:, pl.ds(i * _LANES, _LANES)],
                                     io_sem.at[i])

    copies = [pltpu.make_async_copy(src, dst, weight_sem.at[i]) for i, (src, dst) in enumerate((
        (mem0_hbm, mem0_ref), (wot_hbm.bitcast(jnp.uint32), wo_stage),
        (w1_hbm.bitcast(jnp.uint32), up_stage.at[0]), (w3_hbm.bitcast(jnp.uint32), up_stage.at[1]),
        (w2t_hbm.bitcast(jnp.uint32), down_stage)))]

    def store_tile(u):
        def store(i, words):
            w_ref[u, i] = words
        return store

    def unpacked(words):
        return pltpu.bitcast(words, jnp.bfloat16).astype(jnp.float32)

    for i in range(n_io):
        x_copy(i).start()
    for g in range(4):
        for c in qkv_copies(g):
            c.start()
    for c in copies:
        c.start()
    for i in range(n_io):
        x_copy(i).wait()
    pl.loop(0, n_io)(transpose_in)
    for g in range(4):
        for c in qkv_copies(g):
            c.wait()

    @pl.loop(0, 12)
    def _(u):
        def source(c, row):
            words = qkv_stage[u, c // 2, row:row + _HALF, :]
            words = words & jnp.uint32(0xFFFF0000) if c % 2 else words << 16
            return pltpu.bitcast(words, jnp.float32)
        _lay_out(source, store_tile(u), False)

    copies[0].wait()
    copies[1].wait()

    @pl.loop(0, 4)
    def _(g):
        _lay_out(lambda c, row: unpacked(wo_stage[8 * g + c, row // 2:(row + _HALF) // 2, :]),
                 store_tile(12 + g), True)

    mem0 = mem0_ref[...].astype(jnp.float32)
    mem0 = jnp.concatenate([mem0, mem0[:, _TAIL * _LANES:]], axis=1)
    mem1 = jax.lax.fori_loop(0, _LAG, single_step, mem0)
    for c in copies[2:]:
        c.wait()

    def lanes(tile):
        return pl.ds(pl.multiple_of(tile * _LANES, _LANES), _LANES)

    @pl.loop(0, 9)
    def _(u):
        _lay_out(lambda c, row: unpacked(
            up_stage[c // 4, row // 2:(row + _HALF) // 2, lanes(4 * u + c % 4)]),
            store_tile(16 + u), False)

    def down_source(u):
        return lambda c, row: unpacked(down_stage[row // 2:(row + _HALF) // 2, lanes(8 * u + c)])

    pl.loop(0, 4)(lambda u: _lay_out(down_source(u), store_tile(25 + u), True))
    _lay_out(down_source(4), store_tile(29), True, columns=4)

    first = ffn_alone(0)
    res_ref[:_LAG * seg, :] = first
    store_operands(0, mem_rows, [mem1, mem0])
    store_operands(0, seg_rows, [_layernorm(res_ref[block(_LAG), :]), _layernorm(first[:seg])])
    jax.lax.fori_loop(0, 2, double_step, None)
    last = n_seg - _LAG
    mem2 = jax.lax.fori_loop(1, last // 2, two_steps, mem0)

    n_done = (last // 2 - 4) // 2 + 1
    for i in range(n_done):
        out_copy(i).start()
    ffn_in = [res_ref[block(n_seg - 2, 2), :], res_ref[block(last - 2, 2), :]]
    ffn_out = []
    ffn = _ffn_tasks(ffn_in, w_ref, ffn_out.extend)
    mem2 = single_step(last, mem2, _ORDER_EVEN, ffn)
    mem2 = single_step(last + 1, mem2, _ORDER_ODD, ffn)
    res_ref[block(n_seg - 2, 2), :] = ffn_in[0] + ffn_out[0]
    res_ref[block(last - 2, 2), :] = ffn_in[1] + ffn_out[1]
    jax.lax.fori_loop(last + 2, n_seg, single_step, mem2)
    for i in range(n_done, n_io - 1):
        transpose_out(i, res_ref[i * _LANES:(i + 1) * _LANES, :])
        out_copy(i).start()
    transpose_out(n_io - 1, ffn_alone(last))
    out_copy(n_io - 1).start()
    for i in range(n_io):
        out_copy(i).wait()


@functools.partial(jax.jit, static_argnames=("A_seg_len",))
def pallas_interleave_layers__memory_aug_recurrent_mem_tr__glu_gated_swiglu__prompt_kernel(
    A_x: jax.Array,
    A_mem0: jax.Array,
    A_Wq: jax.Array,
    A_Wk: jax.Array,
    A_Wv: jax.Array,
    A_Wo: jax.Array,
    A_seg_len: int,
    B_x: jax.Array,
    B_w1: jax.Array,
    B_w3: jax.Array,
    B_w2: jax.Array,
):
    del B_x
    _, n_tok, d_model = A_x.shape
    n_mem = A_mem0.shape[1]
    _, n_heads, d_head = A_Wq.shape
    d_ff = B_w1.shape[1]
    assert A_x.shape[0] == 1 and _LAG * A_seg_len == _LANES and n_mem == 8
    assert d_model == _TAIL * _LANES + _HALF and d_head == _LANES
    assert n_heads == 32 and d_ff == 36 * _LANES
    hbm = pl.BlockSpec(memory_space=pltpu.HBM)
    out_t = pl.pallas_call(
        functools.partial(_kernel, seg=A_seg_len),
        out_shape=jax.ShapeDtypeStruct((d_model, n_tok), A_x.dtype),
        in_specs=[hbm] * 9,
        out_specs=hbm,
        scratch_shapes=[
            pltpu.VMEM((n_mem, d_model), A_mem0.dtype),
            pltpu.VMEM((n_tok // _LANES, d_model, _LANES), A_x.dtype),
            pltpu.VMEM((n_tok, d_model + _HALF), jnp.float32),
            pltpu.VMEM((2, len(_OPERANDS), n_mem + A_seg_len, _LANES), jnp.float32),
            pltpu.VMEM((30, len(_PASSES), _HALF, _LANES), jnp.uint32),
            pltpu.VMEM((12, 4, d_model, d_head), jnp.uint32),
            pltpu.VMEM((n_heads, d_model // 2, d_head), jnp.uint32),
            pltpu.VMEM((2, d_model // 2, d_ff), jnp.uint32),
            pltpu.VMEM((d_model // 2, d_ff), jnp.uint32),
            pltpu.SemaphoreType.DMA((48,)),
            pltpu.SemaphoreType.DMA((5,)),
            pltpu.SemaphoreType.DMA((n_tok // _LANES,)),
        ],
        compiler_params=pltpu.CompilerParams(vmem_limit_bytes=120 * 1024 * 1024),
    )(A_x.reshape(n_tok, d_model).T, A_mem0.reshape(n_mem, d_model), A_Wq, A_Wk, A_Wv,
      A_Wo.transpose(0, 2, 1), B_w1, B_w3, B_w2.T)
    return out_t.T.reshape(A_x.shape)
```

```python
import functools
import math
from typing import NamedTuple

import jax
import jax.numpy as jnp
import jax.experimental.pallas as pl
import jax.experimental.pallas.tpu as pltpu

_EPS = 1e-05
_MASKED = -1000000000.0
_LOG2E = math.log2(math.e)
_LANES = 128
_HALF = _LANES // 2
_TAIL = 4
_COLUMNS = 8
_GROUPS = 4
_UP, _DOWN, _UNITS = 16, 25, 30
_LAG = 4
_EARLY = 32
_FLAGS = {"XLA_TPU_FORCE_LP_LLO_SCHEDULER": True}
_ORDER_EVEN = (
    "Q0 N K0 V0*8+S0 Q1*4+G0*4 A0 K1 O0 V1*8+S1 G1 A1 Q2 O1 K2 V2*8+S2 G2 A2 Q3 O2 K3 V3*8+S3 "
    "G3 A3 G8 O3 D4 G4:20")
_ORDER_ODD = (
    "Q0*4+G4*4 K0 V0*8+S0 G5 A0 Q1 O0 K1 V1*8+S1 G6 A1 Q2 O1 K2 G7 V2*8+S2 D0 A2 Q3 O2 K3 "
    "V3*8+S3 D1 D2 A3 D3 F O3")
_ORDER_EVEN_EARLY = _ORDER_EVEN
_ORDER_ODD_EARLY = _ORDER_ODD
_ORDER_DOUBLE = "Q0 K0 V0*8+S0 Q1 K1 A0 V1*8+S1 Q2 K2 A1 V2*8+S2 Q3 K3 A2 V3*8+S3 O0 O1 A3 O2 O3"
_ORDER_SINGLE = "Q0 K0 V0*4+S0 Q1 K1 A0 V1*4+S1 Q2 K2 A1 V2*4+S2 Q3 K3 A2 V3*4+S3 O0 O1 A3 O2 O3"
_ORDER_FFN = "N G0 G1 G2 D0 G3 G4 D1 G5 G8 G6 D4 G7 D2 D3 F"
_ORDER_LOAD = "E0*4+L1 W2 E1*4+L2 W0 W3 E2*4+L0+L3"


class _Pass(NamedTuple):
    low: tuple
    high: tuple
    w_low: tuple
    w_high: tuple
    wide: tuple
    common: bool = False


def _scheme():
    x, y = 0, 1
    a = lambda d: d
    b = lambda d: 4 + d
    rest = lambda d: [e for e in range(4) if e != d]
    neg = lambda terms: tuple((-s, *t) for s, *t in terms)

    def whole(narrow, weight, wide):
        return _Pass(narrow, narrow, weight, weight, wide)

    def m1(d, e):
        return whole(((1, x, d), (1, y, e)), ((1, b(e), d), (1, a(d), e)),
                     ((1, y, a(d)), (1, x, b(e))))

    def m2(d, e):
        return whole(((1, y, min(d, e)), (1, y, max(d, e))), ((1, b(e), d),),
                     ((1, y, b(e)), (-1, y, a(d))))

    def m3(d):
        return whole(((1, x, d),), ((1, a(d), d), *((-1, a(d), e) for e in rest(d))),
                     ((1, x, a(d)), (1, y, a(d))))

    def m4(d):
        return whole(((1, y, d),), ((1, b(d), d), *((-1, b(d), e) for e in rest(d))),
                     ((1, y, b(d)), (1, x, b(d))))

    def m5(d, e):
        return whole(((1, x, min(d, e)), (1, x, max(d, e))), ((1, a(d), e),),
                     ((1, x, a(d)), (-1, x, b(e))))

    def m6(d):
        return whole(((1, y, d), (-1, x, d)), ((1, a(d), d), *((1, b(e), d) for e in rest(d))),
                     ((1, y, a(d)),))

    def m7(d):
        return whole(((1, y, d), (-1, x, d)), ((-1, b(d), d), *((-1, a(e), d) for e in rest(d))),
                     ((1, x, b(d)),))

    def with_tails(p, p_rows, p_columns, q, q_rows, q_columns):
        tail = lambda columns: tuple((1, c, _TAIL) for c in columns)
        return [
            _Pass(p.low, p.high, q.w_low, p.w_high, p.wide + q.wide, common=True),
            _Pass(p.low, ((1, p_rows, _TAIL),), p.w_low + neg(q.w_low), tail(p_columns), p.wide),
            _Pass(((1, q_rows, _TAIL),), q.high, tail(q_columns), q.w_high + neg(p.w_high), q.wide)]

    def near(d, e):
        return [*with_tails(m5(d, e), x, [a(d)], m5(e, d), x, [a(e)]), m3(d),
                *with_tails(m2(d, e), y, [b(e)], m2(e, d), y, [b(d)]), m3(e),
                *with_tails(m6(d), y, [a(d), b(e)], m7(d), x, [b(d), a(e)]), m1(d, e),
                *with_tails(m7(e), x, [b(e), a(d)], m6(e), y, [a(e), b(d)]), m1(e, d)]

    far = lambda d, e: [m5(d, e), m1(d, e), m2(d, e)]
    return (*near(0, 1), *far(0, 2), *far(0, 3), *far(1, 2), *far(1, 3),
            m4(2), m4(3), *near(2, 3),
            m4(0), *far(2, 0), *far(3, 0), m4(1), *far(2, 1), *far(3, 1))


_PASSES = _scheme()


def _selected(single, columns=_COLUMNS):
    for i, p in enumerate(_PASSES):
        if single:
            p = p._replace(
                wide=tuple((s, 0, c) for s, r, c in p.wide if r == c // 4 and c < columns),
                low=tuple((s, 0, d) for s, _, d in p.low),
                high=tuple((s, 0, d) for s, _, d in p.high))
        if p.wide:
            yield i, p


def _operand_keys(single):
    return tuple(dict.fromkeys((p.low, p.high) for _, p in _selected(single)))


def _signed_sum(terms):
    terms = sorted(terms, key=lambda t: -t[0])
    total = terms[0][1] if terms[0][0] > 0 else -terms[0][1]
    for sign, value in terms[1:]:
        total = total + value if sign > 0 else total - value
    return total


def _accumulate(sums, key, sign, value):
    if key not in sums:
        sums[key] = (sign, value)
    elif sums[key][0] == sign:
        sums[key] = (sign, sums[key][1] + value)
    else:
        sums[key] = (1, value - sums[key][1] if sign > 0 else sums[key][1] - value)


def _pack(x):
    return pltpu.bitcast(x.astype(jnp.bfloat16), jnp.uint32)


def _unpack(words):
    return pltpu.bitcast(words, jnp.bfloat16)


def _low_lanes(rows):
    return jax.lax.broadcasted_iota(jnp.int32, (rows, _LANES), 1) < _HALF


def _blocks(x):
    return [x[:, d * _LANES:(d + 1) * _LANES] for d in range(_TAIL + 1)]


def _store_operands(ref, row_blocks):
    blocks = [_blocks(x) for x in row_blocks]
    low_lanes = _low_lanes(row_blocks[0].shape[0])
    total = functools.cache(lambda terms: _signed_sum([(s, blocks[r][d]) for s, r, d in terms]))
    for i, (low, high) in enumerate(_operand_keys(len(row_blocks) == 1)):
        operand = total(low) if low == high else jnp.where(low_lanes, total(low), total(high))
        ref[i] = _pack(operand) if ref.dtype == jnp.uint32 else operand


def _dot(a, b):
    return jnp.dot(a, b, preferred_element_type=jnp.float32)


def _expand(operands_ref, tiles_ref, out, single=False):
    keys = _operand_keys(single)
    sums, common = {}, []
    for i, p in _selected(single):
        operand = operands_ref[keys.index((p.low, p.high))]
        if operand.dtype == jnp.uint32:
            operand = _unpack(operand)
        product = _dot(operand, _unpack(tiles_ref[i]))
        if p.common:
            common = [product, product]
        else:
            if common:
                product = product + common.pop()
            for s, r, c in p.wide:
                _accumulate(sums, (r, c), s, product)
        yield
    assert all(sign > 0 for sign, _ in sums.values())
    out.update({key: value for key, (_, value) in sums.items()})


def _contract(load, tiles_ref, sums, single=False, columns=_COLUMNS):
    held = []
    for i, p in _selected(single, columns):
        product = _dot(_signed_sum([(s, load(r, c)) for s, r, c in p.wide]),
                       _unpack(tiles_ref[i]))
        if p.common or held:
            held.append((p, product))
        if len(held) == 3:
            (p, common), (p1, first), (p2, second) = held
            held = []
            product = common + jnp.where(_low_lanes(common.shape[0]), first, second)
            _accumulate(sums, (p1.high[0][1], _TAIL, 1), 1, first)
            _accumulate(sums, (p2.low[0][1], _TAIL, 0), 1, second)
        if not held:
            for s, r, d in p.low:
                _accumulate(sums, (r, d), s, product)
        yield


def _contracted(sums, r):
    assert all(sign > 0 for sign, _ in sums.values())
    low, high = sums[r, _TAIL, 0][1], sums[r, _TAIL, 1][1]
    tail = jnp.where(_low_lanes(low.shape[0]), low, high)
    tail = tail + pltpu.roll(tail, _HALF, 1)
    return jnp.concatenate([sums[r, d][1] for d in range(_TAIL)] + [tail], axis=1)


def _lay_out(source, tiles_ref, transposed, columns=_COLUMNS):
    def half(terms, offset):
        parts = [(s, source(c, d * _LANES + (0 if d == _TAIL else offset))) for s, c, d in terms]
        if len(parts) > 1:
            parts = [(s, part.astype(jnp.float32)) for s, part in parts]
        return _signed_sum(parts).astype(jnp.bfloat16)

    for i, p in _selected(columns < _COLUMNS, columns):
        low, high = half(p.w_low, 0), half(p.w_high, _HALF)
        if transposed:
            tiles_ref[i] = _pack(jnp.concatenate([low, high], axis=0).T)
        else:
            tiles_ref[i, :_HALF // 2, :] = _pack(low)
            tiles_ref[i, _HALF // 2:, :] = _pack(high)
        yield


def _layernorm(x):
    low_lanes = _low_lanes(x.shape[0])

    def mean(v):
        *full, tail = _blocks(v)
        total = functools.reduce(jnp.add, full) + jnp.where(low_lanes, tail, 0.0)
        return jnp.sum(total, axis=-1, keepdims=True) / (_TAIL * _LANES + _HALF)

    d = x - mean(x)
    return d * jax.lax.rsqrt(mean(d * d) + _EPS)


def _silu(x):
    half = 0.5 * x
    return half + half * jnp.tanh(half)


def _reciprocal(x):
    r = pl.reciprocal(x, approx=True)
    return r * (2.0 - x * r)


def _attention_masks(pieces, rows, n_mem):
    total = sum(end - first for first, end in pieces)

    def index(axis):
        i = jax.lax.broadcasted_iota(jnp.int32, (total, total), axis)
        at, original = 0, i
        for first, end in pieces:
            original = jnp.where(i >= at, i + (first - at), original)
            at += end - first
        return original

    i, j = index(0), index(1)
    if total == rows:
        return (i < n_mem) | (i >= j), _MASKED * _LOG2E
    same = (i >= rows) == (j >= rows)
    visible = (i < n_mem) | ((i >= rows) & (i < rows + n_mem)) | (i >= j)
    fill = jnp.where(same, _MASKED * _LOG2E, -jnp.inf).astype(jnp.float32)
    return same & visible, fill


def _attention_tasks(layers, n_mem, operands_ref, w_ref, heads_ref, outs, known=None):
    single = len(layers) == 1
    rows = layers[0].shape[0]
    if known:
        skipped = (rows - n_mem) // 2
        moved = rows + n_mem + skipped // 2
        pieces = [(0, n_mem), (n_mem + skipped, rows), (rows + n_mem, moved),
                  (rows, rows + n_mem), (moved, 2 * rows), (n_mem, n_mem + skipped)]
        both = jnp.concatenate(layers, axis=0)
        _store_operands(operands_ref, [
            jnp.concatenate([both[first:end] for first, end in part], axis=0)
            for part in (pieces[:3], pieces[3:5])])
    else:
        pieces = [(0, len(layers) * rows)]
        _store_operands(operands_ref, layers)
    visible, fill = _attention_masks(pieces, rows, n_mem)
    scale = _LANES ** -0.5 * _LOG2E
    qkv, probs, sums = {}, {}, {}

    def stacked(u, h, streamed=False):
        value = jnp.concatenate([qkv[u][r, h] for r in range(len(layers))], axis=0)
        if not (single and streamed):
            value = value.astype(jnp.bfloat16)
        return jnp.concatenate([value, known(u, h)], axis=0) if known else value

    def project(u):
        qkv[u] = {}
        yield from _expand(operands_ref, w_ref.at[u], qkv[u], single)

    def scores(g):
        for h in range(_COLUMNS):
            s = jax.lax.dot_general(stacked(4 * g, h, True), stacked(4 * g + 1, h),
                                    (((1,), (1,)), ((), ())), preferred_element_type=jnp.float32)
            s = jnp.where(visible, s * scale, fill)
            p = jnp.exp2(s - jnp.max(s, axis=-1, keepdims=True))
            p = p * _reciprocal(jnp.sum(p, axis=-1, keepdims=True))
            probs[g, h] = p if single else p.astype(jnp.bfloat16)
            yield

    def values(g):
        for h in range(_COLUMNS):
            o, at = _dot(probs[g, h], stacked(4 * g + 2, h)), 0
            for first, end in pieces:
                heads_ref[_COLUMNS * g + h, first:end, :] = o[at:at + end - first]
                at += end - first
            yield

    def output(g):
        yield from _contract(lambda r, h: heads_ref[_COLUMNS * g + h, r * rows:(r + 1) * rows, :],
                             w_ref.at[4 * g + 3], sums, single)
        if g == _GROUPS - 1:
            outs.extend(_contracted(sums, r) for r in range(len(layers)))

    tasks = {}
    for g in range(_GROUPS):
        tasks.update({f"Q{g}": project(4 * g), f"K{g}": project(4 * g + 1),
                      f"V{g}": project(4 * g + 2), f"S{g}": scores(g), f"A{g}": values(g),
                      f"O{g}": output(g)})
    return tasks


def _ffn_tasks(row_blocks, operands_ref, w_ref, hidden_ref, result):
    rows = row_blocks[0].shape[0]
    sums = {}

    def prepare():
        _store_operands(operands_ref, [_layernorm(x) for x in row_blocks])
        yield

    def gated(u):
        both = {}
        yield from _expand(operands_ref, w_ref.at[_UP + u], both)
        for c in range(4):
            for r in range(2):
                hidden_ref[4 * u + c, r * rows:(r + 1) * rows, :] = (
                    _silu(both[r, c]) * both[r, 4 + c])

    def down(u):
        yield from _contract(lambda r, c: hidden_ref[_COLUMNS * u + c, r * rows:(r + 1) * rows, :],
                             w_ref.at[_DOWN + u], sums)

    def down_rest(u):
        rest = {}
        yield from _contract(lambda r, c: hidden_ref[_COLUMNS * u + c], w_ref.at[_DOWN + u], rest,
                             single=True, columns=4)
        for (_, *key), (sign, value) in rest.items():
            for r in range(2):
                _accumulate(sums, (r, *key), sign, value[r * rows:(r + 1) * rows])

    def finish():
        result([_contracted(sums, r) for r in range(2)])
        yield

    return {"N": prepare(), "F": finish(), "D4": down_rest(4),
            **{f"G{u}": gated(u) for u in range(_DOWN - _UP)},
            **{f"D{u}": down(u) for u in range(4)}}


def _passes(order, tasks):
    done = object()
    for item in order.split():
        names, _, turns = item.partition(":")
        running = [(tasks[name], int(count or 1))
                   for name, _, count in (part.partition("*") for part in names.split("+"))]
        turn = 0
        while running and (not turns or turn < int(turns)):
            for task, count in tuple(running):
                for _ in range(count):
                    if next(task, done) is done:
                        running.remove((task, count))
                        break
                    yield
            turn += 1


def _emit(order, tasks):
    for _ in _passes(order, tasks):
        pass


def _chain(*tasks):
    for task in tasks:
        yield from task


def _kernel(xt_hbm, mem0_hbm, wq_hbm, wk_hbm, wv_hbm, wot_hbm, w1_hbm, w3_hbm, w2t_hbm,
            outt_hbm, mem0_ref, io_ref, res_ref, h_ref, operands_ref, short_operands_ref,
            ffn_operands_ref, heads_ref, hidden_ref, early_ref, w_ref, stage_ref,
            stage_sem, mem_sem, io_sem, *, seg):
    d_model, n_tok = xt_hbm.shape
    n_mem = mem0_ref.shape[0]
    n_seg = n_tok // seg
    n_io = n_tok // _LANES
    mem_rows, seg_rows = slice(0, n_mem), slice(n_mem, n_mem + seg)

    def block(r, n=1):
        return pl.ds(pl.multiple_of(r * seg, seg), n * seg)

    def lanes(i):
        return pl.ds(pl.multiple_of(i * _LANES, _LANES), _LANES)

    def transpose_in(i):
        x = io_ref[i].astype(jnp.float32)
        res_ref[lanes(i), :] = jnp.concatenate([x, x[_TAIL * _LANES:]], axis=0).T

    def transpose_out(i, x):
        io_ref[i] = x.T[:d_model].astype(io_ref.dtype)

    def single_passes(r, order, others):
        x = res_ref[block(r), :]
        following = res_ref[block(jnp.minimum(r + 1, n_seg - 1)), :]
        outs = []
        yield from _passes(order, {**others, **_attention_tasks(
            [h_ref[0]], n_mem, operands_ref, w_ref, heads_ref, outs)})
        h_ref[0, seg_rows, :] = _layernorm(following)
        h_ref[0, mem_rows, :] = outs[0][mem_rows]
        res_ref[block(r), :] = x + outs[0][seg_rows]

    def double_tasks(b, layers, outs, early):
        if not early:
            return _attention_tasks(layers, n_mem, operands_ref, w_ref, heads_ref, outs)
        words = pl.ds(pl.multiple_of(b * (seg // 4), seg // 4), seg // 4)
        return _attention_tasks(layers, n_mem, short_operands_ref, w_ref, heads_ref, outs,
                                lambda u, h: _unpack(early_ref[u - u // 4, h, words, :]))

    def double_step(b):
        xs = [res_ref[block(b + _LAG, 2), :], res_ref[block(b, 2), :]]
        outs = []
        _emit(_ORDER_DOUBLE, double_tasks(b, [h_ref[0], h_ref[1]], outs, True))
        for i, r in enumerate((b + _LAG, b)):
            h_ref[i, seg_rows, :] = _layernorm(xs[i][seg:])
            h_ref[i, mem_rows, :] = outs[i][mem_rows]
            res_ref[block(r), :] = xs[i][:seg] + outs[i][seg_rows]

    def two_steps(j, early):
        b = 2 * j
        xs = [res_ref[block(b + _LAG + 1), :], res_ref[block(b + 1), :]]
        ffn_in = [res_ref[block(b + 2, 2), :], res_ref[block(b - 2, 2), :]]
        following = res_ref[block(jnp.minimum(b + _LAG + 2, n_seg - 1)), :]
        if not early:
            transpose_out(j - _EARLY // 2, res_ref[lanes(j - _EARLY // 2), :])
        even, odd = [], []

        def ffn_done(ys):
            for r, y in zip((b + 2, b - 2), ys):
                res_ref[block(r, 2), :] += y
            h_ref[1, seg_rows, :] = _layernorm(res_ref[block(b + 2), :])

        ffn = _ffn_tasks(ffn_in, ffn_operands_ref.at[0], w_ref, hidden_ref, ffn_done)
        _emit(_ORDER_EVEN_EARLY if early else _ORDER_EVEN,
              {**ffn, **double_tasks(b, [h_ref[0], h_ref[1]], even, early)})
        h_ref[0, seg_rows, :] = _layernorm(following)
        for r, o in zip((b + _LAG, b), even):
            res_ref[block(r), :] += o[seg_rows]
        layers = [jnp.concatenate([o[mem_rows], _layernorm(x)], axis=0) for o, x in zip(even, xs)]
        _emit(_ORDER_ODD_EARLY if early else _ORDER_ODD,
              {**ffn, **double_tasks(b + 1, layers, odd, early)})
        for i, r in enumerate((b + _LAG, b)):
            h_ref[i, mem_rows, :] = odd[i][mem_rows]
            res_ref[block(r + 1), :] = xs[i] + odd[i][seg_rows]

    def ffn_passes(first, result):
        xs = [res_ref[block(first, 2), :], res_ref[block(first + 2, 2), :]]
        return _passes(_ORDER_FFN, _ffn_tasks(
            xs, ffn_operands_ref.at[0], w_ref, hidden_ref,
            lambda ys: result(jnp.concatenate([x + y for x, y in zip(xs, ys)], axis=0))))

    def slot(batch, i):
        return 4 * (batch % 2) + i

    def start_columns(s, columns):
        for c, src in enumerate(columns):
            rows = pl.ds(c * src.shape[0], src.shape[0])
            pltpu.make_async_copy(src, stage_ref.at[s, rows], stage_sem.at[s]).start()

    def start_attention(g, i):
        if i < 3:
            words = (wq_hbm, wk_hbm, wv_hbm)[i].bitcast(jnp.uint32)
            start_columns(slot(g, i), [words.at[:, 4 * g + p, :] for p in range(4)])
        else:
            words = wot_hbm.bitcast(jnp.uint32)
            start_columns(slot(g, i), [words.at[_COLUMNS * g + c] for c in range(_COLUMNS)])

    def start_ffn(batch, i, columns=_COLUMNS):
        if i < 2:
            start_columns(slot(batch, i), [
                w.bitcast(jnp.uint32).at[:, lanes(4 * (2 * batch + i) + c)]
                for w in (w1_hbm, w3_hbm) for c in range(4)])
        else:
            start_columns(slot(batch, i), [
                w2t_hbm.bitcast(jnp.uint32).at[:, lanes(_COLUMNS * batch + c)]
                for c in range(columns)])

    def wait_slot(s, columns=_COLUMNS):
        filled = stage_ref.at[s, pl.ds(0, columns * d_model // 2)]
        pltpu.make_async_copy(filled, filled, stage_sem.at[s]).wait()

    def lay_out_heads(g, i):
        def source(c, row):
            words = stage_ref[slot(g, i), pl.ds(c // 2 * d_model + row, _HALF), :]
            words = words & jnp.uint32(0xFFFF0000) if c % 2 else words << 16
            return pltpu.bitcast(words, jnp.float32)

        return _lay_out(source, w_ref.at[4 * g + i], False)

    def lay_out_rows(s, u, transposed, columns=_COLUMNS):
        return _lay_out(
            lambda c, row: _unpack(stage_ref[s, pl.ds((c * d_model + row) // 2, _HALF // 2), :]),
            w_ref.at[u], transposed, columns)

    def x_copy(i):
        return pltpu.make_async_copy(xt_hbm.at[:, lanes(i)], io_ref.at[i], io_sem.at[i])

    def out_copy(i):
        return pltpu.make_async_copy(io_ref.at[i], outt_hbm.at[:, lanes(i)], io_sem.at[i])

    n_chunks = ffn_operands_ref.shape[0]
    n_late = (n_io - 2 * n_chunks) // _GROUPS

    def late_tiles(g):
        return [(2 * n_chunks + 1 + n_late * g + i) % n_io for i in range(n_late)]

    def load_group(g):
        def project(i):
            for chunk in range(n_chunks):
                out = {}
                yield from _expand(ffn_operands_ref.at[chunk], w_ref.at[4 * g + i], out)
                for (r, c), value in out.items():
                    early_ref[3 * g + i, c, pl.ds((2 * chunk + r) * seg, seg), :] = _pack(value)

        def arrive(i):
            if i == 0:
                pl.when(g + 1 < _GROUPS)(lambda: wait_slot(slot(g + 1, 0)))
                pl.when(g + 2 < _GROUPS)(lambda: start_attention(g + 2, 0))
                pl.when(g + 2 == _GROUPS)(lambda: start_ffn(0, 0))
            else:
                wait_slot(slot(g, i))
                pl.when(g + 1 < _GROUPS)(lambda: start_attention(g + 1, i))
                if i < 3:
                    pl.when(g + 1 == _GROUPS)(lambda: start_ffn(0, i))
            yield

        for i in late_tiles(g):
            x_copy(i).start()
        _emit("W1 " + _ORDER_LOAD, {
            **{f"E{i}": project(i) for i in range(3)}, **{f"W{i}": arrive(i) for i in range(4)},
            "L0": lay_out_heads(jnp.minimum(g + 1, _GROUPS - 1), 0),
            "L1": lay_out_heads(g, 1), "L2": lay_out_heads(g, 2),
            "L3": lay_out_rows(slot(g, 3), 4 * g + 3, True)})
        for i in late_tiles(g):
            x_copy(i).wait()
        for i in late_tiles(g):
            transpose_in(i)

    def first_step(r):
        for i in range(3):
            wait_slot(slot(r, i))
        start_ffn(r + 1, 0)
        pl.when(r + 1 < _LAG)(lambda: start_ffn(r + 1, 1))
        pl.when(r + 1 < _LAG)(lambda: start_ffn(r + 1, 2))
        pl.when(r + 1 == _LAG)(lambda: start_ffn(_LAG, 2, 4))
        _emit("P*7+L*2", {
            "P": single_passes(r, _ORDER_SINGLE, {}),
            "L": _passes("L0+L1+L2", {
                "L0": lay_out_rows(slot(r, 0), _UP + 2 * r, False),
                "L1": lay_out_rows(slot(r, 1), _UP + 2 * r + 1, False),
                "L2": lay_out_rows(slot(r, 2), _DOWN + r, True)})})

    mem_copy = pltpu.make_async_copy(mem0_hbm, mem0_ref, mem_sem.at[0])
    start_attention(0, 0)
    for i in range(1, 2 * n_chunks + 1):
        x_copy(i).start()
    mem_copy.start()
    wait_slot(0)
    start_attention(0, 1)
    _emit("L", {"L": lay_out_heads(0, 0)})
    start_attention(0, 2)

    @pl.loop(0, n_chunks)
    def _early_operands(chunk):
        tiles = [2 * chunk + 1, 2 * chunk + 2]
        for i in tiles:
            x_copy(i).wait()
        for i in tiles:
            transpose_in(i)
        _store_operands(ffn_operands_ref.at[chunk], [
            _layernorm(jnp.concatenate(
                [res_ref[pl.ds(pl.multiple_of(i * _LANES + r * seg, seg), seg // 2), :]
                 for r in range(_LANES // seg)], axis=0)) for i in tiles])

    start_attention(1, 0)
    start_attention(0, 3)
    pl.loop(0, _GROUPS)(load_group)
    mem_copy.wait()
    mem0 = mem0_ref[...].astype(jnp.float32)
    mem0 = jnp.concatenate([mem0, mem0[:, _TAIL * _LANES:]], axis=1)
    h_ref[0] = jnp.concatenate([mem0, _layernorm(res_ref[block(0), :])], axis=0)
    h_ref[1, mem_rows, :] = mem0
    pl.loop(0, _LAG)(first_step)
    wait_slot(slot(_LAG, 0))
    wait_slot(slot(_LAG, 2), 4)

    def first_done(x):
        res_ref[:_LAG * seg, :] = x
        h_ref[1, seg_rows, :] = _layernorm(x[:seg])

    _emit("P*5+L", {"P": ffn_passes(0, first_done), "L": _chain(
        lay_out_rows(slot(_LAG, 0), _DOWN - 1, False),
        lay_out_rows(slot(_LAG, 2), _UNITS - 1, True, 4))})
    pl.loop(0, 2)(double_step)
    last = n_seg - _LAG
    pl.loop(1, _EARLY // 2)(functools.partial(two_steps, early=True))
    pl.loop(_EARLY // 2, last // 2)(functools.partial(two_steps, early=False))

    n_done = (last - _EARLY) // 2 - 1
    for i in range(n_done):
        out_copy(i).start()
    h_ref[0] = h_ref[1]
    ffn_in = [res_ref[block(n_seg - 2, 2), :], res_ref[block(last - 2, 2), :]]

    def ffn_done(ys):
        res_ref[block(n_seg - 2, 2), :] += ys[0]
        res_ref[block(last - 2, 2), :] += ys[1]

    ffn = _ffn_tasks(ffn_in, ffn_operands_ref.at[0], w_ref, hidden_ref, ffn_done)
    _emit("P", {"P": _chain(single_passes(last, _ORDER_EVEN, ffn),
                            single_passes(last + 1, _ORDER_ODD, ffn))})
    h_ref[0, seg_rows, :] = _layernorm(res_ref[block(last + 2), :])

    @pl.loop(0, 2)
    def _last_steps(i):
        transpose_out(n_done + i, res_ref[lanes(n_done + i), :])
        _emit("P", {"P": single_passes(last + 2 + i, _ORDER_SINGLE, {})})
        out_copy(n_done + i).start()

    _emit("P", {"P": ffn_passes(last, functools.partial(transpose_out, n_io - 1))})
    out_copy(n_io - 1).start()
    for i in range(n_io):
        out_copy(i).wait()


@functools.partial(jax.jit, static_argnames=("A_seg_len",))
def pallas_interleave_layers__memory_aug_recurrent_mem_tr__glu_gated_swiglu__prompt_kernel(
    A_x: jax.Array,
    A_mem0: jax.Array,
    A_Wq: jax.Array,
    A_Wk: jax.Array,
    A_Wv: jax.Array,
    A_Wo: jax.Array,
    A_seg_len: int,
    B_x: jax.Array,
    B_w1: jax.Array,
    B_w3: jax.Array,
    B_w2: jax.Array,
):
    del B_x
    _, n_tok, d_model = A_x.shape
    n_mem = A_mem0.shape[1]
    _, n_heads, d_head = A_Wq.shape
    d_ff = B_w1.shape[1]
    seg = A_seg_len
    assert A_x.shape[0] == 1 and _LAG * seg == _LANES and n_mem == 8 and n_tok == 64 * seg
    assert d_model == _TAIL * _LANES + _HALF and d_head == _LANES
    assert n_heads == _GROUPS * _COLUMNS and d_ff == 4 * (_DOWN - _UP) * _LANES
    n_operands = len(_operand_keys(False))
    hbm = pl.BlockSpec(memory_space=pltpu.HBM)
    out_t = pl.pallas_call(
        functools.partial(_kernel, seg=seg),
        out_shape=jax.ShapeDtypeStruct((d_model, n_tok), A_x.dtype),
        in_specs=[hbm] * 9,
        out_specs=hbm,
        scratch_shapes=[
            pltpu.VMEM((n_mem, d_model), A_mem0.dtype),
            pltpu.VMEM((n_tok // _LANES, d_model, _LANES), A_x.dtype),
            pltpu.VMEM((n_tok, d_model + _HALF), jnp.float32),
            pltpu.VMEM((2, n_mem + seg, d_model + _HALF), jnp.float32),
            pltpu.VMEM((n_operands, n_mem + seg, _LANES), jnp.float32),
            pltpu.VMEM((n_operands, seg // 2, _LANES), jnp.uint32),
            pltpu.VMEM((_EARLY // 8, n_operands, seg, _LANES), jnp.uint32),
            pltpu.VMEM((n_heads, 2 * (n_mem + seg), d_head), jnp.float32),
            pltpu.VMEM((d_ff // _LANES, 4 * seg, _LANES), jnp.float32),
            pltpu.VMEM((3 * _GROUPS, _COLUMNS, _EARLY * seg // 4, d_head), jnp.uint32),
            pltpu.VMEM((_UNITS, len(_PASSES), _HALF, _LANES), jnp.uint32),
            pltpu.VMEM((8, _COLUMNS * d_model // 2, _LANES), jnp.uint32),
            pltpu.SemaphoreType.DMA((8,)),
            pltpu.SemaphoreType.DMA((1,)),
            pltpu.SemaphoreType.DMA((n_tok // _LANES,)),
        ],
        compiler_params=pltpu.CompilerParams(vmem_limit_bytes=110 * 1024 * 1024, flags=_FLAGS),
    )(A_x.reshape(n_tok, d_model).T, A_mem0.reshape(n_mem, d_model), A_Wq, A_Wk, A_Wv,
      A_Wo.transpose(0, 2, 1), B_w1, B_w3, B_w2.T)
    return out_t.T.reshape(A_x.shape)
```

```python
import functools
import math
from typing import NamedTuple

import jax
import jax.numpy as jnp
import jax.experimental.pallas as pl
import jax.experimental.pallas.tpu as pltpu

_EPS = 1e-05
_MASKED = -1000000000.0
_LOG2E = math.log2(math.e)
_LANES = 128
_HALF = _LANES // 2
_TAIL = 4
_COLUMNS = 8
_GROUPS = 4
_UP, _DOWN, _UNITS = 16, 25, 30
_SLICE = 32
_PENDING = 1
_EVEN = 0
_LAG = 4
_EARLY = 32
_FLAGS = {"XLA_TPU_FORCE_LP_LLO_SCHEDULER": True}
_ORDER_EVEN = (
    "Q0 N K0 V0*8+S0 Q1*4+G0*4 A0 K1 O0 V1*8+S1 G1 A1 Q2 O1 K2 V2*8+S2 G2 A2 Q3 O2 K3 V3*8+S3 "
    "G3 A3 G8 O3 D4 G4:20")
_ORDER_ODD = (
    "Q0*4+G4*4 K0 V0*8+S0 G5 A0 Q1 O0 K1 V1*8+S1 G6 A1 Q2 O1 K2 G7 V2*8+S2 D0 A2 Q3 O2 K3 "
    "V3*8+S3 D1 D2 A3 D3 F O3")
_ORDER_EVEN_SINGLE = _ORDER_EVEN
_ORDER_ODD_SINGLE = _ORDER_ODD
_ORDER_DOUBLE = "Q0 K0 V0*8+S0 Q1 K1 A0 V1*8+S1 Q2 K2 A1 V2*8+S2 Q3 K3 A2 V3*8+S3 O0 O1 A3 O2 O3"
_ORDER_SINGLE = "Q0 K0 V0*4+S0 Q1 K1 A0 V1*4+S1 Q2 K2 A1 V2*4+S2 Q3 K3 A2 V3*4+S3 O0 O1 A3 O2 O3"
_ORDER_FFN = "N G0 G1 G2 D0 G3 G4 D1 G5 G8 G6 D4 G7 D2 D3 F"
_ORDER_LOAD = "E0+L1*20 W2 W3 E1+L2*20+L3*10:240 E1 L2 W0 E2+L0*20+L3*10"
_ORDER_FIRST = "P:12 P+L*24"
_ORDER_FIRST_FFN = "P+L*12"


class _Pass(NamedTuple):
    low: tuple
    high: tuple
    w_low: tuple
    w_high: tuple
    wide: tuple
    common: bool = False


def _scheme():
    x, y = 0, 1
    a = lambda d: d
    b = lambda d: 4 + d
    rest = lambda d: [e for e in range(4) if e != d]

    def whole(narrow, weight, wide):
        return _Pass(narrow, narrow, weight, weight, wide)

    def m1(d, e):
        return whole(((1, x, d), (1, y, e)), ((1, b(e), d), (1, a(d), e)),
                     ((1, y, a(d)), (1, x, b(e))))

    def m2(d, e):
        return whole(((1, y, min(d, e)), (1, y, max(d, e))), ((1, b(e), d),),
                     ((1, y, b(e)), (-1, y, a(d))))

    def m3(d):
        return whole(((1, x, d),), ((1, a(d), d), *((-1, a(d), e) for e in rest(d))),
                     ((1, x, a(d)), (1, y, a(d))))

    def m4(d):
        return whole(((1, y, d),), ((1, b(d), d), *((-1, b(d), e) for e in rest(d))),
                     ((1, y, b(d)), (1, x, b(d))))

    def m5(d, e):
        return whole(((1, x, min(d, e)), (1, x, max(d, e))), ((1, a(d), e),),
                     ((1, x, a(d)), (-1, x, b(e))))

    def m6(d):
        return whole(((1, y, d), (-1, x, d)), ((1, a(d), d), *((1, b(e), d) for e in rest(d))),
                     ((1, y, a(d)),))

    def m7(d):
        return whole(((1, y, d), (-1, x, d)), ((-1, b(d), d), *((-1, a(e), d) for e in rest(d))),
                     ((1, x, b(d)),))

    def with_tails(p, p_rows, p_columns, q, q_rows, q_columns):
        tail = lambda columns: tuple((1, c, _TAIL) for c in columns)
        return [
            _Pass(p.low, p.high, q.w_low, p.w_high, p.wide + q.wide, common=True),
            _Pass(p.low, ((1, p_rows, _TAIL),), p.w_low, tail(p_columns), p.wide),
            _Pass(((1, q_rows, _TAIL),), q.high, tail(q_columns), q.w_high, q.wide)]

    def near(d, e):
        return [*with_tails(m5(d, e), x, [a(d)], m5(e, d), x, [a(e)]), m3(d),
                *with_tails(m2(d, e), y, [b(e)], m2(e, d), y, [b(d)]), m3(e),
                *with_tails(m6(d), y, [a(d), b(e)], m7(d), x, [b(d), a(e)]), m1(d, e),
                *with_tails(m7(e), x, [b(e), a(d)], m6(e), y, [a(e), b(d)]), m1(e, d)]

    far = lambda d, e: [m5(d, e), m1(d, e), m2(d, e)]
    return (*near(0, 1), *far(0, 2), *far(0, 3), *far(1, 2), *far(1, 3),
            m4(2), m4(3), *near(2, 3),
            m4(0), *far(2, 0), *far(3, 0), m4(1), *far(2, 1), *far(3, 1))


_PASSES = _scheme()


def _selected(single, columns=_COLUMNS):
    for i, p in enumerate(_PASSES):
        if single:
            p = p._replace(
                wide=tuple((s, 0, c) for s, r, c in p.wide if r == c // 4 and c < columns),
                low=tuple((s, 0, d) for s, _, d in p.low),
                high=tuple((s, 0, d) for s, _, d in p.high))
        if p.wide:
            yield i, p


def _operand_keys(single):
    return tuple(dict.fromkeys((p.low, p.high) for _, p in _selected(single)))


def _signed_sum(terms):
    terms = sorted(terms, key=lambda t: -t[0])
    total = terms[0][1] if terms[0][0] > 0 else -terms[0][1]
    for sign, value in terms[1:]:
        total = total + value if sign > 0 else total - value
    return total


def _accumulate(sums, key, sign, value):
    if key not in sums:
        sums[key] = (sign, value)
    elif sums[key][0] == sign:
        sums[key] = (sign, sums[key][1] + value)
    else:
        sums[key] = (1, value - sums[key][1] if sign > 0 else sums[key][1] - value)


def _pack(x):
    return pltpu.bitcast(x.astype(jnp.bfloat16), jnp.uint32)


def _unpack(words):
    return pltpu.bitcast(words, jnp.bfloat16)


def _low_lanes(rows):
    return jax.lax.broadcasted_iota(jnp.int32, (rows, _LANES), 1) < _HALF


def _blocks(x):
    return [x[:, d * _LANES:(d + 1) * _LANES] for d in range(_TAIL + 1)]


def _store_operands(ref, row_blocks):
    blocks = [_blocks(x) for x in row_blocks]
    low_lanes = _low_lanes(row_blocks[0].shape[0])
    total = functools.cache(lambda terms: _signed_sum([(s, blocks[r][d]) for s, r, d in terms]))
    for i, (low, high) in enumerate(_operand_keys(len(row_blocks) == 1)):
        ref[i] = total(low) if low == high else jnp.where(low_lanes, total(low), total(high))


def _dot(a, b):
    return jnp.dot(a, b, preferred_element_type=jnp.float32)


def _expand(operands_ref, tiles_ref, out, single=False):
    keys = _operand_keys(single)
    sums, common = {}, []
    for i, p in _selected(single):
        product = _dot(operands_ref[keys.index((p.low, p.high))], _unpack(tiles_ref[i]))
        if p.common:
            common = [product, product]
        else:
            if common:
                product = product + common.pop()
            for s, r, c in p.wide:
                _accumulate(sums, (r, c), s, product)
        yield
    assert all(sign > 0 for sign, _ in sums.values())
    out.update({key: value for key, (_, value) in sums.items()})


def _contract(load, tiles_ref, sums, single=False, columns=_COLUMNS):
    held = []
    for i, p in _selected(single, columns):
        product = _dot(_signed_sum([(s, load(r, c)) for s, r, c in p.wide]),
                       _unpack(tiles_ref[i]))
        if p.common or held:
            held.append((p, product))
        if len(held) == 3:
            (p, common), (p1, first), (p2, second) = held
            held = []
            product = common + jnp.where(_low_lanes(common.shape[0]), first, second)
            _accumulate(sums, (p1.high[0][1], _TAIL, 1), 1, first)
            _accumulate(sums, (p2.low[0][1], _TAIL, 0), 1, second)
        if not held:
            for s, r, d in p.low:
                _accumulate(sums, (r, d), s, product)
        yield


def _contracted(sums, r):
    assert all(sign > 0 for sign, _ in sums.values())
    low, high = sums[r, _TAIL, 0][1], sums[r, _TAIL, 1][1]
    tail = jnp.where(_low_lanes(low.shape[0]), low, high)
    tail = tail + pltpu.roll(tail, _HALF, 1)
    return jnp.concatenate([sums[r, d][1] for d in range(_TAIL)] + [tail], axis=1)


def _lay_out(source, copy, tiles_ref, transposed, columns=_COLUMNS):
    rows = _HALF if transposed else _SLICE
    chosen = list(_selected(columns < _COLUMNS, columns))
    parts, pending = {}, []

    def put(i, at, value):
        if not transposed:
            tiles_ref[i, at // 2:(at + rows) // 2, :] = _pack(value)
        elif i not in parts:
            parts[i] = value
        else:
            halves = [parts.pop(i), value][::1 if at else -1]
            if halves[0].dtype != halves[1].dtype:
                halves = [half.astype(jnp.float32) for half in halves]
            pending.append((i, jnp.concatenate(halves, axis=0).astype(jnp.bfloat16).T))
            if len(pending) > _PENDING:
                i, tile = pending.pop(0)
                tiles_ref[i] = _pack(tile)

    for n, (i, p) in enumerate(chosen):
        for at in range(0, _LANES, rows):
            high = at // _HALF
            if n > high and chosen[n - 1 - high][1].common:
                continue
            first = lambda d: d * _LANES + (at % _HALF if d == _TAIL else at)
            total = lambda terms: _signed_sum([(s, source(c, first(d), rows)) for s, c, d in terms])
            terms = (p.w_low, p.w_high)[high]
            work = 4 * len(terms) + 3
            if p.common:
                k, other = chosen[n + 1 + high]
                value = total(terms)
                put(i, at, value)
                put(k, at, total((other.w_low, other.w_high)[high]) - value)
                work *= 2
            elif len(terms) == 1:
                put(i, at, copy(terms[0][1], first(terms[0][2]), rows))
                work = 3
            else:
                put(i, at, total(terms))
            for _ in range((_EVEN if transposed and _EVEN else work) * rows // 16):
                yield
    for i, tile in pending:
        tiles_ref[i] = _pack(tile)


def _layernorm(x):
    low_lanes = _low_lanes(x.shape[0])

    def mean(v):
        *full, tail = _blocks(v)
        total = functools.reduce(jnp.add, full) + jnp.where(low_lanes, tail, 0.0)
        return jnp.sum(total, axis=-1, keepdims=True) / (_TAIL * _LANES + _HALF)

    d = x - mean(x)
    return d * jax.lax.rsqrt(mean(d * d) + _EPS)


def _silu(x):
    half = 0.5 * x
    return half + half * jnp.tanh(half)


def _reciprocal(x):
    r = pl.reciprocal(x, approx=True)
    return r * (2.0 - x * r)


def _attention_masks(n_layers, rows, n_mem):
    i = jax.lax.broadcasted_iota(jnp.int32, (n_layers * rows, n_layers * rows), 0)
    j = jax.lax.broadcasted_iota(jnp.int32, (n_layers * rows, n_layers * rows), 1)
    if n_layers == 1:
        return (i < n_mem) | (i >= j), _MASKED * _LOG2E
    same = (i >= rows) == (j >= rows)
    visible = (i < n_mem) | ((i >= rows) & (i < rows + n_mem)) | (i >= j)
    fill = jnp.where(same, _MASKED * _LOG2E, -jnp.inf).astype(jnp.float32)
    return same & visible, fill


def _attention_tasks(layers, n_mem, operands_ref, w_ref, heads_ref, outs, known=None):
    single = len(layers) == 1
    rows = layers[0].shape[0]
    skipped = (rows - n_mem) // 2
    kept = rows - skipped // 2
    if known:
        first, second = layers
        layers = [jnp.concatenate([first[:n_mem], first[n_mem + skipped:], second[kept:]], axis=0),
                  second[:kept]]
    _store_operands(operands_ref, layers)
    visible, fill = _attention_masks(len(layers), rows, n_mem)
    scale = _LANES ** -0.5 * _LOG2E
    qkv, probs, sums = {}, {}, {}

    def stacked(u, h, streamed=False):
        parts = [qkv[u][r, h] for r in range(len(layers))]
        if known:
            x, y = parts
            parts = [x[:n_mem], known(u, h), x[n_mem:rows - skipped], y, x[rows - skipped:]]
        value = jnp.concatenate(parts, axis=0)
        return value if single and streamed else value.astype(jnp.bfloat16)

    def project(u):
        qkv[u] = {}
        yield from _expand(operands_ref, w_ref.at[u], qkv[u], single)

    def scores(g):
        for h in range(_COLUMNS):
            s = jax.lax.dot_general(stacked(4 * g, h, True), stacked(4 * g + 1, h),
                                    (((1,), (1,)), ((), ())), preferred_element_type=jnp.float32)
            s = jnp.where(visible, s * scale, fill)
            p = jnp.exp2(s - jnp.max(s, axis=-1, keepdims=True))
            p = p * _reciprocal(jnp.sum(p, axis=-1, keepdims=True))
            probs[g, h] = p if single else p.astype(jnp.bfloat16)
            yield

    def values(g):
        for h in range(_COLUMNS):
            heads_ref[_COLUMNS * g + h, :len(layers) * rows, :] = _dot(
                probs[g, h], stacked(4 * g + 2, h))
            yield

    def output(g):
        yield from _contract(lambda r, h: heads_ref[_COLUMNS * g + h, r * rows:(r + 1) * rows, :],
                             w_ref.at[4 * g + 3], sums, single)
        if g == _GROUPS - 1:
            outs.extend(_contracted(sums, r) for r in range(len(layers)))

    tasks = {}
    for g in range(_GROUPS):
        tasks.update({f"Q{g}": project(4 * g), f"K{g}": project(4 * g + 1),
                      f"V{g}": project(4 * g + 2), f"S{g}": scores(g), f"A{g}": values(g),
                      f"O{g}": output(g)})
    return tasks


def _ffn_tasks(row_blocks, operands_ref, w_ref, hidden_ref, result):
    rows = row_blocks[0].shape[0]
    sums = {}

    def prepare():
        _store_operands(operands_ref, [_layernorm(x) for x in row_blocks])
        yield

    def gated(u):
        both = {}
        yield from _expand(operands_ref, w_ref.at[_UP + u], both)
        for c in range(4):
            for r in range(2):
                hidden_ref[4 * u + c, r * rows:(r + 1) * rows, :] = (
                    _silu(both[r, c]) * both[r, 4 + c])

    def down(u):
        yield from _contract(lambda r, c: hidden_ref[_COLUMNS * u + c, r * rows:(r + 1) * rows, :],
                             w_ref.at[_DOWN + u], sums)

    def down_rest(u):
        rest = {}
        yield from _contract(lambda r, c: hidden_ref[_COLUMNS * u + c], w_ref.at[_DOWN + u], rest,
                             single=True, columns=4)
        for (_, *key), (sign, value) in rest.items():
            for r in range(2):
                _accumulate(sums, (r, *key), sign, value[r * rows:(r + 1) * rows])

    def finish():
        result([_contracted(sums, r) for r in range(2)])
        yield

    return {"N": prepare(), "F": finish(), "D4": down_rest(4),
            **{f"G{u}": gated(u) for u in range(_DOWN - _UP)},
            **{f"D{u}": down(u) for u in range(4)}}


def _passes(order, tasks):
    done = object()
    for item in order.split():
        names, _, turns = item.partition(":")
        running = [(tasks[name], int(count or 1))
                   for name, _, count in (part.partition("*") for part in names.split("+"))]
        turn = 0
        while running and (not turns or turn < int(turns)):
            for task, count in tuple(running):
                for _ in range(count):
                    if next(task, done) is done:
                        running.remove((task, count))
                        break
                    yield
            turn += 1


def _emit(order, tasks):
    for _ in _passes(order, tasks):
        pass


def _chain(*tasks):
    for task in tasks:
        yield from task


def _kernel(xt_hbm, mem0_hbm, wq_hbm, wk_hbm, wv_hbm, wot_hbm, w1_hbm, w3_hbm, w2t_hbm,
            outt_hbm, mem0_ref, io_ref, res_ref, h_ref, operands_ref, short_operands_ref,
            ffn_operands_ref, heads_ref, hidden_ref, early_ref, w_ref, qkv_stage, wo_stage,
            ffn_stage, attention_sem, ffn_sem, mem_sem, io_sem, *, seg):
    d_model, n_tok = xt_hbm.shape
    n_mem = mem0_ref.shape[0]
    n_seg = n_tok // seg
    n_io = n_tok // _LANES
    mem_rows, seg_rows = slice(0, n_mem), slice(n_mem, n_mem + seg)

    def block(r, n=1):
        return pl.ds(pl.multiple_of(r * seg, seg), n * seg)

    def lanes(i):
        return pl.ds(pl.multiple_of(i * _LANES, _LANES), _LANES)

    def transpose_in(i):
        x = io_ref[i].astype(jnp.float32)
        res_ref[lanes(i), :] = jnp.concatenate([x, x[_TAIL * _LANES:]], axis=0).T

    def transpose_out(i, x):
        io_ref[i] = x.T[:d_model].astype(io_ref.dtype)

    def single_passes(r, order, others):
        x = res_ref[block(r), :]
        following = res_ref[block(jnp.minimum(r + 1, n_seg - 1)), :]
        outs = []
        yield from _passes(order, {**others, **_attention_tasks(
            [h_ref[0]], n_mem, operands_ref, w_ref, heads_ref, outs)})
        h_ref[0, seg_rows, :] = _layernorm(following)
        h_ref[0, mem_rows, :] = outs[0][mem_rows]
        res_ref[block(r), :] = x + outs[0][seg_rows]

    def double_tasks(layers, outs, early=None):
        if early is None:
            return _attention_tasks(layers, n_mem, operands_ref, w_ref, heads_ref, outs)
        rows = pl.ds(pl.multiple_of(early * (seg // 2), seg // 2), seg // 2)
        return _attention_tasks(layers, n_mem, short_operands_ref, w_ref, heads_ref, outs,
                                lambda u, h: early_ref[u - u // 4, h, rows, :])

    def double_step(b):
        xs = [res_ref[block(b + _LAG, 2), :], res_ref[block(b, 2), :]]
        outs = []
        _emit(_ORDER_DOUBLE, double_tasks([h_ref[0], h_ref[1]], outs, 2 - b))
        for i, r in enumerate((b + _LAG, b)):
            h_ref[i, seg_rows, :] = _layernorm(xs[i][seg:])
            h_ref[i, mem_rows, :] = outs[i][mem_rows]
            res_ref[block(r), :] = xs[i][:seg] + outs[i][seg_rows]

    def two_steps(j):
        b = 2 * j
        xs = [res_ref[block(b + _LAG + 1), :], res_ref[block(b + 1), :]]
        ffn_in = [res_ref[block(b + 2, 2), :], res_ref[block(b - 2, 2), :]]
        following = res_ref[block(jnp.minimum(b + _LAG + 2, n_seg - 1)), :]
        tile = jnp.maximum(j - 3, 0) // 2
        transpose_out(tile, res_ref[lanes(tile), :])
        even, odd = [], []

        def ffn_done(ys):
            for r, y in zip((b + 2, b - 2), ys):
                res_ref[block(r, 2), :] += y
            h_ref[1, seg_rows, :] = _layernorm(res_ref[block(b + 2), :])

        ffn = _ffn_tasks(ffn_in, ffn_operands_ref.at[0], w_ref, hidden_ref, ffn_done)
        _emit(_ORDER_EVEN, {**ffn, **double_tasks([h_ref[0], h_ref[1]], even, j + _LAG // 2)})
        h_ref[0, seg_rows, :] = _layernorm(following)
        for r, o in zip((b + _LAG, b), even):
            res_ref[block(r), :] += o[seg_rows]
        layers = [jnp.concatenate([o[mem_rows], _layernorm(x)], axis=0) for o, x in zip(even, xs)]
        _emit(_ORDER_ODD, {**ffn, **double_tasks(layers, odd)})
        for i, r in enumerate((b + _LAG, b)):
            h_ref[i, mem_rows, :] = odd[i][mem_rows]
            res_ref[block(r + 1), :] = xs[i] + odd[i][seg_rows]

    def ffn_passes(first, result):
        xs = [res_ref[block(first, 2), :], res_ref[block(first + 2, 2), :]]
        return _passes(_ORDER_FFN, _ffn_tasks(
            xs, ffn_operands_ref.at[0], w_ref, hidden_ref,
            lambda ys: result(jnp.concatenate([x + y for x, y in zip(xs, ys)], axis=0))))

    def attention_copies(g, i):
        sem = attention_sem.at[4 * (g % 2) + i]
        if i == 3:
            heads = wot_hbm.bitcast(jnp.uint32).at[pl.ds(_COLUMNS * g, _COLUMNS)]
            return [pltpu.make_async_copy(heads, wo_stage, sem)]
        words = (wq_hbm, wk_hbm, wv_hbm)[i].bitcast(jnp.uint32)
        return [pltpu.make_async_copy(words.at[:, 4 * g + p, :], qkv_stage.at[g % 2, i, p], sem)
                for p in range(4)]

    def ffn_copies(batch, columns=_COLUMNS):
        width = columns * _LANES
        source = pl.ds(pl.multiple_of(batch * _COLUMNS * _LANES, _LANES), width)
        return [pltpu.make_async_copy(w.bitcast(jnp.uint32).at[:, source],
                                      ffn_stage.at[batch % 2, i, :, pl.ds(0, width)],
                                      ffn_sem.at[3 * (batch % 2) + i])
                for i, w in enumerate((w1_hbm, w3_hbm, w2t_hbm))]

    def start(copies):
        for c in copies:
            c.start()

    def wait(copies):
        for c in copies:
            c.wait()

    def lay_out_heads(g, i, u):
        def source(c, first, n):
            words = qkv_stage[g % 2, i, c // 2, pl.ds(first, n), :]
            words = words & jnp.uint32(0xFFFF0000) if c % 2 else words << 16
            return pltpu.bitcast(words, jnp.float32)

        def copy(c, first, n):
            even, odd = (qkv_stage[g % 2, i, c // 2, pl.ds(first + k, n // 2, stride=2), :]
                         for k in range(2))
            if c % 2:
                return _unpack((even >> 16) | (odd & jnp.uint32(0xFFFF0000)))
            return _unpack((even & jnp.uint32(0xFFFF)) | (odd << 16))

        return _lay_out(source, copy, w_ref.at[u], False)

    def lay_out_rows(words, u, transposed, columns=_COLUMNS):
        copy = lambda c, first, n: _unpack(words(c, pl.ds(first // 2, n // 2)))
        return _lay_out(lambda *at: copy(*at).astype(jnp.float32), copy, w_ref.at[u], transposed,
                        columns)

    def lay_out_up(batch, i):
        return lay_out_rows(
            lambda c, rows: ffn_stage[batch % 2, c // 4, rows, pl.ds((4 * i + c % 4) * _LANES, _LANES)],
            _UP + 2 * batch + i, False)

    def lay_out_down(batch, columns=_COLUMNS):
        return lay_out_rows(
            lambda c, rows: ffn_stage[batch % 2, 2, rows, pl.ds(c * _LANES, _LANES)],
            _DOWN + batch, True, columns)

    def x_copy(i):
        return pltpu.make_async_copy(xt_hbm.at[:, lanes(i)], io_ref.at[i], io_sem.at[i])

    def out_copy(i):
        return pltpu.make_async_copy(io_ref.at[i], outt_hbm.at[:, lanes(i)], io_sem.at[i])

    n_chunks = ffn_operands_ref.shape[0]

    def load_group(g):
        def project(i):
            for chunk in range(n_chunks):
                out = {}
                yield from _expand(ffn_operands_ref.at[chunk], w_ref.at[4 * g + i], out)
                for (r, c), value in out.items():
                    early_ref[3 * g + i, c, pl.ds((2 * chunk + r) * 2 * seg, 2 * seg), :] = value

        def arrive(i):
            if i == 0:
                pl.when(g + 1 < _GROUPS)(lambda: wait(attention_copies(g + 1, 0)))
            else:
                wait(attention_copies(g, i))
            yield

        start(attention_copies(g, 3))
        pl.when(g + 1 < _GROUPS)(
            lambda: start(attention_copies(g + 1, 1) + attention_copies(g + 1, 2)))
        pl.when(g + 2 < _GROUPS)(lambda: start(attention_copies(g + 2, 0)))
        pl.when(g + 1 == _GROUPS)(lambda: start(ffn_copies(0)))
        following = jnp.minimum(g + 1, _GROUPS - 1)
        same = jnp.minimum(g, _GROUPS - 1)
        _emit("W1 " + _ORDER_LOAD, {
            **{f"E{i}": project(i) for i in range(3)}, **{f"W{i}": arrive(i) for i in range(4)},
            "L0": lay_out_heads(following, 0, 4 * following),
            "L1": lay_out_heads(g, 1, 4 * same + 1), "L2": lay_out_heads(g, 2, 4 * same + 2),
            "L3": lay_out_rows(lambda c, rows: wo_stage[c, rows, :], 4 * same + 3, True)})

    def first_step(r):
        wait(ffn_copies(r))
        pl.when(r + 1 < _LAG)(lambda: start(ffn_copies(r + 1)))
        pl.when(r + 1 == _LAG)(lambda: start(ffn_copies(_LAG, 4)))
        _emit(_ORDER_FIRST, {
            "P": single_passes(r, _ORDER_SINGLE, {}),
            "L": _passes("U*2+D", {"U": _chain(lay_out_up(r, 0), lay_out_up(r, 1)),
                                   "D": lay_out_down(r)})})

    mem_copy = pltpu.make_async_copy(mem0_hbm, mem0_ref, mem_sem.at[0])
    start(attention_copies(0, 0))
    for i in range(n_io):
        x_copy(i).start()
    mem_copy.start()
    wait(attention_copies(0, 0))
    start(attention_copies(0, 1))
    _emit("L", {"L": lay_out_heads(0, 0, 0)})
    start(attention_copies(0, 2))

    @pl.loop(0, n_chunks)
    def _early_operands(chunk):
        tiles = [n_io // n_chunks * chunk + i for i in range(n_io // n_chunks)]
        for i in tiles:
            x_copy(i).wait()
        for i in tiles:
            transpose_in(i)
        segments = [2 * (8 * chunk + e) for e in range(8)]
        segments[1] = jnp.where(chunk == 0, _LAG + 1, segments[1])
        halves = [res_ref[pl.ds(pl.multiple_of(r * seg, seg), seg // 2), :] for r in segments]
        _store_operands(ffn_operands_ref.at[chunk], [
            _layernorm(jnp.concatenate(part, axis=0)) for part in (halves[:4], halves[4:])])

    start(attention_copies(1, 0))
    pl.loop(0, _GROUPS)(load_group)
    mem_copy.wait()
    mem0 = mem0_ref[...].astype(jnp.float32)
    mem0 = jnp.concatenate([mem0, mem0[:, _TAIL * _LANES:]], axis=1)
    h_ref[0] = jnp.concatenate([mem0, _layernorm(res_ref[block(0), :])], axis=0)
    h_ref[1, mem_rows, :] = mem0
    pl.loop(0, _LAG)(first_step)
    wait(ffn_copies(_LAG, 4))

    def first_done(x):
        res_ref[:_LAG * seg, :] = x
        h_ref[1, seg_rows, :] = _layernorm(x[:seg])

    _emit(_ORDER_FIRST_FFN, {"P": ffn_passes(0, first_done),
                             "L": _chain(lay_out_up(_LAG, 0), lay_out_down(_LAG, 4))})
    pl.loop(0, 2)(double_step)
    last = n_seg - _LAG
    pl.loop(1, last // 2)(two_steps)

    n_done = n_io - 3
    for i in range(n_done):
        out_copy(i).start()
    h_ref[0] = h_ref[1]
    ffn_in = [res_ref[block(n_seg - 2, 2), :], res_ref[block(last - 2, 2), :]]

    def ffn_done(ys):
        res_ref[block(n_seg - 2, 2), :] += ys[0]
        res_ref[block(last - 2, 2), :] += ys[1]

    ffn = _ffn_tasks(ffn_in, ffn_operands_ref.at[0], w_ref, hidden_ref, ffn_done)
    _emit("P", {"P": _chain(single_passes(last, _ORDER_EVEN_SINGLE, ffn),
                            single_passes(last + 1, _ORDER_ODD_SINGLE, ffn))})
    h_ref[0, seg_rows, :] = _layernorm(res_ref[block(last + 2), :])

    @pl.loop(0, 2)
    def _last_steps(i):
        transpose_out(n_done + i, res_ref[lanes(n_done + i), :])
        _emit("P", {"P": single_passes(last + 2 + i, _ORDER_SINGLE, {})})
        out_copy(n_done + i).start()

    _emit("P", {"P": ffn_passes(last, functools.partial(transpose_out, n_io - 1))})
    out_copy(n_io - 1).start()
    for i in range(n_io):
        out_copy(i).wait()


@functools.partial(jax.jit, static_argnames=("A_seg_len",))
def pallas_interleave_layers__memory_aug_recurrent_mem_tr__glu_gated_swiglu__prompt_kernel(
    A_x: jax.Array,
    A_mem0: jax.Array,
    A_Wq: jax.Array,
    A_Wk: jax.Array,
    A_Wv: jax.Array,
    A_Wo: jax.Array,
    A_seg_len: int,
    B_x: jax.Array,
    B_w1: jax.Array,
    B_w3: jax.Array,
    B_w2: jax.Array,
):
    del B_x
    _, n_tok, d_model = A_x.shape
    n_mem = A_mem0.shape[1]
    _, n_heads, d_head = A_Wq.shape
    d_ff = B_w1.shape[1]
    seg = A_seg_len
    assert A_x.shape[0] == 1 and _LAG * seg == _LANES and n_mem == 8 and n_tok == 64 * seg
    assert d_model == _TAIL * _LANES + _HALF and d_head == _LANES
    assert n_heads == _GROUPS * _COLUMNS and d_ff == 4 * (_DOWN - _UP) * _LANES
    n_operands = len(_operand_keys(False))
    hbm = pl.BlockSpec(memory_space=pltpu.HBM)
    out_t = pl.pallas_call(
        functools.partial(_kernel, seg=seg),
        out_shape=jax.ShapeDtypeStruct((d_model, n_tok), A_x.dtype),
        in_specs=[hbm] * 9,
        out_specs=hbm,
        scratch_shapes=[
            pltpu.VMEM((n_mem, d_model), A_mem0.dtype),
            pltpu.VMEM((n_tok // _LANES, d_model, _LANES), A_x.dtype),
            pltpu.VMEM((n_tok, d_model + _HALF), jnp.float32),
            pltpu.VMEM((2, n_mem + seg, d_model + _HALF), jnp.float32),
            pltpu.VMEM((n_operands, n_mem + seg, _LANES), jnp.float32),
            pltpu.VMEM((n_operands, seg, _LANES), jnp.float32),
            pltpu.VMEM((_EARLY // 8, n_operands, 2 * seg, _LANES), jnp.float32),
            pltpu.VMEM((n_heads, 2 * (n_mem + seg), d_head), jnp.float32),
            pltpu.VMEM((d_ff // _LANES, 4 * seg, _LANES), jnp.float32),
            pltpu.VMEM((3 * _GROUPS, _COLUMNS, _EARLY * seg // 2, d_head), jnp.float32),
            pltpu.VMEM((_UNITS, len(_PASSES), _HALF, _LANES), jnp.uint32),
            pltpu.VMEM((2, 3, _COLUMNS // 2, d_model, d_head), jnp.uint32),
            pltpu.VMEM((_COLUMNS, d_model // 2, d_head), jnp.uint32),
            pltpu.VMEM((2, 3, d_model // 2, _COLUMNS * _LANES), jnp.uint32),
            pltpu.SemaphoreType.DMA((8,)),
            pltpu.SemaphoreType.DMA((6,)),
            pltpu.SemaphoreType.DMA((1,)),
            pltpu.SemaphoreType.DMA((n_tok // _LANES,)),
        ],
        compiler_params=pltpu.CompilerParams(vmem_limit_bytes=124 * 1024 * 1024, flags=_FLAGS,
                                             disable_bounds_checks=True),
    )(A_x.reshape(n_tok, d_model).T, A_mem0.reshape(n_mem, d_model), A_Wq, A_Wk, A_Wv,
      A_Wo.transpose(0, 2, 1), B_w1, B_w3, B_w2.T)
    return out_t.T.reshape(A_x.shape)
```

```python
import functools
import math
from typing import NamedTuple

import jax
import jax.numpy as jnp
import jax.experimental.pallas as pl
import jax.experimental.pallas.tpu as pltpu

_EPS = 1e-05
_MASKED = -1000000000.0
_LOG2E = math.log2(math.e)
_LANES = 128
_HALF = _LANES // 2
_TAIL = 4
_COLUMNS = 8
_GROUPS = 4
_UP, _DOWN, _UNITS = 16, 25, 30
_PENDING = 2
_EVEN = (8, 26)
_UP_ROWS = 32
_ORDER_L = "U*2+D"
_CARRY = False
_LAG = 4
_EARLY = 32
_FLAGS = {"XLA_TPU_FORCE_LP_LLO_SCHEDULER": True}
_ORDER_EVEN = "N X Q0 K0 V0 Q1 G0*8+S0 K1 A0 V1 G1*8+S1 O0 Q2 A1 K2 O1 V2 G2*8+S2 Q3 A2 K3 O2 V3 G3*8+S3 G8 A3 D4 O3 G4"
_ORDER_ODD = "Q0 K0 V0*8+S0 G5 A0 G6 Q1 G7 K1 D0 V1*8+S1 D1 A1 D2 Q2 D3 F X K2 V2*8+S2 Q3 A2 K3 V3*8+S3 O0 O1 A3 O2 O3"
_ORDER_EVEN_SINGLE = (
    "Q0 N K0 V0*4+S0 Q1 K1 G0 A0 V1*4+S1 O0 G1 A1 Q2 K2 V2*4+S2 O1 G2 A2 Q3 K3 V3*4+S3 X O2 "
    "G3 A3 G8 O3 D4 G4")
_ORDER_ODD_SINGLE = (
    "Q0 K0 V0*4+S0 G5 A0 Q1 K1 V1*4+S1 G6 A1 Q2 K2 G7 V2*4+S2 D0 A2 Q3 K3 "
    "V3*4+S3 D1 D2 A3 D3 F X O0 O1 O2 O3")
_ORDER_DOUBLE = "Q0 K0 Q1 K1 V0*8+S0 Q2 K2 V1*8+S1 A0 Q3 K3 V2 A1 O0*8+S2 V3 X O1*6+S3 A2 O2:30 A3 O2 O3"
_ORDER_SINGLE = "Q0 K0 V0*4+S0 Q1 K1 A0 V1*4+S1 Q2 K2 A1 V2*4+S2 Q3 K3 A2 V3*4+S3 X O0 O1 A3 O2 O3"
_ORDER_FFN = "N G0 G1 G2 D0 G3 G4 D1 G5 G8 G6 D4 G7 D2 D3 F"
_ORDER_LOAD = "E0+L1*21 W2 W3 E1+L2*21+L3*10:240 E1 L2 W0 E2+L0*21+L3*11"
_ORDER_FIRST = "P:4 P+L*24"
_ORDER_FIRST_FFN = "P:20 P+L*14"


class _Pass(NamedTuple):
    low: tuple
    high: tuple
    w_low: tuple
    w_high: tuple
    wide: tuple
    common: bool = False


def _scheme():
    x, y = 0, 1
    a = lambda d: d
    b = lambda d: 4 + d
    rest = lambda d: [e for e in range(4) if e != d]

    def whole(narrow, weight, wide):
        return _Pass(narrow, narrow, weight, weight, wide)

    def m1(d, e):
        return whole(((1, x, d), (1, y, e)), ((1, b(e), d), (1, a(d), e)),
                     ((1, y, a(d)), (1, x, b(e))))

    def m2(d, e):
        return whole(((1, y, min(d, e)), (1, y, max(d, e))), ((1, b(e), d),),
                     ((1, y, b(e)), (-1, y, a(d))))

    def m3(d):
        return whole(((1, x, d),), ((1, a(d), d), *((-1, a(d), e) for e in rest(d))),
                     ((1, x, a(d)), (1, y, a(d))))

    def m4(d):
        return whole(((1, y, d),), ((1, b(d), d), *((-1, b(d), e) for e in rest(d))),
                     ((1, y, b(d)), (1, x, b(d))))

    def m5(d, e):
        return whole(((1, x, min(d, e)), (1, x, max(d, e))), ((1, a(d), e),),
                     ((1, x, a(d)), (-1, x, b(e))))

    def m6(d):
        return whole(((1, y, d), (-1, x, d)), ((1, a(d), d), *((1, b(e), d) for e in rest(d))),
                     ((1, y, a(d)),))

    def m7(d):
        return whole(((1, y, d), (-1, x, d)), ((-1, b(d), d), *((-1, a(e), d) for e in rest(d))),
                     ((1, x, b(d)),))

    def with_tails(p, p_rows, p_columns, q, q_rows, q_columns):
        tail = lambda columns: tuple((1, c, _TAIL) for c in columns)
        return [
            _Pass(p.low, p.high, q.w_low, p.w_high, p.wide + q.wide, common=True),
            _Pass(p.low, ((1, p_rows, _TAIL),), p.w_low, tail(p_columns), p.wide),
            _Pass(((1, q_rows, _TAIL),), q.high, tail(q_columns), q.w_high, q.wide)]

    def near(d, e):
        return [*with_tails(m5(d, e), x, [a(d)], m5(e, d), x, [a(e)]), m3(d),
                *with_tails(m2(d, e), y, [b(e)], m2(e, d), y, [b(d)]), m3(e),
                *with_tails(m6(d), y, [a(d), b(e)], m7(d), x, [b(d), a(e)]), m1(d, e),
                *with_tails(m7(e), x, [b(e), a(d)], m6(e), y, [a(e), b(d)]), m1(e, d)]

    far = lambda d, e: [m5(d, e), m1(d, e), m2(d, e)]
    return (*near(0, 1), *far(0, 2), *far(0, 3), *far(1, 2), *far(1, 3),
            m4(2), m4(3), *near(2, 3),
            m4(0), *far(2, 0), *far(3, 0), m4(1), *far(2, 1), *far(3, 1))


_PASSES = _scheme()


def _selected(single, columns=_COLUMNS):
    for i, p in enumerate(_PASSES):
        if single:
            p = p._replace(
                wide=tuple((s, 0, c) for s, r, c in p.wide if r == c // 4 and c < columns),
                low=tuple((s, 0, d) for s, _, d in p.low),
                high=tuple((s, 0, d) for s, _, d in p.high))
        if p.wide:
            yield i, p


def _operand_keys(single):
    return tuple(dict.fromkeys((p.low, p.high) for _, p in _selected(single)))


def _signed_sum(terms):
    terms = sorted(terms, key=lambda t: -t[0])
    total = terms[0][1] if terms[0][0] > 0 else -terms[0][1]
    for sign, value in terms[1:]:
        total = total + value if sign > 0 else total - value
    return total


def _accumulate(sums, key, sign, value):
    if key not in sums:
        sums[key] = (sign, value)
    elif sums[key][0] == sign:
        sums[key] = (sign, sums[key][1] + value)
    else:
        sums[key] = (1, value - sums[key][1] if sign > 0 else sums[key][1] - value)


def _pack(x):
    return pltpu.bitcast(x.astype(jnp.bfloat16), jnp.uint32)


def _unpack(words):
    return pltpu.bitcast(words, jnp.bfloat16)


def _low_lanes(rows):
    return jax.lax.broadcasted_iota(jnp.int32, (rows, _LANES), 1) < _HALF


def _blocks(x):
    return [x[:, d * _LANES:(d + 1) * _LANES] for d in range(_TAIL + 1)]


def _store_operands(ref, first, row_blocks):
    blocks = [_blocks(x) for x in row_blocks]
    rows = row_blocks[0].shape[0]
    low_lanes = _low_lanes(rows)
    total = functools.cache(lambda terms: _signed_sum([(s, blocks[r][d]) for s, r, d in terms]))
    for i, (low, high) in enumerate(_operand_keys(len(row_blocks) == 1)):
        ref[i, pl.ds(first, rows), :] = (
            total(low) if low == high else jnp.where(low_lanes, total(low), total(high)))


def _dot(a, b):
    return jnp.dot(a, b, preferred_element_type=jnp.float32)


def _expand(operands_ref, tiles_ref, out, single=False):
    keys = _operand_keys(single)
    sums, common = {}, []
    for i, p in _selected(single):
        product = _dot(operands_ref[keys.index((p.low, p.high))], _unpack(tiles_ref[i]))
        if p.common:
            common = [product, product]
        else:
            if common:
                product = product + common.pop()
            for s, r, c in p.wide:
                _accumulate(sums, (r, c), s, product)
        yield
    assert all(sign > 0 for sign, _ in sums.values())
    out.update({key: value for key, (_, value) in sums.items()})


def _contract(load, tiles_ref, sums, single=False, columns=_COLUMNS):
    held = []
    for i, p in _selected(single, columns):
        product = _dot(_signed_sum([(s, load(r, c)) for s, r, c in p.wide]),
                       _unpack(tiles_ref[i]))
        if p.common or held:
            held.append((p, product))
        if len(held) == 3:
            (p, common), (p1, first), (p2, second) = held
            held = []
            product = common + jnp.where(_low_lanes(common.shape[0]), first, second)
            _accumulate(sums, (p1.high[0][1], _TAIL, 1), 1, first)
            _accumulate(sums, (p2.low[0][1], _TAIL, 0), 1, second)
        if not held:
            for s, r, d in p.low:
                _accumulate(sums, (r, d), s, product)
        yield


def _residual(row_blocks):
    return {(r, d) if d < _TAIL else (r, d, 0): (1, block)
            for r, x in enumerate(row_blocks) for d, block in enumerate(_blocks(x))}


def _contracted(sums, r):
    assert all(sign > 0 for sign, _ in sums.values())
    low, high = sums[r, _TAIL, 0][1], sums[r, _TAIL, 1][1]
    tail = jnp.where(_low_lanes(low.shape[0]), low, high)
    tail = tail + pltpu.roll(tail, _HALF, 1)
    return jnp.concatenate([sums[r, d][1] for d in range(_TAIL)] + [tail], axis=1)


def _weight_sums(source, copy, starts, columns=_COLUMNS):
    chosen = list(_selected(columns < _COLUMNS, columns))
    for n, (i, p) in enumerate(chosen):
        for high in range(2):
            if n > high and chosen[n - 1 - high][1].common:
                continue
            for at in starts:
                first = lambda d: d * _LANES + at + (0 if d == _TAIL else high * _HALF)
                total = lambda terms: _signed_sum([(s, source(c, first(d))) for s, c, d in terms])
                terms = (p.w_low, p.w_high)[high]
                if len(terms) == 1:
                    yield i, high * _HALF + at, copy(terms[0][1], first(terms[0][2])), 0
                else:
                    value = total(terms)
                    yield i, high * _HALF + at, value, len(terms)
                if p.common:
                    k, other = chosen[n + 1 + high]
                    value = value if len(terms) > 1 else total(terms)
                    yield (k, high * _HALF + at, total((other.w_low, other.w_high)[high]) - value,
                           len(terms) + 1)


def _lay_out(sums, tiles_ref):
    for i, first, value, terms in sums:
        tiles_ref[i, pl.ds(pl.multiple_of(first // 2, 8), value.shape[0] // 2), :] = _pack(value)
        yield from range((4 * terms + 3) * value.shape[0] // 16)


def _lay_out_transposed(sums, tiles_ref):
    halves, pending = {}, []
    for i, first, value, terms in sums:
        halves[i, first] = value
        if (i, _HALF - first) in halves:
            pair = [halves[i, 0], halves[i, _HALF]]
            if pair[0].dtype != pair[1].dtype:
                pair = [half.astype(jnp.float32) for half in pair]
            pending.append((i, jnp.concatenate(pair, axis=0).astype(jnp.bfloat16).T))
        if len(pending) > _PENDING:
            k, tile = pending.pop(0)
            tiles_ref[k] = _pack(tile)
        yield from range(_EVEN[0] * terms + _EVEN[1])
    for k, tile in pending:
        tiles_ref[k] = _pack(tile)


def _layernorm(x):
    low_lanes = _low_lanes(x.shape[0])

    def mean(v):
        *full, tail = _blocks(v)
        total = functools.reduce(jnp.add, full) + jnp.where(low_lanes, tail, 0.0)
        return jnp.sum(total, axis=-1, keepdims=True) / (_TAIL * _LANES + _HALF)

    d = x - mean(x)
    return d * jax.lax.rsqrt(mean(d * d) + _EPS)


def _silu(x):
    half = 0.5 * x
    return half + half * jnp.tanh(half)


def _reciprocal(x):
    r = pl.reciprocal(x, approx=True)
    return r * (2.0 - x * r)


def _attention_masks(n_layers, rows, n_mem):
    i = jax.lax.broadcasted_iota(jnp.int32, (n_layers * rows, n_layers * rows), 0)
    j = jax.lax.broadcasted_iota(jnp.int32, (n_layers * rows, n_layers * rows), 1)
    if n_layers == 1:
        return (i < n_mem) | (i >= j), _MASKED * _LOG2E
    same = (i >= rows) == (j >= rows)
    visible = (i < n_mem) | ((i >= rows) & (i < rows + n_mem)) | (i >= j)
    fill = jnp.where(same, _MASKED * _LOG2E, -jnp.inf).astype(jnp.float32)
    return same & visible, fill


def _attention_tasks(xs, operands_ref, w_ref, heads_ref, outs, known=None):
    n_layers, rows = len(xs), heads_ref.shape[1] // 2
    single, n_mem = n_layers == 1, rows - xs[0].shape[0]
    visible, fill = _attention_masks(n_layers, rows, n_mem)
    scale = _LANES ** -0.5 * _LOG2E
    qkv, probs = {}, {}
    sums = _residual([jnp.concatenate([jnp.zeros_like(x[:n_mem]), x], axis=0) for x in xs])

    def stacked(u, h, streamed=False):
        parts = [qkv[u][r, h] for r in range(n_layers)]
        if known:
            (x, y), moved = parts, (rows + n_mem) // 2
            parts = [x[:n_mem], known(u, h), x[n_mem:moved], y, x[moved:]]
        value = jnp.concatenate(parts, axis=0)
        return value if single and streamed else value.astype(jnp.bfloat16)

    def project(u):
        qkv[u] = {}
        yield from _expand(operands_ref, w_ref.at[u], qkv[u], single)

    def scores(g):
        for h in range(_COLUMNS):
            s = jax.lax.dot_general(stacked(4 * g, h, True), stacked(4 * g + 1, h),
                                    (((1,), (1,)), ((), ())), preferred_element_type=jnp.float32)
            s = jnp.where(visible, s * scale, fill)
            p = jnp.exp2(s - jnp.max(s, axis=-1, keepdims=True))
            p = p * _reciprocal(jnp.sum(p, axis=-1, keepdims=True))
            probs[g, h] = p if single else p.astype(jnp.bfloat16)
            yield

    def values(g):
        for h in range(_COLUMNS):
            heads_ref[_COLUMNS * g + h, :n_layers * rows, :] = _dot(
                probs[g, h], stacked(4 * g + 2, h))
            yield

    def output(g):
        yield from _contract(lambda r, h: heads_ref[_COLUMNS * g + h, r * rows:(r + 1) * rows, :],
                             w_ref.at[4 * g + 3], sums, single)
        if g == _GROUPS - 1:
            outs.extend(_contracted(sums, r) for r in range(n_layers))

    tasks = {}
    for g in range(_GROUPS):
        tasks.update({f"Q{g}": project(4 * g), f"K{g}": project(4 * g + 1),
                      f"V{g}": project(4 * g + 2), f"S{g}": scores(g), f"A{g}": values(g),
                      f"O{g}": output(g)})
    return tasks


def _ffn_tasks(xs, operands_ref, w_ref, hidden_ref, result):
    rows = operands_ref.shape[1]
    sums = _residual(xs)

    def gated(u):
        both = {}
        yield from _expand(operands_ref, w_ref.at[_UP + u], both)
        for c in range(4):
            for r in range(2):
                hidden_ref[4 * u + c, r * rows:(r + 1) * rows, :] = (
                    _silu(both[r, c]) * both[r, 4 + c])

    def down(u):
        yield from _contract(lambda r, c: hidden_ref[_COLUMNS * u + c, r * rows:(r + 1) * rows, :],
                             w_ref.at[_DOWN + u], sums)

    def down_rest(u):
        rest = {}
        yield from _contract(lambda r, c: hidden_ref[_COLUMNS * u + c], w_ref.at[_DOWN + u], rest,
                             single=True, columns=4)
        for (_, *key), (sign, value) in rest.items():
            for r in range(2):
                _accumulate(sums, (r, *key), sign, value[r * rows:(r + 1) * rows])

    def finish():
        result([_contracted(sums, r) for r in range(2)])
        yield

    return {"F": finish(), "D4": down_rest(4),
            **{f"G{u}": gated(u) for u in range(_DOWN - _UP)},
            **{f"D{u}": down(u) for u in range(4)}}


def _passes(order, tasks):
    done = object()
    for item in order.split():
        names, _, turns = item.partition(":")
        running = [(tasks[name], int(count or 1))
                   for name, _, count in (part.partition("*") for part in names.split("+"))]
        turn = 0
        while running and (not turns or turn < int(turns)):
            for task, count in tuple(running):
                for _ in range(count):
                    if next(task, done) is done:
                        running.remove((task, count))
                        break
                    yield
            turn += 1


def _run(*tasks):
    for _ in _chain(*tasks):
        pass


def _emit(order, tasks):
    _run(_passes(order, tasks))


def _chain(*tasks):
    for task in tasks:
        yield from task


def _kernel(xt_hbm, mem0_hbm, wq_hbm, wk_hbm, wv_hbm, wot_hbm, w1_hbm, w3_hbm, w2t_hbm,
            outt_hbm, mem0_ref, io_ref, res_ref, mem_ref, operands_ref, heads_ref, hidden_ref, early_ref, w_ref, qkv_stage, wo_stage,
            ffn_stage, attention_sem, ffn_sem, mem_sem, io_sem, *, seg):
    d_model, n_tok = xt_hbm.shape
    n_mem = mem0_ref.shape[0]
    n_seg = n_tok // seg
    n_io = n_tok // _LANES

    def window(r, n):
        return res_ref.at[pl.ds(pl.multiple_of((r + _LAG) * seg, seg), n * seg)]

    def block(r, n=1):
        return pl.ds(r * seg, n * seg)

    def lanes(i):
        return pl.ds(pl.multiple_of(i * _LANES, _LANES), _LANES)

    def transpose_in(i):
        x = io_ref[i].astype(jnp.float32)
        res_ref[lanes(i + 1), :] = jnp.concatenate([x, x[_TAIL * _LANES:]], axis=0).T

    def transpose_out(i, x):
        io_ref[i] = x.T[:d_model].astype(io_ref.dtype)

    full, short, chunks = 0, n_mem + seg, n_mem + 2 * seg
    full_ref = operands_ref.at[:, pl.ds(full, n_mem + seg)]
    chunk_ref = lambda i: operands_ref.at[:, pl.ds(chunks + 2 * seg * i, 2 * seg)]

    def prepare(ref, first, starts):
        for i, rows in enumerate(starts):
            _store_operands(operands_ref, first + 8 * i,
                            [_layernorm(ref[pl.ds(r, 8), :]) for r in rows])
        yield

    def prepare_full(ref, blocks):
        return prepare(ref, full + n_mem, [[r * seg + i for r in blocks] for i in range(0, seg, 8)])

    def prepare_short(ref, first, second):
        x = [first * seg + i for i in range(seg // 2, seg, 8)] + [(second + 1) * seg - 8]
        if _CARRY:
            for i, r in enumerate(x):
                mem_ref[0, pl.ds(n_mem + 8 * i, 8), :] = _layernorm(ref[pl.ds(r, 8), :])
                mem_ref[1, pl.ds(n_mem + 8 * i, 8), :] = _layernorm(ref[pl.ds(second * seg + 8 * i, 8), :])
                yield
        else:
            yield from prepare(ref, short + n_mem, [[r, second * seg + 8 * i] for i, r in enumerate(x)])

    def prepare_ffn(ref, blocks):
        return prepare(ref, chunks, [[r * seg + i for r in blocks] for i in range(0, 2 * seg, 8)])

    def attention(order, ref, blocks, others, early=None):
        xs, outs = [ref[block(r), :] for r in blocks], []
        for at in range(0, seg if _CARRY and early is not None else n_mem, 8):
            _store_operands(operands_ref, (full if early is None else short) + at,
                            [mem_ref[i, at:at + 8] for i in range(len(blocks))])
        if early is None:
            tasks = _attention_tasks(xs, full_ref, w_ref, heads_ref, outs)
        else:
            rows = pl.ds(pl.multiple_of(early * (seg // 2), seg // 2), seg // 2)
            tasks = _attention_tasks(
                xs, operands_ref.at[:, pl.ds(short, seg)], w_ref, heads_ref, outs,
                lambda u, h: early_ref[u - u // 4, h, rows, :])
        yield from _passes(order, {**others, **tasks})
        for i, r in enumerate(blocks):
            mem_ref[i, :n_mem] = outs[i][:n_mem]
            ref[block(r), :] = outs[i][n_mem:]

    def ffn_tasks(ref, blocks, result=None):
        def update(ys):
            for r, y in zip(blocks, ys):
                ref[block(r, 2), :] = y

        return {"N": prepare_ffn(ref, blocks), **_ffn_tasks(
            [ref[block(r, 2), :] for r in blocks], chunk_ref(0), w_ref, hidden_ref,
            result or update)}

    def double_step(b):
        ref = window(b, _LAG + 2)
        _run(attention(_ORDER_DOUBLE, ref, [_LAG, 0], {"X": prepare_short(ref, _LAG + 1, 1)}, 2 - b))

    def two_steps(j):
        b = 6
        ref = window(2 * j - b, b + _LAG + 3)
        transpose_out(jnp.where((j % 2 == 1) & (j > 1), (j - 3) // 2, n_io - 1), ref[block(0, 4), :])
        ffn = ffn_tasks(ref, [b + 2, b - 2])
        _run(attention(_ORDER_EVEN, ref, [b + _LAG, b],
                       {**ffn, "X": prepare_full(ref, [b + _LAG + 1, b + 1])}, j + _LAG // 2),
             attention(_ORDER_ODD, ref, [b + _LAG + 1, b + 1],
                       {**ffn, "X": prepare_short(ref, b + _LAG + 2, b + 2)}))

    def attention_copies(g, i):
        sem = attention_sem.at[4 * (g % 2) + i]
        if i == 3:
            heads = wot_hbm.bitcast(jnp.uint32).at[pl.ds(_COLUMNS * g, _COLUMNS)]
            return [pltpu.make_async_copy(heads, wo_stage, sem)]
        words = (wq_hbm, wk_hbm, wv_hbm)[i].bitcast(jnp.uint32)
        return [pltpu.make_async_copy(words.at[:, 4 * g + p, :], qkv_stage.at[g % 2, i, p], sem)
                for p in range(4)]

    def ffn_copies(batch, columns=_COLUMNS):
        width = columns * _LANES
        source = pl.ds(pl.multiple_of(batch * _COLUMNS * _LANES, _LANES), width)
        return [pltpu.make_async_copy(w.bitcast(jnp.uint32).at[:, source],
                                      ffn_stage.at[batch % 2, i, :, pl.ds(0, width)],
                                      ffn_sem.at[3 * (batch % 2) + i])
                for i, w in enumerate((w1_hbm, w3_hbm, w2t_hbm))]

    def start(copies):
        for c in copies:
            c.start()

    def wait(copies):
        for c in copies:
            c.wait()

    def lay_out_heads(g, i, u, starts=range(0, _HALF, 16)):
        def source(c, first):
            words = qkv_stage[g % 2, i, c // 2, pl.ds(pl.multiple_of(first, 16), 16), :]
            words = words & jnp.uint32(0xFFFF0000) if c % 2 else words << 16
            return pltpu.bitcast(words, jnp.float32)

        def copy(c, first):
            even, odd = (qkv_stage[g % 2, i, c // 2, pl.ds(first + k, 8, stride=2), :]
                         for k in range(2))
            if c % 2:
                return _unpack((even >> 16) | (odd & jnp.uint32(0xFFFF0000)))
            return _unpack((even & jnp.uint32(0xFFFF)) | (odd << 16))

        return _lay_out(_weight_sums(source, copy, starts), w_ref.at[u])

    def lay_out_rows(words, u, transposed, columns=_COLUMNS):
        rows = _HALF if transposed else _UP_ROWS
        copy = lambda c, first: _unpack(words(c, pl.ds(first // 2, rows // 2)))
        sums = _weight_sums(lambda *at: copy(*at).astype(jnp.float32), copy,
                            range(0, _HALF, rows), columns)
        return (_lay_out_transposed if transposed else _lay_out)(sums, w_ref.at[u])

    def lay_out_up(batch, i):
        return lay_out_rows(
            lambda c, rows: ffn_stage[batch % 2, c // 4, rows, pl.ds((4 * i + c % 4) * _LANES, _LANES)],
            _UP + 2 * batch + i, False)

    def lay_out_down(batch, columns=_COLUMNS):
        return lay_out_rows(
            lambda c, rows: ffn_stage[batch % 2, 2, rows, pl.ds(c * _LANES, _LANES)],
            _DOWN + batch, True, columns)

    def x_copy(i):
        return pltpu.make_async_copy(xt_hbm.at[:, lanes(i)], io_ref.at[i], io_sem.at[i])

    def out_copy(i):
        return pltpu.make_async_copy(io_ref.at[i], outt_hbm.at[:, lanes(i)], io_sem.at[i])

    n_chunks = _EARLY // 8

    def load_group(g):
        def project(i):
            for chunk in range(n_chunks):
                out = {}
                yield from _expand(chunk_ref(chunk), w_ref.at[4 * g + i], out)
                for (r, c), value in out.items():
                    early_ref[3 * g + i, c, pl.ds((2 * chunk + r) * 2 * seg, 2 * seg), :] = value

        def arrive(i):
            if i == 0:
                pl.when(g + 1 < _GROUPS)(lambda: wait(attention_copies(g + 1, 0)))
            else:
                wait(attention_copies(g, i))
            yield

        start(attention_copies(g, 3))
        pl.when(g + 1 < _GROUPS)(
            lambda: start(attention_copies(g + 1, 1) + attention_copies(g + 1, 2)))
        pl.when(g + 2 < _GROUPS)(lambda: start(attention_copies(g + 2, 0)))
        pl.when(g + 2 >= _GROUPS)(lambda: start(ffn_copies(g + 2 - _GROUPS)))
        following = jnp.minimum(g + 1, _GROUPS - 1)
        same = jnp.minimum(g, _GROUPS - 1)
        _emit("W1 " + _ORDER_LOAD, {
            **{f"E{i}": project(i) for i in range(3)}, **{f"W{i}": arrive(i) for i in range(4)},
            "L0": lay_out_heads(following, 0, 4 * following),
            "L1": lay_out_heads(g, 1, 4 * same + 1), "L2": lay_out_heads(g, 2, 4 * same + 2),
            "L3": lay_out_rows(lambda c, rows: wo_stage[c, rows, :], 4 * same + 3, True)})

    def first_step(r):
        ref = window(r, 2)
        wait(ffn_copies(r))
        _emit(_ORDER_FIRST, {
            "P": attention(_ORDER_SINGLE, ref, [0], {"X": prepare_full(ref, [1])}),
            "L": _passes(_ORDER_L, {"U": _chain(lay_out_up(r, 0), lay_out_up(r, 1)),
                                   "D": lay_out_down(r)})})
        pl.when(r + 2 < _LAG)(lambda: start(ffn_copies(r + 2)))
        pl.when(r + 2 == _LAG)(lambda: start(ffn_copies(_LAG, 4)))

    mem_copy = pltpu.make_async_copy(mem0_hbm, mem0_ref, mem_sem.at[0])
    per_chunk = n_io // n_chunks
    start(attention_copies(0, 0) + [x_copy(i) for i in range(per_chunk)] + [mem_copy])
    for spare in (window(-_LAG, _LAG), window(n_seg, 1)):
        spare[...] = jnp.zeros(spare.shape, spare.dtype)
    wait(attention_copies(0, 0))

    @pl.loop(0, n_chunks)
    def _early_operands(chunk):
        tiles = [per_chunk * chunk + i for i in range(per_chunk)]
        pl.when(chunk + 1 < n_chunks)(lambda: start([x_copy(i + per_chunk) for i in tiles]))
        pl.when(chunk == 1)(lambda: start(attention_copies(0, 1)))
        pl.when(chunk == n_chunks - 1)(lambda: start(attention_copies(0, 2)))
        wait([x_copy(i) for i in tiles])
        _run(lay_out_heads(0, 0, 0, starts=[16 * chunk]))
        for i in tiles:
            transpose_in(i)
        segments = [2 * (8 * chunk + e) for e in range(8)]
        segments[1] = jnp.where(chunk == 0, _LAG + 1, segments[1])
        halves = [window(r, 1)[:seg // 2, :] for r in segments]
        _store_operands(operands_ref, pl.multiple_of(chunks + 2 * seg * chunk, 8), [
            _layernorm(jnp.concatenate(part, axis=0)) for part in (halves[:4], halves[4:])])

    start(attention_copies(1, 0))
    pl.loop(0, _GROUPS)(load_group)
    mem_copy.wait()
    mem0 = mem0_ref[...].astype(jnp.float32)
    mem0 = jnp.concatenate([mem0, mem0[:, _TAIL * _LANES:]], axis=1)
    mem_ref[0, :n_mem] = mem_ref[1, :n_mem] = mem0
    whole = window(0, n_seg)
    _run(prepare_full(whole, [0]))
    pl.loop(0, _LAG)(first_step)
    wait(ffn_copies(_LAG, 4))
    _emit(_ORDER_FIRST_FFN, {"P": _passes(_ORDER_FFN, ffn_tasks(whole, [0, 2])),
                             "L": _chain(lay_out_up(_LAG, 0), lay_out_down(_LAG, 4))})
    _run(prepare_short(whole, _LAG, 0))
    pl.loop(0, 2)(double_step)
    last = n_seg - _LAG
    pl.loop(1, last // 2)(two_steps)

    n_done = n_io - 3
    for i in range(n_done):
        out_copy(i).start()
    mem_ref[0, :n_mem] = mem_ref[1, :n_mem]
    ffn = ffn_tasks(whole, [n_seg - 2, last - 2])
    _run(prepare_full(whole, [last]),
         attention(_ORDER_EVEN_SINGLE, whole, [last],
                   {**ffn, "X": prepare_full(whole, [last + 1])}),
         attention(_ORDER_ODD_SINGLE, whole, [last + 1],
                   {**ffn, "X": prepare_full(whole, [last + 2])}))

    @pl.loop(0, 2)
    def _last_steps(i):
        transpose_out(n_done + i, res_ref[lanes(n_done + i + 1), :])
        ref = window(last + 2 + i, 2)
        _run(attention(_ORDER_SINGLE, ref, [0], {"X": prepare_full(ref, [1])}))
        out_copy(n_done + i).start()

    _emit(_ORDER_FFN, ffn_tasks(whole, [last, last + 2],
                                lambda ys: transpose_out(n_io - 1, jnp.concatenate(ys, axis=0))))
    out_copy(n_io - 1).start()
    for i in range(n_io):
        out_copy(i).wait()


@functools.partial(jax.jit, static_argnames=("A_seg_len",))
def pallas_interleave_layers__memory_aug_recurrent_mem_tr__glu_gated_swiglu__prompt_kernel(
    A_x: jax.Array,
    A_mem0: jax.Array,
    A_Wq: jax.Array,
    A_Wk: jax.Array,
    A_Wv: jax.Array,
    A_Wo: jax.Array,
    A_seg_len: int,
    B_x: jax.Array,
    B_w1: jax.Array,
    B_w3: jax.Array,
    B_w2: jax.Array,
):
    del B_x
    _, n_tok, d_model = A_x.shape
    n_mem = A_mem0.shape[1]
    _, n_heads, d_head = A_Wq.shape
    d_ff = B_w1.shape[1]
    seg = A_seg_len
    assert A_x.shape[0] == 1 and _LAG * seg == _LANES and n_mem == 8 and n_tok == 64 * seg
    assert d_model == _TAIL * _LANES + _HALF and d_head == _LANES
    assert n_heads == _GROUPS * _COLUMNS and d_ff == 4 * (_DOWN - _UP) * _LANES
    n_operands = len(_operand_keys(False))
    hbm = pl.BlockSpec(memory_space=pltpu.HBM)
    out_t = pl.pallas_call(
        functools.partial(_kernel, seg=seg),
        out_shape=jax.ShapeDtypeStruct((d_model, n_tok), A_x.dtype),
        in_specs=[hbm] * 9,
        out_specs=hbm,
        scratch_shapes=[
            pltpu.VMEM((n_mem, d_model), A_mem0.dtype),
            pltpu.VMEM((n_tok // _LANES, d_model, _LANES), A_x.dtype),
            pltpu.VMEM((n_tok + (_LAG + 1) * seg, d_model + _HALF), jnp.float32),
            pltpu.VMEM((2, seg, d_model + _HALF), jnp.float32),
            pltpu.VMEM((n_operands, n_mem + 2 * seg + _EARLY * seg // 4, _LANES), jnp.float32),
            pltpu.VMEM((n_heads, 2 * (n_mem + seg), d_head), jnp.float32),
            pltpu.VMEM((d_ff // _LANES, 4 * seg, _LANES), jnp.float32),
            pltpu.VMEM((3 * _GROUPS, _COLUMNS, _EARLY * seg // 2, d_head), jnp.float32),
            pltpu.VMEM((_UNITS, len(_PASSES), _HALF, _LANES), jnp.uint32),
            pltpu.VMEM((2, 3, _COLUMNS // 2, d_model, d_head), jnp.uint32),
            pltpu.VMEM((_COLUMNS, d_model // 2, d_head), jnp.uint32),
            pltpu.VMEM((2, 3, d_model // 2, _COLUMNS * _LANES), jnp.uint32),
            pltpu.SemaphoreType.DMA((8,)),
            pltpu.SemaphoreType.DMA((6,)),
            pltpu.SemaphoreType.DMA((1,)),
            pltpu.SemaphoreType.DMA((n_tok // _LANES,)),
        ],
        compiler_params=pltpu.CompilerParams(vmem_limit_bytes=124 * 1024 * 1024, flags=_FLAGS,
                                             disable_bounds_checks=True),
    )(A_x.reshape(n_tok, d_model).T, A_mem0.reshape(n_mem, d_model), A_Wq, A_Wk, A_Wv,
      A_Wo.transpose(0, 2, 1), B_w1, B_w3, B_w2.T)
    return out_t.T.reshape(A_x.shape)
```

```python
import functools
import math
from typing import NamedTuple

import jax
import jax.numpy as jnp
import jax.experimental.pallas as pl
import jax.experimental.pallas.tpu as pltpu

_EPS = 1e-05
_MASKED = -1000000000.0
_LOG2E = math.log2(math.e)
_LANES = 128
_HALF = _LANES // 2
_TAIL = 4
_COLUMNS = 8
_GROUPS = 4
_UP, _DOWN, _UNITS = 16, 25, 30
_PENDING = 2
_EVEN = (8, 26)
_UP_ROWS = 32
_ORDER_L = "U*2+D"
_SHORT = "bfloat16"
_CHUNK = "bfloat16"
_LAG = 4
_EARLY = 32
_FLAGS = {"XLA_TPU_FORCE_LP_LLO_SCHEDULER": True}
_ORDER_EVEN = "N X Q0 K0 V0 Q1 G0*8+S0 K1 A0 V1 G1*8+S1 O0 Q2 A1 K2 O1 V2 G2*8+S2 Q3 A2 K3 O2 V3 G3*8+S3 G8 A3 D4 O3 G4"
_ORDER_ODD = "Q0 K0 V0*8+S0 G5 A0 G6 Q1 G7 K1 D0 V1*8+S1 D1 A1 D2 Q2 D3 F X K2 V2*8+S2 Q3 A2 K3 V3*8+S3 O0 O1 A3 O2 O3"
_ORDER_EVEN_SINGLE = (
    "Q0 N K0 V0*4+S0 Q1 K1 G0 A0 V1*4+S1 O0 G1 A1 Q2 K2 V2*4+S2 O1 G2 A2 Q3 K3 V3*4+S3 X O2 "
    "G3 A3 G8 O3 D4 G4")
_ORDER_ODD_SINGLE = (
    "Q0 K0 V0*4+S0 G5 A0 Q1 K1 V1*4+S1 G6 A1 Q2 K2 G7 V2*4+S2 D0 A2 Q3 K3 "
    "V3*4+S3 D1 D2 A3 D3 F X O0 O1 O2 O3")
_ORDER_DOUBLE = "Q0 K0 Q1 K1 V0*8+S0 Q2 K2 V1*8+S1 A0 Q3 K3 V2 A1 O0*8+S2 V3 X O1*6+S3 A2 O2:30 A3 O2 O3"
_ORDER_SINGLE = "Q0 K0 V0*4+S0 Q1 K1 A0 V1*4+S1 Q2 K2 A1 V2*4+S2 Q3 K3 A2 V3*4+S3 X O0 O1 A3 O2 O3"
_ORDER_FFN = "N G0 G1 G2 D0 G3 G4 D1 G5 G8 G6 D4 G7 D2 D3 F"
_ORDER_LOAD = "E0+L1*21 W2 W3 E1+L2*21+L3*10:240 E1 L2 W0 E2+L0*21+L3*11"
_ORDER_FIRST = "P:4 P+L*24"
_ORDER_FIRST_FFN = "P:20 P+L*14"


class _Pass(NamedTuple):
    low: tuple
    high: tuple
    w_low: tuple
    w_high: tuple
    wide: tuple
    common: bool = False


def _scheme():
    x, y = 0, 1
    a = lambda d: d
    b = lambda d: 4 + d
    rest = lambda d: [e for e in range(4) if e != d]

    def whole(narrow, weight, wide):
        return _Pass(narrow, narrow, weight, weight, wide)

    def m1(d, e):
        return whole(((1, x, d), (1, y, e)), ((1, b(e), d), (1, a(d), e)),
                     ((1, y, a(d)), (1, x, b(e))))

    def m2(d, e):
        return whole(((1, y, min(d, e)), (1, y, max(d, e))), ((1, b(e), d),),
                     ((1, y, b(e)), (-1, y, a(d))))

    def m3(d):
        return whole(((1, x, d),), ((1, a(d), d), *((-1, a(d), e) for e in rest(d))),
                     ((1, x, a(d)), (1, y, a(d))))

    def m4(d):
        return whole(((1, y, d),), ((1, b(d), d), *((-1, b(d), e) for e in rest(d))),
                     ((1, y, b(d)), (1, x, b(d))))

    def m5(d, e):
        return whole(((1, x, min(d, e)), (1, x, max(d, e))), ((1, a(d), e),),
                     ((1, x, a(d)), (-1, x, b(e))))

    def m6(d):
        return whole(((1, y, d), (-1, x, d)), ((1, a(d), d), *((1, b(e), d) for e in rest(d))),
                     ((1, y, a(d)),))

    def m7(d):
        return whole(((1, y, d), (-1, x, d)), ((-1, b(d), d), *((-1, a(e), d) for e in rest(d))),
                     ((1, x, b(d)),))

    def with_tails(p, p_rows, p_columns, q, q_rows, q_columns):
        tail = lambda columns: tuple((1, c, _TAIL) for c in columns)
        return [
            _Pass(p.low, p.high, q.w_low, p.w_high, p.wide + q.wide, common=True),
            _Pass(p.low, ((1, p_rows, _TAIL),), p.w_low, tail(p_columns), p.wide),
            _Pass(((1, q_rows, _TAIL),), q.high, tail(q_columns), q.w_high, q.wide)]

    def near(d, e):
        return [*with_tails(m5(d, e), x, [a(d)], m5(e, d), x, [a(e)]), m3(d),
                *with_tails(m2(d, e), y, [b(e)], m2(e, d), y, [b(d)]), m3(e),
                *with_tails(m6(d), y, [a(d), b(e)], m7(d), x, [b(d), a(e)]), m1(d, e),
                *with_tails(m7(e), x, [b(e), a(d)], m6(e), y, [a(e), b(d)]), m1(e, d)]

    far = lambda d, e: [m5(d, e), m1(d, e), m2(d, e)]
    return (*near(0, 1), *far(0, 2), *far(0, 3), *far(1, 2), *far(1, 3),
            m4(2), m4(3), *near(2, 3),
            m4(0), *far(2, 0), *far(3, 0), m4(1), *far(2, 1), *far(3, 1))


_PASSES = _scheme()


def _selected(single, columns=_COLUMNS):
    for i, p in enumerate(_PASSES):
        if single:
            p = p._replace(
                wide=tuple((s, 0, c) for s, r, c in p.wide if r == c // 4 and c < columns),
                low=tuple((s, 0, d) for s, _, d in p.low),
                high=tuple((s, 0, d) for s, _, d in p.high))
        if p.wide:
            yield i, p


def _operand_keys(single):
    return tuple(dict.fromkeys((p.low, p.high) for _, p in _selected(single)))


def _signed_sum(terms):
    terms = sorted(terms, key=lambda t: -t[0])
    total = terms[0][1] if terms[0][0] > 0 else -terms[0][1]
    for sign, value in terms[1:]:
        total = total + value if sign > 0 else total - value
    return total


def _accumulate(sums, key, sign, value):
    if key not in sums:
        sums[key] = (sign, value)
    elif sums[key][0] == sign:
        sums[key] = (sign, sums[key][1] + value)
    else:
        sums[key] = (1, value - sums[key][1] if sign > 0 else sums[key][1] - value)


def _unpack(words):
    return pltpu.bitcast(words, jnp.bfloat16)


def _load(ref, i):
    return _unpack(ref.bitcast(jnp.uint32)[i]) if ref.dtype == jnp.bfloat16 else ref[i]


def _store(ref, i, first, value):
    rows = value.shape[0]
    if value.dtype == jnp.bfloat16:
        ref.bitcast(jnp.uint32)[i, pl.ds(first // 2, rows // 2), :] = pltpu.bitcast(value, jnp.uint32)
    else:
        ref[i, pl.ds(first, rows), :] = value.astype(ref.dtype)


def _low_lanes(rows):
    return jax.lax.broadcasted_iota(jnp.int32, (rows, _LANES), 1) < _HALF


def _blocks(x):
    return [x[:, d * _LANES:(d + 1) * _LANES] for d in range(_TAIL + 1)]


def _store_operands(ref, first, row_blocks):
    blocks = [_blocks(x) for x in row_blocks]
    rows = row_blocks[0].shape[0]
    low_lanes = _low_lanes(rows)
    total = functools.cache(lambda terms: _signed_sum([(s, blocks[r][d]) for s, r, d in terms]))
    for i, (low, high) in enumerate(_operand_keys(len(row_blocks) == 1)):
        _store(ref, i, first,
               total(low) if low == high else jnp.where(low_lanes, total(low), total(high)))


def _dot(a, b):
    return jnp.dot(a, b, preferred_element_type=jnp.float32)


def _expand(operands_ref, tiles_ref, out, single=False):
    keys = _operand_keys(single)
    sums, common = {}, []
    for i, p in _selected(single):
        product = _dot(_load(operands_ref, keys.index((p.low, p.high))), _load(tiles_ref, i))
        if p.common:
            common = [product, product]
        else:
            if common:
                product = product + common.pop()
            for s, r, c in p.wide:
                _accumulate(sums, (r, c), s, product)
        yield
    assert all(sign > 0 for sign, _ in sums.values())
    out.update({key: value for key, (_, value) in sums.items()})


def _contract(load, tiles_ref, sums, single=False, columns=_COLUMNS):
    held = []
    for i, p in _selected(single, columns):
        product = _dot(_signed_sum([(s, load(r, c)) for s, r, c in p.wide]),
                       _load(tiles_ref, i))
        if p.common or held:
            held.append((p, product))
        if len(held) == 3:
            (p, common), (p1, first), (p2, second) = held
            held = []
            product = common + jnp.where(_low_lanes(common.shape[0]), first, second)
            _accumulate(sums, (p1.high[0][1], _TAIL, 1), 1, first)
            _accumulate(sums, (p2.low[0][1], _TAIL, 0), 1, second)
        if not held:
            for s, r, d in p.low:
                _accumulate(sums, (r, d), s, product)
        yield


def _residual(row_blocks):
    return {(r, d) if d < _TAIL else (r, d, 0): (1, block)
            for r, x in enumerate(row_blocks) for d, block in enumerate(_blocks(x))}


def _contracted(sums, r):
    assert all(sign > 0 for sign, _ in sums.values())
    low, high = sums[r, _TAIL, 0][1], sums[r, _TAIL, 1][1]
    tail = jnp.where(_low_lanes(low.shape[0]), low, high)
    tail = tail + pltpu.roll(tail, _HALF, 1)
    return jnp.concatenate([sums[r, d][1] for d in range(_TAIL)] + [tail], axis=1)


def _weight_sums(source, copy, starts, columns=_COLUMNS):
    chosen = list(_selected(columns < _COLUMNS, columns))
    for n, (i, p) in enumerate(chosen):
        for high in range(2):
            if n > high and chosen[n - 1 - high][1].common:
                continue
            for at in starts:
                first = lambda d: d * _LANES + at + (0 if d == _TAIL else high * _HALF)
                total = lambda terms: _signed_sum([(s, source(c, first(d))) for s, c, d in terms])
                terms = (p.w_low, p.w_high)[high]
                if len(terms) == 1:
                    yield i, high * _HALF + at, copy(terms[0][1], first(terms[0][2])), 0
                else:
                    value = total(terms)
                    yield i, high * _HALF + at, value, len(terms)
                if p.common:
                    k, other = chosen[n + 1 + high]
                    value = value if len(terms) > 1 else total(terms)
                    yield (k, high * _HALF + at, total((other.w_low, other.w_high)[high]) - value,
                           len(terms) + 1)


def _lay_out(sums, tiles_ref):
    for i, first, value, terms in sums:
        _store(tiles_ref, i, pl.multiple_of(first, 16), value)
        yield from range((4 * terms + 3) * value.shape[0] // 16)


def _lay_out_transposed(sums, tiles_ref):
    halves, pending = {}, []
    for i, first, value, terms in sums:
        halves[i, first] = value
        if (i, _HALF - first) in halves:
            pair = [halves[i, 0], halves[i, _HALF]]
            if pair[0].dtype != pair[1].dtype:
                pair = [half.astype(jnp.float32) for half in pair]
            pending.append((i, jnp.concatenate(pair, axis=0).astype(jnp.bfloat16).T))
        if len(pending) > _PENDING:
            k, tile = pending.pop(0)
            _store(tiles_ref, k, 0, tile)
        yield from range(_EVEN[0] * terms + _EVEN[1])
    for k, tile in pending:
        _store(tiles_ref, k, 0, tile)


def _layernorm(x):
    low_lanes = _low_lanes(x.shape[0])

    def mean(v):
        *full, tail = _blocks(v)
        total = functools.reduce(jnp.add, full) + jnp.where(low_lanes, tail, 0.0)
        return jnp.sum(total, axis=-1, keepdims=True) / (_TAIL * _LANES + _HALF)

    d = x - mean(x)
    return d * jax.lax.rsqrt(mean(d * d) + _EPS)


def _silu(x):
    half = 0.5 * x
    return half + half * jnp.tanh(half)


def _reciprocal(x):
    r = pl.reciprocal(x, approx=True)
    return r * (2.0 - x * r)


def _attention_masks(n_layers, rows, n_mem):
    i = jax.lax.broadcasted_iota(jnp.int32, (n_layers * rows, n_layers * rows), 0)
    j = jax.lax.broadcasted_iota(jnp.int32, (n_layers * rows, n_layers * rows), 1)
    if n_layers == 1:
        return (i < n_mem) | (i >= j), _MASKED * _LOG2E
    same = (i >= rows) == (j >= rows)
    visible = (i < n_mem) | ((i >= rows) & (i < rows + n_mem)) | (i >= j)
    fill = jnp.where(same, _MASKED * _LOG2E, -jnp.inf).astype(jnp.float32)
    return same & visible, fill


def _attention_tasks(xs, operands_ref, w_ref, heads_ref, outs, known=None):
    n_layers, rows = len(xs), heads_ref.shape[1] // 2
    single, n_mem = n_layers == 1, rows - xs[0].shape[0]
    visible, fill = _attention_masks(n_layers, rows, n_mem)
    scale = _LANES ** -0.5 * _LOG2E
    qkv, probs = {}, {}
    sums = _residual([jnp.concatenate([jnp.zeros_like(x[:n_mem]), x], axis=0) for x in xs])

    def stacked(u, h, streamed=False):
        parts = [qkv[u][r, h] for r in range(n_layers)]
        if known:
            (x, y), moved = parts, (rows + n_mem) // 2
            parts = [x[:n_mem], known(u, h), x[n_mem:moved], y, x[moved:]]
        value = jnp.concatenate(parts, axis=0)
        return value if single and streamed else value.astype(jnp.bfloat16)

    def project(u):
        qkv[u] = {}
        yield from _expand(operands_ref, w_ref.at[u], qkv[u], single)

    def scores(g):
        for h in range(_COLUMNS):
            s = jax.lax.dot_general(stacked(4 * g, h, True), stacked(4 * g + 1, h),
                                    (((1,), (1,)), ((), ())), preferred_element_type=jnp.float32)
            s = jnp.where(visible, s * scale, fill)
            p = jnp.exp2(s - jnp.max(s, axis=-1, keepdims=True))
            p = p * _reciprocal(jnp.sum(p, axis=-1, keepdims=True))
            probs[g, h] = p if single else p.astype(jnp.bfloat16)
            yield

    def values(g):
        for h in range(_COLUMNS):
            heads_ref[_COLUMNS * g + h, :n_layers * rows, :] = _dot(
                probs[g, h], stacked(4 * g + 2, h))
            yield

    def output(g):
        yield from _contract(lambda r, h: heads_ref[_COLUMNS * g + h, r * rows:(r + 1) * rows, :],
                             w_ref.at[4 * g + 3], sums, single)
        if g == _GROUPS - 1:
            outs.extend(_contracted(sums, r) for r in range(n_layers))

    tasks = {}
    for g in range(_GROUPS):
        tasks.update({f"Q{g}": project(4 * g), f"K{g}": project(4 * g + 1),
                      f"V{g}": project(4 * g + 2), f"S{g}": scores(g), f"A{g}": values(g),
                      f"O{g}": output(g)})
    return tasks


def _ffn_tasks(xs, operands_ref, w_ref, hidden_ref, result):
    rows = operands_ref.shape[1]
    sums = _residual(xs)

    def gated(u):
        both = {}
        yield from _expand(operands_ref, w_ref.at[_UP + u], both)
        for c in range(4):
            for r in range(2):
                hidden_ref[4 * u + c, r * rows:(r + 1) * rows, :] = (
                    _silu(both[r, c]) * both[r, 4 + c])

    def down(u):
        yield from _contract(lambda r, c: hidden_ref[_COLUMNS * u + c, r * rows:(r + 1) * rows, :],
                             w_ref.at[_DOWN + u], sums)

    def down_rest(u):
        rest = {}
        yield from _contract(lambda r, c: hidden_ref[_COLUMNS * u + c], w_ref.at[_DOWN + u], rest,
                             single=True, columns=4)
        for (_, *key), (sign, value) in rest.items():
            for r in range(2):
                _accumulate(sums, (r, *key), sign, value[r * rows:(r + 1) * rows])

    def finish():
        result([_contracted(sums, r) for r in range(2)])
        yield

    return {"F": finish(), "D4": down_rest(4),
            **{f"G{u}": gated(u) for u in range(_DOWN - _UP)},
            **{f"D{u}": down(u) for u in range(4)}}


def _passes(order, tasks):
    done = object()
    for item in order.split():
        names, _, turns = item.partition(":")
        running = [(tasks[name], int(count or 1))
                   for name, _, count in (part.partition("*") for part in names.split("+"))]
        turn = 0
        while running and (not turns or turn < int(turns)):
            for task, count in tuple(running):
                for _ in range(count):
                    if next(task, done) is done:
                        running.remove((task, count))
                        break
                    yield
            turn += 1


def _run(*tasks):
    for _ in _chain(*tasks):
        pass


def _emit(order, tasks):
    _run(_passes(order, tasks))


def _chain(*tasks):
    for task in tasks:
        yield from task


def _kernel(xt_hbm, mem0_hbm, wq_hbm, wk_hbm, wv_hbm, wot_hbm, w1_hbm, w3_hbm, w2t_hbm,
            outt_hbm, mem0_ref, io_ref, res_ref, mem_ref, full_ref, short_ref, chunks_ref, heads_ref, hidden_ref, early_ref, w_ref, x_stage, qkv_stage, wo_stage,
            ffn_stage, x_sem, attention_sem, ffn_sem, mem_sem, io_sem, *, seg):
    d_model, n_tok = xt_hbm.shape
    n_mem = mem0_hbm.shape[0]
    n_seg = n_tok // seg
    n_io = n_tok // _LANES

    def window(r, n):
        return res_ref.at[pl.ds(pl.multiple_of((r + _LAG) * seg, seg), n * seg)]

    def block(r, n=1):
        return pl.ds(r * seg, n * seg)

    def lanes(i):
        return pl.ds(pl.multiple_of(i * _LANES, _LANES), _LANES)

    def transpose_out(i, x):
        io_ref[i] = x.T[:d_model].astype(io_ref.dtype)

    def prepare(ref, operands_ref, first, starts, rows=8):
        for i, pair in enumerate(starts):
            _store_operands(operands_ref, first + rows * i,
                            [_layernorm(ref[pl.ds(r, rows), :]) for r in pair])
        yield

    def prepare_full(ref, blocks):
        return prepare(ref, full_ref, n_mem,
                       [[r * seg + i for r in blocks] for i in range(0, seg, 8)])

    def prepare_short(ref, first, second):
        x = _layernorm(ref[pl.ds(first * seg + seg // 2, seg // 2), :])
        y = _layernorm(ref[block(second), :])
        mem_ref[0, n_mem:] = jnp.concatenate([x, y[seg - n_mem:]], axis=0)
        mem_ref[1, n_mem:] = y[:seg - n_mem]
        yield

    def prepare_ffn(ref, blocks):
        return prepare(ref, chunks_ref.at[0], 0,
                       [[r * seg + i for r in blocks] for i in range(0, 2 * seg, 16)], 16)

    def attention(order, ref, blocks, others, early=None):
        xs, outs = [ref[block(r), :] for r in blocks], []
        operands_ref = full_ref if early is None else short_ref
        _store_operands(operands_ref, 0, [
            mem_ref[i, :n_mem if early is None else seg] for i in range(len(blocks))])
        known = None if early is None else lambda u, h: early_ref[early, u - u // 4, h]
        tasks = _attention_tasks(xs, operands_ref, w_ref, heads_ref, outs, known)
        yield from _passes(order, {**others, **tasks})
        for i, r in enumerate(blocks):
            mem_ref[i, :n_mem] = outs[i][:n_mem]
            ref[block(r), :] = outs[i][n_mem:]

    def ffn_tasks(ref, blocks, result=None):
        def update(ys):
            for r, y in zip(blocks, ys):
                ref[block(r, 2), :] = y

        return {"N": prepare_ffn(ref, blocks), **_ffn_tasks(
            [ref[block(r, 2), :] for r in blocks], chunks_ref.at[0], w_ref, hidden_ref,
            result or update)}

    def double_step(b):
        ref = window(b, _LAG + 2)
        _run(attention(_ORDER_DOUBLE, ref, [_LAG, 0], {"X": prepare_short(ref, _LAG + 1, 1)}, 2 - b))

    def two_steps(j):
        b = 6
        ref = window(2 * j - b, b + _LAG + 3)
        transpose_out(jnp.where((j % 2 == 1) & (j > 1), (j - 3) // 2, n_io - 1), ref[block(0, 4), :])
        ffn = ffn_tasks(ref, [b + 2, b - 2])
        _run(attention(_ORDER_EVEN, ref, [b + _LAG, b],
                       {**ffn, "X": prepare_full(ref, [b + _LAG + 1, b + 1])}, j + _LAG // 2),
             attention(_ORDER_ODD, ref, [b + _LAG + 1, b + 1],
                       {**ffn, "X": prepare_short(ref, b + _LAG + 2, b + 2)}))

    def attention_copies(g, i):
        sem = attention_sem.at[4 * (g % 2) + i]
        if i == 3:
            heads = wot_hbm.bitcast(jnp.uint32).at[pl.ds(_COLUMNS * g, _COLUMNS)]
            return [pltpu.make_async_copy(heads, wo_stage, sem)]
        words = (wq_hbm, wk_hbm, wv_hbm)[i].bitcast(jnp.uint32)
        return [pltpu.make_async_copy(words.at[:, 4 * g + p, :], qkv_stage.at[g % 2, i, p], sem)
                for p in range(4)]

    def ffn_copies(batch, columns=_COLUMNS):
        width = columns * _LANES
        source = pl.ds(pl.multiple_of(batch * _COLUMNS * _LANES, _LANES), width)
        return [pltpu.make_async_copy(w.bitcast(jnp.uint32).at[:, source],
                                      ffn_stage.at[batch % 2, i, :, pl.ds(0, width)],
                                      ffn_sem.at[3 * (batch % 2) + i])
                for i, w in enumerate((w1_hbm, w3_hbm, w2t_hbm))]

    def start(copies):
        for c in copies:
            c.start()

    def wait(copies):
        for c in copies:
            c.wait()

    def lay_out_heads(g, i, u, starts=range(0, _HALF, 16)):
        def source(c, first):
            words = qkv_stage[g % 2, i, c // 2, pl.ds(pl.multiple_of(first, 16), 16), :]
            words = words & jnp.uint32(0xFFFF0000) if c % 2 else words << 16
            return pltpu.bitcast(words, jnp.float32)

        return _lay_out(_weight_sums(source, source, starts), w_ref.at[u])

    def lay_out_rows(words, u, transposed, columns=_COLUMNS):
        rows = _HALF if transposed else _UP_ROWS
        copy = lambda c, first: _unpack(words(c, pl.ds(first // 2, rows // 2)))
        sums = _weight_sums(lambda *at: copy(*at).astype(jnp.float32), copy,
                            range(0, _HALF, rows), columns)
        return (_lay_out_transposed if transposed else _lay_out)(sums, w_ref.at[u])

    def lay_out_up(batch, i):
        return lay_out_rows(
            lambda c, rows: ffn_stage[batch % 2, c // 4, rows, pl.ds((4 * i + c % 4) * _LANES, _LANES)],
            _UP + 2 * batch + i, False)

    def lay_out_down(batch, columns=_COLUMNS):
        return lay_out_rows(
            lambda c, rows: ffn_stage[batch % 2, 2, rows, pl.ds(c * _LANES, _LANES)],
            _DOWN + batch, True, columns)

    def x_copy(chunk):
        width = x_stage.shape[2]
        columns = pl.ds(pl.multiple_of(chunk * width, width), width)
        return pltpu.make_async_copy(xt_hbm.at[:, columns], x_stage.at[chunk], x_sem.at[chunk])

    def out_copy(i):
        return pltpu.make_async_copy(io_ref.at[i], outt_hbm.at[:, lanes(i)], io_sem.at[i])

    n_chunks = _EARLY // 8

    def load_group(g):
        def project(i):
            for chunk in range(n_chunks):
                out = {}
                yield from _expand(chunks_ref.at[chunk], w_ref.at[4 * g + i], out)
                for (r, c), value in out.items():
                    for e in range(4):
                        early_ref[8 * chunk + 4 * r + e, 3 * g + i, c] = (
                            value[e * seg // 2:(e + 1) * seg // 2])

        def arrive(i):
            if i == 0:
                pl.when(g + 1 < _GROUPS)(lambda: wait(attention_copies(g + 1, 0)))
            else:
                wait(attention_copies(g, i))
            yield

        start(attention_copies(g, 3))
        pl.when(g + 1 < _GROUPS)(
            lambda: start([c for i in range(3) for c in attention_copies(g + 1, i)]))
        pl.when(g + 2 >= _GROUPS)(lambda: start(ffn_copies(g + 2 - _GROUPS)))
        following = jnp.minimum(g + 1, _GROUPS - 1)
        same = jnp.minimum(g, _GROUPS - 1)
        _emit("W1 " + _ORDER_LOAD, {
            **{f"E{i}": project(i) for i in range(3)}, **{f"W{i}": arrive(i) for i in range(4)},
            "L0": lay_out_heads(following, 0, 4 * following),
            "L1": lay_out_heads(g, 1, 4 * same + 1), "L2": lay_out_heads(g, 2, 4 * same + 2),
            "L3": lay_out_rows(lambda c, rows: wo_stage[c, rows, :], 4 * same + 3, True)})

    def first_step(r):
        ref = window(r, 2)
        wait(ffn_copies(r))
        _emit(_ORDER_FIRST, {
            "P": attention(_ORDER_SINGLE, ref, [0], {"X": prepare_full(ref, [1])}),
            "L": _passes(_ORDER_L, {"U": _chain(lay_out_up(r, 0), lay_out_up(r, 1)),
                                   "D": lay_out_down(r)})})
        pl.when(r + 2 < _LAG)(lambda: start(ffn_copies(r + 2)))
        pl.when(r + 2 == _LAG)(lambda: start(ffn_copies(_LAG, 4)))

    mem_copy = pltpu.make_async_copy(mem0_hbm, mem0_ref.at[0], mem_sem.at[0])
    start([x_copy(0)] + attention_copies(0, 0))
    for spare in (window(-_LAG, _LAG), window(n_seg, 1)):
        spare[...] = jnp.zeros(spare.shape, spare.dtype)
    wait(attention_copies(0, 0)[:2])
    x_copy(1).start()
    wait(attention_copies(0, 0)[2:])
    start([x_copy(i) for i in range(2, n_chunks)])

    @pl.loop(0, n_chunks)
    def _early_operands(chunk):
        pl.when(chunk == 1)(lambda: start(attention_copies(0, 1) + [mem_copy]))
        pl.when(chunk == 2)(lambda: start(attention_copies(0, 2)))
        wait([x_copy(chunk)])
        _run(lay_out_heads(0, 0, 0, starts=[16 * chunk]))
        x = x_stage[chunk].astype(jnp.float32)
        x = jnp.concatenate([x, x[_TAIL * _LANES:]], axis=0).T
        window(n_seg // n_chunks * chunk, n_seg // n_chunks)[...] = x
        halves = [x[2 * e * seg:2 * e * seg + seg // 2] for e in range(8)]
        halves[1] = jnp.where(chunk == 0, x[(_LAG + 1) * seg:(_LAG + 1) * seg + seg // 2], halves[1])
        _store_operands(chunks_ref.at[chunk], 0, [
            _layernorm(jnp.concatenate(part, axis=0)) for part in (halves[:4], halves[4:])])

    pl.loop(0, _GROUPS)(load_group)
    mem_copy.wait()
    mem0 = mem0_ref[0].astype(jnp.float32)
    mem0 = jnp.concatenate([mem0, mem0[:, _TAIL * _LANES:]], axis=1)
    mem_ref[0, :n_mem] = mem_ref[1, :n_mem] = mem0
    whole = window(0, n_seg)
    _run(prepare_full(whole, [0]))
    pl.loop(0, _LAG)(first_step)
    wait(ffn_copies(_LAG, 4))
    _emit(_ORDER_FIRST_FFN, {"P": _passes(_ORDER_FFN, ffn_tasks(whole, [0, 2])),
                             "L": _chain(lay_out_up(_LAG, 0), lay_out_down(_LAG, 4))})
    _run(prepare_short(whole, _LAG, 0))
    pl.loop(0, 2)(double_step)
    last = n_seg - _LAG
    pl.loop(1, last // 2)(two_steps)

    n_done = n_io - 3
    for i in range(n_done):
        out_copy(i).start()
    mem_ref[0, :n_mem] = mem_ref[1, :n_mem]
    ffn = ffn_tasks(whole, [n_seg - 2, last - 2])
    _run(prepare_full(whole, [last]),
         attention(_ORDER_EVEN_SINGLE, whole, [last],
                   {**ffn, "X": prepare_full(whole, [last + 1])}),
         attention(_ORDER_ODD_SINGLE, whole, [last + 1],
                   {**ffn, "X": prepare_full(whole, [last + 2])}))

    @pl.loop(0, 2)
    def _last_steps(i):
        transpose_out(n_done + i, res_ref[lanes(n_done + i + 1), :])
        ref = window(last + 2 + i, 2)
        _run(attention(_ORDER_SINGLE, ref, [0], {"X": prepare_full(ref, [1])}))
        out_copy(n_done + i).start()

    _emit(_ORDER_FFN, ffn_tasks(whole, [last, last + 2],
                                lambda ys: transpose_out(n_io - 1, jnp.concatenate(ys, axis=0))))
    out_copy(n_io - 1).start()
    for i in range(n_io):
        out_copy(i).wait()


@functools.partial(jax.jit, static_argnames=("A_seg_len",))
def pallas_interleave_layers__memory_aug_recurrent_mem_tr__glu_gated_swiglu__prompt_kernel(
    A_x: jax.Array,
    A_mem0: jax.Array,
    A_Wq: jax.Array,
    A_Wk: jax.Array,
    A_Wv: jax.Array,
    A_Wo: jax.Array,
    A_seg_len: int,
    B_x: jax.Array,
    B_w1: jax.Array,
    B_w3: jax.Array,
    B_w2: jax.Array,
):
    del B_x
    _, n_tok, d_model = A_x.shape
    n_mem = A_mem0.shape[1]
    _, n_heads, d_head = A_Wq.shape
    d_ff = B_w1.shape[1]
    seg = A_seg_len
    assert A_x.shape[0] == 1 and _LAG * seg == _LANES and n_mem == 8 and n_tok == 64 * seg
    assert d_model == _TAIL * _LANES + _HALF and d_head == _LANES
    assert n_heads == _GROUPS * _COLUMNS and d_ff == 4 * (_DOWN - _UP) * _LANES
    n_operands = len(_operand_keys(False))
    hbm = pl.BlockSpec(memory_space=pltpu.HBM)
    out_t = pl.pallas_call(
        functools.partial(_kernel, seg=seg),
        out_shape=jax.ShapeDtypeStruct((d_model, n_tok), A_x.dtype),
        in_specs=[hbm] * 9,
        out_specs=hbm,
        scratch_shapes=[
            pltpu.VMEM((2, n_mem, d_model), A_mem0.dtype),
            pltpu.VMEM((n_tok // _LANES, d_model, _LANES), A_x.dtype),
            pltpu.VMEM((n_tok + (_LAG + 1) * seg, d_model + _HALF), jnp.float32),
            pltpu.VMEM((2, seg, d_model + _HALF), jnp.float32),
            pltpu.VMEM((n_operands, n_mem + seg, _LANES), jnp.float32),
            pltpu.VMEM((n_operands, seg, _LANES), jnp.dtype(_SHORT)),
            pltpu.VMEM((_EARLY // 8, n_operands, 2 * seg, _LANES), jnp.dtype(_CHUNK)),
            pltpu.VMEM((n_heads, 2 * (n_mem + seg), d_head), jnp.float32),
            pltpu.VMEM((d_ff // _LANES, 4 * seg, _LANES), jnp.float32),
            pltpu.VMEM((_EARLY, 3 * _GROUPS, _COLUMNS, seg // 2, d_head), jnp.float32),
            pltpu.VMEM((_UNITS, len(_PASSES), _LANES, _LANES), jnp.bfloat16),
            pltpu.VMEM((_EARLY // 8, d_model, 8 * n_tok // _EARLY), A_x.dtype),
            pltpu.VMEM((2, 3, _COLUMNS // 2, d_model, d_head), jnp.uint32),
            pltpu.VMEM((_COLUMNS, d_model // 2, d_head), jnp.uint32),
            pltpu.VMEM((2, 3, d_model // 2, _COLUMNS * _LANES), jnp.uint32),
            pltpu.SemaphoreType.DMA((_EARLY // 8,)),
            pltpu.SemaphoreType.DMA((8,)),
            pltpu.SemaphoreType.DMA((6,)),
            pltpu.SemaphoreType.DMA((1,)),
            pltpu.SemaphoreType.DMA((n_tok // _LANES,)),
        ],
        compiler_params=pltpu.CompilerParams(vmem_limit_bytes=124 * 1024 * 1024, flags=_FLAGS,
                                             disable_bounds_checks=True),
    )(A_x.reshape(n_tok, d_model).T, A_mem0.reshape(n_mem, d_model), A_Wq, A_Wk, A_Wv,
      A_Wo.transpose(0, 2, 1), B_w1, B_w3, B_w2.T)
    return out_t.T.reshape(A_x.shape)
```

```python
import functools
import math
from typing import NamedTuple

import jax
import jax.numpy as jnp
import jax.experimental.pallas as pl
import jax.experimental.pallas.tpu as pltpu

_EPS = 1e-05
_MASKED = -1000000000.0
_LOG2E = math.log2(math.e)
_LANES = 128
_HALF = _LANES // 2
_TAIL = 4
_COLUMNS = 8
_GROUPS = 4
_UP, _DOWN, _UNITS = 16, 25, 30
_PENDING = 2
_EVEN = (8, 26)
_UP_ROWS = 32
_ORDER_L = "U*2+D"
_SHORT = "bfloat16"
_CHUNK = "bfloat16"
_LAG = 4
_EARLY = 32
_FLAGS = {"XLA_TPU_FORCE_LP_LLO_SCHEDULER": True}
_ORDER_EVEN = "N X Q0 K0 V0 Q1 G0*8+S0 K1 A0 V1 G1*8+S1 O0 Q2 A1 K2 O1 V2 G2*8+S2 Q3 A2 K3 O2 V3 G3*8+S3 G8 A3 D4 O3 G4"
_ORDER_ODD = "Q0 K0 V0*8+S0 G5 A0 G6 Q1 G7 K1 D0 V1*8+S1 D1 A1 D2 Q2 D3 F X K2 V2*8+S2 Q3 A2 K3 V3*8+S3 O0 O1 A3 O2 O3"
_ORDER_EVEN_SINGLE = (
    "Q0 N K0 V0*4+S0 Q1 K1 G0 A0 V1*4+S1 O0 G1 A1 Q2 K2 V2*4+S2 O1 G2 A2 Q3 K3 V3*4+S3 X O2 "
    "G3 A3 G8 O3 D4 G4")
_ORDER_ODD_SINGLE = (
    "Q0 K0 V0*4+S0 G5 A0 Q1 K1 V1*4+S1 G6 A1 Q2 K2 G7 V2*4+S2 D0 A2 Q3 K3 "
    "V3*4+S3 D1 D2 A3 D3 F X O0 O1 O2 O3")
_ORDER_DOUBLE = "Q0 K0 Q1 K1 V0*8+S0 Q2 K2 V1*8+S1 A0 Q3 K3 V2 A1 O0*8+S2 V3 X O1*6+S3 A2 O2:30 A3 O2 O3"
_ORDER_SINGLE = "Q0 K0 V0*4+S0 Q1 K1 A0 V1*4+S1 Q2 K2 A1 V2*4+S2 Q3 K3 A2 V3*4+S3 X O0 O1 A3 O2 O3"
_ORDER_FFN = "N G0 G1 G2 D0 G3 G4 D1 G5 G6 G8 G7 D2 D4 D3 F"
_ORDER_LOAD = "E0+L1*21 W2 W3 E1+L2*21+L3*10:240 E1 L2 W0 E2+L0*21+L3*11"
_ORDER_FIRST = "P:4 P+L*24"
_ORDER_FIRST_FFN = "P:20 P+L*15"


class _Pass(NamedTuple):
    low: tuple
    high: tuple
    w_low: tuple
    w_high: tuple
    wide: tuple
    common: bool = False


def _scheme(columns):
    x, y, n = 0, 1, columns // 2
    a = lambda d: d % n
    b = lambda d: n + d % n
    rest = lambda d: [e for e in range(4) if e != d and e // n == d // n]

    def whole(narrow, weight, wide):
        return _Pass(narrow, narrow, weight, weight, wide)

    def m1(d, e):
        return whole(((1, x, d), (1, y, e)), ((1, b(e), d), (1, a(d), e)),
                     ((1, y, a(d)), (1, x, b(e))))

    def m2(d, e):
        return whole(((1, y, min(d, e)), (1, y, max(d, e))), ((1, b(e), d),),
                     ((1, y, b(e)), (-1, y, a(d))))

    def m3(d):
        return whole(((1, x, d),), ((1, a(d), d), *((-1, a(d), e) for e in rest(d))),
                     ((1, x, a(d)), (1, y, a(d))))

    def m4(d):
        return whole(((1, y, d),), ((1, b(d), d), *((-1, b(d), e) for e in rest(d))),
                     ((1, y, b(d)), (1, x, b(d))))

    def m5(d, e):
        return whole(((1, x, min(d, e)), (1, x, max(d, e))), ((1, a(d), e),),
                     ((1, x, a(d)), (-1, x, b(e))))

    def m6(d):
        return whole(((1, y, d), (-1, x, d)), ((1, a(d), d), *((1, b(e), d) for e in rest(d))),
                     ((1, y, a(d)),))

    def m7(d):
        return whole(((1, y, d), (-1, x, d)), ((-1, b(d), d), *((-1, a(e), d) for e in rest(d))),
                     ((1, x, b(d)),))

    def with_tails(p, p_rows, p_columns, q, q_rows, q_columns):
        tail = lambda columns: tuple((1, c, _TAIL) for c in columns)
        return [
            _Pass(p.low, p.high, q.w_low, p.w_high, p.wide + q.wide, common=True),
            _Pass(p.low, ((1, p_rows, _TAIL),), p.w_low, tail(p_columns), p.wide),
            _Pass(((1, q_rows, _TAIL),), q.high, tail(q_columns), q.w_high, q.wide)]

    def near(d, e):
        return [*with_tails(m5(d, e), x, [a(d)], m5(e, d), x, [a(e)]), m3(d),
                *with_tails(m2(d, e), y, [b(e)], m2(e, d), y, [b(d)]), m3(e),
                *with_tails(m6(d), y, [a(d), b(e)], m7(d), x, [b(d), a(e)]), m1(d, e),
                *with_tails(m7(e), x, [b(e), a(d)], m6(e), y, [a(e), b(d)]), m1(e, d)]

    far = lambda d, e: [m5(d, e), m1(d, e), m2(d, e)]
    if columns < _COLUMNS:
        return (*near(0, 1), m4(0), m4(1), *far(2, 3), *far(3, 2),
                *(m(d) for d in (2, 3) for m in (m3, m4, m6, m7)))
    return (*near(0, 1), *far(0, 2), *far(0, 3), *far(1, 2), *far(1, 3),
            m4(2), m4(3), *near(2, 3),
            m4(0), *far(2, 0), *far(3, 0), m4(1), *far(2, 1), *far(3, 1))


def _selected(single, columns=_COLUMNS):
    for i, p in enumerate(_scheme(columns)):
        if single:
            p = p._replace(wide=tuple((s, 0, c) for s, r, c in p.wide if r == c // 4),
                           low=tuple((s, 0, d) for s, _, d in p.low),
                           high=tuple((s, 0, d) for s, _, d in p.high))
        if p.wide:
            yield i, p


def _operand_keys(single):
    return tuple(dict.fromkeys((p.low, p.high) for _, p in _selected(single)))


def _signed_sum(terms):
    terms = sorted(terms, key=lambda t: -t[0])
    total = terms[0][1] if terms[0][0] > 0 else -terms[0][1]
    for sign, value in terms[1:]:
        total = total + value if sign > 0 else total - value
    return total


def _accumulate(sums, key, sign, value):
    if key not in sums:
        sums[key] = (sign, value)
    elif sums[key][0] == sign:
        sums[key] = (sign, sums[key][1] + value)
    else:
        sums[key] = (1, value - sums[key][1] if sign > 0 else sums[key][1] - value)


def _unpack(words):
    return pltpu.bitcast(words, jnp.bfloat16)


def _load(ref, i):
    return _unpack(ref.bitcast(jnp.uint32)[i]) if ref.dtype == jnp.bfloat16 else ref[i]


def _store(ref, i, first, value):
    rows = value.shape[0]
    if value.dtype == jnp.bfloat16:
        ref.bitcast(jnp.uint32)[i, pl.ds(first // 2, rows // 2), :] = pltpu.bitcast(value, jnp.uint32)
    else:
        ref[i, pl.ds(first, rows), :] = value.astype(ref.dtype)


def _low_lanes(rows):
    return jax.lax.broadcasted_iota(jnp.int32, (rows, _LANES), 1) < _HALF


def _blocks(x):
    return [x[:, d * _LANES:(d + 1) * _LANES] for d in range(_TAIL + 1)]


def _store_operands(ref, first, row_blocks):
    blocks = [_blocks(x) for x in row_blocks]
    rows = row_blocks[0].shape[0]
    low_lanes = _low_lanes(rows)
    total = functools.cache(lambda terms: _signed_sum([(s, blocks[r][d]) for s, r, d in terms]))
    for i, (low, high) in enumerate(_operand_keys(len(row_blocks) == 1)):
        _store(ref, i, first,
               total(low) if low == high else jnp.where(low_lanes, total(low), total(high)))


def _dot(a, b):
    return jnp.dot(a, b, preferred_element_type=jnp.float32)


def _expand(operands_ref, tiles_ref, out, single=False):
    keys = _operand_keys(single)
    sums, common = {}, []
    for i, p in _selected(single):
        product = _dot(_load(operands_ref, keys.index((p.low, p.high))), _load(tiles_ref, i))
        if p.common:
            common = [product, product]
        else:
            if common:
                product = product + common.pop()
            for s, r, c in p.wide:
                _accumulate(sums, (r, c), s, product)
        yield
    assert all(sign > 0 for sign, _ in sums.values())
    out.update({key: value for key, (_, value) in sums.items()})


def _contract(load, tiles_ref, sums, single=False, columns=_COLUMNS):
    held = []
    for i, p in _selected(single, columns):
        product = _dot(_signed_sum([(s, load(r, c)) for s, r, c in p.wide]),
                       _load(tiles_ref, i))
        if p.common or held:
            held.append((p, product))
        if len(held) == 3:
            (p, common), (p1, first), (p2, second) = held
            held = []
            product = common + jnp.where(_low_lanes(common.shape[0]), first, second)
            _accumulate(sums, (p1.high[0][1], _TAIL, 1), 1, first)
            _accumulate(sums, (p2.low[0][1], _TAIL, 0), 1, second)
        if not held:
            for s, r, d in p.low:
                _accumulate(sums, (r, d), s, product)
        yield


def _residual(row_blocks):
    return {(r, d) if d < _TAIL else (r, d, 0): (1, block)
            for r, x in enumerate(row_blocks) for d, block in enumerate(_blocks(x))}


def _contracted(sums, r):
    assert all(sign > 0 for sign, _ in sums.values())
    low, high = sums[r, _TAIL, 0][1], sums[r, _TAIL, 1][1]
    tail = jnp.where(_low_lanes(low.shape[0]), low, high)
    tail = tail + pltpu.roll(tail, _HALF, 1)
    return jnp.concatenate([sums[r, d][1] for d in range(_TAIL)] + [tail], axis=1)


def _weight_sums(source, copy, starts, columns=_COLUMNS):
    chosen = list(_selected(False, columns))
    for n, (i, p) in enumerate(chosen):
        for high in range(2):
            if n > high and chosen[n - 1 - high][1].common:
                continue
            for at in starts:
                first = lambda d: d * _LANES + at + (0 if d == _TAIL else high * _HALF)
                total = lambda terms: _signed_sum([(s, source(c, first(d))) for s, c, d in terms])
                terms = (p.w_low, p.w_high)[high]
                if len(terms) == 1:
                    yield i, high * _HALF + at, copy(terms[0][1], first(terms[0][2])), 0
                else:
                    value = total(terms)
                    yield i, high * _HALF + at, value, len(terms)
                if p.common:
                    k, other = chosen[n + 1 + high]
                    value = value if len(terms) > 1 else total(terms)
                    yield (k, high * _HALF + at, total((other.w_low, other.w_high)[high]) - value,
                           len(terms) + 1)


def _lay_out(sums, tiles_ref):
    for i, first, value, terms in sums:
        _store(tiles_ref, i, pl.multiple_of(first, 16), value)
        yield from range((4 * terms + 3) * value.shape[0] // 16)


def _lay_out_transposed(sums, tiles_ref):
    halves, pending = {}, []
    for i, first, value, terms in sums:
        halves[i, first] = value
        if (i, _HALF - first) in halves:
            pair = [halves[i, 0], halves[i, _HALF]]
            if pair[0].dtype != pair[1].dtype:
                pair = [half.astype(jnp.float32) for half in pair]
            pending.append((i, jnp.concatenate(pair, axis=0).astype(jnp.bfloat16).T))
        if len(pending) > _PENDING:
            k, tile = pending.pop(0)
            _store(tiles_ref, k, 0, tile)
        yield from range(_EVEN[0] * terms + _EVEN[1])
    for k, tile in pending:
        _store(tiles_ref, k, 0, tile)


def _layernorm(x):
    low_lanes = _low_lanes(x.shape[0])

    def mean(v):
        *full, tail = _blocks(v)
        total = functools.reduce(jnp.add, full) + jnp.where(low_lanes, tail, 0.0)
        return jnp.sum(total, axis=-1, keepdims=True) / (_TAIL * _LANES + _HALF)

    d = x - mean(x)
    return d * jax.lax.rsqrt(mean(d * d) + _EPS)


def _silu(x):
    half = 0.5 * x
    return half + half * jnp.tanh(half)


def _reciprocal(x):
    r = pl.reciprocal(x, approx=True)
    return r * (2.0 - x * r)


def _attention_masks(n_layers, rows, n_mem):
    i = jax.lax.broadcasted_iota(jnp.int32, (n_layers * rows, n_layers * rows), 0)
    j = jax.lax.broadcasted_iota(jnp.int32, (n_layers * rows, n_layers * rows), 1)
    if n_layers == 1:
        return (i < n_mem) | (i >= j), _MASKED * _LOG2E
    same = (i >= rows) == (j >= rows)
    visible = (i < n_mem) | ((i >= rows) & (i < rows + n_mem)) | (i >= j)
    fill = jnp.where(same, _MASKED * _LOG2E, -jnp.inf).astype(jnp.float32)
    return same & visible, fill


def _attention_tasks(xs, operands_ref, w_ref, heads_ref, outs, known=None):
    n_layers, rows = len(xs), heads_ref.shape[1] // 2
    single, n_mem = n_layers == 1, rows - xs[0].shape[0]
    visible, fill = _attention_masks(n_layers, rows, n_mem)
    scale = _LANES ** -0.5 * _LOG2E
    qkv, probs = {}, {}
    sums = _residual([jnp.concatenate([jnp.zeros_like(x[:n_mem]), x], axis=0) for x in xs])

    def stacked(u, h, streamed=False):
        parts = [qkv[u][r, h] for r in range(n_layers)]
        if known:
            (x, y), moved = parts, (rows + n_mem) // 2
            parts = [x[:n_mem], known(u, h), x[n_mem:moved], y, x[moved:]]
        value = jnp.concatenate(parts, axis=0)
        return value if single and streamed else value.astype(jnp.bfloat16)

    def project(u):
        qkv[u] = {}
        yield from _expand(operands_ref, w_ref.at[u], qkv[u], single)

    def scores(g):
        for h in range(_COLUMNS):
            s = jax.lax.dot_general(stacked(4 * g, h, True), stacked(4 * g + 1, h),
                                    (((1,), (1,)), ((), ())), preferred_element_type=jnp.float32)
            s = jnp.where(visible, s * scale, fill)
            p = jnp.exp2(s - jnp.max(s, axis=-1, keepdims=True))
            p = p * _reciprocal(jnp.sum(p, axis=-1, keepdims=True))
            probs[g, h] = p if single else p.astype(jnp.bfloat16)
            yield

    def values(g):
        for h in range(_COLUMNS):
            heads_ref[_COLUMNS * g + h, :n_layers * rows, :] = _dot(
                probs[g, h], stacked(4 * g + 2, h))
            yield

    def output(g):
        yield from _contract(lambda r, h: heads_ref[_COLUMNS * g + h, r * rows:(r + 1) * rows, :],
                             w_ref.at[4 * g + 3], sums, single)
        if g == _GROUPS - 1:
            outs.extend(_contracted(sums, r) for r in range(n_layers))

    tasks = {}
    for g in range(_GROUPS):
        tasks.update({f"Q{g}": project(4 * g), f"K{g}": project(4 * g + 1),
                      f"V{g}": project(4 * g + 2), f"S{g}": scores(g), f"A{g}": values(g),
                      f"O{g}": output(g)})
    return tasks


def _ffn_tasks(xs, operands_ref, w_ref, hidden_ref, result):
    rows = operands_ref.shape[1]
    sums = _residual(xs)

    def gated(u):
        both = {}
        yield from _expand(operands_ref, w_ref.at[_UP + u], both)
        for c in range(4):
            for r in range(2):
                hidden_ref[4 * u + c, r * rows:(r + 1) * rows, :] = (
                    _silu(both[r, c]) * both[r, 4 + c])

    def down(u):
        yield from _contract(lambda r, c: hidden_ref[_COLUMNS * u + c, r * rows:(r + 1) * rows, :],
                             w_ref.at[_DOWN + u], sums,
                             columns=min(_COLUMNS, hidden_ref.shape[0] - _COLUMNS * u))

    def finish():
        result([_contracted(sums, r) for r in range(2)])
        yield

    return {"F": finish(),
            **{f"G{u}": gated(u) for u in range(_DOWN - _UP)},
            **{f"D{u}": down(u) for u in range(_UNITS - _DOWN)}}


def _passes(order, tasks):
    done = object()
    for item in order.split():
        names, _, turns = item.partition(":")
        running = [(tasks[name], int(count or 1))
                   for name, _, count in (part.partition("*") for part in names.split("+"))]
        turn = 0
        while running and (not turns or turn < int(turns)):
            for task, count in tuple(running):
                for _ in range(count):
                    if next(task, done) is done:
                        running.remove((task, count))
                        break
                    yield
            turn += 1


def _run(*tasks):
    for _ in _chain(*tasks):
        pass


def _emit(order, tasks):
    _run(_passes(order, tasks))


def _chain(*tasks):
    for task in tasks:
        yield from task


def _kernel(xt_hbm, mem0_hbm, wq_hbm, wk_hbm, wv_hbm, wot_hbm, w1_hbm, w3_hbm, w2t_hbm,
            outt_hbm, mem0_ref, io_ref, res_ref, mem_ref, full_ref, short_ref, chunks_ref, heads_ref, hidden_ref, early_ref, w_ref, x_stage, qkv_stage, wo_stage,
            ffn_stage, x_sem, attention_sem, ffn_sem, mem_sem, io_sem, *, seg):
    d_model, n_tok = xt_hbm.shape
    n_mem = mem0_hbm.shape[0]
    n_seg = n_tok // seg
    n_io = n_tok // _LANES

    def window(r, n):
        return res_ref.at[pl.ds(pl.multiple_of((r + _LAG) * seg, seg), n * seg)]

    def block(r, n=1):
        return pl.ds(r * seg, n * seg)

    def lanes(i):
        return pl.ds(pl.multiple_of(i * _LANES, _LANES), _LANES)

    def transpose_out(i, x):
        io_ref[i] = x.T[:d_model].astype(io_ref.dtype)

    def prepare(ref, operands_ref, first, starts, rows=8):
        for i, pair in enumerate(starts):
            _store_operands(operands_ref, first + rows * i,
                            [_layernorm(ref[pl.ds(r, rows), :]) for r in pair])
        yield

    def prepare_full(ref, blocks):
        return prepare(ref, full_ref, n_mem,
                       [[r * seg + i for r in blocks] for i in range(0, seg, 8)])

    def prepare_short(ref, first, second):
        x = _layernorm(ref[pl.ds(first * seg + seg // 2, seg // 2), :])
        y = _layernorm(ref[block(second), :])
        mem_ref[0, n_mem:] = jnp.concatenate([x, y[seg - n_mem:]], axis=0)
        mem_ref[1, n_mem:] = y[:seg - n_mem]
        yield

    def prepare_ffn(ref, blocks):
        return prepare(ref, chunks_ref.at[0], 0,
                       [[r * seg + i for r in blocks] for i in range(0, 2 * seg, 16)], 16)

    def attention(order, ref, blocks, others, early=None):
        xs, outs = [ref[block(r), :] for r in blocks], []
        operands_ref = full_ref if early is None else short_ref
        _store_operands(operands_ref, 0, [
            mem_ref[i, :n_mem if early is None else seg] for i in range(len(blocks))])
        known = None if early is None else lambda u, h: early_ref[early, u - u // 4, h]
        tasks = _attention_tasks(xs, operands_ref, w_ref, heads_ref, outs, known)
        yield from _passes(order, {**others, **tasks})
        for i, r in enumerate(blocks):
            mem_ref[i, :n_mem] = outs[i][:n_mem]
            ref[block(r), :] = outs[i][n_mem:]

    def ffn_tasks(ref, blocks, result=None):
        def update(ys):
            for r, y in zip(blocks, ys):
                ref[block(r, 2), :] = y

        return {"N": prepare_ffn(ref, blocks), **_ffn_tasks(
            [ref[block(r, 2), :] for r in blocks], chunks_ref.at[0], w_ref, hidden_ref,
            result or update)}

    def double_step(b):
        ref = window(b, _LAG + 2)
        _run(attention(_ORDER_DOUBLE, ref, [_LAG, 0], {"X": prepare_short(ref, _LAG + 1, 1)}, 2 - b))

    def two_steps(j):
        b = 6
        ref = window(2 * j - b, b + _LAG + 3)
        transpose_out(jnp.where((j % 2 == 1) & (j > 1), (j - 3) // 2, n_io - 1), ref[block(0, 4), :])
        ffn = ffn_tasks(ref, [b + 2, b - 2])
        _run(attention(_ORDER_EVEN, ref, [b + _LAG, b],
                       {**ffn, "X": prepare_full(ref, [b + _LAG + 1, b + 1])}, j + _LAG // 2),
             attention(_ORDER_ODD, ref, [b + _LAG + 1, b + 1],
                       {**ffn, "X": prepare_short(ref, b + _LAG + 2, b + 2)}))

    def attention_copies(g, i):
        sem = attention_sem.at[4 * (g % 2) + i]
        if i == 3:
            heads = wot_hbm.bitcast(jnp.uint32).at[pl.ds(_COLUMNS * g, _COLUMNS)]
            return [pltpu.make_async_copy(heads, wo_stage, sem)]
        words = (wq_hbm, wk_hbm, wv_hbm)[i].bitcast(jnp.uint32)
        return [pltpu.make_async_copy(words.at[:, 4 * g + p, :], qkv_stage.at[g % 2, i, p], sem)
                for p in range(4)]

    def ffn_copies(batch, columns=_COLUMNS):
        width = columns * _LANES
        source = pl.ds(pl.multiple_of(batch * _COLUMNS * _LANES, _LANES), width)
        return [pltpu.make_async_copy(w.bitcast(jnp.uint32).at[:, source],
                                      ffn_stage.at[batch % 3, i, :, pl.ds(0, width)],
                                      ffn_sem.at[3 * (batch % 3) + i])
                for i, w in enumerate((w1_hbm, w3_hbm, w2t_hbm))]

    def start(copies):
        for c in copies:
            c.start()

    def wait(copies):
        for c in copies:
            c.wait()

    def lay_out_heads(g, i, u, starts=range(0, _HALF, 16)):
        def source(c, first):
            words = qkv_stage[g % 2, i, c // 2, pl.ds(pl.multiple_of(first, 16), 16), :]
            words = words & jnp.uint32(0xFFFF0000) if c % 2 else words << 16
            return pltpu.bitcast(words, jnp.float32)

        return _lay_out(_weight_sums(source, source, starts), w_ref.at[u])

    def lay_out_rows(words, u, transposed, columns=_COLUMNS):
        rows = _HALF if transposed else _UP_ROWS
        copy = lambda c, first: _unpack(words(c, pl.ds(first // 2, rows // 2)))
        sums = _weight_sums(lambda *at: copy(*at).astype(jnp.float32), copy,
                            range(0, _HALF, rows), columns)
        return (_lay_out_transposed if transposed else _lay_out)(sums, w_ref.at[u])

    def lay_out_up(batch, i):
        return lay_out_rows(
            lambda c, rows: ffn_stage[batch % 3, c // 4, rows, pl.ds((4 * i + c % 4) * _LANES, _LANES)],
            _UP + 2 * batch + i, False)

    def lay_out_down(batch, columns=_COLUMNS):
        return lay_out_rows(
            lambda c, rows: ffn_stage[batch % 3, 2, rows, pl.ds(c * _LANES, _LANES)],
            _DOWN + batch, True, columns)

    def x_copy(chunk):
        width = x_stage.shape[2]
        columns = pl.ds(pl.multiple_of(chunk * width, width), width)
        return pltpu.make_async_copy(xt_hbm.at[:, columns], x_stage.at[chunk], x_sem.at[chunk])

    def out_copy(i):
        return pltpu.make_async_copy(io_ref.at[i], outt_hbm.at[:, lanes(i)], io_sem.at[i])

    n_chunks = _EARLY // 8

    def load_group(g):
        def project(i):
            for chunk in range(n_chunks):
                out = {}
                yield from _expand(chunks_ref.at[chunk], w_ref.at[4 * g + i], out)
                for (r, c), value in out.items():
                    for e in range(4):
                        early_ref[8 * chunk + 4 * r + e, 3 * g + i, c] = (
                            value[e * seg // 2:(e + 1) * seg // 2])

        def arrive(i):
            if i == 0:
                pl.when(g + 1 < _GROUPS)(lambda: wait(attention_copies(g + 1, 0)))
            else:
                wait(attention_copies(g, i))
            if i == 3:
                pl.when(g + 1 < _GROUPS)(
                    lambda: start(attention_copies(g + 1, 1) + attention_copies(g + 1, 2)))
            if i in (3, 0):
                pl.when(g + 1 == _GROUPS)(lambda: start(ffn_copies(int(i == 0))))
            yield

        start(attention_copies(g, 3))
        pl.when(g + 1 < _GROUPS)(lambda: start(attention_copies(g + 1, 0)))
        following = jnp.minimum(g + 1, _GROUPS - 1)
        same = jnp.minimum(g, _GROUPS - 1)
        _emit("W1 " + _ORDER_LOAD, {
            **{f"E{i}": project(i) for i in range(3)}, **{f"W{i}": arrive(i) for i in range(4)},
            "L0": lay_out_heads(following, 0, 4 * following),
            "L1": lay_out_heads(g, 1, 4 * same + 1), "L2": lay_out_heads(g, 2, 4 * same + 2),
            "L3": lay_out_rows(lambda c, rows: wo_stage[c, rows, :], 4 * same + 3, True)})

    def first_step(r):
        ref = window(r, 2)
        pl.when(r + 2 < _LAG)(lambda: start(ffn_copies(r + 2)))
        pl.when(r + 2 == _LAG)(lambda: start(ffn_copies(_LAG, 4)))
        wait(ffn_copies(r))
        _emit(_ORDER_FIRST, {
            "P": attention(_ORDER_SINGLE, ref, [0], {"X": prepare_full(ref, [1])}),
            "L": _passes(_ORDER_L, {"U": _chain(lay_out_up(r, 0), lay_out_up(r, 1)),
                                   "D": lay_out_down(r)})})

    mem_copy = pltpu.make_async_copy(mem0_hbm, mem0_ref.at[0], mem_sem.at[0])
    first = attention_copies(0, 0)
    start([x_copy(0)] + first)
    for spare in (window(-_LAG, _LAG), window(n_seg, 1)):
        spare[...] = jnp.zeros(spare.shape, spare.dtype)
    wait(first[:2])
    x_copy(1).start()
    wait(first[2:])
    start([x_copy(i) for i in range(2, n_chunks)] + [mem_copy])

    @pl.loop(0, n_chunks)
    def _early_operands(chunk):
        pl.when(chunk == 1)(lambda: start(attention_copies(0, 1)))
        pl.when(chunk == 3)(lambda: start(attention_copies(0, 2)))
        wait([x_copy(chunk)])
        _run(lay_out_heads(0, 0, 0, starts=[16 * chunk]))
        x = x_stage[chunk].astype(jnp.float32)
        x = jnp.concatenate([x, x[_TAIL * _LANES:]], axis=0).T
        window(n_seg // n_chunks * chunk, n_seg // n_chunks)[...] = x
        halves = [x[2 * e * seg:2 * e * seg + seg // 2] for e in range(8)]
        halves[1] = jnp.where(chunk == 0, x[(_LAG + 1) * seg:(_LAG + 1) * seg + seg // 2], halves[1])
        _store_operands(chunks_ref.at[chunk], 0, [
            _layernorm(jnp.concatenate(part, axis=0)) for part in (halves[:4], halves[4:])])

    pl.loop(0, _GROUPS)(load_group)
    mem_copy.wait()
    mem0 = mem0_ref[0].astype(jnp.float32)
    mem0 = jnp.concatenate([mem0, mem0[:, _TAIL * _LANES:]], axis=1)
    mem_ref[0, :n_mem] = mem_ref[1, :n_mem] = mem0
    whole = window(0, n_seg)
    _run(prepare_full(whole, [0]))
    pl.loop(0, _LAG)(first_step)
    wait(ffn_copies(_LAG, 4))
    _emit(_ORDER_FIRST_FFN, {"P": _passes(_ORDER_FFN, ffn_tasks(whole, [0, 2])),
                             "L": _chain(lay_out_up(_LAG, 0), lay_out_down(_LAG, 4))})
    _run(prepare_short(whole, _LAG, 0))
    pl.loop(0, 2)(double_step)
    last = n_seg - _LAG
    pl.loop(1, last // 2)(two_steps)

    n_done = n_io - 3
    for i in range(n_done):
        out_copy(i).start()
    mem_ref[0, :n_mem] = mem_ref[1, :n_mem]
    ffn = ffn_tasks(whole, [n_seg - 2, last - 2])
    _run(prepare_full(whole, [last]),
         attention(_ORDER_EVEN_SINGLE, whole, [last],
                   {**ffn, "X": prepare_full(whole, [last + 1])}),
         attention(_ORDER_ODD_SINGLE, whole, [last + 1],
                   {**ffn, "X": prepare_full(whole, [last + 2])}))

    @pl.loop(0, 2)
    def _last_steps(i):
        transpose_out(n_done + i, res_ref[lanes(n_done + i + 1), :])
        ref = window(last + 2 + i, 2)
        _run(attention(_ORDER_SINGLE, ref, [0], {"X": prepare_full(ref, [1])}))
        out_copy(n_done + i).start()

    _emit(_ORDER_FFN, ffn_tasks(whole, [last, last + 2],
                                lambda ys: transpose_out(n_io - 1, jnp.concatenate(ys, axis=0))))
    out_copy(n_io - 1).start()
    for i in range(n_io):
        out_copy(i).wait()


@functools.partial(jax.jit, static_argnames=("A_seg_len",))
def pallas_interleave_layers__memory_aug_recurrent_mem_tr__glu_gated_swiglu__prompt_kernel(
    A_x: jax.Array,
    A_mem0: jax.Array,
    A_Wq: jax.Array,
    A_Wk: jax.Array,
    A_Wv: jax.Array,
    A_Wo: jax.Array,
    A_seg_len: int,
    B_x: jax.Array,
    B_w1: jax.Array,
    B_w3: jax.Array,
    B_w2: jax.Array,
):
    del B_x
    _, n_tok, d_model = A_x.shape
    n_mem = A_mem0.shape[1]
    _, n_heads, d_head = A_Wq.shape
    d_ff = B_w1.shape[1]
    seg = A_seg_len
    assert A_x.shape[0] == 1 and _LAG * seg == _LANES and n_mem == 8 and n_tok == 64 * seg
    assert d_model == _TAIL * _LANES + _HALF and d_head == _LANES
    assert n_heads == _GROUPS * _COLUMNS and d_ff == 4 * (_DOWN - _UP) * _LANES
    n_operands = len(_operand_keys(False))
    hbm = pl.BlockSpec(memory_space=pltpu.HBM)
    out_t = pl.pallas_call(
        functools.partial(_kernel, seg=seg),
        out_shape=jax.ShapeDtypeStruct((d_model, n_tok), A_x.dtype),
        in_specs=[hbm] * 9,
        out_specs=hbm,
        scratch_shapes=[
            pltpu.VMEM((16, n_mem, d_model), A_mem0.dtype),
            pltpu.VMEM((n_tok // _LANES, d_model, _LANES), A_x.dtype),
            pltpu.VMEM((n_tok + (_LAG + 1) * seg, d_model + _HALF), jnp.float32),
            pltpu.VMEM((2, seg, d_model + _HALF), jnp.float32),
            pltpu.VMEM((n_operands, n_mem + seg, _LANES), jnp.float32),
            pltpu.VMEM((n_operands, seg, _LANES), jnp.dtype(_SHORT)),
            pltpu.VMEM((_EARLY // 8, n_operands, 2 * seg, _LANES), jnp.dtype(_CHUNK)),
            pltpu.VMEM((n_heads, 2 * (n_mem + seg), d_head), jnp.float32),
            pltpu.VMEM((d_ff // _LANES, 4 * seg, _LANES), jnp.float32),
            pltpu.VMEM((_EARLY, 3 * _GROUPS, _COLUMNS, seg // 2, d_head), jnp.float32),
            pltpu.VMEM((_UNITS, len(_scheme(_COLUMNS)), _LANES, _LANES), jnp.bfloat16),
            pltpu.VMEM((_EARLY // 8, d_model, 8 * n_tok // _EARLY), A_x.dtype),
            pltpu.VMEM((2, 3, _COLUMNS // 2, d_model, d_head), jnp.uint32),
            pltpu.VMEM((_COLUMNS, d_model // 2, d_head), jnp.uint32),
            pltpu.VMEM((3, 3, d_model // 2, _COLUMNS * _LANES), jnp.uint32),
            pltpu.SemaphoreType.DMA((_EARLY // 8,)),
            pltpu.SemaphoreType.DMA((8,)),
            pltpu.SemaphoreType.DMA((9,)),
            pltpu.SemaphoreType.DMA((1,)),
            pltpu.SemaphoreType.DMA((n_tok // _LANES,)),
        ],
        compiler_params=pltpu.CompilerParams(vmem_limit_bytes=124 * 1024 * 1024, flags=_FLAGS,
                                             disable_bounds_checks=True),
    )(A_x.reshape(n_tok, d_model).T, A_mem0.reshape(n_mem, d_model), A_Wq, A_Wk, A_Wv,
      A_Wo.transpose(0, 2, 1), B_w1, B_w3, B_w2.T)
    return out_t.T.reshape(A_x.shape)
```

```python
import functools
import math
from typing import NamedTuple

import jax
import jax.numpy as jnp
import jax.experimental.pallas as pl
import jax.experimental.pallas.tpu as pltpu

_EPS = 1e-05
_MASKED = -1000000000.0
_LOG2E = math.log2(math.e)
_LANES = 128
_HALF = _LANES // 2
_TAIL = 4
_COLUMNS = 8
_MEMBERS = 4
_WQ, _WK, _WV, _WO, _UP, _DOWN, _FAMILIES = 0, 1, 2, 3, 4, 6, 7
_LAG = 4
_CHUNKS = 4
_ORDER_EVEN = (
    "N X Q0 K0 G0*4+V0*4 Q1 G1*10+S0 K1 A0 V1 G2*6+S1 Q2 A1 K2 V2 G3*6+S2 Q3 A2 K3 V3 G4*6+S3 "
    "O0 A3+O1*6 G8 O2 O3 D4")
_ORDER_ODD = (
    "Q0 K0 V0*10+S0 G5 A0 G6 Q1 G7 K1 D0 V1*6+S1 D1 A1 D2 Q2 D3 F X K2 V2*6+S2 Q3 A2 K3 "
    "V3*6+S3 O0 O1 A3+O2*4 O3")
_ORDER_EVEN_SINGLE = (
    "Q0 N K0 V0*4+S0 Q1 K1 G0 A0 V1*4+S1 O0 G1 A1 Q2 K2 V2*4+S2 O1 G2 A2 Q3 K3 V3*4+S3 X O2 "
    "G3 A3 G8 O3 D4 G4")
_ORDER_ODD_SINGLE = (
    "Q0 K0 V0*4+S0 G5 A0 Q1 K1 V1*4+S1 G6 A1 Q2 K2 G7 V2*4+S2 D0 A2 Q3 K3 "
    "V3*4+S3 D1 D2 A3 D3 F X O0 O1 O2 O3")
_ORDER_DOUBLE = (
    "Q0 K0 Q1 K1 V0*10+S0 Q2 K2 V1*6+S1 A0 Q3 K3 V2 A1 O0*6+S2 V3 X O1*6+S3 A2 O2:30 A3 O2 O3")
_ORDER_SINGLE = (
    "Q0 K0 V0*4+S0 Q1 K1 A0 V1*4+S1 Q2 K2 A1 V2*4+S2 Q3 K3 A2 V3*4+S3 X O0 O1 A3 O2 O3")
_ORDER_FFN = "N G0 G1 G2 D0 G3 G4 D1 G5 G6 G7 G8 D2 D4 D3 F"
_ORDER_SHARED = "E+L*18+O*13"
_ORDER_LOAD = "W1 E0+L1*28 W2 E1+L2*28+L3*12:208 E1 L2 W0 E2+L0*28+L3*12"
_ORDER_FIRST = "P:8 P+L*28"
_ORDER_FIRST_FFN = "P:20 P+L*15"


class _Pass(NamedTuple):
    low: tuple
    high: tuple
    w_low: tuple
    w_high: tuple
    wide: tuple
    common: bool = False


@functools.cache
def _scheme(kind, shift=0):
    x, y, n = 0, 1, 4 if kind in ("member", "alone") else 2
    a = lambda d: d % n + shift
    b = lambda d: d % n + shift + (2 if kind == "narrow" else 4)
    rest = lambda d: [e for e in range(4) if e != d and e // n == d // n]

    def whole(narrow, weight, wide):
        return _Pass(tuple(sorted(narrow)), tuple(sorted(narrow)), weight, weight, wide)

    def m1(d, e):
        return whole(((1, x, d), (1, y, e)), ((1, b(e), d), (1, a(d), e)),
                     ((1, y, a(d)), (1, x, b(e))))

    def m2(d, e):
        return whole(((1, y, d), (1, y, e)), ((1, b(e), d),), ((1, y, b(e)), (-1, y, a(d))))

    def m3(d):
        return whole(((1, x, d),), ((1, a(d), d), *((-1, a(d), e) for e in rest(d))),
                     ((1, x, a(d)), (1, y, a(d))))

    def m4(d):
        return whole(((1, y, d),), ((1, b(d), d), *((-1, b(d), e) for e in rest(d))),
                     ((1, y, b(d)), (1, x, b(d))))

    def m5(d, e):
        return whole(((1, x, d), (1, x, e)), ((1, a(d), e),), ((1, x, a(d)), (-1, x, b(e))))

    def m6(d):
        return whole(((1, y, d), (-1, x, d)), ((1, a(d), d), *((1, b(e), d) for e in rest(d))),
                     ((1, y, a(d)),))

    def m7(d):
        return whole(((1, y, d), (-1, x, d)), ((-1, b(d), d), *((-1, a(e), d) for e in rest(d))),
                     ((1, x, b(d)),))

    def with_tails(p, p_rows, p_columns, q, q_rows, q_columns):
        tail = lambda columns: tuple((1, c, _TAIL) for c in columns)
        return [_Pass(p.low, p.high, q.w_low, p.w_high, p.wide + q.wide, common=True),
                _Pass(p.low, ((1, p_rows, _TAIL),), p.w_low, tail(p_columns), p.wide),
                _Pass(((1, q_rows, _TAIL),), q.high, tail(q_columns), q.w_high, q.wide)]

    def pair_with_tails(d, e):
        return [*with_tails(m5(d, e), x, [a(d)], m5(e, d), x, [a(e)]), m3(d),
                *with_tails(m2(d, e), y, [b(e)], m2(e, d), y, [b(d)]), m3(e),
                *with_tails(m6(d), y, [a(d), b(e)], m7(d), x, [b(d), a(e)]), m1(d, e), m4(d),
                *with_tails(m7(e), x, [b(e), a(d)], m6(e), y, [a(e), b(d)]), m1(e, d), m4(e)]

    edge = lambda d, e: [m5(d, e), m1(d, e), m2(d, e)]
    pair = lambda d, e: [m3(d), m6(d), *edge(d, e), m7(e), m4(e),
                         m3(e), m6(e), *edge(e, d), m7(d), m4(d)]
    if kind == "shared":
        return (*pair(0, 1), *(() if shift else _scheme(kind, 2)))
    if kind == "narrow":
        return (*pair_with_tails(0, 1), *pair(2, 3))
    ends = pair if kind == "member" else pair_with_tails
    return (*ends(0, 1), *edge(0, 2), *edge(0, 3), *edge(1, 2), *edge(1, 3),
            *edge(2, 0), *edge(3, 0), *edge(2, 1), *edge(3, 1), *ends(2, 3))


def _selected(kind, single):
    for i, p in enumerate(_scheme(kind)):
        if single:
            narrow = tuple((s, 0, d) for s, _, d in p.low)
            p = p._replace(low=narrow, high=narrow,
                           wide=tuple((s, 0, c) for s, r, c in p.wide if r == c // 4))
        if p.wide:
            yield i, p


def _tiles(w_ref, kind, family=_FAMILIES, member=_MEMBERS):
    size = lambda name: len(_scheme(name))
    first = family * (_MEMBERS * size("member") + size("shared"))
    if kind in ("member", "shared"):
        first += member * size("member")
    return w_ref.at[pl.ds(first + (size("alone") if kind == "narrow" else 0), size(kind))]


def _tail_for(terms, block):
    return tuple(sorted((s, r, _TAIL if d == block else d) for s, r, d in terms))


@functools.cache
def _operand_keys(single):
    return tuple(dict.fromkeys(_tail_for(p.low, block) for block in (None, 0, 1)
                               for _, p in _selected("member", single)))


def _signed_sum(terms):
    terms = sorted(terms, key=lambda t: -t[0])
    total = terms[0][1] if terms[0][0] > 0 else -terms[0][1]
    for sign, value in terms[1:]:
        total = total + value if sign > 0 else total - value
    return total


def _accumulate(sums, key, sign, value):
    if key not in sums:
        sums[key] = (sign, value)
    elif sums[key][0] == sign:
        sums[key] = (sign, sums[key][1] + value)
    else:
        sums[key] = (1, value - sums[key][1] if sign > 0 else sums[key][1] - value)


def _words(ref):
    return ref.bitcast(jnp.uint32) if ref.dtype == jnp.bfloat16 else ref


def _unpack(words):
    return pltpu.bitcast(words, jnp.bfloat16) if words.dtype == jnp.uint32 else words


def _store(ref, i, first, value):
    rows = value.shape[0]
    if value.dtype == jnp.bfloat16:
        _words(ref)[i, pl.ds(first // 2, rows // 2), :] = pltpu.bitcast(value, jnp.uint32)
    else:
        ref[i, pl.ds(first, rows), :] = value.astype(ref.dtype)


def _lane_half(rows):
    return jax.lax.broadcasted_iota(jnp.int32, (rows, _LANES), 1) // _HALF


def _blocks(x):
    return [x[:, d * _LANES:(d + 1) * _LANES] for d in range(_TAIL + 1)]


def _store_operands(ref, first, row_blocks):
    blocks = [_blocks(x) for x in row_blocks]
    for i, terms in enumerate(_operand_keys(len(row_blocks) == 1)):
        _store(ref, i, first, _signed_sum([(s, blocks[r][d]) for s, r, d in terms]))


def _dot(a, b):
    return jnp.dot(a, b, preferred_element_type=jnp.float32)


def _expand(operands_ref, w_ref, unit, out, single=False):
    operands_ref, tiles_ref = _words(operands_ref), _words(_tiles(w_ref, *unit))
    operand = lambda terms: operands_ref[_operand_keys(single).index(terms)]
    half = _lane_half(operands_ref.shape[1])
    freed = {}
    if unit[0] == "member":
        blocks = [unit[2] // 2] if isinstance(unit[2], int) else range(_MEMBERS // 2)
        freed = {d: half == unit[2] - 2 * d for d in blocks}
    sums, common = {key: (1, value) for key, value in out.items()}, []
    for i, p in _selected(unit[0], single):
        lhs = operand(p.low)
        if p.high != p.low:
            lhs = jnp.where(half == 0, lhs, operand(p.high))
        for d, lanes in freed.items():
            if _tail_for(p.low, d) != p.low:
                lhs = jnp.where(lanes, operand(_tail_for(p.low, d)), lhs)
        product = _dot(_unpack(lhs), _unpack(tiles_ref[i]))
        if p.common:
            common = [product, product]
        else:
            if common:
                product = product + common.pop()
            for s, r, c in p.wide:
                _accumulate(sums, (r, c), s, product)
        yield
    assert all(sign > 0 for sign, _ in sums.values())
    out.update({key: value for key, (_, value) in sums.items()})


def _contract(load, w_ref, unit, sums, single=False):
    tiles_ref = _words(_tiles(w_ref, *unit))
    freed = unit[2] // 2 if unit[0] == "member" else None
    held, mixed = [], {}
    for i, p in _selected(unit[0], single):
        product = _dot(_signed_sum([(s, load(r, c)) for s, r, c in p.wide]),
                       _unpack(tiles_ref[i]))
        if p.common or held:
            held.append((p, product))
        if len(held) == 3:
            (p, common), (p1, first), (p2, second) = held
            held = []
            product = common + jnp.where(_lane_half(common.shape[0]) == 0, first, second)
            _accumulate(sums, (p1.high[0][1], _TAIL, 1), 1, first)
            _accumulate(sums, (p2.low[0][1], _TAIL, 0), 1, second)
        if not held:
            for s, r, d in p.low:
                _accumulate(mixed if d == freed else sums, (r, d), s, product)
        yield
    for (r, d), (s, both) in mixed.items():
        _accumulate(sums, (r, _TAIL, unit[2] % 2), s, both)
        _accumulate(sums, (r, d), s, jnp.where(_lane_half(both.shape[0]) == unit[2] % 2, 0.0, both))


def _residual(row_blocks):
    return {(r, d) if d < _TAIL else (r, d, 0): (1, block)
            for r, x in enumerate(row_blocks) for d, block in enumerate(_blocks(x))}


def _contracted(sums, r):
    assert all(sign > 0 for sign, _ in sums.values())
    low, high = sums[r, _TAIL, 0][1], sums[r, _TAIL, 1][1]
    tail = jnp.where(_lane_half(low.shape[0]) == 0, low, high)
    tail = tail + pltpu.roll(tail, _HALF, 1)
    return jnp.concatenate([sums[r, d][1] for d in range(_TAIL)] + [tail], axis=1)


def _weight_sum(parts):
    return _signed_sum([(s, part.astype(jnp.float32) if len(parts) > 1 else part)
                        for s, part in parts])


def _weight_sums(passes, source, starts):
    for i, p in enumerate(passes):
        for high in range(2):
            if i > high and passes[i - 1 - high].common:
                continue
            for at in starts:
                first = high * _HALF + at
                total = lambda terms: _weight_sum(
                    [(s, source(c, d, at if d == _TAIL else first)) for s, c, d in terms])
                terms = (p.w_low, p.w_high)[high]
                value = total(terms)
                yield i, first, value, len(terms)
                if p.common:
                    other = passes[i + 1 + high]
                    other = total((other.w_low, other.w_high)[high]).astype(jnp.float32)
                    yield i + 1 + high, first, other - value.astype(jnp.float32), len(terms) + 1


def _lay_out(sums, tiles_ref):
    for i, first, value, terms in sums:
        _store(tiles_ref, i, pl.multiple_of(first, 16), value)
        yield from range((4 * terms + 1) * value.shape[0] // 16)


def _lay_out_transposed(sums, tiles_ref):
    halves, pending = {}, []
    for i, first, value, terms in sums:
        halves[i, first] = value
        if (i, _HALF - first) in halves:
            pair = [halves[i, 0], halves[i, _HALF]]
            if pair[0].dtype != pair[1].dtype:
                pair = [half.astype(jnp.float32) for half in pair]
            pending.append((i, jnp.concatenate(pair, axis=0).astype(jnp.bfloat16).T))
        if len(pending) > 2:
            _store(tiles_ref, pending[0][0], 0, pending.pop(0)[1])
        yield from range(8 * terms + 22)
    for i, tile in pending:
        _store(tiles_ref, i, 0, tile)


def _layernorm(x):
    low_lanes = _lane_half(x.shape[0]) == 0

    def mean(v):
        *full, tail = _blocks(v)
        total = functools.reduce(jnp.add, full) + jnp.where(low_lanes, tail, 0.0)
        return jnp.sum(total, axis=-1, keepdims=True) / (_TAIL * _LANES + _HALF)

    d = x - mean(x)
    return d * jax.lax.rsqrt(mean(d * d) + _EPS)


def _silu(x):
    half = 0.5 * x
    return half + half * jnp.tanh(half)


def _reciprocal(x):
    r = pl.reciprocal(x, approx=True)
    return r * (2.0 - x * r)


def _attention_masks(n_layers, rows, n_mem):
    i = jax.lax.broadcasted_iota(jnp.int32, (n_layers * rows, n_layers * rows), 0)
    j = jax.lax.broadcasted_iota(jnp.int32, (n_layers * rows, n_layers * rows), 1)
    if n_layers == 1:
        return (i < n_mem) | (i >= j), _MASKED * _LOG2E
    same = (i >= rows) == (j >= rows)
    visible = (i < n_mem) | ((i >= rows) & (i < rows + n_mem)) | (i >= j)
    fill = jnp.where(same, _MASKED * _LOG2E, -jnp.inf).astype(jnp.float32)
    return same & visible, fill


def _expand_member(operands_ref, w_ref, family, member, shared_ref, out, single=False):
    rows = operands_ref.shape[1]
    if member == 0:
        yield from _expand(operands_ref, w_ref, ("shared", family), out, single)
        for (r, c), value in out.items():
            shared_ref[c, r * rows:(r + 1) * rows, :] = value
    out.update({(r, c): shared_ref[c, r * rows:(r + 1) * rows, :]
                for r in range(1 if single else 2) for c in range(_COLUMNS)})
    yield from _expand(operands_ref, w_ref, ("member", family, member), out, single)


def _store_wide(ref, member, c, rows, value):
    ref[member, c, rows, :] = value
    if member == _MEMBERS - 1:
        ref[_MEMBERS, c, rows, :] = functools.reduce(
            jnp.add, [ref[m, c, rows, :] for m in range(member)] + [value])


def _contract_member(ref, w_ref, family, member, sums, single=False):
    rows = ref.shape[2] // 2
    load = lambda m: lambda r, c: ref[m, c, r * rows:(r + 1) * rows, :]
    yield from _contract(load(member), w_ref, ("member", family, member), sums, single)
    if member == _MEMBERS - 1:
        yield from _contract(load(_MEMBERS), w_ref, ("shared", family), sums, single)


def _attention_tasks(xs, operands_ref, w_ref, wide_ref, outs, known=None):
    n_layers, rows = len(xs), wide_ref.shape[2] // 2
    single, n_mem = n_layers == 1, rows - xs[0].shape[0]
    visible, fill = _attention_masks(n_layers, rows, n_mem)
    scale = _LANES ** -0.5 * _LOG2E
    qkv, probs = {}, {}
    sums = _residual([jnp.concatenate([jnp.zeros_like(x[:n_mem]), x], axis=0) for x in xs])

    def stacked(family, g, h):
        parts = [qkv[family, g][r, h] for r in range(n_layers)]
        if known:
            (x, y), moved = parts, (rows + n_mem) // 2
            parts = [x[:n_mem], known(family, g, h), x[n_mem:moved], y, x[moved:]]
        value = jnp.concatenate(parts, axis=0)
        return value if single and family == _WQ else value.astype(jnp.bfloat16)

    def project(family, g):
        qkv[family, g] = {}
        return _expand_member(operands_ref, w_ref, family, g, wide_ref.at[_MEMBERS + 1 + family],
                              qkv[family, g], single)

    def scores(g):
        for h in range(_COLUMNS):
            s = jax.lax.dot_general(stacked(_WQ, g, h), stacked(_WK, g, h),
                                    (((1,), (1,)), ((), ())), preferred_element_type=jnp.float32)
            s = jnp.where(visible, s * scale, fill)
            p = jnp.exp2(s - jnp.max(s, axis=-1, keepdims=True))
            p = p * _reciprocal(jnp.sum(p, axis=-1, keepdims=True))
            probs[g, h] = p if single else p.astype(jnp.bfloat16)
            yield

    def values(g):
        for h in range(_COLUMNS):
            _store_wide(wide_ref, g, h, slice(0, n_layers * rows),
                        _dot(probs[g, h], stacked(_WV, g, h)))
            yield

    def output(g):
        yield from _contract_member(wide_ref, w_ref, _WO, g, sums, single)
        if g == _MEMBERS - 1:
            outs.extend(_contracted(sums, r) for r in range(n_layers))

    tasks = {}
    for g in range(_MEMBERS):
        tasks.update({f"Q{g}": project(_WQ, g), f"K{g}": project(_WK, g), f"V{g}": project(_WV, g),
                      f"S{g}": scores(g), f"A{g}": values(g), f"O{g}": output(g)})
    return tasks


def _ffn_tasks(xs, operands_ref, w_ref, wide_ref, result):
    rows = operands_ref.shape[1]
    sums = _residual(xs)

    def gated(member, i):
        both = {}
        if member < _MEMBERS:
            yield from _expand_member(operands_ref, w_ref, _UP + i, member,
                                      wide_ref.at[_MEMBERS + 2 + i], both)
        else:
            yield from _expand(operands_ref, w_ref, ("alone",), both)
        for c in range(4):
            for r in range(2):
                _store_wide(wide_ref, member + member // _MEMBERS, 4 * i + c,
                            slice(r * rows, (r + 1) * rows), _silu(both[r, c]) * both[r, 4 + c])

    def finish():
        result([_contracted(sums, r) for r in range(2)])
        yield

    return {"F": finish(), **{f"G{u}": gated(*divmod(u, 2)) for u in range(2 * _MEMBERS + 1)},
            **{f"D{m}": _contract_member(wide_ref, w_ref, _DOWN, m, sums) for m in range(_MEMBERS)},
            "D4": _contract(lambda r, c: wide_ref[_MEMBERS + 1, c, r * rows:(r + 1) * rows, :],
                            w_ref, ("narrow",), sums)}


def _passes(order, tasks):
    done = object()
    for item in order.split():
        names, _, turns = item.partition(":")
        running = [(tasks[name], int(count or 1))
                   for name, _, count in (part.partition("*") for part in names.split("+"))]
        turn = 0
        while running and (not turns or turn < int(turns)):
            for task, count in tuple(running):
                for _ in range(count):
                    if next(task, done) is done:
                        running.remove((task, count))
                        break
                    yield
            turn += 1


def _chain(*tasks):
    for task in tasks:
        yield from task


def _run(*tasks):
    for _ in _chain(*tasks):
        pass


def _kernel(xt_hbm, mem0_hbm, wq_hbm, wk_hbm, wv_hbm, wot_hbm, w1_hbm, w3_hbm, w2t_hbm,
            outt_hbm, out_ref, mem_ref, full_ref, short_ref, chunks_ref, heads_ref, hidden_ref,
            early_ref, w_ref, x_stage, qkv_stage, qkv_shared, wo_stage, wo_shared, ffn_stage,
            ffn_shared, res_ref, mem0_ref, x_sem, attention_sem, ffn_sem, shared_sem, out_sem,
            *, seg):
    d_model, n_tok = xt_hbm.shape
    n_mem = mem0_hbm.shape[0]
    n_seg = n_tok // seg
    n_out = n_tok // _LANES

    def window(r, n):
        return res_ref.at[pl.ds(pl.multiple_of((r + _LAG) * seg, seg), n * seg)]

    def block(r, n=1):
        return pl.ds(r * seg, n * seg)

    def lanes(i, n=1):
        return pl.ds(pl.multiple_of(i * _LANES, _LANES), n * _LANES)

    def transpose_out(i, x):
        out_ref[i] = x.T[:d_model].astype(out_ref.dtype)

    def prepare(ref, blocks, total, operands_ref, first):
        rows = 32 // operands_ref.dtype.itemsize
        for i in range(0, total, rows):
            _store_operands(operands_ref, first + i,
                            [_layernorm(ref[pl.ds(r * seg + i, rows), :]) for r in blocks])
        yield

    def prepare_full(ref, blocks):
        return prepare(ref, blocks, seg, full_ref, n_mem)

    def prepare_short(ref, first, second):
        x = _layernorm(ref[pl.ds(first * seg + seg // 2, seg // 2), :])
        y = _layernorm(ref[block(second), :])
        mem_ref[0, n_mem:] = jnp.concatenate([x, y[seg - n_mem:]], axis=0)
        mem_ref[1, n_mem:] = y[:seg - n_mem]
        yield

    def attention(order, ref, blocks, others, early=None):
        xs, outs = [ref[block(r), :] for r in blocks], []
        operands_ref = full_ref if early is None else short_ref
        _store_operands(operands_ref, 0, [
            mem_ref[i, :n_mem if early is None else seg] for i in range(len(blocks))])
        known = None if early is None else lambda *at: early_ref[(early, *at)]
        tasks = _attention_tasks(xs, operands_ref, w_ref, heads_ref, outs, known)
        yield from _passes(order, {**others, **tasks})
        for i, r in enumerate(blocks):
            mem_ref[i, :n_mem] = outs[i][:n_mem]
            ref[block(r), :] = outs[i][n_mem:]

    def ffn_tasks(ref, blocks, result=None):
        def update(ys):
            for r, y in zip(blocks, ys):
                ref[block(r, 2), :] = y

        return {"N": prepare(ref, blocks, 2 * seg, chunks_ref.at[0], 0), **_ffn_tasks(
            [ref[block(r, 2), :] for r in blocks], chunks_ref.at[0], w_ref, hidden_ref,
            result or update)}

    def double_step(b):
        ref = window(b, _LAG + 2)
        _run(attention(_ORDER_DOUBLE, ref, [_LAG, 0],
                       {"X": prepare_short(ref, _LAG + 1, 1)}, _LAG // 2 - b))

    def two_steps(j):
        b = 6
        ref = window(2 * j - b, b + _LAG + 3)
        transpose_out(jnp.where((j % 2 == 1) & (j > 1), (j - 3) // 2, n_out - 1),
                      ref[block(0, 4), :])
        ffn = ffn_tasks(ref, [b + 2, b - 2])
        _run(attention(_ORDER_EVEN, ref, [b + _LAG, b],
                       {**ffn, "X": prepare_full(ref, [b + _LAG + 1, b + 1])}, j + _LAG // 2),
             attention(_ORDER_ODD, ref, [b + _LAG + 1, b + 1],
                       {**ffn, "X": prepare_short(ref, b + _LAG + 2, b + 2)}))

    qkv_words = [_words(w) for w in (wq_hbm, wk_hbm, wv_hbm)]
    ffn_words = [_words(w) for w in (w1_hbm, w3_hbm, w2t_hbm)]
    pairs = _COLUMNS // 2

    def attention_copies(family, g):
        sem = attention_sem.at[family]
        if family == _WO:
            heads = _words(wot_hbm).at[pl.ds(_COLUMNS * g, _COLUMNS)]
            return [pltpu.make_async_copy(heads, wo_stage, sem)]
        return [pltpu.make_async_copy(qkv_words[family].at[:, pairs * g + p, :],
                                      qkv_stage.at[family, p], sem) for p in range(pairs)]

    def ffn_copies(m, columns=_COLUMNS):
        return [pltpu.make_async_copy(w.at[:, lanes(_COLUMNS * m, columns)],
                                      ffn_stage.at[m % 3, i, :, lanes(0, columns)],
                                      ffn_sem.at[3 * (m % 3) + i])
                for i, w in enumerate(ffn_words)]

    def shared_copies(which):
        ends = []
        for m in range(_MEMBERS):
            rows, words = pl.ds(m * _HALF, _HALF), pl.ds(m * _HALF // 2, _HALF // 2)
            if which == 0:
                ends += [(w.at[rows, pairs * m + p, :], qkv_shared.at[i, p, rows])
                         for i, w in enumerate(qkv_words) for p in range(pairs)]
            elif which == 1:
                ends += [(_words(wot_hbm).at[pl.ds(_COLUMNS * m, _COLUMNS), words],
                          wo_shared.at[:, words])]
            else:
                ends += [(w.at[words, lanes(_COLUMNS * m, _COLUMNS)], ffn_shared.at[i, words])
                         for i, w in enumerate(ffn_words)]
        return [pltpu.make_async_copy(*pair, shared_sem.at[which]) for pair in ends]

    def x_copy(chunk):
        columns = lanes(n_out // _CHUNKS * chunk, n_out // _CHUNKS)
        return pltpu.make_async_copy(xt_hbm.at[:, columns], x_stage.at[chunk], x_sem.at[chunk])

    def out_copy(i):
        return pltpu.make_async_copy(out_ref.at[i], outt_hbm.at[:, lanes(i)], out_sem.at[i])

    def start(copies):
        for c in copies:
            c.start()

    def wait(copies):
        for c in copies:
            c.wait()

    def head_pairs(ref):
        def source(c, d, first):
            words = ref[c // 2, pl.ds(pl.multiple_of(d * _LANES + first, 16), 16), :]
            words = words & jnp.uint32(0xFFFF0000) if c % 2 else words << 16
            return pltpu.bitcast(words, jnp.float32)
        return source

    def row_pairs(words, rows):
        return lambda c, d, first: _unpack(words(c, pl.ds(pl.multiple_of((d * _LANES + first) >> 1, 8), rows // 2)))

    def member_sums(own, shared, m, rows, starts=None):
        moved = [jnp.where(m == h, (2 * _TAIL - h) * _HALF, 0) for h in range(_MEMBERS)]
        zero = [jnp.where(m == h, (_MEMBERS - h) * _HALF, 0) for h in range(_MEMBERS)]

        def source(c, d, high, first):
            first = high * _HALF + first
            if d >= _MEMBERS // 2:
                return own(c, d, first)
            return (own(c, d, first + moved[2 * d + high]).astype(jnp.float32)
                    - shared(c, d, first + zero[2 * d + high]).astype(jnp.float32))

        for i, p in enumerate(_scheme("member")):
            for high in range(2):
                for first in starts or range(0, _HALF, rows):
                    value = _weight_sum([(s, source(c, d, high, first)) for s, c, d in p.w_low])
                    yield i, high * _HALF + first, value, sum(1 + (d < 2) for _, _, d in p.w_low)

    def lay_out_heads(family, g, starts=None):
        sums = member_sums(head_pairs(qkv_stage.at[family]), head_pairs(qkv_shared.at[family]),
                           g, 16, starts)
        return _lay_out(sums, _tiles(w_ref, "member", family, g))

    def lay_out_shared_half(lay_out, words, rows, family, i):
        n = len(_scheme("shared")) // 2
        sums = _weight_sums(_scheme("shared")[:n], row_pairs(words, rows), range(0, _HALF, rows))
        return lay_out(sums, _tiles(w_ref, "shared", family).at[pl.ds(n * i, n)])

    def up_words(ref, first):
        return lambda c, rows: ref[c // 4, rows, lanes(first + c % 4)]

    def down_words(ref):
        return lambda c, rows: ref[2, rows, lanes(c)]

    def project_early(chunk, unit):
        at = lambda r, g, c: (pl.ds(8 * chunk + 4 * r, 4), unit[1], g, c)
        out = {}
        if unit[0] == "member":
            out = {(r, c): early_ref[at(r, _MEMBERS - 1, c)].reshape(2 * seg, _LANES)
                   for r in range(2) for c in range(_COLUMNS)}
        yield from _expand(chunks_ref.at[chunk], w_ref, unit, out)
        for (r, c), value in out.items():
            early_ref[at(r, unit[2] if unit[0] == "member" else _MEMBERS - 1, c)] = (
                value.reshape(4, seg // 2, _LANES))

    def load_chunk(chunk):
        pl.when(chunk == 1)(lambda: start(attention_copies(_WQ, 0) + shared_copies(1)))
        pl.when(chunk == 3)(lambda: start(attention_copies(_WK, 0)))
        wait([x_copy(chunk)])
        for family in (_WQ, _WK, _WV):
            sums = _weight_sums(_scheme("shared"), head_pairs(qkv_shared.at[family]), [16 * chunk])
            _run(_lay_out(sums, _tiles(w_ref, "shared", family)))
        x = x_stage[chunk].astype(jnp.float32)
        x = jnp.concatenate([x, x[_TAIL * _LANES:]], axis=0).T
        window(n_seg // _CHUNKS * chunk, n_seg // _CHUNKS)[...] = x
        half = lambda r: x[r * seg:r * seg + seg // 2]
        halves = [half(2 * e) for e in range(8)]
        halves[1] = jnp.where(chunk == 0, half(_LAG + 1), halves[1])
        _store_operands(chunks_ref.at[chunk], 0, [
            _layernorm(jnp.concatenate(part, axis=0)) for part in (halves[:4], halves[4:])])

    def project_shared(chunk):
        _run(_passes(_ORDER_SHARED, {
            "E": _chain(*(project_early(chunk, ("shared", f)) for f in (_WQ, _WK, _WV))),
            "L": lay_out_heads(_WQ, 0, [16 * chunk]),
            "O": lay_out_shared_half(
                _lay_out_transposed, lambda c, rows: wo_shared[c + 2 * (chunk % 2), rows, :],
                _HALF, _WO, chunk % 2)}))

    def load_group(g):
        more = g + 1 < _MEMBERS

        def arrive(family):
            if family == _WK:
                start(attention_copies(_WO, g))
                pl.when(more)(lambda: start(attention_copies(_WQ, g + 1)))
                pl.when(~more)(lambda: start(shared_copies(2)))
                wait(attention_copies(_WK, g))
            elif family == _WV:
                wait(attention_copies(_WV, g) + attention_copies(_WO, g))
                pl.when(more)(lambda: start(attention_copies(_WK, g + 1)))
                pl.when(~more)(lambda: start(ffn_copies(0)))
            else:
                pl.when(more)(lambda: wait(attention_copies(_WQ, g + 1)))
                pl.when(more)(lambda: start(attention_copies(_WV, g + 1)))
                pl.when(~more)(lambda: start(ffn_copies(1)))
            yield

        same = jnp.minimum(g, _MEMBERS - 1)
        wo_sums = member_sums(row_pairs(lambda c, rows: wo_stage[c, rows, :], _HALF),
                              row_pairs(lambda c, rows: wo_shared[c, rows, :], _HALF), g, _HALF)
        _run(_passes(_ORDER_LOAD, {
            **{f"E{f}": _chain(*(project_early(chunk, ("member", f, g)) for chunk in range(_CHUNKS)))
               for f in (_WQ, _WK, _WV)},
            **{f"W{f}": arrive(f) for f in (_WQ, _WK, _WV)},
            "L0": lay_out_heads(_WQ, jnp.minimum(g + 1, _MEMBERS - 1)),
            "L1": lay_out_heads(_WK, same), "L2": lay_out_heads(_WV, same),
            "L3": _lay_out_transposed(wo_sums, _tiles(w_ref, "member", _WO, same))}))

    def first_step(m):
        pl.when(m + 2 < _MEMBERS)(lambda: start(ffn_copies(m + 2)))
        pl.when(m + 2 == _MEMBERS)(lambda: start(ffn_copies(_MEMBERS, 4)))
        wait(ffn_copies(m))
        ref, stage = window(m, 2), ffn_stage.at[m % 3]
        up = [_lay_out(member_sums(row_pairs(up_words(stage, 4 * i), 32),
                                   row_pairs(up_words(ffn_shared, 4 * i), 32), m, 32),
                       _tiles(w_ref, "member", _UP + i, m)) for i in range(2)]
        shared = lay_out_shared_half(_lay_out, up_words(ffn_shared, 2 * m), 32, _UP + m // 2, m % 2)
        down = _lay_out_transposed(
            member_sums(row_pairs(down_words(stage), _HALF),
                        row_pairs(down_words(ffn_shared), _HALF), m, _HALF),
            _tiles(w_ref, "member", _DOWN, m))
        _run(_passes(_ORDER_FIRST, {
            "P": attention(_ORDER_SINGLE, ref, [0], {"X": prepare_full(ref, [1])}),
            "L": _passes("U*2+D", {"U": _chain(shared, *up), "D": down})}))

    def first_ffn():
        stage = ffn_stage.at[_MEMBERS % 3]
        down = lambda kind, ref, *family: _lay_out_transposed(
            _weight_sums(_scheme(kind), row_pairs(down_words(ref), _HALF), [0]),
            _tiles(w_ref, kind, *family))
        up = _lay_out(_weight_sums(_scheme("alone"), row_pairs(up_words(stage, 0), 32), [0, 32]),
                      _tiles(w_ref, "alone"))
        _run(_passes(_ORDER_FIRST_FFN, {
            "P": _passes(_ORDER_FFN, ffn_tasks(window(0, _LAG), [0, 2])),
            "L": _chain(up, down("narrow", stage), down("shared", ffn_shared, _DOWN))}))

    def last_steps():
        ref = window(n_seg - _LAG - 2, _LAG + 2)
        ffn = ffn_tasks(ref, [_LAG, 0])
        _run(prepare_full(ref, [2]),
             attention(_ORDER_EVEN_SINGLE, ref, [2], {**ffn, "X": prepare_full(ref, [3])}),
             attention(_ORDER_ODD_SINGLE, ref, [3], {**ffn, "X": prepare_full(ref, [4])}))

    def last_step(i):
        tile = n_out - 3 + i
        transpose_out(tile, window(_LANES // seg * tile, _LANES // seg)[...])
        ref = window(n_seg - 2 + i, 2)
        _run(attention(_ORDER_SINGLE, ref, [0], {"X": prepare_full(ref, [1])}))
        out_copy(tile).start()

    def last_ffn():
        _run(_passes(_ORDER_FFN, ffn_tasks(
            window(n_seg - _LAG, _LAG), [0, 2],
            lambda ys: transpose_out(n_out - 1, jnp.concatenate(ys, axis=0)))))

    mem_copy = pltpu.make_async_copy(mem0_hbm, mem0_ref, shared_sem.at[3])
    start([x_copy(0)] + shared_copies(0) + [x_copy(1)])
    behind = pl.ds(_MEMBERS * _HALF // 2, _HALF // 2)
    for spare in (window(-_LAG, _LAG), window(n_seg, 1), wo_shared.at[:, behind],
                  ffn_shared.at[:, behind], qkv_shared.at[:, :, pl.ds(_MEMBERS * _HALF, _HALF)]):
        spare[...] = jnp.zeros(spare.shape, spare.dtype)
    wait(shared_copies(0))
    start([x_copy(i) for i in range(2, _CHUNKS)] + [mem_copy])
    pl.loop(0, _CHUNKS)(load_chunk)
    mem_copy.wait()
    mem0 = mem0_ref[...].astype(jnp.float32)
    mem_ref[0, :n_mem] = mem_ref[1, :n_mem] = jnp.concatenate(
        [mem0, mem0[:, _TAIL * _LANES:]], axis=1)
    _run(prepare_full(window(0, 1), [0]))
    start(attention_copies(_WV, 0))
    wait(attention_copies(_WQ, 0) + shared_copies(1))
    pl.loop(0, _CHUNKS)(project_shared)
    pl.loop(0, _MEMBERS)(load_group)
    wait(shared_copies(2))
    pl.loop(0, _LAG)(first_step)
    wait(ffn_copies(_MEMBERS, 4))
    first_ffn()
    _run(prepare_short(window(0, _LAG + 1), _LAG, 0))
    pl.loop(0, 2)(double_step)
    pl.loop(1, (n_seg - _LAG) // 2)(two_steps)
    start([out_copy(i) for i in range(n_out - 3)])
    mem_ref[0, :n_mem] = mem_ref[1, :n_mem]
    last_steps()
    pl.loop(0, 2)(last_step)
    last_ffn()
    out_copy(n_out - 1).start()
    wait([out_copy(i) for i in range(n_out)])


@functools.partial(jax.jit, static_argnames=("A_seg_len",))
def pallas_interleave_layers__memory_aug_recurrent_mem_tr__glu_gated_swiglu__prompt_kernel(
    A_x: jax.Array,
    A_mem0: jax.Array,
    A_Wq: jax.Array,
    A_Wk: jax.Array,
    A_Wv: jax.Array,
    A_Wo: jax.Array,
    A_seg_len: int,
    B_x: jax.Array,
    B_w1: jax.Array,
    B_w3: jax.Array,
    B_w2: jax.Array,
):
    del B_x
    _, n_tok, d_model = A_x.shape
    n_mem = A_mem0.shape[1]
    _, n_heads, d_head = A_Wq.shape
    seg = A_seg_len
    assert A_x.shape[0] == 1 and _LAG * seg == _LANES and n_mem == 8
    assert n_tok == 16 * _CHUNKS * seg and d_model == _TAIL * _LANES + _HALF and d_head == _LANES
    assert n_heads == _MEMBERS * _COLUMNS and B_w1.shape[1] == (n_heads + 4) * _LANES
    n_operands = pl.cdiv(len(_operand_keys(False)), 8) * 8
    n_tiles = (_FAMILIES * (_MEMBERS * len(_scheme("member")) + len(_scheme("shared")))
               + len(_scheme("alone")) + len(_scheme("narrow")))
    shared_rows = (_MEMBERS + 1) * _HALF
    hbm = pl.BlockSpec(memory_space=pltpu.HBM)
    out_t = pl.pallas_call(
        functools.partial(_kernel, seg=seg),
        out_shape=jax.ShapeDtypeStruct((d_model, n_tok), A_x.dtype),
        in_specs=[hbm] * 9,
        out_specs=hbm,
        scratch_shapes=[
            pltpu.VMEM((n_tok // _LANES, d_model, _LANES), A_x.dtype),
            pltpu.VMEM((2, seg, d_model + _HALF), jnp.float32),
            pltpu.VMEM((n_operands, n_mem + seg, _LANES), jnp.float32),
            pltpu.VMEM((n_operands, seg, _LANES), jnp.bfloat16),
            pltpu.VMEM((_CHUNKS, n_operands, 2 * seg, _LANES), jnp.bfloat16),
            pltpu.VMEM((_MEMBERS + 4, _COLUMNS, 2 * (n_mem + seg), _LANES), jnp.float32),
            pltpu.VMEM((_MEMBERS + 4, _COLUMNS, 4 * seg, _LANES), jnp.float32),
            pltpu.VMEM((8 * _CHUNKS, 3, _MEMBERS, _COLUMNS, seg // 2, _LANES), jnp.float32),
            pltpu.VMEM((n_tiles, _LANES, _LANES), jnp.bfloat16),
            pltpu.VMEM((_CHUNKS, d_model, n_tok // _CHUNKS), A_x.dtype),
            pltpu.VMEM((3, _COLUMNS // 2, d_model, _LANES), jnp.uint32),
            pltpu.VMEM((3, _COLUMNS // 2, shared_rows, _LANES), jnp.uint32),
            pltpu.VMEM((_COLUMNS, d_model // 2, _LANES), jnp.uint32),
            pltpu.VMEM((_COLUMNS, shared_rows // 2, _LANES), jnp.uint32),
            pltpu.VMEM((3, 3, d_model // 2, _COLUMNS * _LANES), jnp.uint32),
            pltpu.VMEM((3, shared_rows // 2, _COLUMNS * _LANES), jnp.uint32),
            pltpu.VMEM((n_tok + 2 * _LAG * seg, d_model + _HALF), jnp.float32),
            pltpu.VMEM((n_mem, d_model), A_mem0.dtype),
            pltpu.SemaphoreType.DMA((_CHUNKS,)),
            pltpu.SemaphoreType.DMA((4,)),
            pltpu.SemaphoreType.DMA((9,)),
            pltpu.SemaphoreType.DMA((4,)),
            pltpu.SemaphoreType.DMA((n_tok // _LANES,)),
        ],
        compiler_params=pltpu.CompilerParams(
            vmem_limit_bytes=126 * 1024 * 1024, disable_bounds_checks=True,
            flags={"XLA_TPU_FORCE_LP_LLO_SCHEDULER": True}),
    )(A_x.reshape(n_tok, d_model).T, A_mem0.reshape(n_mem, d_model), A_Wq, A_Wk, A_Wv,
      A_Wo.transpose(0, 2, 1), B_w1, B_w3, B_w2.T)
    return out_t.T.reshape(A_x.shape)
```

```python
import functools
import math
from typing import NamedTuple

import jax
import jax.numpy as jnp
import jax.experimental.pallas as pl
import jax.experimental.pallas.tpu as pltpu

_EPS = 1e-05
_MASKED = -1000000000.0
_LOG2E = math.log2(math.e)
_LANES = 128
_HALF = _LANES // 2
_TAIL = 4
_COLUMNS = 8
_MEMBERS = 4
_WQ, _WK, _WV, _WO, _UP, _DOWN, _FAMILIES = 0, 1, 2, 3, 4, 6, 7
_LAG = 4
_CHUNKS = 4
_ORDER_EVEN = (
    "N X Q0 K0 G0*4+V0*4 Q1 G1*10+S0 K1 A0 V1 G2*6+S1 Q2 A1 K2 V2 G3*6+S2 Q3 A2 K3 V3 G4*6+S3 "
    "O0 A3+O1*6 G8 O2 O3 D4")
_ORDER_ODD = (
    "Q0 K0 V0*10+S0 G5 A0 G6 Q1 G7 K1 D0 V1*6+S1 D1 A1 D2 Q2 D3 F X K2 V2*6+S2 Q3 A2 K3 "
    "V3*6+S3 O0 O1 A3+O2*4 O3")
_ORDER_EVEN_SINGLE = (
    "Q0 N K0 V0*4+S0 Q1 K1 G0 A0 V1*4+S1 O0 G1 A1 Q2 K2 V2*4+S2 O1 G2 A2 Q3 K3 V3*4+S3 X O2 "
    "G3 A3 G8 O3 D4 G4")
_ORDER_ODD_SINGLE = (
    "Q0 K0 V0*4+S0 G5 A0 Q1 K1 V1*4+S1 G6 A1 Q2 K2 G7 V2*4+S2 D0 A2 Q3 K3 "
    "V3*4+S3 D1 D2 A3 D3 F X O0 O1 O2 O3")
_ORDER_DOUBLE = (
    "Q0 K0 Q1 K1 V0*10+S0 Q2 K2 V1*6+S1 A0 Q3 K3 V2 A1 O0*6+S2 V3 X O1*6+S3 A2 O2:30 A3 O2 O3")
_ORDER_SINGLE = (
    "Q0 K0 V0*4+S0 Q1 K1 A0 V1*4+S1 Q2 K2 A1 V2*4+S2 Q3 K3 A2 V3*4+S3 X O0 O1 A3 O2 O3")
_ORDER_FFN = "N G0 G1 G2 D0 G3 G4 D1 G5 G6 G7 G8 D2 D4 D3 F"
_ORDER_SHARED = "E+L*18"
_ORDER_LOAD = "W1 E0+L1*28+L4*5 W2 E1+L2*28+L3*12:208 E1 L2 W0 E2+L0*28+L3*12"
_ORDER_FIRST = "P:8 P+L*28"
_ORDER_FIRST_FFN = "P:20 P+L*15"


class _Pass(NamedTuple):
    low: tuple
    high: tuple
    w_low: tuple
    w_high: tuple
    wide: tuple
    common: bool = False


@functools.cache
def _scheme(kind, shift=0):
    x, y, n = 0, 1, 4 if kind in ("member", "alone") else 2
    a = lambda d: d % n + shift
    b = lambda d: d % n + shift + (2 if kind == "narrow" else 4)
    rest = lambda d: [e for e in range(4) if e != d and e // n == d // n]

    def whole(narrow, weight, wide):
        return _Pass(tuple(sorted(narrow)), tuple(sorted(narrow)), weight, weight, wide)

    def m1(d, e):
        return whole(((1, x, d), (1, y, e)), ((1, b(e), d), (1, a(d), e)),
                     ((1, y, a(d)), (1, x, b(e))))

    def m2(d, e):
        return whole(((1, y, d), (1, y, e)), ((1, b(e), d),), ((1, y, b(e)), (-1, y, a(d))))

    def m3(d):
        return whole(((1, x, d),), ((1, a(d), d), *((-1, a(d), e) for e in rest(d))),
                     ((1, x, a(d)), (1, y, a(d))))

    def m4(d):
        return whole(((1, y, d),), ((1, b(d), d), *((-1, b(d), e) for e in rest(d))),
                     ((1, y, b(d)), (1, x, b(d))))

    def m5(d, e):
        return whole(((1, x, d), (1, x, e)), ((1, a(d), e),), ((1, x, a(d)), (-1, x, b(e))))

    def m6(d):
        return whole(((1, y, d), (-1, x, d)), ((1, a(d), d), *((1, b(e), d) for e in rest(d))),
                     ((1, y, a(d)),))

    def m7(d):
        return whole(((1, y, d), (-1, x, d)), ((-1, b(d), d), *((-1, a(e), d) for e in rest(d))),
                     ((1, x, b(d)),))

    def with_tails(p, p_rows, p_columns, q, q_rows, q_columns):
        tail = lambda columns: tuple((1, c, _TAIL) for c in columns)
        return [_Pass(p.low, p.high, q.w_low, p.w_high, p.wide + q.wide, common=True),
                _Pass(p.low, ((1, p_rows, _TAIL),), p.w_low, tail(p_columns), p.wide),
                _Pass(((1, q_rows, _TAIL),), q.high, tail(q_columns), q.w_high, q.wide)]

    def pair_with_tails(d, e):
        return [*with_tails(m5(d, e), x, [a(d)], m5(e, d), x, [a(e)]), m3(d),
                *with_tails(m2(d, e), y, [b(e)], m2(e, d), y, [b(d)]), m3(e),
                *with_tails(m6(d), y, [a(d), b(e)], m7(d), x, [b(d), a(e)]), m1(d, e), m4(d),
                *with_tails(m7(e), x, [b(e), a(d)], m6(e), y, [a(e), b(d)]), m1(e, d), m4(e)]

    edge = lambda d, e: [m5(d, e), m1(d, e), m2(d, e)]
    pair = lambda d, e: [m3(d), m6(d), *edge(d, e), m7(e), m4(e),
                         m3(e), m6(e), *edge(e, d), m7(d), m4(d)]
    if kind == "shared":
        return (*pair(0, 1), *(() if shift else _scheme(kind, 2)))
    if kind == "narrow":
        return (*pair_with_tails(0, 1), *pair(2, 3))
    ends = pair if kind == "member" else pair_with_tails
    return (*ends(0, 1), *edge(0, 2), *edge(0, 3), *edge(1, 2), *edge(1, 3),
            *edge(2, 0), *edge(3, 0), *edge(2, 1), *edge(3, 1), *ends(2, 3))


def _selected(kind, single):
    for i, p in enumerate(_scheme(kind)):
        if single:
            narrow = tuple((s, 0, d) for s, _, d in p.low)
            p = p._replace(low=narrow, high=narrow,
                           wide=tuple((s, 0, c) for s, r, c in p.wide if r == c // 4))
        if p.wide:
            yield i, p


def _tiles(w_ref, kind, family=_FAMILIES, member=_MEMBERS):
    size = lambda name: len(_scheme(name))
    first = family * (_MEMBERS * size("member") + size("shared"))
    if kind in ("member", "shared"):
        first += member * size("member")
    return w_ref.at[pl.ds(first + (size("alone") if kind == "narrow" else 0), size(kind))]


def _tail_for(terms, block):
    return tuple(sorted((s, r, _TAIL if d == block else d) for s, r, d in terms))


@functools.cache
def _operand_keys(single):
    return tuple(dict.fromkeys(_tail_for(p.low, block) for block in (None, 0, 1)
                               for _, p in _selected("member", single)))


def _signed_sum(terms):
    terms = sorted(terms, key=lambda t: -t[0])
    total = terms[0][1] if terms[0][0] > 0 else -terms[0][1]
    for sign, value in terms[1:]:
        total = total + value if sign > 0 else total - value
    return total


def _accumulate(sums, key, sign, value):
    if key not in sums:
        sums[key] = (sign, value)
    elif sums[key][0] == sign:
        sums[key] = (sign, sums[key][1] + value)
    else:
        sums[key] = (1, value - sums[key][1] if sign > 0 else sums[key][1] - value)


def _words(ref):
    return ref.bitcast(jnp.uint32) if ref.dtype == jnp.bfloat16 else ref


def _unpack(words):
    return pltpu.bitcast(words, jnp.bfloat16) if words.dtype == jnp.uint32 else words


def _store(ref, i, first, value):
    rows = value.shape[0]
    if value.dtype == jnp.bfloat16:
        _words(ref)[i, pl.ds(first // 2, rows // 2), :] = pltpu.bitcast(value, jnp.uint32)
    else:
        ref[i, pl.ds(first, rows), :] = value.astype(ref.dtype)


def _lane_half(rows):
    return jax.lax.broadcasted_iota(jnp.int32, (rows, _LANES), 1) // _HALF


def _blocks(x):
    return [x[:, d * _LANES:(d + 1) * _LANES] for d in range(_TAIL + 1)]


def _store_operands(ref, first, row_blocks):
    blocks = [_blocks(x) for x in row_blocks]
    for i, terms in enumerate(_operand_keys(len(row_blocks) == 1)):
        _store(ref, i, first, _signed_sum([(s, blocks[r][d]) for s, r, d in terms]))


def _dot(a, b):
    return jnp.dot(a, b, preferred_element_type=jnp.float32)


def _expand(operands_ref, w_ref, unit, out, single=False):
    operands_ref, tiles_ref = _words(operands_ref), _words(_tiles(w_ref, *unit))
    operand = lambda terms: operands_ref[_operand_keys(single).index(terms)]
    half = _lane_half(operands_ref.shape[1])
    freed = {}
    if unit[0] == "member":
        blocks = [unit[2] // 2] if isinstance(unit[2], int) else range(_MEMBERS // 2)
        freed = {d: half == unit[2] - 2 * d for d in blocks}
    sums, common = {key: (1, value) for key, value in out.items()}, []
    for i, p in _selected(unit[0], single):
        lhs = operand(p.low)
        if p.high != p.low:
            lhs = jnp.where(half == 0, lhs, operand(p.high))
        for d, lanes in freed.items():
            if _tail_for(p.low, d) != p.low:
                lhs = jnp.where(lanes, operand(_tail_for(p.low, d)), lhs)
        product = _dot(_unpack(lhs), _unpack(tiles_ref[i]))
        if p.common:
            common = [product, product]
        else:
            if common:
                product = product + common.pop()
            for s, r, c in p.wide:
                _accumulate(sums, (r, c), s, product)
        yield
    assert all(sign > 0 for sign, _ in sums.values())
    out.update({key: value for key, (_, value) in sums.items()})


def _contract(load, w_ref, unit, sums, single=False):
    tiles_ref = _words(_tiles(w_ref, *unit))
    freed = unit[2] // 2 if unit[0] == "member" else None
    held, mixed = [], {}
    for i, p in _selected(unit[0], single):
        product = _dot(_signed_sum([(s, load(r, c)) for s, r, c in p.wide]),
                       _unpack(tiles_ref[i]))
        if p.common or held:
            held.append((p, product))
        if len(held) == 3:
            (p, common), (p1, first), (p2, second) = held
            held = []
            product = common + jnp.where(_lane_half(common.shape[0]) == 0, first, second)
            _accumulate(sums, (p1.high[0][1], _TAIL, 1), 1, first)
            _accumulate(sums, (p2.low[0][1], _TAIL, 0), 1, second)
        if not held:
            for s, r, d in p.low:
                _accumulate(mixed if d == freed else sums, (r, d), s, product)
        yield
    for (r, d), (s, both) in mixed.items():
        _accumulate(sums, (r, _TAIL, unit[2] % 2), s, both)
        _accumulate(sums, (r, d), s, jnp.where(_lane_half(both.shape[0]) == unit[2] % 2, 0.0, both))


def _residual(row_blocks):
    return {(r, d) if d < _TAIL else (r, d, 0): (1, block)
            for r, x in enumerate(row_blocks) for d, block in enumerate(_blocks(x))}


def _contracted(sums, r):
    assert all(sign > 0 for sign, _ in sums.values())
    low, high = sums[r, _TAIL, 0][1], sums[r, _TAIL, 1][1]
    tail = jnp.where(_lane_half(low.shape[0]) == 0, low, high)
    tail = tail + pltpu.roll(tail, _HALF, 1)
    return jnp.concatenate([sums[r, d][1] for d in range(_TAIL)] + [tail], axis=1)


def _weight_sum(parts):
    return _signed_sum([(s, part.astype(jnp.float32) if len(parts) > 1 else part)
                        for s, part in parts])


def _weight_sums(passes, source, starts):
    for i, p in enumerate(passes):
        for high in range(2):
            if i > high and passes[i - 1 - high].common:
                continue
            for at in starts:
                first = high * _HALF + at
                total = lambda terms: _weight_sum(
                    [(s, source(c, d, at if d == _TAIL else first)) for s, c, d in terms])
                terms = (p.w_low, p.w_high)[high]
                value = total(terms)
                yield i, first, value, len(terms)
                if p.common:
                    other = passes[i + 1 + high]
                    other = total((other.w_low, other.w_high)[high]).astype(jnp.float32)
                    yield i + 1 + high, first, other - value.astype(jnp.float32), len(terms) + 1


def _lay_out(sums, tiles_ref):
    for i, first, value, terms in sums:
        _store(tiles_ref, i, pl.multiple_of(first, 16), value)
        yield from range((4 * terms + 1) * value.shape[0] // 16)


def _lay_out_transposed(sums, tiles_ref):
    halves, pending = {}, []
    for i, first, value, terms in sums:
        halves[i, first] = value
        if (i, _HALF - first) in halves:
            pair = [halves[i, 0], halves[i, _HALF]]
            if pair[0].dtype != pair[1].dtype:
                pair = [half.astype(jnp.float32) for half in pair]
            pending.append((i, jnp.concatenate(pair, axis=0).astype(jnp.bfloat16).T))
        if len(pending) > 2:
            _store(tiles_ref, pending[0][0], 0, pending.pop(0)[1])
        yield from range(8 * terms + 22)
    for i, tile in pending:
        _store(tiles_ref, i, 0, tile)


def _layernorm(x):
    low_lanes = _lane_half(x.shape[0]) == 0

    def mean(v):
        *full, tail = _blocks(v)
        total = functools.reduce(jnp.add, full) + jnp.where(low_lanes, tail, 0.0)
        return jnp.sum(total, axis=-1, keepdims=True) / (_TAIL * _LANES + _HALF)

    d = x - mean(x)
    return d * jax.lax.rsqrt(mean(d * d) + _EPS)


def _silu(x):
    half = 0.5 * x
    return half + half * jnp.tanh(half)


def _reciprocal(x):
    r = pl.reciprocal(x, approx=True)
    return r * (2.0 - x * r)


def _attention_masks(n_layers, rows, n_mem):
    i = jax.lax.broadcasted_iota(jnp.int32, (n_layers * rows, n_layers * rows), 0)
    j = jax.lax.broadcasted_iota(jnp.int32, (n_layers * rows, n_layers * rows), 1)
    if n_layers == 1:
        return (i < n_mem) | (i >= j), _MASKED * _LOG2E
    same = (i >= rows) == (j >= rows)
    visible = (i < n_mem) | ((i >= rows) & (i < rows + n_mem)) | (i >= j)
    fill = jnp.where(same, _MASKED * _LOG2E, -jnp.inf).astype(jnp.float32)
    return same & visible, fill


def _expand_member(operands_ref, w_ref, family, member, shared_ref, out, single=False):
    rows = operands_ref.shape[1]
    if member == 0:
        yield from _expand(operands_ref, w_ref, ("shared", family), out, single)
        for (r, c), value in out.items():
            shared_ref[c, r * rows:(r + 1) * rows, :] = value
    out.update({(r, c): shared_ref[c, r * rows:(r + 1) * rows, :]
                for r in range(1 if single else 2) for c in range(_COLUMNS)})
    yield from _expand(operands_ref, w_ref, ("member", family, member), out, single)


def _store_wide(ref, member, c, rows, value):
    ref[member, c, rows, :] = value
    if member == _MEMBERS - 1:
        ref[_MEMBERS, c, rows, :] = functools.reduce(
            jnp.add, [ref[m, c, rows, :] for m in range(member)] + [value])


def _contract_member(ref, w_ref, family, member, sums, single=False):
    rows = ref.shape[2] // 2
    load = lambda m: lambda r, c: ref[m, c, r * rows:(r + 1) * rows, :]
    yield from _contract(load(member), w_ref, ("member", family, member), sums, single)
    if member == _MEMBERS - 1:
        yield from _contract(load(_MEMBERS), w_ref, ("shared", family), sums, single)


def _attention_tasks(xs, operands_ref, w_ref, wide_ref, outs, known=None):
    n_layers, rows = len(xs), wide_ref.shape[2] // 2
    single, n_mem = n_layers == 1, rows - xs[0].shape[0]
    visible, fill = _attention_masks(n_layers, rows, n_mem)
    scale = _LANES ** -0.5 * _LOG2E
    qkv, probs = {}, {}
    sums = _residual([jnp.concatenate([jnp.zeros_like(x[:n_mem]), x], axis=0) for x in xs])

    def stacked(family, g, h):
        parts = [qkv[family, g][r, h] for r in range(n_layers)]
        if known:
            (x, y), moved = parts, (rows + n_mem) // 2
            parts = [x[:n_mem], known(family, g, h), x[n_mem:moved], y, x[moved:]]
        value = jnp.concatenate(parts, axis=0)
        return value if single and family == _WQ else value.astype(jnp.bfloat16)

    def project(family, g):
        qkv[family, g] = {}
        return _expand_member(operands_ref, w_ref, family, g, wide_ref.at[_MEMBERS + 1 + family],
                              qkv[family, g], single)

    def scores(g):
        for h in range(_COLUMNS):
            s = jax.lax.dot_general(stacked(_WQ, g, h), stacked(_WK, g, h),
                                    (((1,), (1,)), ((), ())), preferred_element_type=jnp.float32)
            s = jnp.where(visible, s * scale, fill)
            p = jnp.exp2(s - jnp.max(s, axis=-1, keepdims=True))
            p = p * _reciprocal(jnp.sum(p, axis=-1, keepdims=True))
            probs[g, h] = p if single else p.astype(jnp.bfloat16)
            yield

    def values(g):
        for h in range(_COLUMNS):
            _store_wide(wide_ref, g, h, slice(0, n_layers * rows),
                        _dot(probs[g, h], stacked(_WV, g, h)))
            yield

    def output(g):
        yield from _contract_member(wide_ref, w_ref, _WO, g, sums, single)
        if g == _MEMBERS - 1:
            outs.extend(_contracted(sums, r) for r in range(n_layers))

    tasks = {}
    for g in range(_MEMBERS):
        tasks.update({f"Q{g}": project(_WQ, g), f"K{g}": project(_WK, g), f"V{g}": project(_WV, g),
                      f"S{g}": scores(g), f"A{g}": values(g), f"O{g}": output(g)})
    return tasks


def _ffn_tasks(xs, operands_ref, w_ref, wide_ref, result):
    rows = operands_ref.shape[1]
    sums = _residual(xs)

    def gated(member, i):
        both = {}
        if member < _MEMBERS:
            yield from _expand_member(operands_ref, w_ref, _UP + i, member,
                                      wide_ref.at[_MEMBERS + 2 + i], both)
        else:
            yield from _expand(operands_ref, w_ref, ("alone",), both)
        for c in range(4):
            for r in range(2):
                _store_wide(wide_ref, member + member // _MEMBERS, 4 * i + c,
                            slice(r * rows, (r + 1) * rows), _silu(both[r, c]) * both[r, 4 + c])

    def finish():
        result([_contracted(sums, r) for r in range(2)])
        yield

    return {"F": finish(), **{f"G{u}": gated(*divmod(u, 2)) for u in range(2 * _MEMBERS + 1)},
            **{f"D{m}": _contract_member(wide_ref, w_ref, _DOWN, m, sums) for m in range(_MEMBERS)},
            "D4": _contract(lambda r, c: wide_ref[_MEMBERS + 1, c, r * rows:(r + 1) * rows, :],
                            w_ref, ("narrow",), sums)}


def _passes(order, tasks):
    done = object()
    for item in order.split():
        names, _, turns = item.partition(":")
        running = [(tasks[name], int(count or 1))
                   for name, _, count in (part.partition("*") for part in names.split("+"))]
        turn = 0
        while running and (not turns or turn < int(turns)):
            for task, count in tuple(running):
                for _ in range(count):
                    if next(task, done) is done:
                        running.remove((task, count))
                        break
                    yield
            turn += 1


def _chain(*tasks):
    for task in tasks:
        yield from task


def _run(*tasks):
    for _ in _chain(*tasks):
        pass


def _kernel(xt_hbm, mem0_hbm, wq_hbm, wk_hbm, wv_hbm, wot_hbm, w1_hbm, w3_hbm, w2t_hbm,
            outt_hbm, out_ref, mem_ref, full_ref, short_ref, chunks_ref, heads_ref, hidden_ref,
            early_ref, w_ref, x_stage, qkv_stage, qkv_shared, wo_stage, wo_shared, ffn_stage,
            ffn_shared, res_ref, mem0_ref, x_sem, attention_sem, ffn_sem, shared_sem, out_sem,
            *, seg):
    d_model, n_tok = xt_hbm.shape
    n_mem = mem0_hbm.shape[0]
    n_seg = n_tok // seg
    n_out = n_tok // _LANES

    def window(r, n):
        return res_ref.at[pl.ds(pl.multiple_of((r + _LAG) * seg, seg), n * seg)]

    def block(r, n=1):
        return pl.ds(r * seg, n * seg)

    def lanes(i, n=1):
        return pl.ds(pl.multiple_of(i * _LANES, _LANES), n * _LANES)

    def transpose_out(i, x):
        out_ref[i] = x.T[:d_model].astype(out_ref.dtype)

    def prepare(ref, blocks, total, operands_ref, first):
        rows = 32 // operands_ref.dtype.itemsize
        for i in range(0, total, rows):
            _store_operands(operands_ref, first + i,
                            [_layernorm(ref[pl.ds(r * seg + i, rows), :]) for r in blocks])
        yield

    def prepare_full(ref, blocks):
        return prepare(ref, blocks, seg, full_ref, n_mem)

    def prepare_short(ref, first, second):
        x = _layernorm(ref[pl.ds(first * seg + seg // 2, seg // 2), :])
        y = _layernorm(ref[block(second), :])
        mem_ref[0, n_mem:] = jnp.concatenate([x, y[seg - n_mem:]], axis=0)
        mem_ref[1, n_mem:] = y[:seg - n_mem]
        yield

    def attention(order, ref, blocks, others, early=None):
        xs, outs = [ref[block(r), :] for r in blocks], []
        operands_ref = full_ref if early is None else short_ref
        _store_operands(operands_ref, 0, [
            mem_ref[i, :n_mem if early is None else seg] for i in range(len(blocks))])
        known = None if early is None else lambda *at: early_ref[(early, *at)]
        tasks = _attention_tasks(xs, operands_ref, w_ref, heads_ref, outs, known)
        yield from _passes(order, {**others, **tasks})
        for i, r in enumerate(blocks):
            mem_ref[i, :n_mem] = outs[i][:n_mem]
            ref[block(r), :] = outs[i][n_mem:]

    def ffn_tasks(ref, blocks, result=None):
        def update(ys):
            for r, y in zip(blocks, ys):
                ref[block(r, 2), :] = y

        return {"N": prepare(ref, blocks, 2 * seg, chunks_ref.at[0], 0), **_ffn_tasks(
            [ref[block(r, 2), :] for r in blocks], chunks_ref.at[0], w_ref, hidden_ref,
            result or update)}

    def double_step(b):
        ref = window(b, _LAG + 2)
        _run(attention(_ORDER_DOUBLE, ref, [_LAG, 0],
                       {"X": prepare_short(ref, _LAG + 1, 1)}, _LAG // 2 - b))

    def two_steps(j):
        b = 6
        ref = window(2 * j - b, b + _LAG + 3)
        transpose_out(jnp.where((j % 2 == 1) & (j > 1), (j - 3) // 2, n_out - 1),
                      ref[block(0, 4), :])
        ffn = ffn_tasks(ref, [b + 2, b - 2])
        _run(attention(_ORDER_EVEN, ref, [b + _LAG, b],
                       {**ffn, "X": prepare_full(ref, [b + _LAG + 1, b + 1])}, j + _LAG // 2),
             attention(_ORDER_ODD, ref, [b + _LAG + 1, b + 1],
                       {**ffn, "X": prepare_short(ref, b + _LAG + 2, b + 2)}))

    qkv_words = [_words(w) for w in (wq_hbm, wk_hbm, wv_hbm)]
    ffn_words = [_words(w) for w in (w1_hbm, w3_hbm, w2t_hbm)]
    pairs = _COLUMNS // 2

    def attention_copies(family, g):
        sem = attention_sem.at[family]
        if family == _WO:
            heads = _words(wot_hbm).at[pl.ds(_COLUMNS * g, _COLUMNS)]
            return [pltpu.make_async_copy(heads, wo_stage, sem)]
        return [pltpu.make_async_copy(qkv_words[family].at[:, pairs * g + p, :],
                                      qkv_stage.at[family, p], sem) for p in range(pairs)]

    def ffn_copies(m, columns=_COLUMNS):
        return [pltpu.make_async_copy(w.at[:, lanes(_COLUMNS * m, columns)],
                                      ffn_stage.at[m % 3, i, :, lanes(0, columns)],
                                      ffn_sem.at[3 * (m % 3) + i])
                for i, w in enumerate(ffn_words)]

    def shared_copies(which):
        ends = []
        for m in range(_MEMBERS):
            rows, words = pl.ds(m * _HALF, _HALF), pl.ds(m * _HALF // 2, _HALF // 2)
            if which == 0:
                ends += [(w.at[rows, pairs * m + p, :], qkv_shared.at[i, p, rows])
                         for i, w in enumerate(qkv_words) for p in range(pairs)]
            elif which == 1:
                ends += [(_words(wot_hbm).at[pl.ds(_COLUMNS * m, _COLUMNS), words],
                          wo_shared.at[:, words])]
            else:
                ends += [(w.at[words, lanes(_COLUMNS * m, _COLUMNS)], ffn_shared.at[i, words])
                         for i, w in enumerate(ffn_words)]
        return [pltpu.make_async_copy(*pair, shared_sem.at[which]) for pair in ends]

    def x_copy(chunk):
        columns = lanes(n_out // _CHUNKS * chunk, n_out // _CHUNKS)
        return pltpu.make_async_copy(xt_hbm.at[:, columns], x_stage.at[chunk], x_sem.at[chunk])

    def out_copy(i):
        return pltpu.make_async_copy(out_ref.at[i], outt_hbm.at[:, lanes(i)], out_sem.at[i])

    def start(copies):
        for c in copies:
            c.start()

    def wait(copies):
        for c in copies:
            c.wait()

    def head_pairs(ref):
        def source(c, d, first):
            words = ref[c // 2, pl.ds(pl.multiple_of(d * _LANES + first, 16), 16), :]
            words = words & jnp.uint32(0xFFFF0000) if c % 2 else words << 16
            return pltpu.bitcast(words, jnp.float32)
        return source

    def row_pairs(words, rows):
        return lambda c, d, first: _unpack(words(c, pl.ds(pl.multiple_of((d * _LANES + first) >> 1, 8), rows // 2)))

    def member_sums(own, shared, m, rows, starts=None):
        moved = [jnp.where(m == h, (2 * _TAIL - h) * _HALF, 0) for h in range(_MEMBERS)]
        zero = [jnp.where(m == h, (_MEMBERS - h) * _HALF, 0) for h in range(_MEMBERS)]

        def source(c, d, high, first):
            first = high * _HALF + first
            if d >= _MEMBERS // 2:
                return own(c, d, first)
            return (own(c, d, first + moved[2 * d + high]).astype(jnp.float32)
                    - shared(c, d, first + zero[2 * d + high]).astype(jnp.float32))

        for i, p in enumerate(_scheme("member")):
            for high in range(2):
                for first in starts or range(0, _HALF, rows):
                    value = _weight_sum([(s, source(c, d, high, first)) for s, c, d in p.w_low])
                    yield i, high * _HALF + first, value, sum(1 + (d < 2) for _, _, d in p.w_low)

    def lay_out_heads(family, g, starts=None):
        sums = member_sums(head_pairs(qkv_stage.at[family]), head_pairs(qkv_shared.at[family]),
                           g, 16, starts)
        return _lay_out(sums, _tiles(w_ref, "member", family, g))

    def lay_out_shared_half(lay_out, words, rows, family, i):
        n = len(_scheme("shared")) // 2
        sums = _weight_sums(_scheme("shared")[:n], row_pairs(words, rows), range(0, _HALF, rows))
        return lay_out(sums, _tiles(w_ref, "shared", family).at[pl.ds(n * i, n)])

    def up_words(ref, first):
        return lambda c, rows: ref[c // 4, rows, lanes(first + c % 4)]

    def down_words(ref):
        return lambda c, rows: ref[2, rows, lanes(c)]

    def project_early(chunk, unit):
        at = lambda r, g, c: (pl.ds(8 * chunk + 4 * r, 4), unit[1], g, c)
        out = {}
        if unit[0] == "member":
            out = {(r, c): early_ref[at(r, _MEMBERS - 1, c)].reshape(2 * seg, _LANES)
                   for r in range(2) for c in range(_COLUMNS)}
        yield from _expand(chunks_ref.at[chunk], w_ref, unit, out)
        for (r, c), value in out.items():
            early_ref[at(r, unit[2] if unit[0] == "member" else _MEMBERS - 1, c)] = (
                value.reshape(4, seg // 2, _LANES))

    def load_chunk(chunk):
        pl.when(chunk == 1)(lambda: start(attention_copies(_WQ, 0)))
        wait([x_copy(chunk)])
        for family in (_WQ, _WK, _WV):
            sums = _weight_sums(_scheme("shared"), head_pairs(qkv_shared.at[family]), [16 * chunk])
            _run(_lay_out(sums, _tiles(w_ref, "shared", family)))
        x = x_stage[chunk].astype(jnp.float32)
        x = jnp.concatenate([x, x[_TAIL * _LANES:]], axis=0).T
        window(n_seg // _CHUNKS * chunk, n_seg // _CHUNKS)[...] = x
        half = lambda r: x[r * seg:r * seg + seg // 2]
        halves = [half(2 * e) for e in range(8)]
        halves[1] = jnp.where(chunk == 0, half(_LAG + 1), halves[1])
        _store_operands(chunks_ref.at[chunk], 0, [
            _layernorm(jnp.concatenate(part, axis=0)) for part in (halves[:4], halves[4:])])

    def project_shared(chunk):
        _run(_passes(_ORDER_SHARED, {
            "E": _chain(*(project_early(chunk, ("shared", f)) for f in (_WQ, _WK, _WV))),
            "L": lay_out_heads(_WQ, 0, [16 * chunk])}))

    def load_group(g):
        more = g + 1 < _MEMBERS

        def arrive(family):
            if family == _WK:
                start(attention_copies(_WO, g))
                pl.when(more)(lambda: start(attention_copies(_WQ, g + 1)))
                pl.when(~more)(lambda: start(ffn_copies(0)))
                wait(attention_copies(_WK, g))
            elif family == _WV:
                wait(attention_copies(_WV, g) + attention_copies(_WO, g))
                pl.when(more)(lambda: start(attention_copies(_WK, g + 1)))
                pl.when(~more)(lambda: start(ffn_copies(1)))
            else:
                pl.when(more)(lambda: wait(attention_copies(_WQ, g + 1)))
                pl.when(more)(lambda: start(attention_copies(_WV, g + 1)))
                pl.when(g == 1)(lambda: start(shared_copies(2)))
            yield

        same = jnp.minimum(g, _MEMBERS - 1)
        wo_sums = member_sums(row_pairs(lambda c, rows: wo_stage[c, rows, :], _HALF),
                              row_pairs(lambda c, rows: wo_shared[c, rows, :], _HALF), g, _HALF)
        _run(_passes(_ORDER_LOAD, {
            **{f"E{f}": _chain(*(project_early(chunk, ("member", f, g)) for chunk in range(_CHUNKS)))
               for f in (_WQ, _WK, _WV)},
            **{f"W{f}": arrive(f) for f in (_WQ, _WK, _WV)},
            "L0": lay_out_heads(_WQ, jnp.minimum(g + 1, _MEMBERS - 1)),
            "L1": lay_out_heads(_WK, same), "L2": lay_out_heads(_WV, same),
            "L3": _lay_out_transposed(wo_sums, _tiles(w_ref, "member", _WO, same)),
            "L4": lay_out_shared_half(
                _lay_out_transposed, lambda c, rows: wo_shared[c + 2 * (g % 2), rows, :], _HALF,
                _WO, g % 2)}))

    def first_step(m):
        pl.when(m + 2 < _MEMBERS)(lambda: start(ffn_copies(m + 2)))
        pl.when(m + 2 == _MEMBERS)(lambda: start(ffn_copies(_MEMBERS, 4)))
        wait(ffn_copies(m))
        ref, stage = window(m, 2), ffn_stage.at[m % 3]
        up = [_lay_out(member_sums(row_pairs(up_words(stage, 4 * i), 32),
                                   row_pairs(up_words(ffn_shared, 4 * i), 32), m, 32),
                       _tiles(w_ref, "member", _UP + i, m)) for i in range(2)]
        shared = lay_out_shared_half(_lay_out, up_words(ffn_shared, 2 * m), 32, _UP + m // 2, m % 2)
        down = _lay_out_transposed(
            member_sums(row_pairs(down_words(stage), _HALF),
                        row_pairs(down_words(ffn_shared), _HALF), m, _HALF),
            _tiles(w_ref, "member", _DOWN, m))
        _run(_passes(_ORDER_FIRST, {
            "P": attention(_ORDER_SINGLE, ref, [0], {"X": prepare_full(ref, [1])}),
            "L": _passes("U*2+D", {"U": _chain(shared, *up), "D": down})}))

    def first_ffn():
        stage = ffn_stage.at[_MEMBERS % 3]
        down = lambda kind, ref, *family: _lay_out_transposed(
            _weight_sums(_scheme(kind), row_pairs(down_words(ref), _HALF), [0]),
            _tiles(w_ref, kind, *family))
        up = _lay_out(_weight_sums(_scheme("alone"), row_pairs(up_words(stage, 0), 32), [0, 32]),
                      _tiles(w_ref, "alone"))
        _run(_passes(_ORDER_FIRST_FFN, {
            "P": _passes(_ORDER_FFN, ffn_tasks(window(0, _LAG), [0, 2])),
            "L": _chain(up, down("narrow", stage), down("shared", ffn_shared, _DOWN))}))

    def last_steps():
        ref = window(n_seg - _LAG - 2, _LAG + 2)
        ffn = ffn_tasks(ref, [_LAG, 0])
        _run(prepare_full(ref, [2]),
             attention(_ORDER_EVEN_SINGLE, ref, [2], {**ffn, "X": prepare_full(ref, [3])}),
             attention(_ORDER_ODD_SINGLE, ref, [3], {**ffn, "X": prepare_full(ref, [4])}))

    def last_step(i):
        tile = n_out - 3 + i
        transpose_out(tile, window(_LANES // seg * tile, _LANES // seg)[...])
        ref = window(n_seg - 2 + i, 2)
        _run(attention(_ORDER_SINGLE, ref, [0], {"X": prepare_full(ref, [1])}))
        out_copy(tile).start()

    def last_ffn():
        _run(_passes(_ORDER_FFN, ffn_tasks(
            window(n_seg - _LAG, _LAG), [0, 2],
            lambda ys: transpose_out(n_out - 1, jnp.concatenate(ys, axis=0)))))

    mem_copy = pltpu.make_async_copy(mem0_hbm, mem0_ref.at[0], shared_sem.at[3])
    start([x_copy(0)] + shared_copies(0) + [x_copy(1)])
    behind = pl.ds(_MEMBERS * _HALF // 2, _HALF // 2)
    for spare in (window(-_LAG, _LAG), window(n_seg, 1), wo_shared.at[:, behind],
                  ffn_shared.at[:, behind], qkv_shared.at[:, :, pl.ds(_MEMBERS * _HALF, _HALF)]):
        spare[...] = jnp.zeros(spare.shape, spare.dtype)
    wait(shared_copies(0))
    start([x_copy(i) for i in range(2, _CHUNKS)] + [mem_copy])
    pl.loop(0, _CHUNKS)(load_chunk)
    mem_copy.wait()
    mem0 = mem0_ref[0].astype(jnp.float32)
    mem_ref[0, :n_mem] = mem_ref[1, :n_mem] = jnp.concatenate(
        [mem0, mem0[:, _TAIL * _LANES:]], axis=1)
    _run(prepare_full(window(0, 1), [0]))
    start(shared_copies(1) + attention_copies(_WK, 0))
    wait(attention_copies(_WQ, 0))
    start(attention_copies(_WV, 0))
    pl.loop(0, _CHUNKS)(project_shared)
    wait(shared_copies(1))
    pl.loop(0, _MEMBERS)(load_group)
    wait(shared_copies(2))
    pl.loop(0, _LAG)(first_step)
    wait(ffn_copies(_MEMBERS, 4))
    first_ffn()
    _run(prepare_short(window(0, _LAG + 1), _LAG, 0))
    pl.loop(0, 2)(double_step)
    pl.loop(1, (n_seg - _LAG) // 2)(two_steps)
    start([out_copy(i) for i in range(n_out - 3)])
    mem_ref[0, :n_mem] = mem_ref[1, :n_mem]
    last_steps()
    pl.loop(0, 2)(last_step)
    last_ffn()
    out_copy(n_out - 1).start()
    wait([out_copy(i) for i in range(n_out)])


@functools.partial(jax.jit, static_argnames=("A_seg_len",))
def pallas_interleave_layers__memory_aug_recurrent_mem_tr__glu_gated_swiglu__prompt_kernel(
    A_x: jax.Array,
    A_mem0: jax.Array,
    A_Wq: jax.Array,
    A_Wk: jax.Array,
    A_Wv: jax.Array,
    A_Wo: jax.Array,
    A_seg_len: int,
    B_x: jax.Array,
    B_w1: jax.Array,
    B_w3: jax.Array,
    B_w2: jax.Array,
):
    del B_x
    _, n_tok, d_model = A_x.shape
    n_mem = A_mem0.shape[1]
    _, n_heads, d_head = A_Wq.shape
    seg = A_seg_len
    assert A_x.shape[0] == 1 and _LAG * seg == _LANES and n_mem == 8
    assert n_tok == 16 * _CHUNKS * seg and d_model == _TAIL * _LANES + _HALF and d_head == _LANES
    assert n_heads == _MEMBERS * _COLUMNS and B_w1.shape[1] == (n_heads + 4) * _LANES
    n_operands = pl.cdiv(len(_operand_keys(False)), 8) * 8
    n_tiles = (_FAMILIES * (_MEMBERS * len(_scheme("member")) + len(_scheme("shared")))
               + len(_scheme("alone")) + len(_scheme("narrow")))
    shared_rows = (_MEMBERS + 1) * _HALF
    hbm = pl.BlockSpec(memory_space=pltpu.HBM)
    out_t = pl.pallas_call(
        functools.partial(_kernel, seg=seg),
        out_shape=jax.ShapeDtypeStruct((d_model, n_tok), A_x.dtype),
        in_specs=[hbm] * 9,
        out_specs=hbm,
        scratch_shapes=[
            pltpu.VMEM((n_tok // _LANES, d_model, _LANES), A_x.dtype),
            pltpu.VMEM((2, seg, d_model + _HALF), jnp.float32),
            pltpu.VMEM((n_operands, n_mem + seg, _LANES), jnp.float32),
            pltpu.VMEM((n_operands, seg, _LANES), jnp.bfloat16),
            pltpu.VMEM((_CHUNKS, n_operands, 2 * seg, _LANES), jnp.bfloat16),
            pltpu.VMEM((_MEMBERS + 4, _COLUMNS, 2 * (n_mem + seg), _LANES), jnp.float32),
            pltpu.VMEM((_MEMBERS + 4, _COLUMNS, 4 * seg, _LANES), jnp.float32),
            pltpu.VMEM((8 * _CHUNKS, 3, _MEMBERS, _COLUMNS, seg // 2, _LANES), jnp.float32),
            pltpu.VMEM((n_tiles, _LANES, _LANES), jnp.bfloat16),
            pltpu.VMEM((_CHUNKS, d_model, n_tok // _CHUNKS), A_x.dtype),
            pltpu.VMEM((3, _COLUMNS // 2, d_model, _LANES), jnp.uint32),
            pltpu.VMEM((3, _COLUMNS // 2, shared_rows, _LANES), jnp.uint32),
            pltpu.VMEM((_COLUMNS, d_model // 2, _LANES), jnp.uint32),
            pltpu.VMEM((_COLUMNS, shared_rows // 2, _LANES), jnp.uint32),
            pltpu.VMEM((3, 3, d_model // 2, _COLUMNS * _LANES), jnp.uint32),
            pltpu.VMEM((3, shared_rows // 2, _COLUMNS * _LANES), jnp.uint32),
            pltpu.VMEM((n_tok + 2 * _LAG * seg, d_model + _HALF), jnp.float32),
            pltpu.VMEM((16, n_mem, d_model), A_mem0.dtype),
            pltpu.SemaphoreType.DMA((_CHUNKS,)),
            pltpu.SemaphoreType.DMA((4,)),
            pltpu.SemaphoreType.DMA((9,)),
            pltpu.SemaphoreType.DMA((4,)),
            pltpu.SemaphoreType.DMA((n_tok // _LANES,)),
        ],
        compiler_params=pltpu.CompilerParams(
            vmem_limit_bytes=126 * 1024 * 1024, disable_bounds_checks=True,
            flags={"XLA_TPU_FORCE_LP_LLO_SCHEDULER": True}),
    )(A_x.reshape(n_tok, d_model).T, A_mem0.reshape(n_mem, d_model), A_Wq, A_Wk, A_Wv,
      A_Wo.transpose(0, 2, 1), B_w1, B_w3, B_w2.T)
    return out_t.T.reshape(A_x.shape)
```

```python
import functools
import math
from typing import NamedTuple

import jax
import jax.numpy as jnp
import jax.experimental.pallas as pl
import jax.experimental.pallas.tpu as pltpu

_EPS = 1e-05
_MASKED = -1000000000.0
_LOG2E = math.log2(math.e)
_LANES = 128
_HALF = _LANES // 2
_TAIL = 4
_COLUMNS = 8
_MEMBERS = 4
_WQ, _WK, _WV, _WO, _UP, _DOWN, _FAMILIES = 0, 1, 2, 3, 4, 6, 7
_LAG = 4
_CHUNKS = 4
_ORDER_EVEN = (
    "N X Q0 K0 V0*10+S0 Q1 A0 K1 V1*6+S1 Q2 A1 K2 V2*6+S2 Q3 A2 K3 O0 O1 O2 G0 G1*10+S3 V3 G8 "
    "A3+G2*6 G3 O3 D4")
_ORDER_ODD = (
    "Q0 K0 G4 G5 V0 D0*6+S0 Q1 A0 K1 G6 G7 V1 D1*6+S1 Q2 A1 K2 V2 D2*6+S2 Q3 A2 K3 V3 O0*6+S3 "
    "D3 F X A3+O1*6 O2 O3")
_ORDER_EVEN_SINGLE = (
    "Q0 N K0 V0*4+S0 Q1 K1 G0 A0 V1*4+S1 O0 G1 A1 Q2 K2 V2*4+S2 O1 G2 A2 Q3 K3 V3*4+S3 X O2 "
    "G3 A3 G8 O3 D4 G4")
_ORDER_ODD_SINGLE = (
    "Q0 K0 V0*4+S0 G5 A0 Q1 K1 V1*4+S1 G6 A1 Q2 K2 G7 V2*4+S2 D0 A2 Q3 K3 "
    "D1 D2 D3 F X V3*4+S3 O0 O1 A3 O2 O3")
_ORDER_DOUBLE = (
    "Q0 K0 Q1 K1 V0*10+S0 Q2 K2 V1*6+S1 A0 Q3 K3 V2 A1 O0*6+S2 V3 X O1*6+S3 A2 O2:30 A3 O2 O3")
_ORDER_SINGLE = (
    "Q0 K0 V0*4+S0 Q1 K1 A0 V1*4+S1 Q2 K2 A1 V2*4+S2 Q3 K3 A2 V3*4+S3 X O0 O1 A3 O2 O3")
_ORDER_FFN = "N G0 G1 G2 D0 G3 G4 D1 G5 G6 G7 G8 D2 D4 D3 F"
_ORDER_SHARED = "E+L*13"
_ORDER_LOAD = "W1 E0+L1*20+L4*5 W2 E1+L2*20+L3*12:208 E1 L2 W0 E2+L0*20+L3*12"
_ORDER_FIRST = "P:8 P+L*23"
_ORDER_FIRST_FFN = "P:20 P+L*15"


class _Pass(NamedTuple):
    low: tuple
    high: tuple
    w_low: tuple
    w_high: tuple
    wide: tuple
    common: bool = False


@functools.cache
def _scheme(kind, shift=0):
    x, y, n = 0, 1, 4 if kind in ("member", "alone") else 2
    a = lambda d: d % n + shift
    b = lambda d: d % n + shift + (2 if kind == "narrow" else 4)
    rest = lambda d: [e for e in range(4) if e != d and e // n == d // n]

    def whole(narrow, weight, wide):
        return _Pass(tuple(sorted(narrow)), tuple(sorted(narrow)), weight, weight, wide)

    def m1(d, e):
        return whole(((1, x, d), (1, y, e)), ((1, b(e), d), (1, a(d), e)),
                     ((1, y, a(d)), (1, x, b(e))))

    def m2(d, e):
        return whole(((1, y, d), (1, y, e)), ((1, b(e), d),), ((1, y, b(e)), (-1, y, a(d))))

    def m3(d):
        return whole(((1, x, d),), ((1, a(d), d), *((-1, a(d), e) for e in rest(d))),
                     ((1, x, a(d)), (1, y, a(d))))

    def m4(d):
        return whole(((1, y, d),), ((1, b(d), d), *((-1, b(d), e) for e in rest(d))),
                     ((1, y, b(d)), (1, x, b(d))))

    def m5(d, e):
        return whole(((1, x, d), (1, x, e)), ((1, a(d), e),), ((1, x, a(d)), (-1, x, b(e))))

    def m6(d):
        return whole(((1, y, d), (-1, x, d)), ((1, a(d), d), *((1, b(e), d) for e in rest(d))),
                     ((1, y, a(d)),))

    def m7(d):
        return whole(((1, y, d), (-1, x, d)), ((-1, b(d), d), *((-1, a(e), d) for e in rest(d))),
                     ((1, x, b(d)),))

    def with_tails(p, p_rows, p_columns, q, q_rows, q_columns):
        tail = lambda columns: tuple((1, c, _TAIL) for c in columns)
        return [_Pass(p.low, p.high, q.w_low, p.w_high, p.wide + q.wide, common=True),
                _Pass(p.low, ((1, p_rows, _TAIL),), p.w_low, tail(p_columns), p.wide),
                _Pass(((1, q_rows, _TAIL),), q.high, tail(q_columns), q.w_high, q.wide)]

    def pair_with_tails(d, e):
        return [*with_tails(m5(d, e), x, [a(d)], m5(e, d), x, [a(e)]), m3(d),
                *with_tails(m2(d, e), y, [b(e)], m2(e, d), y, [b(d)]), m3(e),
                *with_tails(m6(d), y, [a(d), b(e)], m7(d), x, [b(d), a(e)]), m1(d, e), m4(d),
                *with_tails(m7(e), x, [b(e), a(d)], m6(e), y, [a(e), b(d)]), m1(e, d), m4(e)]

    edge = lambda d, e: [m5(d, e), m1(d, e), m2(d, e)]
    pair = lambda d, e: [m3(d), m6(d), *edge(d, e), m7(e), m4(e),
                         m3(e), m6(e), *edge(e, d), m7(d), m4(d)]
    if kind == "shared":
        return (*pair(0, 1), *(() if shift else _scheme(kind, 2)))
    if kind == "narrow":
        return (*pair_with_tails(0, 1), *pair(2, 3))
    ends = pair if kind == "member" else pair_with_tails
    return (*ends(0, 1), *edge(0, 2), *edge(0, 3), *edge(1, 2), *edge(1, 3),
            *edge(2, 0), *edge(3, 0), *edge(2, 1), *edge(3, 1), *ends(2, 3))


def _selected(kind, single):
    for i, p in enumerate(_scheme(kind)):
        if single:
            narrow = tuple((s, 0, d) for s, _, d in p.low)
            p = p._replace(low=narrow, high=narrow,
                           wide=tuple((s, 0, c) for s, r, c in p.wide if r == c // 4))
        if p.wide:
            yield i, p


def _tiles(w_refs, kind, family=_FAMILIES, member=_MEMBERS, skip=0):
    size = lambda name: len(_scheme(name)) // 2
    first = family * (_MEMBERS * size("member") + size("shared")) + skip
    if kind in ("member", "shared"):
        first += member * size("member")
    first += size("alone") if kind == "narrow" else 0
    return lambda i: (w_refs[i % 2], first + i // 2)


def _tail_for(terms, block):
    return tuple(sorted((s, r, _TAIL if d == block else d) for s, r, d in terms))


@functools.cache
def _operand_keys(single):
    return tuple(dict.fromkeys(_tail_for(p.low, block) for block in (None, 0, 1)
                               for _, p in _selected("member", single)))


def _signed_sum(terms):
    terms = sorted(terms, key=lambda t: -t[0])
    total = terms[0][1] if terms[0][0] > 0 else -terms[0][1]
    for sign, value in terms[1:]:
        total = total + value if sign > 0 else total - value
    return total


def _accumulate(sums, key, sign, value):
    if key not in sums:
        sums[key] = (sign, value)
    elif sums[key][0] == sign:
        sums[key] = (sign, sums[key][1] + value)
    else:
        sums[key] = (1, value - sums[key][1] if sign > 0 else sums[key][1] - value)


def _words(ref):
    return ref.bitcast(jnp.uint32) if ref.dtype == jnp.bfloat16 else ref


def _unpack(words):
    return pltpu.bitcast(words, jnp.bfloat16) if words.dtype == jnp.uint32 else words


def _load(ref, i):
    return _unpack(_words(ref)[i])


def _store(ref, i, first, value):
    rows = value.shape[0]
    if value.dtype == jnp.bfloat16:
        _words(ref)[i, pl.ds(first // 2, rows // 2), :] = pltpu.bitcast(value, jnp.uint32)
    else:
        ref[i, pl.ds(first, rows), :] = value.astype(ref.dtype)


def _lane_half(rows):
    return jax.lax.broadcasted_iota(jnp.int32, (rows, _LANES), 1) // _HALF


def _blocks(x):
    return [x[:, d * _LANES:(d + 1) * _LANES] for d in range(_TAIL + 1)]


def _store_operands(ref, first, row_blocks):
    blocks = [_blocks(x) for x in row_blocks]
    for i, terms in enumerate(_operand_keys(len(row_blocks) == 1)):
        _store(ref, i, first, _signed_sum([(s, blocks[r][d]) for s, r, d in terms]))


def _dot(a, b):
    return jnp.dot(a, b, preferred_element_type=jnp.float32)


def _expand(operands_ref, w_refs, unit, out, single=False):
    operands_ref, tile = _words(operands_ref), _tiles(w_refs, *unit)
    operand = lambda terms: operands_ref[_operand_keys(single).index(terms)]
    half = _lane_half(operands_ref.shape[1])
    freed = {}
    if unit[0] == "member":
        blocks = [unit[2] // 2] if isinstance(unit[2], int) else range(_MEMBERS // 2)
        freed = {d: half == unit[2] - 2 * d for d in blocks}
    sums, common = {key: (1, value) for key, value in out.items()}, []
    for i, p in _selected(unit[0], single):
        lhs = operand(p.low)
        if p.high != p.low:
            lhs = jnp.where(half == 0, lhs, operand(p.high))
        for d, lanes in freed.items():
            if _tail_for(p.low, d) != p.low:
                lhs = jnp.where(lanes, operand(_tail_for(p.low, d)), lhs)
        product = _dot(_unpack(lhs), _load(*tile(i)))
        if p.common:
            common = [product, product]
        else:
            if common:
                product = product + common.pop()
            for s, r, c in p.wide:
                _accumulate(sums, (r, c), s, product)
        yield
    assert all(sign > 0 for sign, _ in sums.values())
    out.update({key: value for key, (_, value) in sums.items()})


def _contract(load, w_refs, unit, sums, single=False):
    tile = _tiles(w_refs, *unit)
    freed = unit[2] // 2 if unit[0] == "member" else None
    held, mixed = [], {}
    for i, p in _selected(unit[0], single):
        product = _dot(_signed_sum([(s, load(r, c)) for s, r, c in p.wide]),
                       _load(*tile(i)))
        if p.common or held:
            held.append((p, product))
        if len(held) == 3:
            (p, common), (p1, first), (p2, second) = held
            held = []
            product = common + jnp.where(_lane_half(common.shape[0]) == 0, first, second)
            _accumulate(sums, (p1.high[0][1], _TAIL, 1), 1, first)
            _accumulate(sums, (p2.low[0][1], _TAIL, 0), 1, second)
        if not held:
            for s, r, d in p.low:
                _accumulate(mixed if d == freed else sums, (r, d), s, product)
        yield
    for (r, d), (s, both) in mixed.items():
        _accumulate(sums, (r, _TAIL, unit[2] % 2), s, both)
        _accumulate(sums, (r, d), s, jnp.where(_lane_half(both.shape[0]) == unit[2] % 2, 0.0, both))


def _residual(row_blocks):
    return {(r, d) if d < _TAIL else (r, d, 0): (1, block)
            for r, x in enumerate(row_blocks) for d, block in enumerate(_blocks(x))}


def _contracted(sums, r):
    assert all(sign > 0 for sign, _ in sums.values())
    low, high = sums[r, _TAIL, 0][1], sums[r, _TAIL, 1][1]
    tail = jnp.where(_lane_half(low.shape[0]) == 0, low, high)
    tail = tail + pltpu.roll(tail, _HALF, 1)
    return jnp.concatenate([sums[r, d][1] for d in range(_TAIL)] + [tail], axis=1)


def _weight_sum(parts):
    return _signed_sum([(s, part.astype(jnp.float32) if len(parts) > 1 else part)
                        for s, part in parts])


def _weight_sums(passes, source, starts):
    for i, p in enumerate(passes):
        for high in range(2):
            if i > high and passes[i - 1 - high].common:
                continue
            for at in starts:
                first = high * _HALF + at
                total = lambda terms: _weight_sum(
                    [(s, source(c, 2 * d + high * (d < _TAIL), at)) for s, c, d in terms])
                terms = (p.w_low, p.w_high)[high]
                value = total(terms)
                yield i, first, value, len(terms)
                if p.common:
                    other = passes[i + 1 + high]
                    other = total((other.w_low, other.w_high)[high]).astype(jnp.float32)
                    yield i + 1 + high, first, other - value.astype(jnp.float32), len(terms) + 1


def _lay_out(sums, tile):
    for i, first, value, terms in sums:
        _store(*tile(i), pl.multiple_of(first, 16), value)
        yield from range(int(4 * terms + 1) * value.shape[0] // 16)


def _lay_out_transposed(sums, tile):
    halves, pending = {}, []
    for i, first, value, terms in sums:
        halves[i, first] = value
        if (i, _HALF - first) in halves:
            pair = [halves[i, 0], halves[i, _HALF]]
            if pair[0].dtype != pair[1].dtype:
                pair = [half.astype(jnp.float32) for half in pair]
            pending.append((i, jnp.concatenate(pair, axis=0).astype(jnp.bfloat16).T))
        if len(pending) > 2:
            _store(*tile(pending[0][0]), 0, pending.pop(0)[1])
        yield from range(int(8 * terms + 22))
    for i, value in pending:
        _store(*tile(i), 0, value)


def _layernorm(x):
    low_lanes = _lane_half(x.shape[0]) == 0

    def mean(v):
        *full, tail = _blocks(v)
        total = functools.reduce(jnp.add, full) + jnp.where(low_lanes, tail, 0.0)
        return jnp.sum(total, axis=-1, keepdims=True) / (_TAIL * _LANES + _HALF)

    d = x - mean(x)
    return d * jax.lax.rsqrt(mean(d * d) + _EPS)


def _silu(x):
    half = 0.5 * x
    return half + half * jnp.tanh(half)


def _reciprocal(x):
    r = pl.reciprocal(x, approx=True)
    return r * (2.0 - x * r)


def _attention_masks(n_layers, rows, n_mem):
    i = jax.lax.broadcasted_iota(jnp.int32, (n_layers * rows, n_layers * rows), 0)
    j = jax.lax.broadcasted_iota(jnp.int32, (n_layers * rows, n_layers * rows), 1)
    if n_layers == 1:
        return (i < n_mem) | (i >= j), _MASKED * _LOG2E
    same = (i >= rows) == (j >= rows)
    visible = (i < n_mem) | ((i >= rows) & (i < rows + n_mem)) | (i >= j)
    fill = jnp.where(same, _MASKED * _LOG2E, -jnp.inf).astype(jnp.float32)
    return same & visible, fill


def _expand_member(operands_ref, w_refs, family, member, shared_ref, out, single=False):
    rows = operands_ref.shape[1]
    if member == 0:
        yield from _expand(operands_ref, w_refs, ("shared", family), out, single)
        for (r, c), value in out.items():
            shared_ref[c, r * rows:(r + 1) * rows, :] = value
    out.update({(r, c): shared_ref[c, r * rows:(r + 1) * rows, :]
                for r in range(1 if single else 2) for c in range(_COLUMNS)})
    yield from _expand(operands_ref, w_refs, ("member", family, member), out, single)


def _store_wide(ref, member, c, rows, value):
    ref[member, c, rows, :] = value
    if member == _MEMBERS - 1:
        ref[_MEMBERS, c, rows, :] = functools.reduce(
            jnp.add, [ref[m, c, rows, :] for m in range(member)] + [value])


def _contract_member(ref, w_refs, family, member, sums, single=False):
    rows = ref.shape[2] // 2
    load = lambda m: lambda r, c: ref[m, c, r * rows:(r + 1) * rows, :]
    yield from _contract(load(member), w_refs, ("member", family, member), sums, single)
    if member == _MEMBERS - 1:
        yield from _contract(load(_MEMBERS), w_refs, ("shared", family), sums, single)


def _attention_tasks(xs, operands_ref, w_refs, qkv_ref, wide_ref, outs, known=None):
    n_layers, rows = len(xs), wide_ref.shape[2] // 2
    single, n_mem = n_layers == 1, rows - xs[0].shape[0]
    visible, fill = _attention_masks(n_layers, rows, n_mem)
    scale = _LANES ** -0.5 * _LOG2E
    qkv, probs = {}, {}
    sums = _residual([jnp.concatenate([jnp.zeros_like(x[:n_mem]), x], axis=0) for x in xs])

    def project(family, g):
        out = {}
        yield from _expand_member(operands_ref, w_refs, family, g,
                                  wide_ref.at[_MEMBERS + 1 + family], out, single)
        for h in range(_COLUMNS):
            if single:
                qkv[family, g, h] = out[0, h] if family == _WQ else out[0, h].astype(jnp.bfloat16)
                continue
            parts = x, y = out[0, h], out[1, h]
            if known:
                moved = (rows + n_mem) // 2
                parts = [x[:n_mem], known(family, g, h), x[n_mem:moved], y, x[moved:]]
            qkv_ref[family, g, h] = jnp.concatenate(parts, axis=0).astype(qkv_ref.dtype)

    def stacked(*at):
        return qkv[at] if single else _load(qkv_ref, at)

    def scores(g):
        for h in range(_COLUMNS):
            s = jax.lax.dot_general(stacked(_WQ, g, h), stacked(_WK, g, h),
                                    (((1,), (1,)), ((), ())), preferred_element_type=jnp.float32)
            s = jnp.where(visible, s * scale, fill)
            p = jnp.exp2(s - jnp.max(s, axis=-1, keepdims=True))
            p = p * _reciprocal(jnp.sum(p, axis=-1, keepdims=True))
            probs[g, h] = p if single else p.astype(jnp.bfloat16)
            yield

    def values(g):
        for h in range(_COLUMNS):
            _store_wide(wide_ref, g, h, slice(0, n_layers * rows),
                        _dot(probs[g, h], stacked(_WV, g, h)))
            yield

    def output(g):
        yield from _contract_member(wide_ref, w_refs, _WO, g, sums, single)
        if g == _MEMBERS - 1:
            outs.extend(_contracted(sums, r) for r in range(n_layers))

    tasks = {}
    for g in range(_MEMBERS):
        tasks.update({f"Q{g}": project(_WQ, g), f"K{g}": project(_WK, g), f"V{g}": project(_WV, g),
                      f"S{g}": scores(g), f"A{g}": values(g), f"O{g}": output(g)})
    return tasks


def _ffn_tasks(xs, operands_ref, w_refs, wide_ref, result):
    rows = operands_ref.shape[1]
    sums = _residual(xs)

    def gated(member, i):
        both = {}
        if member < _MEMBERS:
            yield from _expand_member(operands_ref, w_refs, _UP + i, member,
                                      wide_ref.at[_MEMBERS + 2 + i], both)
        else:
            yield from _expand(operands_ref, w_refs, ("alone",), both)
        for c in range(4):
            for r in range(2):
                _store_wide(wide_ref, member + member // _MEMBERS, 4 * i + c,
                            slice(r * rows, (r + 1) * rows), _silu(both[r, c]) * both[r, 4 + c])

    def finish():
        result([_contracted(sums, r) for r in range(2)])
        yield

    return {"F": finish(), **{f"G{u}": gated(*divmod(u, 2)) for u in range(2 * _MEMBERS + 1)},
            **{f"D{m}": _contract_member(wide_ref, w_refs, _DOWN, m, sums) for m in range(_MEMBERS)},
            "D4": _contract(lambda r, c: wide_ref[_MEMBERS + 1, c, r * rows:(r + 1) * rows, :],
                            w_refs, ("narrow",), sums)}


def _passes(order, tasks):
    done = object()
    for item in order.split():
        names, _, turns = item.partition(":")
        running = [(tasks[name], int(count or 1))
                   for name, _, count in (part.partition("*") for part in names.split("+"))]
        turn = 0
        while running and (not turns or turn < int(turns)):
            for task, count in tuple(running):
                for _ in range(count):
                    if next(task, done) is done:
                        running.remove((task, count))
                        break
                    yield
            turn += 1


def _chain(*tasks):
    for task in tasks:
        yield from task


def _run(*tasks):
    for _ in _chain(*tasks):
        pass


def _kernel(xt_hbm, mem0_hbm, wq_hbm, wk_hbm, wv_hbm, wot_hbm, w1_hbm, w3_hbm, w2t_hbm,
            outt_hbm, out_ref, h_ref, full_ref, short_ref, chunks_ref, qkv_ref, heads_ref, hidden_ref,
            early_ref, w_refs, x_stage, qkv_stage, qkv_shared, wo_stage, wo_shared, ffn_stage,
            ffn_shared, res_ref, mem0_ref, x_sem, attention_sem, ffn_sem, shared_sem, out_sem,
            *, seg):
    d_model, n_tok = xt_hbm.shape
    n_mem = mem0_hbm.shape[0]
    n_seg = n_tok // seg
    n_out = n_tok // _LANES

    def window(r, n):
        return res_ref.at[pl.ds(pl.multiple_of((r + _LAG) * seg, seg), n * seg)]

    def block(r, n=1):
        return pl.ds(r * seg, n * seg)

    def lanes(i, n=1):
        return pl.ds(pl.multiple_of(i * _LANES, _LANES), n * _LANES)

    def transpose_out(i, x):
        out_ref[i] = x.T[:d_model].astype(out_ref.dtype)

    def prepare(ref, blocks):
        for i, r in enumerate(blocks):
            h_ref[i, n_mem:] = _layernorm(ref[block(r), :])
        yield

    def attention(order, ref, blocks, others, early=None):
        xs, outs = [ref[block(r), :] for r in blocks], []
        hs = [h_ref[i] for i in range(len(blocks))]
        operands_ref, known = full_ref, None
        if early is not None:
            operands_ref, known = short_ref, lambda *at: early_ref[(early, *at)]
            hs = [jnp.concatenate([hs[0][:n_mem], hs[0][n_mem + seg // 2:], hs[1][seg:]], axis=0),
                  hs[1][:seg]]
        _store_operands(operands_ref, 0, hs)
        tasks = _attention_tasks(xs, operands_ref, w_refs, qkv_ref, heads_ref, outs, known)
        yield from _passes(order, {**others, **tasks})
        for i, r in enumerate(blocks):
            h_ref[i, :n_mem] = outs[i][:n_mem]
            ref[block(r), :] = outs[i][n_mem:]

    def ffn_tasks(ref, blocks, result=None):
        def update(ys):
            for r, y in zip(blocks, ys):
                ref[block(r, 2), :] = y

        def operands():
            for i in range(0, 2 * seg, 16):
                _store_operands(chunks_ref.at[0], i,
                                [_layernorm(ref[pl.ds(r * seg + i, 16), :]) for r in blocks])
            yield

        return {"N": operands(), **_ffn_tasks(
            [ref[block(r, 2), :] for r in blocks], chunks_ref.at[0], w_refs, hidden_ref,
            result or update)}

    def double_step(b):
        ref = window(b, _LAG + 2)
        _run(attention(_ORDER_DOUBLE, ref, [_LAG, 0],
                       {"X": prepare(ref, [_LAG + 1, 1])}, 1 + b))

    def two_steps(j):
        b = 6
        ref = window(2 * j - b, b + _LAG + 3)
        transpose_out(jnp.where((j % 2 == 1) & (j > 1), (j - 3) // 2, n_out - 1),
                      ref[block(0, 4), :])
        ffn = ffn_tasks(ref, [b + 2, b - 2])
        _run(attention(_ORDER_EVEN, ref, [b + _LAG, b],
                       {**ffn, "X": prepare(ref, [b + _LAG + 1, b + 1])}),
             attention(_ORDER_ODD, ref, [b + _LAG + 1, b + 1],
                       {**ffn, "X": prepare(ref, [b + _LAG + 2, b + 2])}, j + _LAG // 2))

    qkv_words = [_words(w) for w in (wq_hbm, wk_hbm, wv_hbm)]
    ffn_words = [_words(w) for w in (w1_hbm, w3_hbm, w2t_hbm)]
    pairs = _COLUMNS // 2

    def attention_copies(family, g):
        sem = attention_sem.at[family]
        if family == _WO:
            heads = _words(wot_hbm).at[pl.ds(_COLUMNS * g, _COLUMNS)]
            return [pltpu.make_async_copy(heads, wo_stage, sem)]
        return [pltpu.make_async_copy(qkv_words[family].at[:, pairs * g + p, :],
                                      qkv_stage.at[family, p], sem) for p in range(pairs)]

    def ffn_copies(m, columns=_COLUMNS):
        return [pltpu.make_async_copy(w.at[:, lanes(_COLUMNS * m, columns)],
                                      ffn_stage.at[m % 3, i, :, lanes(0, columns)],
                                      ffn_sem.at[3 * (m % 3) + i])
                for i, w in enumerate(ffn_words)]

    def shared_copies(which):
        ends = []
        for m in range(_MEMBERS):
            rows, words = pl.ds(m * _HALF, _HALF), pl.ds(m * _HALF // 2, _HALF // 2)
            if which == 0:
                ends += [(w.at[rows, pairs * m + p, :], qkv_shared.at[i, p, rows])
                         for i, w in enumerate(qkv_words) for p in range(pairs)]
            elif which == 1:
                ends += [(_words(wot_hbm).at[pl.ds(_COLUMNS * m, _COLUMNS), words],
                          wo_shared.at[:, words])]
            else:
                ends += [(w.at[words, lanes(_COLUMNS * m, _COLUMNS)], ffn_shared.at[i, words])
                         for i, w in enumerate(ffn_words)]
        return [pltpu.make_async_copy(*pair, shared_sem.at[which]) for pair in ends]

    def x_copy(chunk):
        columns = lanes(n_out // _CHUNKS * chunk, n_out // _CHUNKS)
        return pltpu.make_async_copy(xt_hbm.at[:, columns], x_stage.at[chunk], x_sem.at[chunk])

    def out_copy(i):
        return pltpu.make_async_copy(out_ref.at[i], outt_hbm.at[:, lanes(i)], out_sem.at[i])

    def start(copies):
        for c in copies:
            c.start()

    def wait(copies):
        for c in copies:
            c.wait()

    def head_pairs(ref):
        def source(c, half, first):
            rows = ref.at[c // 2, pl.ds(pl.multiple_of(half * _HALF, _HALF), _HALF)]
            words = rows[pl.ds(pl.multiple_of(first, 16), 16), :]
            words = words & jnp.uint32(0xFFFF0000) if c % 2 else words << 16
            return pltpu.bitcast(words, jnp.float32)
        return source

    def row_pairs(column, rows):
        def source(c, half, first):
            ref, at = column(c)
            words = ref.at[pl.ds(pl.multiple_of(half * (_HALF // 2), _HALF // 2), _HALF // 2)]
            return _unpack(words[pl.ds(first // 2, rows // 2), at])
        return source

    def member_sums(own, shared, m, rows, starts=None):
        places = [(jnp.where(m == h, 2 * _TAIL, h), jnp.where(m == h, _MEMBERS, h))
                  for h in range(_MEMBERS)]

        def source(c, d, high, first):
            if 2 * d >= _MEMBERS:
                return own(c, 2 * d + high, first)
            mine, theirs = places[2 * d + high]
            return (own(c, mine, first).astype(jnp.float32)
                    - shared(c, theirs, first).astype(jnp.float32))

        sets = {}
        for i, p in enumerate(_scheme("member")):
            owners = {c if c < 4 else d for _, c, d in p.w_low}
            key = -1 - min(owners) if len(owners) == 1 and rows < _HALF else i
            sets.setdefault(key, []).append((len(p.w_low), i, p))
        for tiles in sets.values():
            for high in range(2):
                for first in starts or range(0, _HALF, rows):
                    loaded = {}
                    for *_, i, p in sorted(tiles):
                        new = [(c, d) for _, c, d in p.w_low if (c, d) not in loaded]
                        loaded.update({at: source(*at, high, first) for at in new})
                        value = _weight_sum([(s, loaded[c, d]) for s, c, d in p.w_low])
                        work = len(p.w_low) + sum(1 + 2 * (d < 2) for _, d in new)
                        yield i, high * _HALF + first, value, work / 2

    def lay_out_heads(family, g, starts=None):
        sums = member_sums(head_pairs(qkv_stage.at[family]), head_pairs(qkv_shared.at[family]),
                           g, 16, starts)
        return _lay_out(sums, _tiles(w_refs, "member", family, g))

    def lay_out_shared_half(lay_out, words, rows, family, i):
        n = len(_scheme("shared")) // 2
        sums = _weight_sums(_scheme("shared")[:n], row_pairs(words, rows), range(0, _HALF, rows))
        return lay_out(sums, _tiles(w_refs, "shared", family, skip=n // 2 * i))

    def up_words(ref, first):
        return lambda c: (ref.at[c // 4], lanes(first + c % 4))

    def down_words(ref):
        return lambda c: (ref.at[2], lanes(c))

    def project_early(chunk, unit):
        at = lambda r, g, c: (pl.ds(8 * chunk + 4 * r, 4), unit[1], g, c)
        out = {}
        if unit[0] == "member":
            out = {(r, c): early_ref[at(r, _MEMBERS - 1, c)].reshape(2 * seg, _LANES)
                   for r in range(2) for c in range(_COLUMNS)}
        yield from _expand(chunks_ref.at[chunk], w_refs, unit, out)
        for (r, c), value in out.items():
            early_ref[at(r, unit[2] if unit[0] == "member" else _MEMBERS - 1, c)] = (
                value.reshape(4, seg // 2, _LANES))

    def load_chunk(chunk):
        pl.when(chunk == 1)(lambda: start(attention_copies(_WQ, 0)))
        wait([x_copy(chunk)])
        for family in (_WQ, _WK, _WV):
            sums = _weight_sums(_scheme("shared"), head_pairs(qkv_shared.at[family]), [16 * chunk])
            _run(_lay_out(sums, _tiles(w_refs, "shared", family)))
        x = x_stage[chunk].astype(jnp.float32)
        x = jnp.concatenate([x, x[_TAIL * _LANES:]], axis=0).T
        window(n_seg // _CHUNKS * chunk, n_seg // _CHUNKS)[...] = x
        half = lambda r: x[r * seg:r * seg + seg // 2]
        halves = [half(2 * e + 1) for e in range(8)]
        halves[1] = jnp.where(chunk == 0, half(_LAG), halves[1])
        _store_operands(chunks_ref.at[chunk], 0, [
            _layernorm(jnp.concatenate(part, axis=0)) for part in (halves[:4], halves[4:])])

    def project_shared(chunk):
        _run(_passes(_ORDER_SHARED, {
            "E": _chain(*(project_early(chunk, ("shared", f)) for f in (_WQ, _WK, _WV))),
            "L": lay_out_heads(_WQ, 0, [16 * chunk])}))

    def load_group(g):
        more = g + 1 < _MEMBERS

        def arrive(family):
            if family == _WK:
                start(attention_copies(_WO, g))
                pl.when(more)(lambda: start(attention_copies(_WQ, g + 1)))
                pl.when(~more)(lambda: start(ffn_copies(0)))
                wait(attention_copies(_WK, g))
            elif family == _WV:
                wait(attention_copies(_WV, g) + attention_copies(_WO, g))
                pl.when(more)(lambda: start(attention_copies(_WK, g + 1)))
                pl.when(~more)(lambda: start(ffn_copies(1)))
            else:
                pl.when(more)(lambda: wait(attention_copies(_WQ, g + 1)))
                pl.when(more)(lambda: start(attention_copies(_WV, g + 1)))
                pl.when(g == 1)(lambda: start(shared_copies(2)))
            yield

        same = jnp.minimum(g, _MEMBERS - 1)
        wo_sums = member_sums(row_pairs(lambda c: (wo_stage.at[c], slice(None)), _HALF),
                              row_pairs(lambda c: (wo_shared.at[c], slice(None)), _HALF), g, _HALF)
        _run(_passes(_ORDER_LOAD, {
            **{f"E{f}": _chain(*(project_early(chunk, ("member", f, g)) for chunk in range(_CHUNKS)))
               for f in (_WQ, _WK, _WV)},
            **{f"W{f}": arrive(f) for f in (_WQ, _WK, _WV)},
            "L0": lay_out_heads(_WQ, jnp.minimum(g + 1, _MEMBERS - 1)),
            "L1": lay_out_heads(_WK, same), "L2": lay_out_heads(_WV, same),
            "L3": _lay_out_transposed(wo_sums, _tiles(w_refs, "member", _WO, same)),
            "L4": lay_out_shared_half(
                _lay_out_transposed, lambda c: (wo_shared.at[c + 2 * (g % 2)], slice(None)), _HALF,
                _WO, g % 2)}))

    def first_step(m):
        pl.when(m + 2 < _MEMBERS)(lambda: start(ffn_copies(m + 2)))
        pl.when(m + 2 == _MEMBERS)(lambda: start(ffn_copies(_MEMBERS, 4)))
        wait(ffn_copies(m))
        ref, stage = window(m, 2), ffn_stage.at[m % 3]
        up = [_lay_out(member_sums(row_pairs(up_words(stage, 4 * i), 16),
                                   row_pairs(up_words(ffn_shared, 4 * i), 16), m, 16),
                       _tiles(w_refs, "member", _UP + i, m)) for i in range(2)]
        shared = lay_out_shared_half(_lay_out, up_words(ffn_shared, 2 * m), 16, _UP + m // 2, m % 2)
        down = _lay_out_transposed(
            member_sums(row_pairs(down_words(stage), _HALF),
                        row_pairs(down_words(ffn_shared), _HALF), m, _HALF),
            _tiles(w_refs, "member", _DOWN, m))
        _run(_passes(_ORDER_FIRST, {
            "P": attention(_ORDER_SINGLE, ref, [0], {"X": prepare(ref, [1])}),
            "L": _passes("U*9+D*5", {"U": _chain(shared, *up), "D": down})}))

    def first_ffn():
        stage = ffn_stage.at[_MEMBERS % 3]
        down = lambda kind, ref, *family: _lay_out_transposed(
            _weight_sums(_scheme(kind), row_pairs(down_words(ref), _HALF), [0]),
            _tiles(w_refs, kind, *family))
        up = _lay_out(_weight_sums(_scheme("alone"), row_pairs(up_words(stage, 0), 32), [0, 32]),
                      _tiles(w_refs, "alone"))
        _run(_passes(_ORDER_FIRST_FFN, {
            "P": _passes(_ORDER_FFN, ffn_tasks(window(0, _LAG), [0, 2])),
            "L": _chain(up, down("narrow", stage), down("shared", ffn_shared, _DOWN))}))

    def last_steps():
        ref = window(n_seg - _LAG - 2, _LAG + 2)
        ffn = ffn_tasks(ref, [_LAG, 0])
        _run(attention(_ORDER_EVEN_SINGLE, ref, [2], {**ffn, "X": prepare(ref, [3])}),
             attention(_ORDER_ODD_SINGLE, ref, [3], {**ffn, "X": prepare(ref, [4])}))

    def last_step(i):
        tile = n_out - 3 + i
        transpose_out(tile, window(_LANES // seg * tile, _LANES // seg)[...])
        ref = window(n_seg - 2 + i, 2)
        _run(attention(_ORDER_SINGLE, ref, [0], {"X": prepare(ref, [1])}))
        out_copy(tile).start()

    def last_ffn():
        _run(_passes(_ORDER_FFN, ffn_tasks(
            window(n_seg - _LAG, _LAG), [0, 2],
            lambda ys: transpose_out(n_out - 1, jnp.concatenate(ys, axis=0)))))

    mem_copy = pltpu.make_async_copy(mem0_hbm, mem0_ref.at[0], shared_sem.at[3])
    start([x_copy(0)] + shared_copies(0) + [x_copy(1)])
    behind = pl.ds(_MEMBERS * _HALF // 2, _HALF // 2)
    for spare in (window(-_LAG, _LAG), window(n_seg, 1), wo_shared.at[:, behind],
                  ffn_shared.at[:, behind], qkv_shared.at[:, :, pl.ds(_MEMBERS * _HALF, _HALF)]):
        spare[...] = jnp.zeros(spare.shape, spare.dtype)
    wait(shared_copies(0))
    start([x_copy(i) for i in range(2, _CHUNKS)] + [mem_copy])
    pl.loop(0, _CHUNKS)(load_chunk)
    mem_copy.wait()
    mem0 = mem0_ref[0].astype(jnp.float32)
    h_ref[0, :n_mem] = h_ref[1, :n_mem] = jnp.concatenate(
        [mem0, mem0[:, _TAIL * _LANES:]], axis=1)
    _run(prepare(window(0, 1), [0]))
    start(shared_copies(1) + attention_copies(_WK, 0))
    wait(attention_copies(_WQ, 0))
    start(attention_copies(_WV, 0))
    pl.loop(0, _CHUNKS)(project_shared)
    wait(shared_copies(1))
    pl.loop(0, _MEMBERS)(load_group)
    wait(shared_copies(2))
    pl.loop(0, _LAG)(first_step)
    wait(ffn_copies(_MEMBERS, 4))
    first_ffn()
    _run(prepare(window(0, _LAG + 1), [_LAG, 0]))
    pl.loop(0, 2)(double_step)
    pl.loop(1, (n_seg - _LAG) // 2)(two_steps)
    start([out_copy(i) for i in range(n_out - 3)])
    h_ref[0] = h_ref[1]
    last_steps()
    pl.loop(0, 2)(last_step)
    last_ffn()
    out_copy(n_out - 1).start()
    wait([out_copy(i) for i in range(n_out)])


@functools.partial(jax.jit, static_argnames=("A_seg_len",))
def pallas_interleave_layers__memory_aug_recurrent_mem_tr__glu_gated_swiglu__prompt_kernel(
    A_x: jax.Array,
    A_mem0: jax.Array,
    A_Wq: jax.Array,
    A_Wk: jax.Array,
    A_Wv: jax.Array,
    A_Wo: jax.Array,
    A_seg_len: int,
    B_x: jax.Array,
    B_w1: jax.Array,
    B_w3: jax.Array,
    B_w2: jax.Array,
):
    del B_x
    _, n_tok, d_model = A_x.shape
    n_mem = A_mem0.shape[1]
    _, n_heads, d_head = A_Wq.shape
    seg = A_seg_len
    assert A_x.shape[0] == 1 and _LAG * seg == _LANES and n_mem == 8
    assert n_tok == 16 * _CHUNKS * seg and d_model == _TAIL * _LANES + _HALF and d_head == _LANES
    assert n_heads == _MEMBERS * _COLUMNS and B_w1.shape[1] == (n_heads + 4) * _LANES
    n_operands = pl.cdiv(len(_operand_keys(False)), 8) * 8
    n_tiles = (_FAMILIES * (_MEMBERS * len(_scheme("member")) + len(_scheme("shared")))
               + len(_scheme("alone")) + len(_scheme("narrow")))
    shared_rows = (_MEMBERS + 1) * _HALF
    hbm = pl.BlockSpec(memory_space=pltpu.HBM)
    out_t = pl.pallas_call(
        functools.partial(_kernel, seg=seg),
        out_shape=jax.ShapeDtypeStruct((d_model, n_tok), A_x.dtype),
        in_specs=[hbm] * 9,
        out_specs=hbm,
        scratch_shapes=[
            pltpu.VMEM((n_tok // _LANES, d_model, _LANES), A_x.dtype),
            pltpu.VMEM((8, n_mem + seg, d_model + _HALF), jnp.float32),
            pltpu.VMEM((n_operands, n_mem + seg, _LANES), jnp.float32),
            pltpu.VMEM((n_operands, seg, _LANES), jnp.bfloat16),
            pltpu.VMEM((_CHUNKS, n_operands, 2 * seg, _LANES), jnp.bfloat16),
            pltpu.VMEM((3, _MEMBERS, _COLUMNS, 2 * (n_mem + seg), _LANES), jnp.bfloat16),
            pltpu.VMEM((_MEMBERS + 4, _COLUMNS, 2 * (n_mem + seg), _LANES), jnp.float32),
            pltpu.VMEM((_MEMBERS + 4, _COLUMNS, 4 * seg, _LANES), jnp.float32),
            pltpu.VMEM((8 * _CHUNKS, 3, _MEMBERS, _COLUMNS, seg // 2, _LANES), jnp.float32),
            [pltpu.VMEM((n_tiles // 2, _LANES, _LANES), jnp.bfloat16)] * 2,
            pltpu.VMEM((_CHUNKS, d_model, n_tok // _CHUNKS), A_x.dtype),
            pltpu.VMEM((3, _COLUMNS // 2, d_model, _LANES), jnp.uint32),
            pltpu.VMEM((3, _COLUMNS // 2, shared_rows, _LANES), jnp.uint32),
            pltpu.VMEM((_COLUMNS, d_model // 2, _LANES), jnp.uint32),
            pltpu.VMEM((_COLUMNS, shared_rows // 2, _LANES), jnp.uint32),
            pltpu.VMEM((3, 3, d_model // 2, _COLUMNS * _LANES), jnp.uint32),
            pltpu.VMEM((3, shared_rows // 2, _COLUMNS * _LANES), jnp.uint32),
            pltpu.VMEM((n_tok + 2 * _LAG * seg, d_model + _HALF), jnp.float32),
            pltpu.VMEM((16, n_mem, d_model), A_mem0.dtype),
            pltpu.SemaphoreType.DMA((_CHUNKS,)),
            pltpu.SemaphoreType.DMA((4,)),
            pltpu.SemaphoreType.DMA((9,)),
            pltpu.SemaphoreType.DMA((4,)),
            pltpu.SemaphoreType.DMA((n_tok // _LANES,)),
        ],
        compiler_params=pltpu.CompilerParams(
            vmem_limit_bytes=126 * 1024 * 1024, disable_bounds_checks=True,
            flags={"XLA_TPU_FORCE_LP_LLO_SCHEDULER": True}),
    )(A_x.reshape(n_tok, d_model).T, A_mem0.reshape(n_mem, d_model), A_Wq, A_Wk, A_Wv,
      A_Wo.transpose(0, 2, 1), B_w1, B_w3, B_w2.T)
    return out_t.T.reshape(A_x.shape)
```

```python
import functools
import math
from typing import NamedTuple

import jax
import jax.numpy as jnp
import jax.experimental.pallas as pl
import jax.experimental.pallas.tpu as pltpu

_EPS = 1e-05
_MASKED = -1000000000.0
_LOG2E = math.log2(math.e)
_LANES = 128
_HALF = _LANES // 2
_TAIL = 4
_COLUMNS = 8
_MEMBERS = 4
_WQ, _WK, _WV, _WO, _UP, _DOWN, _FAMILIES = 0, 1, 2, 3, 4, 6, 7
_LAG = 4
_CHUNKS = 4
_ORDER_EVEN = (
    "N X Q0 K0 V0*10+S0 Q1 A0 K1 V1*6+S1 Q2 A1 K2 V2*6+S2 Q3 A2 K3 O0 O1 O2 G0 G1*10+S3 V3 G8 "
    "A3+G2*6 G3 O3 D4")
_ORDER_ODD = (
    "Q0 K0 G4 G5 V0 D0*6+S0 Q1 A0 K1 G6 G7 V1 D1*6+S1 Q2 A1 K2 V2 D2*6+S2 Q3 A2 K3 V3 O0*6+S3 "
    "D3 F X A3+O1*6 O2 O3")
_ORDER_EVEN_SINGLE = (
    "Q0 N K0 V0*4+S0 Q1 K1 G0 A0 V1*4+S1 O0 G1 A1 Q2 K2 V2*4+S2 O1 G2 A2 Q3 K3 V3*4+S3 X O2 "
    "G3 A3 G8 O3 D4 G4")
_ORDER_ODD_SINGLE = (
    "Q0 K0 V0*4+S0 G5 A0 Q1 K1 V1*4+S1 G6 A1 Q2 K2 G7 V2*4+S2 D0 A2 Q3 K3 "
    "D1 D2 D3 F X V3*4+S3 O0 O1 A3 O2 O3")
_ORDER_DOUBLE = (
    "Q0 K0 Q1 K1 V0*10+S0 Q2 K2 V1*6+S1 A0 Q3 K3 V2 A1 O0*6+S2 V3 X O1*6+S3 A2 O2:30 A3 O2 O3")
_ORDER_SINGLE = (
    "Q0 K0 V0*4+S0 Q1 K1 A0 V1*4+S1 Q2 K2 A1 V2*4+S2 Q3 K3 A2 V3*4+S3 X O0 O1 A3 O2 O3")
_ORDER_FFN = "N G0 G1 G2 D0 G3 G4 D1 G5 G6 G7 G8 D2 D4 D3 F"
_ORDER_SHARED = "E+L*13 X"
_ORDER_LOAD = "W1 E0+L1*20+L4*5 W2 E1+L2*20+L3*12:208 E1 L2 W0 E2+L0*20+L3*12"
_ORDER_FIRST = "P:8 P+L*23"
_ORDER_FIRST_FFN = "N G0 G1 G2 G3 G4 G5 G8+D0+D1+D2 G6 G7*2+D4 D3 F"


class _Pass(NamedTuple):
    low: tuple
    high: tuple
    w_low: tuple
    w_high: tuple
    wide: tuple
    common: bool = False


@functools.cache
def _scheme(kind, shift=0):
    x, y, n = 0, 1, 4 if kind in ("member", "alone") else 2
    a = lambda d: d % n + shift
    b = lambda d: d % n + shift + (2 if kind == "narrow" else 4)
    rest = lambda d: [e for e in range(4) if e != d and e // n == d // n]

    def whole(narrow, weight, wide):
        return _Pass(tuple(sorted(narrow)), tuple(sorted(narrow)), weight, weight, wide)

    def m1(d, e):
        return whole(((1, x, d), (1, y, e)), ((1, b(e), d), (1, a(d), e)),
                     ((1, y, a(d)), (1, x, b(e))))

    def m2(d, e):
        return whole(((1, y, d), (1, y, e)), ((1, b(e), d),), ((1, y, b(e)), (-1, y, a(d))))

    def m3(d):
        return whole(((1, x, d),), ((1, a(d), d), *((-1, a(d), e) for e in rest(d))),
                     ((1, x, a(d)), (1, y, a(d))))

    def m4(d):
        return whole(((1, y, d),), ((1, b(d), d), *((-1, b(d), e) for e in rest(d))),
                     ((1, y, b(d)), (1, x, b(d))))

    def m5(d, e):
        return whole(((1, x, d), (1, x, e)), ((1, a(d), e),), ((1, x, a(d)), (-1, x, b(e))))

    def m6(d):
        return whole(((1, y, d), (-1, x, d)), ((1, a(d), d), *((1, b(e), d) for e in rest(d))),
                     ((1, y, a(d)),))

    def m7(d):
        return whole(((1, y, d), (-1, x, d)), ((-1, b(d), d), *((-1, a(e), d) for e in rest(d))),
                     ((1, x, b(d)),))

    def with_tails(p, p_rows, p_columns, q, q_rows, q_columns):
        tail = lambda columns: tuple((1, c, _TAIL) for c in columns)
        return [_Pass(p.low, p.high, q.w_low, p.w_high, p.wide + q.wide, common=True),
                _Pass(p.low, ((1, p_rows, _TAIL),), p.w_low, tail(p_columns), p.wide),
                _Pass(((1, q_rows, _TAIL),), q.high, tail(q_columns), q.w_high, q.wide)]

    def pair_with_tails(d, e):
        return [*with_tails(m5(d, e), x, [a(d)], m5(e, d), x, [a(e)]), m3(d),
                *with_tails(m2(d, e), y, [b(e)], m2(e, d), y, [b(d)]), m3(e),
                *with_tails(m6(d), y, [a(d), b(e)], m7(d), x, [b(d), a(e)]), m1(d, e), m4(d),
                *with_tails(m7(e), x, [b(e), a(d)], m6(e), y, [a(e), b(d)]), m1(e, d), m4(e)]

    edge = lambda d, e: [m5(d, e), m1(d, e), m2(d, e)]
    pair = lambda d, e: [m3(d), m6(d), *edge(d, e), m7(e), m4(e),
                         m3(e), m6(e), *edge(e, d), m7(d), m4(d)]
    if kind == "shared":
        return (*pair(0, 1), *(() if shift else _scheme(kind, 2)))
    if kind == "narrow":
        return (*pair_with_tails(0, 1), *pair(2, 3))
    ends = pair if kind == "member" else pair_with_tails
    return (*ends(0, 1), *edge(0, 2), *edge(0, 3), *edge(1, 2), *edge(1, 3),
            *edge(2, 0), *edge(3, 0), *edge(2, 1), *edge(3, 1), *ends(2, 3))


def _selected(kind, single):
    for i, p in enumerate(_scheme(kind)):
        if single:
            narrow = tuple((s, 0, d) for s, _, d in p.low)
            p = p._replace(low=narrow, high=narrow,
                           wide=tuple((s, 0, c) for s, r, c in p.wide if r == c // 4))
        if p.wide:
            yield i, p


def _tiles(w_refs, kind, family=_FAMILIES, member=_MEMBERS, skip=0):
    size = lambda name: len(_scheme(name)) // 2
    first = family * (_MEMBERS * size("member") + size("shared")) + skip
    if kind in ("member", "shared"):
        first += member * size("member")
    first += size("alone") if kind == "narrow" else 0
    count = size(kind) // (1 if isinstance(skip, int) else 2)
    views = [ref.at[pl.ds(first, count)] for ref in w_refs]
    return lambda i: (views[i % 2], i // 2)


def _tail_for(terms, block):
    return tuple(sorted((s, r, _TAIL if d == block else d) for s, r, d in terms))


@functools.cache
def _operand_keys(single):
    return tuple(dict.fromkeys(_tail_for(p.low, block) for block in (None, 0, 1)
                               for _, p in _selected("member", single)))


def _signed_sum(terms):
    terms = sorted(terms, key=lambda t: -t[0])
    total = terms[0][1] if terms[0][0] > 0 else -terms[0][1]
    for sign, value in terms[1:]:
        total = total + value if sign > 0 else total - value
    return total


def _accumulate(sums, key, sign, value):
    if key not in sums:
        sums[key] = (sign, value)
    elif sums[key][0] == sign:
        sums[key] = (sign, sums[key][1] + value)
    else:
        sums[key] = (1, value - sums[key][1] if sign > 0 else sums[key][1] - value)


def _words(ref):
    return ref.bitcast(jnp.uint32) if ref.dtype == jnp.bfloat16 else ref


def _unpack(words):
    return pltpu.bitcast(words, jnp.bfloat16) if words.dtype == jnp.uint32 else words


def _load(ref, i):
    return _unpack(_words(ref)[i])


def _store(ref, i, first, value):
    rows = value.shape[0]
    if value.dtype == jnp.bfloat16:
        _words(ref)[i, pl.ds(first // 2, rows // 2), :] = pltpu.bitcast(value, jnp.uint32)
    else:
        ref[i, pl.ds(first, rows), :] = value.astype(ref.dtype)


def _lane_half(rows):
    return jax.lax.broadcasted_iota(jnp.int32, (rows, _LANES), 1) // _HALF


def _blocks(x):
    return [x[:, d * _LANES:(d + 1) * _LANES] for d in range(_TAIL + 1)]


def _store_operands(ref, first, row_blocks):
    blocks = [_blocks(x) for x in row_blocks]
    for i, terms in enumerate(_operand_keys(len(row_blocks) == 1)):
        _store(ref, i, first, _signed_sum([(s, blocks[r][d]) for s, r, d in terms]))


def _dot(a, b):
    return jnp.dot(a, b, preferred_element_type=jnp.float32)


def _expand(operands_ref, w_refs, unit, out, single=False):
    operands_ref, tile = _words(operands_ref), _tiles(w_refs, *unit)
    operand = lambda terms: operands_ref[_operand_keys(single).index(terms)]
    half = _lane_half(operands_ref.shape[1])
    freed = {}
    if unit[0] == "member":
        blocks = [unit[2] // 2] if isinstance(unit[2], int) else range(_MEMBERS // 2)
        freed = {d: half == unit[2] - 2 * d for d in blocks}
    sums, common = {key: (1, value) for key, value in out.items()}, []
    for i, p in _selected(unit[0], single):
        lhs = operand(p.low)
        if p.high != p.low:
            lhs = jnp.where(half == 0, lhs, operand(p.high))
        for d, lanes in freed.items():
            if _tail_for(p.low, d) != p.low:
                lhs = jnp.where(lanes, operand(_tail_for(p.low, d)), lhs)
        product = _dot(_unpack(lhs), _load(*tile(i)))
        if p.common:
            common = [product, product]
        else:
            if common:
                product = product + common.pop()
            for s, r, c in p.wide:
                _accumulate(sums, (r, c), s, product)
        yield
    assert all(sign > 0 for sign, _ in sums.values())
    out.update({key: value for key, (_, value) in sums.items()})


def _contract(load, w_refs, unit, sums, single=False):
    tile = _tiles(w_refs, *unit)
    freed = unit[2] // 2 if unit[0] == "member" else None
    held, mixed = [], {}
    for i, p in _selected(unit[0], single):
        product = _dot(_signed_sum([(s, load(r, c)) for s, r, c in p.wide]),
                       _load(*tile(i)))
        if p.common or held:
            held.append((p, product))
        if len(held) == 3:
            (p, common), (p1, first), (p2, second) = held
            held = []
            product = common + jnp.where(_lane_half(common.shape[0]) == 0, first, second)
            _accumulate(sums, (p1.high[0][1], _TAIL, 1), 1, first)
            _accumulate(sums, (p2.low[0][1], _TAIL, 0), 1, second)
        if not held:
            for s, r, d in p.low:
                _accumulate(mixed if d == freed else sums, (r, d), s, product)
        yield
    for (r, d), (s, both) in mixed.items():
        _accumulate(sums, (r, _TAIL, unit[2] % 2), s, both)
        _accumulate(sums, (r, d), s, jnp.where(_lane_half(both.shape[0]) == unit[2] % 2, 0.0, both))


def _residual(row_blocks):
    return {(r, d) if d < _TAIL else (r, d, 0): (1, block)
            for r, x in enumerate(row_blocks) for d, block in enumerate(_blocks(x))}


def _contracted(sums, r):
    assert all(sign > 0 for sign, _ in sums.values())
    low, high = sums[r, _TAIL, 0][1], sums[r, _TAIL, 1][1]
    tail = jnp.where(_lane_half(low.shape[0]) == 0, low, high)
    tail = tail + pltpu.roll(tail, _HALF, 1)
    return jnp.concatenate([sums[r, d][1] for d in range(_TAIL)] + [tail], axis=1)


def _weight_sum(parts):
    return _signed_sum([(s, part.astype(jnp.float32) if len(parts) > 1 else part)
                        for s, part in parts])


def _weight_sums(passes, source, starts):
    for i, p in enumerate(passes):
        for high in range(2):
            if i > high and passes[i - 1 - high].common:
                continue
            for at in starts:
                first = high * _HALF + at
                total = lambda terms: _weight_sum(
                    [(s, source(c, 2 * d + high * (d < _TAIL), at)) for s, c, d in terms])
                terms = (p.w_low, p.w_high)[high]
                value = total(terms)
                yield i, first, value, len(terms)
                if p.common:
                    other = passes[i + 1 + high]
                    other = total((other.w_low, other.w_high)[high]).astype(jnp.float32)
                    yield i + 1 + high, first, other - value.astype(jnp.float32), len(terms) + 1


def _lay_out(sums, tile):
    for i, first, value, terms in sums:
        _store(*tile(i), pl.multiple_of(first, 16), value)
        yield from range(int(4 * terms + 1) * value.shape[0] // 16)


def _lay_out_transposed(sums, tile):
    halves, pending = {}, []
    for i, first, value, terms in sums:
        halves[i, first] = value
        if (i, _HALF - first) in halves:
            pair = [halves[i, 0], halves[i, _HALF]]
            if pair[0].dtype != pair[1].dtype:
                pair = [half.astype(jnp.float32) for half in pair]
            pending.append((i, jnp.concatenate(pair, axis=0).astype(jnp.bfloat16).T))
        if len(pending) > 2:
            _store(*tile(pending[0][0]), 0, pending.pop(0)[1])
        yield from range(int(8 * terms + 22))
    for i, value in pending:
        _store(*tile(i), 0, value)


def _layernorm(x):
    low_lanes = _lane_half(x.shape[0]) == 0

    def mean(v):
        *full, tail = _blocks(v)
        total = functools.reduce(jnp.add, full) + jnp.where(low_lanes, tail, 0.0)
        return jnp.sum(total, axis=-1, keepdims=True) / (_TAIL * _LANES + _HALF)

    d = x - mean(x)
    return d * jax.lax.rsqrt(mean(d * d) + _EPS)


def _silu(x):
    half = 0.5 * x
    return half + half * jnp.tanh(half)


def _reciprocal(x):
    r = pl.reciprocal(x, approx=True)
    return r * (2.0 - x * r)


def _attention_masks(n_layers, rows, n_mem):
    i = jax.lax.broadcasted_iota(jnp.int32, (n_layers * rows, n_layers * rows), 0)
    j = jax.lax.broadcasted_iota(jnp.int32, (n_layers * rows, n_layers * rows), 1)
    if n_layers == 1:
        return (i < n_mem) | (i >= j), _MASKED * _LOG2E
    same = (i >= rows) == (j >= rows)
    visible = (i < n_mem) | ((i >= rows) & (i < rows + n_mem)) | (i >= j)
    fill = jnp.where(same, _MASKED * _LOG2E, -jnp.inf).astype(jnp.float32)
    return same & visible, fill


def _expand_member(operands_ref, w_refs, family, member, shared_ref, out, single=False):
    rows = operands_ref.shape[1]
    if member == 0:
        yield from _expand(operands_ref, w_refs, ("shared", family), out, single)
        for (r, c), value in out.items():
            shared_ref[c, r * rows:(r + 1) * rows, :] = value
    out.update({(r, c): shared_ref[c, r * rows:(r + 1) * rows, :]
                for r in range(1 if single else 2) for c in range(_COLUMNS)})
    yield from _expand(operands_ref, w_refs, ("member", family, member), out, single)


def _store_wide(ref, member, c, rows, value):
    ref[member, c, rows, :] = value
    if member == _MEMBERS - 1:
        ref[_MEMBERS, c, rows, :] = functools.reduce(
            jnp.add, [ref[m, c, rows, :] for m in range(member)] + [value])


def _contract_member(ref, w_refs, family, member, sums, single=False):
    rows = ref.shape[2] // 2
    load = lambda m: lambda r, c: ref[m, c, r * rows:(r + 1) * rows, :]
    yield from _contract(load(member), w_refs, ("member", family, member), sums, single)
    if member == _MEMBERS - 1:
        yield from _contract(load(_MEMBERS), w_refs, ("shared", family), sums, single)


def _attention_tasks(xs, operands_ref, w_refs, qkv_ref, wide_ref, outs, known=None):
    n_layers, rows = len(xs), wide_ref.shape[2] // 2
    single, n_mem = n_layers == 1, rows - xs[0].shape[0]
    visible, fill = _attention_masks(n_layers, rows, n_mem)
    scale = _LANES ** -0.5 * _LOG2E
    qkv, probs = {}, {}
    sums = _residual([jnp.concatenate([jnp.zeros_like(x[:n_mem]), x], axis=0) for x in xs])

    def project(family, g):
        out = {}
        yield from _expand_member(operands_ref, w_refs, family, g,
                                  wide_ref.at[_MEMBERS + 1 + family], out, single)
        for h in range(_COLUMNS):
            if single:
                qkv[family, g, h] = out[0, h] if family == _WQ else out[0, h].astype(jnp.bfloat16)
                continue
            parts = x, y = out[0, h], out[1, h]
            if known:
                moved = (rows + n_mem) // 2
                parts = [x[:n_mem], known(family, g, h), x[n_mem:moved], y, x[moved:]]
            qkv_ref[family, g, h] = jnp.concatenate(parts, axis=0).astype(qkv_ref.dtype)

    def stacked(*at):
        return qkv[at] if single else _load(qkv_ref, at)

    def scores(g):
        for h in range(_COLUMNS):
            s = jax.lax.dot_general(stacked(_WQ, g, h), stacked(_WK, g, h),
                                    (((1,), (1,)), ((), ())), preferred_element_type=jnp.float32)
            s = jnp.where(visible, s * scale, fill)
            p = jnp.exp2(s - jnp.max(s, axis=-1, keepdims=True))
            p = p * _reciprocal(jnp.sum(p, axis=-1, keepdims=True))
            probs[g, h] = p if single else p.astype(jnp.bfloat16)
            yield

    def values(g):
        for h in range(_COLUMNS):
            _store_wide(wide_ref, g, h, slice(0, n_layers * rows),
                        _dot(probs[g, h], stacked(_WV, g, h)))
            yield

    def output(g):
        yield from _contract_member(wide_ref, w_refs, _WO, g, sums, single)
        if g == _MEMBERS - 1:
            outs.extend(_contracted(sums, r) for r in range(n_layers))

    tasks = {}
    for g in range(_MEMBERS):
        tasks.update({f"Q{g}": project(_WQ, g), f"K{g}": project(_WK, g), f"V{g}": project(_WV, g),
                      f"S{g}": scores(g), f"A{g}": values(g), f"O{g}": output(g)})
    return tasks


def _ffn_tasks(xs, operands_ref, w_refs, wide_ref, result):
    rows = operands_ref.shape[1]
    sums = _residual(xs)

    def gated(member, i):
        both = {}
        if member < _MEMBERS:
            yield from _expand_member(operands_ref, w_refs, _UP + i, member,
                                      wide_ref.at[_MEMBERS + 2 + i], both)
        else:
            yield from _expand(operands_ref, w_refs, ("alone",), both)
        for c in range(4):
            for r in range(2):
                _store_wide(wide_ref, member + member // _MEMBERS, 4 * i + c,
                            slice(r * rows, (r + 1) * rows), _silu(both[r, c]) * both[r, 4 + c])

    def finish():
        result([_contracted(sums, r) for r in range(2)])
        yield

    return {"F": finish(), **{f"G{u}": gated(*divmod(u, 2)) for u in range(2 * _MEMBERS + 1)},
            **{f"D{m}": _contract_member(wide_ref, w_refs, _DOWN, m, sums) for m in range(_MEMBERS)},
            "D4": _contract(lambda r, c: wide_ref[_MEMBERS + 1, c, r * rows:(r + 1) * rows, :],
                            w_refs, ("narrow",), sums)}


def _passes(order, tasks):
    done = object()
    for item in order.split():
        names, _, turns = item.partition(":")
        running = [(tasks[name], int(count or 1))
                   for name, _, count in (part.partition("*") for part in names.split("+"))]
        turn = 0
        while running and (not turns or turn < int(turns)):
            for task, count in tuple(running):
                for _ in range(count):
                    if next(task, done) is done:
                        running.remove((task, count))
                        break
                    yield
            turn += 1


def _chain(*tasks):
    for task in tasks:
        yield from task


def _run(*tasks):
    for _ in _chain(*tasks):
        pass


def _kernel(xt_hbm, mem0_hbm, wq_hbm, wk_hbm, wv_hbm, wot_hbm, w1_hbm, w3_hbm, w2t_hbm,
            outt_hbm, out_ref, h_ref, full_ref, short_ref, chunks_ref, qkv_ref, heads_ref, hidden_ref,
            early_ref, w_refs, x_stage, qkv_stage, qkv_shared, wo_stage, wo_shared, ffn_stage,
            ffn_shared, res_ref, mem0_ref, x_sem, attention_sem, ffn_sem, shared_sem, out_sem,
            *, seg):
    d_model, n_tok = xt_hbm.shape
    n_mem = mem0_hbm.shape[0]
    n_seg = n_tok // seg
    n_out = n_tok // _LANES

    def window(r, n):
        return res_ref.at[pl.ds(pl.multiple_of((r + _LAG) * seg, seg), n * seg)]

    def block(r, n=1):
        return pl.ds(r * seg, n * seg)

    def lanes(i, n=1):
        return pl.ds(pl.multiple_of(i * _LANES, _LANES), n * _LANES)

    def transpose_out(i, x):
        out_ref[i] = x.T[:d_model].astype(out_ref.dtype)

    def prepare(ref, blocks):
        for i, r in enumerate(blocks):
            h_ref[i, n_mem:] = _layernorm(ref[block(r), :])
        yield

    def attention(order, ref, blocks, others, early=None):
        xs, outs = [ref[block(r), :] for r in blocks], []
        hs = [h_ref[i] for i in range(len(blocks))]
        operands_ref, known = full_ref, None
        if early is not None:
            operands_ref, known = short_ref, lambda *at: early_ref[(early, *at)]
            hs = [jnp.concatenate([hs[0][:n_mem], hs[0][n_mem + seg // 2:], hs[1][seg:]], axis=0),
                  hs[1][:seg]]
        _store_operands(operands_ref, 0, hs)
        tasks = _attention_tasks(xs, operands_ref, w_refs, qkv_ref, heads_ref, outs, known)
        yield from _passes(order, {**others, **tasks})
        for i, r in enumerate(blocks):
            h_ref[i, :n_mem] = outs[i][:n_mem]
            ref[block(r), :] = outs[i][n_mem:]

    def ffn_tasks(ref, blocks, result=None):
        def update(ys):
            for r, y in zip(blocks, ys):
                ref[block(r, 2), :] = y

        def operands():
            for i in range(0, 2 * seg, 16):
                _store_operands(chunks_ref.at[0], i,
                                [_layernorm(ref[pl.ds(r * seg + i, 16), :]) for r in blocks])
            yield

        return {"N": operands(), **_ffn_tasks(
            [ref[block(r, 2), :] for r in blocks], chunks_ref.at[0], w_refs, hidden_ref,
            result or update)}

    def double_step(b):
        ref = window(b, _LAG + 2)
        _run(attention(_ORDER_DOUBLE, ref, [_LAG, 0],
                       {"X": prepare(ref, [_LAG + 1, 1])}, 1 + b))

    def two_steps(j):
        b = 6
        ref = window(2 * j - b, b + _LAG + 3)
        transpose_out(jnp.where((j % 2 == 1) & (j > 1), (j - 3) // 2, n_out - 1),
                      ref[block(0, 4), :])
        ffn = ffn_tasks(ref, [b + 2, b - 2])
        _run(attention(_ORDER_EVEN, ref, [b + _LAG, b],
                       {**ffn, "X": prepare(ref, [b + _LAG + 1, b + 1])}),
             attention(_ORDER_ODD, ref, [b + _LAG + 1, b + 1],
                       {**ffn, "X": prepare(ref, [b + _LAG + 2, b + 2])}, j + _LAG // 2))

    qkv_words = [_words(w) for w in (wq_hbm, wk_hbm, wv_hbm)]
    ffn_words = [_words(w) for w in (w1_hbm, w3_hbm, w2t_hbm)]
    pairs = _COLUMNS // 2

    def attention_copies(family, g):
        sem = attention_sem.at[family]
        if family == _WO:
            heads = _words(wot_hbm).at[pl.ds(_COLUMNS * g, _COLUMNS)]
            return [pltpu.make_async_copy(heads, wo_stage, sem)]
        return [pltpu.make_async_copy(qkv_words[family].at[:, pairs * g + p, :],
                                      qkv_stage.at[family, p], sem) for p in range(pairs)]

    def ffn_copies(m, columns=_COLUMNS):
        return [pltpu.make_async_copy(w.at[:, lanes(_COLUMNS * m, columns)],
                                      ffn_stage.at[m % 3, i, :, lanes(0, columns)],
                                      ffn_sem.at[3 * (m % 3) + i])
                for i, w in enumerate(ffn_words)]

    def shared_copies(which):
        ends = []
        for m in range(_MEMBERS):
            rows, words = pl.ds(m * _HALF, _HALF), pl.ds(m * _HALF // 2, _HALF // 2)
            if which == 0:
                ends += [(w.at[rows, pairs * m + p, :], qkv_shared.at[i, p, rows])
                         for i, w in enumerate(qkv_words) for p in range(pairs)]
            elif which == 1:
                ends += [(_words(wot_hbm).at[pl.ds(_COLUMNS * m, _COLUMNS), words],
                          wo_shared.at[:, words])]
            else:
                ends += [(w.at[words, lanes(_COLUMNS * m, _COLUMNS)], ffn_shared.at[i, words])
                         for i, w in enumerate(ffn_words)]
        return [pltpu.make_async_copy(*pair, shared_sem.at[which]) for pair in ends]

    def x_copy(chunk):
        columns = lanes(n_out // _CHUNKS * chunk, n_out // _CHUNKS)
        return pltpu.make_async_copy(xt_hbm.at[:, columns], x_stage.at[chunk], x_sem.at[chunk])

    def out_copy(i):
        return pltpu.make_async_copy(out_ref.at[i], outt_hbm.at[:, lanes(i)], out_sem.at[i])

    def start(copies):
        for c in copies:
            c.start()

    def wait(copies):
        for c in copies:
            c.wait()

    def head_pairs(ref):
        def source(c, half, first):
            rows = ref.at[c // 2, pl.ds(pl.multiple_of(half * _HALF, _HALF), _HALF)]
            words = rows[pl.ds(pl.multiple_of(first, 16), 16), :]
            words = words & jnp.uint32(0xFFFF0000) if c % 2 else words << 16
            return pltpu.bitcast(words, jnp.float32)
        return source

    def row_pairs(column, rows):
        def source(c, half, first):
            ref, at = column(c)
            words = ref.at[pl.ds(pl.multiple_of(half * (_HALF // 2), _HALF // 2), _HALF // 2)]
            return _unpack(words[pl.ds(first // 2, rows // 2), at])
        return source

    def member_sums(own, shared, m, rows, starts=None):
        places = [(jnp.where(m == h, 2 * _TAIL, h), jnp.where(m == h, _MEMBERS, h))
                  for h in range(_MEMBERS)]

        def source(c, d, high, first):
            if 2 * d >= _MEMBERS:
                return own(c, 2 * d + high, first)
            mine, theirs = places[2 * d + high]
            return (own(c, mine, first).astype(jnp.float32)
                    - shared(c, theirs, first).astype(jnp.float32))

        sets = {}
        for i, p in enumerate(_scheme("member")):
            owners = {c if c < 4 else d for _, c, d in p.w_low}
            key = -1 - min(owners) if len(owners) == 1 and rows < _HALF else i
            sets.setdefault(key, []).append((len(p.w_low), i, p))
        for tiles in sets.values():
            for high in range(2):
                for first in starts or range(0, _HALF, rows):
                    loaded = {}
                    for *_, i, p in sorted(tiles):
                        new = [(c, d) for _, c, d in p.w_low if (c, d) not in loaded]
                        loaded.update({at: source(*at, high, first) for at in new})
                        value = _weight_sum([(s, loaded[c, d]) for s, c, d in p.w_low])
                        work = len(p.w_low) + sum(1 + 2 * (d < 2) for _, d in new)
                        yield i, high * _HALF + first, value, work / 2

    def lay_out_heads(family, g, starts=None):
        sums = member_sums(head_pairs(qkv_stage.at[family]), head_pairs(qkv_shared.at[family]),
                           g, 16, starts)
        return _lay_out(sums, _tiles(w_refs, "member", family, g))

    def lay_out_shared_half(lay_out, words, rows, family, i):
        n = len(_scheme("shared")) // 2
        sums = _weight_sums(_scheme("shared")[:n], row_pairs(words, rows), range(0, _HALF, rows))
        return lay_out(sums, _tiles(w_refs, "shared", family, skip=n // 2 * i))

    def up_words(ref, first):
        return lambda c: (ref.at[c // 4], lanes(first + c % 4))

    def down_words(ref):
        return lambda c: (ref.at[2], lanes(c))

    def project_early(chunk, unit):
        at = lambda r, g, c: (pl.ds(8 * chunk + 4 * r, 4), unit[1], g, c)
        out = {}
        if unit[0] == "member":
            out = {(r, c): early_ref[at(r, _MEMBERS - 1, c)].reshape(2 * seg, _LANES)
                   for r in range(2) for c in range(_COLUMNS)}
        yield from _expand(chunks_ref.at[chunk], w_refs, unit, out)
        for (r, c), value in out.items():
            early_ref[at(r, unit[2] if unit[0] == "member" else _MEMBERS - 1, c)] = (
                value.reshape(4, seg // 2, _LANES))

    def load_chunk(chunk):
        x = x_stage[chunk].astype(jnp.float32)
        x = jnp.concatenate([x, x[_TAIL * _LANES:]], axis=0).T
        window(n_seg // _CHUNKS * chunk, n_seg // _CHUNKS)[...] = x
        segments = [2 * e + 1 for e in range(8)]
        if isinstance(chunk, int) and chunk == 0:
            segments[1] = _LAG
        for e in range(4):
            _store_operands(chunks_ref.at[chunk], e * seg // 2, [
                _layernorm(x[r * seg:r * seg + seg // 2]) for r in segments[e::4]])
        yield

    def clear(i):
        rows = lambda first, n=1: pl.ds(pl.multiple_of(first + 8 * n * i, 8), 8 * n)
        for spare in (res_ref.at[rows(0, _LAG)], res_ref.at[rows((_LAG + n_seg) * seg)],
                      wo_shared.at[:, rows(_MEMBERS * _HALF // 2)],
                      ffn_shared.at[:, rows(_MEMBERS * _HALF // 2)],
                      qkv_shared.at[:, :, rows(_MEMBERS * _HALF, 2)]):
            spare[...] = jnp.zeros(spare.shape, spare.dtype)

    def lay_out_shared(i):
        for family in (_WQ, _WK, _WV):
            sums = _weight_sums(_scheme("shared"), head_pairs(qkv_shared.at[family]), [16 * i])
            _run(_lay_out(sums, _tiles(w_refs, "shared", family)))

    def project_shared(chunk):
        pl.when(chunk == 1)(lambda: start(shared_copies(1) + attention_copies(_WK, 0)))
        pl.when(chunk == 2)(lambda: start(attention_copies(_WV, 0)))
        pl.when(chunk + 1 < _CHUNKS)(lambda: wait([x_copy(chunk + 1)]))
        _run(_passes(_ORDER_SHARED, {
            "E": _chain(*(project_early(chunk, ("shared", f)) for f in (_WQ, _WK, _WV))),
            "L": lay_out_heads(_WQ, 0, [16 * chunk]),
            "X": load_chunk(jnp.minimum(chunk + 1, _CHUNKS - 1))}))

    def load_group(g):
        more = g + 1 < _MEMBERS

        def arrive(family):
            if family == _WK:
                start(attention_copies(_WO, g))
                pl.when(more)(lambda: start(attention_copies(_WQ, g + 1)))
                pl.when(~more)(lambda: start(shared_copies(2)))
                wait(attention_copies(_WK, g))
            elif family == _WV:
                wait(attention_copies(_WV, g) + attention_copies(_WO, g))
                pl.when(more)(lambda: start(attention_copies(_WK, g + 1)))
                for i, copy in enumerate(ffn_copies(0)):
                    pl.when(g == i)(copy.start)
                pl.when(~more)(lambda: start(ffn_copies(1)))
            else:
                pl.when(more)(lambda: wait(attention_copies(_WQ, g + 1)))
                pl.when(more)(lambda: start(attention_copies(_WV, g + 1)))
            yield

        same = jnp.minimum(g, _MEMBERS - 1)
        wo_sums = member_sums(row_pairs(lambda c: (wo_stage.at[c], slice(None)), _HALF),
                              row_pairs(lambda c: (wo_shared.at[c], slice(None)), _HALF), g, _HALF)
        _run(_passes(_ORDER_LOAD, {
            **{f"E{f}": _chain(*(project_early(chunk, ("member", f, g)) for chunk in range(_CHUNKS)))
               for f in (_WQ, _WK, _WV)},
            **{f"W{f}": arrive(f) for f in (_WQ, _WK, _WV)},
            "L0": lay_out_heads(_WQ, jnp.minimum(g + 1, _MEMBERS - 1)),
            "L1": lay_out_heads(_WK, same), "L2": lay_out_heads(_WV, same),
            "L3": _lay_out_transposed(wo_sums, _tiles(w_refs, "member", _WO, same)),
            "L4": lay_out_shared_half(
                _lay_out_transposed, lambda c: (wo_shared.at[c + 2 * (g % 2)], slice(None)), _HALF,
                _WO, g % 2)}))

    def first_step(m):
        pl.when(m + 2 < _MEMBERS)(lambda: start(ffn_copies(m + 2)))
        pl.when(m + 2 == _MEMBERS)(lambda: start(ffn_copies(_MEMBERS, 4)))
        wait(ffn_copies(m))
        ref, stage = window(m, 2), ffn_stage.at[m % 3]
        up = [_lay_out(member_sums(row_pairs(up_words(stage, 4 * i), 16),
                                   row_pairs(up_words(ffn_shared, 4 * i), 16), m, 16),
                       _tiles(w_refs, "member", _UP + i, m)) for i in range(2)]
        shared = lay_out_shared_half(_lay_out, up_words(ffn_shared, 2 * m), 16, _UP + m // 2, m % 2)
        down = _lay_out_transposed(
            member_sums(row_pairs(down_words(stage), _HALF),
                        row_pairs(down_words(ffn_shared), _HALF), m, _HALF),
            _tiles(w_refs, "member", _DOWN, m))
        _run(_passes(_ORDER_FIRST, {
            "P": attention(_ORDER_SINGLE, ref, [0], {"X": prepare(ref, [1])}),
            "L": _passes("U*9+D*5", {"U": _chain(shared, *up), "D": down})}))

    def first_ffn():
        stage = ffn_stage.at[_MEMBERS % 3]
        down = lambda kind, ref, *family: _lay_out_transposed(
            _weight_sums(_scheme(kind), row_pairs(down_words(ref), _HALF), [0]),
            _tiles(w_refs, kind, *family))
        up = _lay_out(_weight_sums(_scheme("alone"), row_pairs(up_words(stage, 0), 32), [0, 32]),
                      _tiles(w_refs, "alone"))
        _run(up, down("narrow", stage), down("shared", ffn_shared, _DOWN),
             _passes(_ORDER_FIRST_FFN, ffn_tasks(window(0, _LAG), [0, 2])))

    def last_steps():
        ref = window(n_seg - _LAG - 2, _LAG + 2)
        ffn = ffn_tasks(ref, [_LAG, 0])
        _run(attention(_ORDER_EVEN_SINGLE, ref, [2], {**ffn, "X": prepare(ref, [3])}),
             attention(_ORDER_ODD_SINGLE, ref, [3], {**ffn, "X": prepare(ref, [4])}))

    def last_step(i):
        tile = n_out - 3 + i
        transpose_out(tile, window(_LANES // seg * tile, _LANES // seg)[...])
        ref = window(n_seg - 2 + i, 2)
        _run(attention(_ORDER_SINGLE, ref, [0], {"X": prepare(ref, [1])}))
        out_copy(tile).start()

    def last_ffn():
        _run(_passes(_ORDER_FFN, ffn_tasks(
            window(n_seg - _LAG, _LAG), [0, 2],
            lambda ys: transpose_out(n_out - 1, jnp.concatenate(ys, axis=0)))))

    mem_copy = pltpu.make_async_copy(mem0_hbm, mem0_ref.at[0], shared_sem.at[3])
    x_copy(0).start()
    pl.loop(0, 4)(clear)
    start([mem_copy] + shared_copies(0))
    wait([x_copy(0), mem_copy])
    start([x_copy(1)] + attention_copies(_WQ, 0))
    mem0 = mem0_ref[0].astype(jnp.float32)
    h_ref[0, :n_mem] = h_ref[1, :n_mem] = jnp.concatenate(
        [mem0, mem0[:, _TAIL * _LANES:]], axis=1)
    _run(load_chunk(0), prepare(window(0, 1), [0]))
    wait(shared_copies(0))
    pl.loop(0, _HALF // 16)(lay_out_shared)
    x_copy(2).start()
    wait(attention_copies(_WQ, 0))
    x_copy(3).start()
    pl.loop(0, _CHUNKS)(project_shared)
    wait(shared_copies(1))
    pl.loop(0, _MEMBERS)(load_group)
    wait(shared_copies(2))
    pl.loop(0, _LAG)(first_step)
    wait(ffn_copies(_MEMBERS, 4))
    first_ffn()
    _run(prepare(window(0, _LAG + 1), [_LAG, 0]))
    pl.loop(0, 2)(double_step)
    pl.loop(1, (n_seg - _LAG) // 2)(two_steps)
    start([out_copy(i) for i in range(n_out - 3)])
    h_ref[0] = h_ref[1]
    last_steps()
    pl.loop(0, 2)(last_step)
    last_ffn()
    out_copy(n_out - 1).start()
    wait([out_copy(i) for i in range(n_out)])


@functools.partial(jax.jit, static_argnames=("A_seg_len",))
def pallas_interleave_layers__memory_aug_recurrent_mem_tr__glu_gated_swiglu__prompt_kernel(
    A_x: jax.Array,
    A_mem0: jax.Array,
    A_Wq: jax.Array,
    A_Wk: jax.Array,
    A_Wv: jax.Array,
    A_Wo: jax.Array,
    A_seg_len: int,
    B_x: jax.Array,
    B_w1: jax.Array,
    B_w3: jax.Array,
    B_w2: jax.Array,
):
    del B_x
    _, n_tok, d_model = A_x.shape
    n_mem = A_mem0.shape[1]
    _, n_heads, d_head = A_Wq.shape
    seg = A_seg_len
    assert A_x.shape[0] == 1 and _LAG * seg == _LANES and n_mem == 8
    assert n_tok == 16 * _CHUNKS * seg and d_model == _TAIL * _LANES + _HALF and d_head == _LANES
    assert n_heads == _MEMBERS * _COLUMNS and B_w1.shape[1] == (n_heads + 4) * _LANES
    n_operands = pl.cdiv(len(_operand_keys(False)), 8) * 8
    n_tiles = (_FAMILIES * (_MEMBERS * len(_scheme("member")) + len(_scheme("shared")))
               + len(_scheme("alone")) + len(_scheme("narrow")))
    shared_rows = (_MEMBERS + 1) * _HALF
    hbm = pl.BlockSpec(memory_space=pltpu.HBM)
    out_t = pl.pallas_call(
        functools.partial(_kernel, seg=seg),
        out_shape=jax.ShapeDtypeStruct((d_model, n_tok), A_x.dtype),
        in_specs=[hbm] * 9,
        out_specs=hbm,
        scratch_shapes=[
            pltpu.VMEM((n_tok // _LANES, d_model, _LANES), A_x.dtype),
            pltpu.VMEM((8, n_mem + seg, d_model + _HALF), jnp.float32),
            pltpu.VMEM((n_operands, n_mem + seg, _LANES), jnp.float32),
            pltpu.VMEM((n_operands, seg, _LANES), jnp.bfloat16),
            pltpu.VMEM((_CHUNKS, n_operands, 2 * seg, _LANES), jnp.bfloat16),
            pltpu.VMEM((3, _MEMBERS, _COLUMNS, 2 * (n_mem + seg), _LANES), jnp.bfloat16),
            pltpu.VMEM((_MEMBERS + 4, _COLUMNS, 2 * (n_mem + seg), _LANES), jnp.float32),
            pltpu.VMEM((_MEMBERS + 4, _COLUMNS, 4 * seg, _LANES), jnp.float32),
            pltpu.VMEM((8 * _CHUNKS, 3, _MEMBERS, _COLUMNS, seg // 2, _LANES), jnp.float32),
            [pltpu.VMEM((n_tiles // 2, _LANES, _LANES), jnp.bfloat16)] * 2,
            pltpu.VMEM((_CHUNKS, d_model, n_tok // _CHUNKS), A_x.dtype),
            pltpu.VMEM((3, _COLUMNS // 2, d_model, _LANES), jnp.uint32),
            pltpu.VMEM((3, _COLUMNS // 2, shared_rows, _LANES), jnp.uint32),
            pltpu.VMEM((_COLUMNS, d_model // 2, _LANES), jnp.uint32),
            pltpu.VMEM((_COLUMNS, shared_rows // 2, _LANES), jnp.uint32),
            pltpu.VMEM((3, 3, d_model // 2, _COLUMNS * _LANES), jnp.uint32),
            pltpu.VMEM((3, shared_rows // 2, _COLUMNS * _LANES), jnp.uint32),
            pltpu.VMEM((n_tok + 2 * _LAG * seg, d_model + _HALF), jnp.float32),
            pltpu.VMEM((16, n_mem, d_model), A_mem0.dtype),
            pltpu.SemaphoreType.DMA((_CHUNKS,)),
            pltpu.SemaphoreType.DMA((4,)),
            pltpu.SemaphoreType.DMA((9,)),
            pltpu.SemaphoreType.DMA((4,)),
            pltpu.SemaphoreType.DMA((n_tok // _LANES,)),
        ],
        compiler_params=pltpu.CompilerParams(
            vmem_limit_bytes=126 * 1024 * 1024, disable_bounds_checks=True,
            flags={"XLA_TPU_FORCE_LP_LLO_SCHEDULER": True}),
    )(A_x.reshape(n_tok, d_model).T, A_mem0.reshape(n_mem, d_model), A_Wq, A_Wk, A_Wv,
      A_Wo.transpose(0, 2, 1), B_w1, B_w3, B_w2.T)
    return out_t.T.reshape(A_x.shape)
```

```python
import functools
import math
from typing import NamedTuple

import jax
import jax.numpy as jnp
import jax.experimental.pallas as pl
import jax.experimental.pallas.tpu as pltpu

_EPS = 1e-05
_MASKED = -1000000000.0
_LOG2E = math.log2(math.e)
_LANES = 128
_HALF = _LANES // 2
_TAIL = 4
_COLUMNS = 8
_MEMBERS = 4
_WQ, _WK, _WV, _WO, _W1, _W3, _W2, _FAMILIES = range(8)
_LAG = 4
_CHUNKS = 4
_ORDER_EVEN = (
    "N X Q0 K0 V0*10+S0 Q1 A0 K1 V1*6+S1 Q2 K2 V2*6+S2 A1 Q3 A2 O0 O1 O2 K3 G0 U0*10+S3 V3 "
    "A3+G1*6 G4 U4 U1 O3 D4")
_ORDER_ODD = (
    "Q0 K0 G2 U2 D0*6+S0 V0 Q1 A0 K1 G3 U3 V1 D1*6+S1 Q2 A1 K2 V2 D2*6+S2 Q3 K3 V3 O0*4+S3 A2 "
    "D3 F X A3+O1*6 O2 O3")
_ORDER_EVEN_SINGLE = (
    "Q0 N K0 V0*4+S0 Q1 K1 G0 A0 V1*4+S1 O0 U0 A1 Q2 K2 V2*4+S2 O1 G1 A2 Q3 K3 V3*4+S3 X O2 "
    "U1 A3 G4 U4 O3 D4 G2")
_ORDER_ODD_SINGLE = (
    "Q0 K0 V0*4+S0 U2 A0 Q1 K1 V1*4+S1 G3 A1 Q2 K2 U3 V2*4+S2 D0 A2 Q3 K3 "
    "D1 D2 D3 F X V3*4+S3 O0 O1 A3 O2 O3")
_ORDER_DOUBLE = (
    "Q0 K0 Q1 K1 V0*10+S0 Q2 K2 V1*6+S1 A0 Q3 K3 V2 A1 O0*6+S2 V3 X O1*6+S3 A2 O2:30 A3 O2 O3")
_ORDER_SINGLE = (
    "Q0 K0 V0*4+S0 Q1 K1 A0 V1*4+S1 Q2 K2 A1 V2*4+S2 Q3 K3 A2 V3*4+S3 X O0 O1 A3 O2 O3")
_ORDER_FFN = "N G0 U0 G1 D0 U1 G2 D1 U2 G3 U3 G4 U4 D2 D4 D3 F"
_ORDER_SHARED = "E+L*13 X"
_ORDER_LOAD = "W1 E0+L1*20+L4*5 W2 E1+L2*20+L3*12:208 E1 L2 W0 E2+L0*20+L3*12"
_ORDER_FIRST = "P:8 P+L*23"
_ORDER_FIRST_FFN = "N G0 U0 G1 U1 G2 U2 G4+D0*2 U4+D1*2 D2 G3 U3*2+D4 D3 F"


class _Pass(NamedTuple):
    low: tuple
    high: tuple
    w_low: tuple
    w_high: tuple
    wide: tuple
    common: bool = False


@functools.cache
def _scheme(kind, shift=0):
    x, y, n = 0, 1, 4 if kind == "member" else 2
    a = lambda d: d % n + shift
    b = lambda d: d % n + shift + (2 if kind == "narrow" else 4)
    rest = lambda d: [e for e in range(4) if e != d and e // n == d // n]

    def whole(narrow, weight, wide):
        return _Pass(tuple(sorted(narrow)), tuple(sorted(narrow)), weight, weight, wide)

    def m1(d, e):
        return whole(((1, x, d), (1, y, e)), ((1, b(e), d), (1, a(d), e)),
                     ((1, y, a(d)), (1, x, b(e))))

    def m2(d, e):
        return whole(((1, y, d), (1, y, e)), ((1, b(e), d),), ((1, y, b(e)), (-1, y, a(d))))

    def m3(d):
        return whole(((1, x, d),), ((1, a(d), d), *((-1, a(d), e) for e in rest(d))),
                     ((1, x, a(d)), (1, y, a(d))))

    def m4(d):
        return whole(((1, y, d),), ((1, b(d), d), *((-1, b(d), e) for e in rest(d))),
                     ((1, y, b(d)), (1, x, b(d))))

    def m5(d, e):
        return whole(((1, x, d), (1, x, e)), ((1, a(d), e),), ((1, x, a(d)), (-1, x, b(e))))

    def m6(d):
        return whole(((1, y, d), (-1, x, d)), ((1, a(d), d), *((1, b(e), d) for e in rest(d))),
                     ((1, y, a(d)),))

    def m7(d):
        return whole(((1, y, d), (-1, x, d)), ((-1, b(d), d), *((-1, a(e), d) for e in rest(d))),
                     ((1, x, b(d)),))

    def with_tails(p, p_rows, p_columns, q, q_rows, q_columns):
        tail = lambda columns: tuple((1, c, _TAIL) for c in columns)
        return [_Pass(p.low, p.high, q.w_low, p.w_high, p.wide + q.wide, common=True),
                _Pass(p.low, ((1, p_rows, _TAIL),), p.w_low, tail(p_columns), p.wide),
                _Pass(((1, q_rows, _TAIL),), q.high, tail(q_columns), q.w_high, q.wide)]

    def pair_with_tails(d, e):
        return [*with_tails(m5(d, e), x, [a(d)], m5(e, d), x, [a(e)]), m3(d),
                *with_tails(m2(d, e), y, [b(e)], m2(e, d), y, [b(d)]), m3(e),
                *with_tails(m6(d), y, [a(d), b(e)], m7(d), x, [b(d), a(e)]), m1(d, e), m4(d),
                *with_tails(m7(e), x, [b(e), a(d)], m6(e), y, [a(e), b(d)]), m1(e, d), m4(e)]

    edge = lambda d, e: [m5(d, e), m1(d, e), m2(d, e)]
    pair = lambda d, e: [m3(d), m6(d), *edge(d, e), m7(e), m4(e),
                         m3(e), m6(e), *edge(e, d), m7(d), m4(d)]
    if kind == "shared":
        return (*pair(0, 1), *(() if shift else _scheme(kind, 2)))
    if kind == "narrow":
        return (*pair_with_tails(0, 1), *pair(2, 3))
    return (*pair(0, 1), *edge(0, 2), *edge(0, 3), *edge(1, 2), *edge(1, 3),
            *edge(2, 0), *edge(3, 0), *edge(2, 1), *edge(3, 1), *pair(2, 3))


def _selected(kind, single):
    for i, p in enumerate(_scheme(kind)):
        if single:
            narrow = tuple((s, 0, d) for s, _, d in p.low)
            p = p._replace(low=narrow, high=narrow,
                           wide=tuple((s, 0, c) for s, r, c in p.wide if r == c // 4))
        if p.wide:
            yield i, p


def _tiles(w_refs, kind, family, member=_MEMBERS, half=None):
    size = lambda name: len(_scheme(name)) // 2
    per_family = _MEMBERS * size("member") + size("shared")
    first, count = family * per_family + member * size("member"), size(kind)
    if kind == "narrow":
        first = _FAMILIES * per_family + (family - _W1) * count
    if half is not None:
        first, count = first + half * (count // 2), count // 2
    views = [ref.at[pl.ds(first, count)] for ref in w_refs]
    return lambda i: (views[i % 2], i // 2)


def _tail_for(terms, block):
    return tuple(sorted((s, r, _TAIL if d == block else d) for s, r, d in terms))


@functools.cache
def _operand_keys(single):
    return tuple(dict.fromkeys(_tail_for(p.low, block) for block in (None, 0, 1)
                               for _, p in _selected("member", single)))


def _signed_sum(terms):
    terms = sorted(terms, key=lambda t: -t[0])
    total = terms[0][1] if terms[0][0] > 0 else -terms[0][1]
    for sign, value in terms[1:]:
        total = total + value if sign > 0 else total - value
    return total


def _accumulate(sums, key, sign, value):
    if key not in sums:
        sums[key] = (sign, value)
    elif sums[key][0] == sign:
        sums[key] = (sign, sums[key][1] + value)
    else:
        sums[key] = (1, value - sums[key][1] if sign > 0 else sums[key][1] - value)


def _words(ref):
    return ref.bitcast(jnp.uint32) if ref.dtype == jnp.bfloat16 else ref


def _unpack(words):
    return pltpu.bitcast(words, jnp.bfloat16) if words.dtype == jnp.uint32 else words


def _load(ref, i):
    return _unpack(_words(ref)[i])


def _store(ref, i, first, value):
    rows = value.shape[0]
    if value.dtype == jnp.bfloat16:
        _words(ref)[i, pl.ds(first // 2, rows // 2), :] = pltpu.bitcast(value, jnp.uint32)
    else:
        ref[i, pl.ds(first, rows), :] = value.astype(ref.dtype)


def _lane_half(rows):
    return jax.lax.broadcasted_iota(jnp.int32, (rows, _LANES), 1) // _HALF


def _blocks(x):
    return [x[:, d * _LANES:(d + 1) * _LANES] for d in range(_TAIL + 1)]


def _store_operands(ref, first, row_blocks):
    blocks = [_blocks(x) for x in row_blocks]
    for i, terms in enumerate(_operand_keys(len(row_blocks) == 1)):
        _store(ref, i, first, _signed_sum([(s, blocks[r][d]) for s, r, d in terms]))


def _dot(a, b):
    return jnp.dot(a, b, preferred_element_type=jnp.float32)


def _expand(operands_ref, w_refs, unit, out, single=False):
    operands_ref, tile = _words(operands_ref), _tiles(w_refs, *unit)
    operand = lambda terms: operands_ref[_operand_keys(single).index(terms)]
    half = _lane_half(operands_ref.shape[1])
    freed = {}
    if unit[0] == "member":
        blocks = [unit[2] // 2] if isinstance(unit[2], int) else range(_MEMBERS // 2)
        freed = {d: half == unit[2] - 2 * d for d in blocks}
    sums, common = {key: (1, value) for key, value in out.items()}, []
    for i, p in _selected(unit[0], single):
        lhs = operand(p.low)
        if p.high != p.low:
            lhs = jnp.where(half == 0, lhs, operand(p.high))
        for d, lanes in freed.items():
            if _tail_for(p.low, d) != p.low:
                lhs = jnp.where(lanes, operand(_tail_for(p.low, d)), lhs)
        product = _dot(_unpack(lhs), _load(*tile(i)))
        if p.common:
            common = [product, product]
        else:
            if common:
                product = product + common.pop()
            for s, r, c in p.wide:
                _accumulate(sums, (r, c), s, product)
        yield
    assert all(sign > 0 for sign, _ in sums.values())
    out.update({key: value for key, (_, value) in sums.items()})


def _contract(load, w_refs, unit, sums, single=False):
    tile = _tiles(w_refs, *unit)
    freed = unit[2] // 2 if unit[0] == "member" else None
    held, mixed = [], {}
    for i, p in _selected(unit[0], single):
        product = _dot(_signed_sum([(s, load(r, c)) for s, r, c in p.wide]),
                       _load(*tile(i)))
        if p.common or held:
            held.append((p, product))
        if len(held) == 3:
            (p, common), (p1, first), (p2, second) = held
            held = []
            product = common + jnp.where(_lane_half(common.shape[0]) == 0, first, second)
            _accumulate(sums, (p1.high[0][1], _TAIL, 1), 1, first)
            _accumulate(sums, (p2.low[0][1], _TAIL, 0), 1, second)
        if not held:
            for s, r, d in p.low:
                _accumulate(mixed if d == freed else sums, (r, d), s, product)
        yield
    for (r, d), (s, both) in mixed.items():
        _accumulate(sums, (r, _TAIL, unit[2] % 2), s, both)
        _accumulate(sums, (r, d), s, jnp.where(_lane_half(both.shape[0]) == unit[2] % 2, 0.0, both))


def _residual(row_blocks):
    return {(r, d) if d < _TAIL else (r, d, 0): (1, block)
            for r, x in enumerate(row_blocks) for d, block in enumerate(_blocks(x))}


def _contracted(sums, r):
    assert all(sign > 0 for sign, _ in sums.values())
    low, high = sums[r, _TAIL, 0][1], sums[r, _TAIL, 1][1]
    tail = jnp.where(_lane_half(low.shape[0]) == 0, low, high)
    tail = tail + pltpu.roll(tail, _HALF, 1)
    return jnp.concatenate([sums[r, d][1] for d in range(_TAIL)] + [tail], axis=1)


def _weight_sum(parts):
    return _signed_sum([(s, part.astype(jnp.float32) if len(parts) > 1 else part)
                        for s, part in parts])


def _weight_sums(passes, source, starts):
    for i, p in enumerate(passes):
        for high in range(2):
            if i > high and passes[i - 1 - high].common:
                continue
            for at in starts:
                first = high * _HALF + at
                total = lambda terms: _weight_sum(
                    [(s, source(c, 2 * d + high * (d < _TAIL), at)) for s, c, d in terms])
                terms = (p.w_low, p.w_high)[high]
                value = total(terms)
                yield i, first, value, len(terms)
                if p.common:
                    other = passes[i + 1 + high]
                    other = total((other.w_low, other.w_high)[high]).astype(jnp.float32)
                    yield i + 1 + high, first, other - value.astype(jnp.float32), len(terms) + 1


def _lay_out(sums, tile):
    for i, first, value, terms in sums:
        _store(*tile(i), pl.multiple_of(first, 16), value)
        yield from range(int(4 * terms + 1) * value.shape[0] // 16)


def _lay_out_transposed(sums, tile):
    halves, pending = {}, []
    for i, first, value, terms in sums:
        halves[i, first] = value
        if (i, _HALF - first) in halves:
            pair = [halves[i, 0], halves[i, _HALF]]
            if pair[0].dtype != pair[1].dtype:
                pair = [half.astype(jnp.float32) for half in pair]
            pending.append((i, jnp.concatenate(pair, axis=0).astype(jnp.bfloat16).T))
        if len(pending) > 2:
            _store(*tile(pending[0][0]), 0, pending.pop(0)[1])
        yield from range(int(8 * terms + 22))
    for i, value in pending:
        _store(*tile(i), 0, value)


def _layernorm(x):
    low_lanes = _lane_half(x.shape[0]) == 0

    def mean(v):
        *full, tail = _blocks(v)
        total = functools.reduce(jnp.add, full) + jnp.where(low_lanes, tail, 0.0)
        return jnp.sum(total, axis=-1, keepdims=True) / (_TAIL * _LANES + _HALF)

    d = x - mean(x)
    return d * jax.lax.rsqrt(mean(d * d) + _EPS)


def _silu(x):
    half = 0.5 * x
    return half + half * jnp.tanh(half)


def _reciprocal(x):
    r = pl.reciprocal(x, approx=True)
    return r * (2.0 - x * r)


def _attention_masks(n_layers, rows, n_mem):
    i = jax.lax.broadcasted_iota(jnp.int32, (n_layers * rows, n_layers * rows), 0)
    j = jax.lax.broadcasted_iota(jnp.int32, (n_layers * rows, n_layers * rows), 1)
    if n_layers == 1:
        return (i < n_mem) | (i >= j), _MASKED * _LOG2E
    same = (i >= rows) == (j >= rows)
    visible = (i < n_mem) | ((i >= rows) & (i < rows + n_mem)) | (i >= j)
    fill = jnp.where(same, _MASKED * _LOG2E, -jnp.inf).astype(jnp.float32)
    return same & visible, fill


def _expand_member(operands_ref, w_refs, family, member, shared_ref, out, single=False):
    rows = operands_ref.shape[1]
    if member == 0:
        yield from _expand(operands_ref, w_refs, ("shared", family), out, single)
        for (r, c), value in out.items():
            shared_ref[c, r * rows:(r + 1) * rows, :] = value
    out.update({(r, c): shared_ref[c, r * rows:(r + 1) * rows, :]
                for r in range(1 if single else 2) for c in range(_COLUMNS)})
    yield from _expand(operands_ref, w_refs, ("member", family, member), out, single)


def _store_wide(ref, member, c, rows, value):
    ref[member, c, rows, :] = value
    if member == _MEMBERS - 1:
        ref[_MEMBERS, c, rows, :] = functools.reduce(
            jnp.add, [ref[m, c, rows, :] for m in range(member)] + [value])


def _contract_member(ref, w_refs, family, member, sums, single=False):
    rows = ref.shape[2] // 2
    load = lambda m: lambda r, c: ref[m, c, r * rows:(r + 1) * rows, :]
    yield from _contract(load(member), w_refs, ("member", family, member), sums, single)
    if member == _MEMBERS - 1:
        yield from _contract(load(_MEMBERS), w_refs, ("shared", family), sums, single)


def _attention_tasks(xs, operands_ref, w_refs, qkv_ref, wide_ref, outs, known=None):
    n_layers, rows = len(xs), wide_ref.shape[2] // 2
    single, n_mem = n_layers == 1, rows - xs[0].shape[0]
    visible, fill = _attention_masks(n_layers, rows, n_mem)
    scale = _LANES ** -0.5 * _LOG2E
    qkv, probs = {}, {}
    sums = _residual([jnp.concatenate([jnp.zeros_like(x[:n_mem]), x], axis=0) for x in xs])

    def project(family, g):
        out = {}
        yield from _expand_member(operands_ref, w_refs, family, g,
                                  wide_ref.at[_MEMBERS + 1 + family], out, single)
        for h in range(_COLUMNS):
            if single:
                qkv[family, g, h] = out[0, h] if family == _WQ else out[0, h].astype(jnp.bfloat16)
                continue
            parts = x, y = out[0, h], out[1, h]
            if known:
                moved = (rows + n_mem) // 2
                parts = [x[:n_mem], known(family, g, h), x[n_mem:moved], y, x[moved:]]
            qkv_ref[family, g, h] = jnp.concatenate(parts, axis=0).astype(qkv_ref.dtype)

    def stacked(*at):
        return qkv[at] if single else _load(qkv_ref, at)

    def scores(g):
        for h in range(_COLUMNS):
            s = jax.lax.dot_general(stacked(_WQ, g, h), stacked(_WK, g, h),
                                    (((1,), (1,)), ((), ())), preferred_element_type=jnp.float32)
            s = jnp.where(visible, s * scale, fill)
            p = jnp.exp2(s - jnp.max(s, axis=-1, keepdims=True))
            p = p * _reciprocal(jnp.sum(p, axis=-1, keepdims=True))
            probs[g, h] = p if single else p.astype(jnp.bfloat16)
            yield

    def values(g):
        for h in range(_COLUMNS):
            _store_wide(wide_ref, g, h, slice(0, n_layers * rows),
                        _dot(probs[g, h], stacked(_WV, g, h)))
            yield

    def output(g):
        yield from _contract_member(wide_ref, w_refs, _WO, g, sums, single)
        if g == _MEMBERS - 1:
            outs.extend(_contracted(sums, r) for r in range(n_layers))

    tasks = {}
    for g in range(_MEMBERS):
        tasks.update({f"Q{g}": project(_WQ, g), f"K{g}": project(_WK, g), f"V{g}": project(_WV, g),
                      f"S{g}": scores(g), f"A{g}": values(g), f"O{g}": output(g)})
    return tasks


def _ffn_tasks(xs, operands_ref, w_refs, wide_ref, result):
    rows = operands_ref.shape[1]
    sums = _residual(xs)

    def hidden(family, m):
        out, slot = {}, m + m // _MEMBERS
        if m < _MEMBERS:
            yield from _expand_member(operands_ref, w_refs, family, m,
                                      wide_ref.at[_MEMBERS + 2 + family - _W1], out)
        else:
            yield from _expand(operands_ref, w_refs, ("narrow", family), out)
        for (r, c), value in out.items():
            at = slice(r * rows, (r + 1) * rows)
            if family == _W1:
                wide_ref[slot, c, at, :] = _silu(value)
            else:
                _store_wide(wide_ref, slot, c, at, wide_ref[slot, c, at, :] * value)

    def finish():
        result([_contracted(sums, r) for r in range(2)])
        yield

    tasks = {"F": finish(), "D4": _contract(
        lambda r, c: wide_ref[_MEMBERS + 1, c, r * rows:(r + 1) * rows, :], w_refs,
        ("narrow", _W2), sums)}
    for m in range(_MEMBERS + 1):
        tasks.update({f"G{m}": hidden(_W1, m), f"U{m}": hidden(_W3, m)})
    for m in range(_MEMBERS):
        tasks[f"D{m}"] = _contract_member(wide_ref, w_refs, _W2, m, sums)
    return tasks


def _passes(order, tasks):
    done = object()
    for item in order.split():
        names, _, turns = item.partition(":")
        running = [(tasks[name], int(count or 1))
                   for name, _, count in (part.partition("*") for part in names.split("+"))]
        turn = 0
        while running and (not turns or turn < int(turns)):
            for task, count in tuple(running):
                for _ in range(count):
                    if next(task, done) is done:
                        running.remove((task, count))
                        break
                    yield
            turn += 1


def _chain(*tasks):
    for task in tasks:
        yield from task


def _run(*tasks):
    for _ in _chain(*tasks):
        pass


def _kernel(xt_hbm, mem0_hbm, wq_hbm, wk_hbm, wv_hbm, wot_hbm, w1_hbm, w3_hbm, w2t_hbm,
            outt_hbm, out_ref, h_ref, full_ref, short_ref, chunks_ref, qkv_ref, heads_ref, hidden_ref,
            early_ref, w_refs, x_stage, qkv_stage, qkv_shared, wo_stage, wo_shared, ffn_stage,
            ffn_shared, res_ref, mem0_ref, x_sem, attention_sem, ffn_sem, shared_sem, out_sem,
            *, seg):
    d_model, n_tok = xt_hbm.shape
    n_mem = mem0_hbm.shape[0]
    n_seg = n_tok // seg
    n_out = n_tok // _LANES

    def window(r, n):
        return res_ref.at[pl.ds(pl.multiple_of((r + _LAG) * seg, seg), n * seg)]

    def block(r, n=1):
        return pl.ds(r * seg, n * seg)

    def lanes(i, n=1):
        return pl.ds(pl.multiple_of(i * _LANES, _LANES), n * _LANES)

    def transpose_out(i, x):
        out_ref[i] = x.T[:d_model].astype(out_ref.dtype)

    def prepare(ref, blocks):
        for i, r in enumerate(blocks):
            h_ref[i, n_mem:] = _layernorm(ref[block(r), :])
        yield

    def attention(order, ref, blocks, others, early=None):
        xs, outs = [ref[block(r), :] for r in blocks], []
        hs = [h_ref[i] for i in range(len(blocks))]
        operands_ref, known = full_ref, None
        if early is not None:
            operands_ref, known = short_ref, lambda *at: early_ref[(early, *at)]
            hs = [jnp.concatenate([hs[0][:n_mem], hs[0][n_mem + seg // 2:], hs[1][seg:]], axis=0),
                  hs[1][:seg]]
        _store_operands(operands_ref, 0, hs)
        tasks = _attention_tasks(xs, operands_ref, w_refs, qkv_ref, heads_ref, outs, known)
        yield from _passes(order, {**others, **tasks})
        for i, r in enumerate(blocks):
            h_ref[i, :n_mem] = outs[i][:n_mem]
            ref[block(r), :] = outs[i][n_mem:]

    def ffn_tasks(ref, blocks, result=None):
        def update(ys):
            for r, y in zip(blocks, ys):
                ref[block(r, 2), :] = y

        def operands():
            for i in range(0, 2 * seg, 16):
                _store_operands(chunks_ref.at[0], i,
                                [_layernorm(ref[pl.ds(r * seg + i, 16), :]) for r in blocks])
            yield

        return {"N": operands(), **_ffn_tasks(
            [ref[block(r, 2), :] for r in blocks], chunks_ref.at[0], w_refs, hidden_ref,
            result or update)}

    def double_step(b):
        ref = window(b, _LAG + 2)
        _run(attention(_ORDER_DOUBLE, ref, [_LAG, 0],
                       {"X": prepare(ref, [_LAG + 1, 1])}, 1 + b))

    def two_steps(j):
        b = 6
        ref = window(2 * j - b, b + _LAG + 3)
        transpose_out(jnp.where((j % 2 == 1) & (j > 1), (j - 3) // 2, n_out - 1),
                      ref[block(0, 4), :])
        ffn = ffn_tasks(ref, [b + 2, b - 2])
        _run(attention(_ORDER_EVEN, ref, [b + _LAG, b],
                       {**ffn, "X": prepare(ref, [b + _LAG + 1, b + 1])}),
             attention(_ORDER_ODD, ref, [b + _LAG + 1, b + 1],
                       {**ffn, "X": prepare(ref, [b + _LAG + 2, b + 2])}, j + _LAG // 2))

    qkv_words = [_words(w) for w in (wq_hbm, wk_hbm, wv_hbm)]
    ffn_words = [_words(w) for w in (w1_hbm, w3_hbm, w2t_hbm)]
    pairs = _COLUMNS // 2

    def attention_copies(family, g):
        sem = attention_sem.at[family]
        if family == _WO:
            heads = _words(wot_hbm).at[pl.ds(_COLUMNS * g, _COLUMNS)]
            return [pltpu.make_async_copy(heads, wo_stage, sem)]
        return [pltpu.make_async_copy(qkv_words[family].at[:, pairs * g + p, :],
                                      qkv_stage.at[family, p], sem) for p in range(pairs)]

    def ffn_copies(m, columns=_COLUMNS):
        return [pltpu.make_async_copy(w.at[:, lanes(_COLUMNS * m, columns)],
                                      ffn_stage.at[m % 3, i, :, lanes(0, columns)],
                                      ffn_sem.at[3 * (m % 3) + i])
                for i, w in enumerate(ffn_words)]

    def shared_copies(which):
        ends = []
        for m in range(_MEMBERS):
            rows, words = pl.ds(m * _HALF, _HALF), pl.ds(m * _HALF // 2, _HALF // 2)
            if which == 0:
                ends += [(w.at[rows, pairs * m + p, :], qkv_shared.at[i, p, rows])
                         for i, w in enumerate(qkv_words) for p in range(pairs)]
            elif which == 1:
                ends += [(_words(wot_hbm).at[pl.ds(_COLUMNS * m, _COLUMNS), words],
                          wo_shared.at[:, words])]
            else:
                ends += [(w.at[words, lanes(_COLUMNS * m, _COLUMNS)], ffn_shared.at[i, words])
                         for i, w in enumerate(ffn_words)]
        return [pltpu.make_async_copy(*pair, shared_sem.at[which]) for pair in ends]

    def x_copy(chunk):
        columns = lanes(n_out // _CHUNKS * chunk, n_out // _CHUNKS)
        return pltpu.make_async_copy(xt_hbm.at[:, columns], x_stage.at[chunk], x_sem.at[chunk])

    def out_copy(i):
        return pltpu.make_async_copy(out_ref.at[i], outt_hbm.at[:, lanes(i)], out_sem.at[i])

    def start(copies):
        for c in copies:
            c.start()

    def wait(copies):
        for c in copies:
            c.wait()

    def head_pairs(ref):
        def source(c, half, first):
            rows = ref.at[c // 2, pl.ds(pl.multiple_of(half * _HALF, _HALF), _HALF)]
            words = rows[pl.ds(pl.multiple_of(first, 16), 16), :]
            words = words & jnp.uint32(0xFFFF0000) if c % 2 else words << 16
            return pltpu.bitcast(words, jnp.float32)
        return source

    def row_pairs(column, rows):
        def source(c, half, first):
            ref, at = column(c)
            words = ref.at[pl.ds(pl.multiple_of(half * (_HALF // 2), _HALF // 2), _HALF // 2)]
            return _unpack(words[pl.ds(first // 2, rows // 2), at])
        return source

    def member_sums(own, shared, m, rows, starts=None):
        places = [(jnp.where(m == h, 2 * _TAIL, h), jnp.where(m == h, _MEMBERS, h))
                  for h in range(_MEMBERS)]

        def source(c, d, high, first):
            if 2 * d >= _MEMBERS:
                return own(c, 2 * d + high, first)
            mine, theirs = places[2 * d + high]
            return (own(c, mine, first).astype(jnp.float32)
                    - shared(c, theirs, first).astype(jnp.float32))

        sets = {}
        for i, p in enumerate(_scheme("member")):
            owners = {c if c < 4 else d for _, c, d in p.w_low}
            key = -1 - min(owners) if len(owners) == 1 and rows < _HALF else i
            sets.setdefault(key, []).append((len(p.w_low), i, p))
        for tiles in sets.values():
            for high in range(2):
                for first in starts or range(0, _HALF, rows):
                    loaded = {}
                    for *_, i, p in sorted(tiles):
                        new = [(c, d) for _, c, d in p.w_low if (c, d) not in loaded]
                        loaded.update({at: source(*at, high, first) for at in new})
                        value = _weight_sum([(s, loaded[c, d]) for s, c, d in p.w_low])
                        work = len(p.w_low) + sum(1 + 2 * (d < 2) for _, d in new)
                        yield i, high * _HALF + first, value, work / 2

    def lay_out_heads(family, g, starts=None):
        sums = member_sums(head_pairs(qkv_stage.at[family]), head_pairs(qkv_shared.at[family]),
                           g, 16, starts)
        return _lay_out(sums, _tiles(w_refs, "member", family, g))

    def lay_out_shared_half(lay_out, words, rows, family, i):
        n = len(_scheme("shared")) // 2
        sums = _weight_sums(_scheme("shared")[:n], row_pairs(words, rows), range(0, _HALF, rows))
        return lay_out(sums, _tiles(w_refs, "shared", family, half=i))

    def ffn_columns(ref, family, first=0):
        return lambda c: (ref.at[family - _W1], lanes(first + c))

    def project_early(chunk, unit):
        at = lambda r, g, c: (pl.ds(8 * chunk + 4 * r, 4), unit[1], g, c)
        out = {}
        if unit[0] == "member":
            out = {(r, c): early_ref[at(r, _MEMBERS - 1, c)].reshape(2 * seg, _LANES)
                   for r in range(2) for c in range(_COLUMNS)}
        yield from _expand(chunks_ref.at[chunk], w_refs, unit, out)
        for (r, c), value in out.items():
            early_ref[at(r, unit[2] if unit[0] == "member" else _MEMBERS - 1, c)] = (
                value.reshape(4, seg // 2, _LANES))

    def load_chunk(chunk):
        x = x_stage[chunk].astype(jnp.float32)
        x = jnp.concatenate([x, x[_TAIL * _LANES:]], axis=0).T
        window(n_seg // _CHUNKS * chunk, n_seg // _CHUNKS)[...] = x
        segments = [2 * e + 1 for e in range(8)]
        if isinstance(chunk, int) and chunk == 0:
            segments[1] = _LAG
        for e in range(4):
            _store_operands(chunks_ref.at[chunk], e * seg // 2, [
                _layernorm(x[r * seg:r * seg + seg // 2]) for r in segments[e::4]])
        yield

    def clear(i):
        rows = lambda first, n=1: pl.ds(pl.multiple_of(first + 8 * n * i, 8), 8 * n)
        for spare in (res_ref.at[rows(0, _LAG)], res_ref.at[rows((_LAG + n_seg) * seg)],
                      wo_shared.at[:, rows(_MEMBERS * _HALF // 2)],
                      ffn_shared.at[:, rows(_MEMBERS * _HALF // 2)],
                      qkv_shared.at[:, :, rows(_MEMBERS * _HALF, 2)]):
            spare[...] = jnp.zeros(spare.shape, spare.dtype)

    def lay_out_shared(i):
        for family in (_WQ, _WK, _WV):
            sums = _weight_sums(_scheme("shared"), head_pairs(qkv_shared.at[family]), [16 * i])
            _run(_lay_out(sums, _tiles(w_refs, "shared", family)))

    def project_shared(chunk):
        pl.when(chunk == 1)(lambda: start(shared_copies(1) + attention_copies(_WK, 0)))
        pl.when(chunk == 2)(lambda: start(attention_copies(_WV, 0)))
        pl.when(chunk + 1 < _CHUNKS)(lambda: wait([x_copy(chunk + 1)]))
        _run(_passes(_ORDER_SHARED, {
            "E": _chain(*(project_early(chunk, ("shared", f)) for f in (_WQ, _WK, _WV))),
            "L": lay_out_heads(_WQ, 0, [16 * chunk]),
            "X": load_chunk(jnp.minimum(chunk + 1, _CHUNKS - 1))}))

    def load_group(g):
        more = g + 1 < _MEMBERS

        def arrive(family):
            if family == _WK:
                start(attention_copies(_WO, g))
                pl.when(more)(lambda: start(attention_copies(_WQ, g + 1)))
                pl.when(~more)(lambda: start(shared_copies(2)))
                wait(attention_copies(_WK, g))
            elif family == _WV:
                wait(attention_copies(_WV, g) + attention_copies(_WO, g))
                pl.when(more)(lambda: start(attention_copies(_WK, g + 1)))
                for i, copy in enumerate(ffn_copies(0)):
                    pl.when(g == i)(copy.start)
                pl.when(~more)(lambda: start(ffn_copies(1)))
            else:
                pl.when(more)(lambda: wait(attention_copies(_WQ, g + 1)))
                pl.when(more)(lambda: start(attention_copies(_WV, g + 1)))
            yield

        same = jnp.minimum(g, _MEMBERS - 1)
        wo_sums = member_sums(row_pairs(lambda c: (wo_stage.at[c], slice(None)), _HALF),
                              row_pairs(lambda c: (wo_shared.at[c], slice(None)), _HALF), g, _HALF)
        _run(_passes(_ORDER_LOAD, {
            **{f"E{f}": _chain(*(project_early(chunk, ("member", f, g)) for chunk in range(_CHUNKS)))
               for f in (_WQ, _WK, _WV)},
            **{f"W{f}": arrive(f) for f in (_WQ, _WK, _WV)},
            "L0": lay_out_heads(_WQ, jnp.minimum(g + 1, _MEMBERS - 1)),
            "L1": lay_out_heads(_WK, same), "L2": lay_out_heads(_WV, same),
            "L3": _lay_out_transposed(wo_sums, _tiles(w_refs, "member", _WO, same)),
            "L4": lay_out_shared_half(
                _lay_out_transposed, lambda c: (wo_shared.at[c + 2 * (g % 2)], slice(None)), _HALF,
                _WO, g % 2)}))

    def first_step(m):
        pl.when(m + 2 < _MEMBERS)(lambda: start(ffn_copies(m + 2)))
        pl.when(m + 2 == _MEMBERS)(lambda: start(ffn_copies(_MEMBERS, 4)))
        wait(ffn_copies(m))
        ref, stage = window(m, 2), ffn_stage.at[m % 3]
        sums = lambda family, rows: member_sums(
            row_pairs(ffn_columns(stage, family), rows),
            row_pairs(ffn_columns(ffn_shared, family), rows), m, rows)
        up = [_lay_out(sums(f, 16), _tiles(w_refs, "member", f, m)) for f in (_W1, _W3)]
        down = _lay_out_transposed(sums(_W2, _HALF), _tiles(w_refs, "member", _W2, m))
        shared = lay_out_shared_half(_lay_out, ffn_columns(ffn_shared, _W1 + m // 2, 2 * (m % 2)),
                                     16, _W1 + m // 2, m % 2)
        _run(_passes(_ORDER_FIRST, {
            "P": attention(_ORDER_SINGLE, ref, [0], {"X": prepare(ref, [1])}),
            "L": _passes("U*9+D*5", {"U": _chain(shared, *up), "D": down})}))

    def first_ffn():
        stage = ffn_stage.at[_MEMBERS % 3]
        sums = lambda kind, ref, family: _weight_sums(
            _scheme(kind), row_pairs(ffn_columns(ref, family), _HALF), [0])
        _run(*(_lay_out(sums("narrow", stage, f), _tiles(w_refs, "narrow", f)) for f in (_W1, _W3)),
             *(_lay_out_transposed(sums(kind, ref, _W2), _tiles(w_refs, kind, _W2))
               for kind, ref in (("narrow", stage), ("shared", ffn_shared))),
             _passes(_ORDER_FIRST_FFN, ffn_tasks(window(0, _LAG), [0, 2])))

    def last_steps():
        ref = window(n_seg - _LAG - 2, _LAG + 2)
        ffn = ffn_tasks(ref, [_LAG, 0])
        _run(attention(_ORDER_EVEN_SINGLE, ref, [2], {**ffn, "X": prepare(ref, [3])}),
             attention(_ORDER_ODD_SINGLE, ref, [3], {**ffn, "X": prepare(ref, [4])}))

    def last_step(i):
        tile = n_out - 3 + i
        transpose_out(tile, window(_LANES // seg * tile, _LANES // seg)[...])
        ref = window(n_seg - 2 + i, 2)
        _run(attention(_ORDER_SINGLE, ref, [0], {"X": prepare(ref, [1])}))
        out_copy(tile).start()

    def last_ffn():
        _run(_passes(_ORDER_FFN, ffn_tasks(
            window(n_seg - _LAG, _LAG), [0, 2],
            lambda ys: transpose_out(n_out - 1, jnp.concatenate(ys, axis=0)))))

    mem_copy = pltpu.make_async_copy(mem0_hbm, mem0_ref.at[0], shared_sem.at[3])
    x_copy(0).start()
    pl.loop(0, 4)(clear)
    start([mem_copy] + shared_copies(0))
    wait([x_copy(0), mem_copy])
    start([x_copy(1)] + attention_copies(_WQ, 0))
    mem0 = mem0_ref[0].astype(jnp.float32)
    h_ref[0, :n_mem] = h_ref[1, :n_mem] = jnp.concatenate(
        [mem0, mem0[:, _TAIL * _LANES:]], axis=1)
    _run(load_chunk(0), prepare(window(0, 1), [0]))
    wait(shared_copies(0))
    pl.loop(0, _HALF // 16)(lay_out_shared)
    x_copy(2).start()
    wait(attention_copies(_WQ, 0))
    x_copy(3).start()
    pl.loop(0, _CHUNKS)(project_shared)
    wait(shared_copies(1))
    pl.loop(0, _MEMBERS)(load_group)
    wait(shared_copies(2))
    pl.loop(0, _LAG)(first_step)
    wait(ffn_copies(_MEMBERS, 4))
    first_ffn()
    _run(prepare(window(0, _LAG + 1), [_LAG, 0]))
    pl.loop(0, 2)(double_step)
    pl.loop(1, (n_seg - _LAG) // 2)(two_steps)
    start([out_copy(i) for i in range(n_out - 3)])
    h_ref[0] = h_ref[1]
    last_steps()
    pl.loop(0, 2)(last_step)
    last_ffn()
    out_copy(n_out - 1).start()
    wait([out_copy(i) for i in range(n_out)])


@functools.partial(jax.jit, static_argnames=("A_seg_len",))
def pallas_interleave_layers__memory_aug_recurrent_mem_tr__glu_gated_swiglu__prompt_kernel(
    A_x: jax.Array,
    A_mem0: jax.Array,
    A_Wq: jax.Array,
    A_Wk: jax.Array,
    A_Wv: jax.Array,
    A_Wo: jax.Array,
    A_seg_len: int,
    B_x: jax.Array,
    B_w1: jax.Array,
    B_w3: jax.Array,
    B_w2: jax.Array,
):
    del B_x
    _, n_tok, d_model = A_x.shape
    n_mem = A_mem0.shape[1]
    _, n_heads, d_head = A_Wq.shape
    seg = A_seg_len
    assert A_x.shape[0] == 1 and _LAG * seg == _LANES and n_mem == 8
    assert n_tok == 16 * _CHUNKS * seg and d_model == _TAIL * _LANES + _HALF and d_head == _LANES
    assert n_heads == _MEMBERS * _COLUMNS and B_w1.shape[1] == (n_heads + 4) * _LANES
    n_operands = pl.cdiv(len(_operand_keys(False)), 8) * 8
    n_tiles = (_FAMILIES * (_MEMBERS * len(_scheme("member")) + len(_scheme("shared")))
               + 3 * len(_scheme("narrow")))
    shared_rows = (_MEMBERS + 1) * _HALF
    hbm = pl.BlockSpec(memory_space=pltpu.HBM)
    out_t = pl.pallas_call(
        functools.partial(_kernel, seg=seg),
        out_shape=jax.ShapeDtypeStruct((d_model, n_tok), A_x.dtype),
        in_specs=[hbm] * 9,
        out_specs=hbm,
        scratch_shapes=[
            pltpu.VMEM((n_tok // _LANES, d_model, _LANES), A_x.dtype),
            pltpu.VMEM((8, n_mem + seg, d_model + _HALF), jnp.float32),
            pltpu.VMEM((n_operands, n_mem + seg, _LANES), jnp.float32),
            pltpu.VMEM((n_operands, seg, _LANES), jnp.bfloat16),
            pltpu.VMEM((_CHUNKS, n_operands, 2 * seg, _LANES), jnp.bfloat16),
            pltpu.VMEM((3, _MEMBERS, _COLUMNS, 2 * (n_mem + seg), _LANES), jnp.bfloat16),
            pltpu.VMEM((_MEMBERS + 4, _COLUMNS, 2 * (n_mem + seg), _LANES), jnp.float32),
            pltpu.VMEM((_MEMBERS + 4, _COLUMNS, 4 * seg, _LANES), jnp.float32),
            pltpu.VMEM((8 * _CHUNKS, 3, _MEMBERS, _COLUMNS, seg // 2, _LANES), jnp.float32),
            [pltpu.VMEM((n_tiles // 2, _LANES, _LANES), jnp.bfloat16)] * 2,
            pltpu.VMEM((_CHUNKS, d_model, n_tok // _CHUNKS), A_x.dtype),
            pltpu.VMEM((3, _COLUMNS // 2, d_model, _LANES), jnp.uint32),
            pltpu.VMEM((3, _COLUMNS // 2, shared_rows, _LANES), jnp.uint32),
            pltpu.VMEM((_COLUMNS, d_model // 2, _LANES), jnp.uint32),
            pltpu.VMEM((_COLUMNS, shared_rows // 2, _LANES), jnp.uint32),
            pltpu.VMEM((3, 3, d_model // 2, _COLUMNS * _LANES), jnp.uint32),
            pltpu.VMEM((3, shared_rows // 2, _COLUMNS * _LANES), jnp.uint32),
            pltpu.VMEM((n_tok + 2 * _LAG * seg, d_model + _HALF), jnp.float32),
            pltpu.VMEM((16, n_mem, d_model), A_mem0.dtype),
            pltpu.SemaphoreType.DMA((_CHUNKS,)),
            pltpu.SemaphoreType.DMA((4,)),
            pltpu.SemaphoreType.DMA((9,)),
            pltpu.SemaphoreType.DMA((4,)),
            pltpu.SemaphoreType.DMA((n_tok // _LANES,)),
        ],
        compiler_params=pltpu.CompilerParams(
            vmem_limit_bytes=126 * 1024 * 1024,
            flags={"XLA_TPU_FORCE_LP_LLO_SCHEDULER": True}),
    )(A_x.reshape(n_tok, d_model).T, A_mem0.reshape(n_mem, d_model), A_Wq, A_Wk, A_Wv,
      A_Wo.transpose(0, 2, 1), B_w1, B_w3, B_w2.T)
    return out_t.T.reshape(A_x.shape)
```

```python
import functools
import math
from typing import NamedTuple

import jax
import jax.numpy as jnp
import jax.experimental.pallas as pl
import jax.experimental.pallas.tpu as pltpu

_EPS = 1e-05
_MASKED = -1000000000.0
_LOG2E = math.log2(math.e)
_LANES = 128
_HALF = _LANES // 2
_TAIL = 4
_COLUMNS = 8
_MEMBERS = 4
_WQ, _WK, _WV, _WO, _W1, _W3, _W2, _FAMILIES = range(8)
_LAG = 4
_CHUNKS = 4
_ORDER_EVEN = (
    "X Q0+K0 V0*10+S0 Q1 N A0 K1 K2 V1*6+S1 Q2 A1 V2*6+S2 Q3 A2 O0*4+O1*4 O2 K3 G0 U0*10+S3 "
    "V3 A3+G1*6 G4 U4 U1 O3 D4")
_ORDER_ODD = (
    "Q0 K0 G2 D0*6+S0 V0 U2 Q1 A0 K1 G3 V1 D1*6+S1 Q2 U3 A1 K2 V2 D2*6+S2 Q3 K3*7+V3*8 A2 "
    "O0*4+S3 D3 F X A3+O1*6 O2 O3")
_ORDER_EVEN_SINGLE = (
    "Q0 N K0 V0*4+S0 Q1 K1 G0 A0 V1*4+S1 O0 U0 A1 Q2 K2 V2*4+S2 O1 G1 A2 Q3 K3 V3*4+S3 X O2 "
    "U1 A3 G4 U4 O3 D4 G2")
_ORDER_ODD_SINGLE = (
    "Q0 K0 V0*4+S0 U2 A0 Q1 K1 V1*4+S1 G3 A1 Q2 K2 U3 V2*4+S2 D0 A2 Q3 K3 "
    "D1 D2 D3 F X V3*4+S3 O0 O1 A3 O2 O3")
_ORDER_DOUBLE = (
    "Q0 K0 Q1 K1 V0*10+S0 K2 Q2 V1*6+S1 A0 Q3 K3 X O0*6+S2 V3 A1 V2 O1*6+S3 A2 A3+O2*6 O3")
_ORDER_SINGLE = (
    "Q0 K0 V0*4+S0 Q1 K1 A0 V1*4+S1 Q2 K2 A1 V2*4+S2 Q3 K3 A2 V3*4+S3 X O0 O1 A3 O2 O3")
_ORDER_FFN = "N G0 U0 G1 D0 U1 G2 D1 U2 G3 U3 G4 U4 D2 D4 D3 F"
_ORDER_SHARED = "E+L*13 X"
_ORDER_LOAD = (
    "W1 E0:4 E0+L1*19+L4*5 W2 E1:4 E1+L2*19+L3*12:204 E1 L2 W0 E2:4 E2+L0*19+L3*12")
_ORDER_FIRST = "P:8 P+L*23"
_ORDER_FIRST_FFN = "N G0 U0 G1 U1 G2 U2 G4+D0*2 U4+D1*2 D2 G3 U3*2+D4 D3 F"


class _Pass(NamedTuple):
    low: tuple
    high: tuple
    w_low: tuple
    w_high: tuple
    wide: tuple
    common: bool = False


@functools.cache
def _scheme(kind, shift=0):
    x, y, n = 0, 1, 4 if kind == "member" else 2
    a = lambda d: d % n + shift
    b = lambda d: d % n + shift + (2 if kind == "narrow" else 4)
    rest = lambda d: [e for e in range(4) if e != d and e // n == d // n]

    def whole(narrow, weight, wide):
        return _Pass(tuple(sorted(narrow)), tuple(sorted(narrow)), weight, weight, wide)

    def m1(d, e):
        return whole(((1, x, d), (1, y, e)), ((1, b(e), d), (1, a(d), e)),
                     ((1, y, a(d)), (1, x, b(e))))

    def m2(d, e):
        return whole(((1, y, d), (1, y, e)), ((1, b(e), d),), ((1, y, b(e)), (-1, y, a(d))))

    def m3(d):
        return whole(((1, x, d),), ((1, a(d), d), *((-1, a(d), e) for e in rest(d))),
                     ((1, x, a(d)), (1, y, a(d))))

    def m4(d):
        return whole(((1, y, d),), ((1, b(d), d), *((-1, b(d), e) for e in rest(d))),
                     ((1, y, b(d)), (1, x, b(d))))

    def m5(d, e):
        return whole(((1, x, d), (1, x, e)), ((1, a(d), e),), ((1, x, a(d)), (-1, x, b(e))))

    def m6(d):
        return whole(((1, y, d), (-1, x, d)), ((1, a(d), d), *((1, b(e), d) for e in rest(d))),
                     ((1, y, a(d)),))

    def m7(d):
        return whole(((1, y, d), (-1, x, d)), ((-1, b(d), d), *((-1, a(e), d) for e in rest(d))),
                     ((1, x, b(d)),))

    def with_tails(p, p_rows, p_columns, q, q_rows, q_columns):
        tail = lambda columns: tuple((1, c, _TAIL) for c in columns)
        return [_Pass(p.low, p.high, q.w_low, p.w_high, p.wide + q.wide, common=True),
                _Pass(p.low, ((1, p_rows, _TAIL),), p.w_low, tail(p_columns), p.wide),
                _Pass(((1, q_rows, _TAIL),), q.high, tail(q_columns), q.w_high, q.wide)]

    def pair_with_tails(d, e):
        return [*with_tails(m5(d, e), x, [a(d)], m5(e, d), x, [a(e)]), m3(d),
                *with_tails(m2(d, e), y, [b(e)], m2(e, d), y, [b(d)]), m3(e),
                *with_tails(m6(d), y, [a(d), b(e)], m7(d), x, [b(d), a(e)]), m1(d, e), m4(d),
                *with_tails(m7(e), x, [b(e), a(d)], m6(e), y, [a(e), b(d)]), m1(e, d), m4(e)]

    edge = lambda d, e: [m5(d, e), m1(d, e), m2(d, e)]
    pair = lambda d, e: [m3(d), m6(d), *edge(d, e), m7(e), m4(e),
                         m3(e), m6(e), *edge(e, d), m7(d), m4(d)]
    if kind == "shared":
        return (*pair(0, 1), *(() if shift else _scheme(kind, 2)))
    if kind == "narrow":
        return (*pair_with_tails(0, 1), *pair(2, 3))
    edges = ((0, 1), (0, 2), (0, 3), (3, 1), (3, 2), (2, 1), (2, 3), (1, 2), (1, 3),
             (1, 0), (2, 0), (3, 0))
    passes = []
    for i, (d, e) in enumerate(edges):
        if all(d != earlier for earlier, _ in edges[:i]):
            passes += [m3(d), m6(d)]
        if all(e != earlier for _, earlier in edges[:i]):
            passes += [m7(e), m4(e)]
        passes += edge(d, e)
    return tuple(passes)


def _selected(kind, single):
    for i, p in enumerate(_scheme(kind)):
        if single:
            narrow = tuple((s, 0, d) for s, _, d in p.low)
            p = p._replace(low=narrow, high=narrow,
                           wide=tuple((s, 0, c) for s, r, c in p.wide if r == c // 4))
        if p.wide:
            yield i, p


def _tiles(w_refs, kind, family, member=_MEMBERS, half=None):
    size = lambda name: len(_scheme(name)) // 2
    per_family = _MEMBERS * size("member") + size("shared")
    first, count = family * per_family + member * size("member"), size(kind)
    if kind == "narrow":
        first = _FAMILIES * per_family + (family - _W1) * count
    if half is not None:
        first, count = first + half * (count // 2), count // 2
    views = [ref.at[pl.ds(first, count)] for ref in w_refs]
    return lambda i: (views[i % 2], i // 2)


def _tail_for(terms, block):
    return tuple(sorted((s, r, _TAIL if d == block else d) for s, r, d in terms))


@functools.cache
def _operand_keys(single):
    return tuple(dict.fromkeys(_tail_for(p.low, block) for block in (None, 0, 1)
                               for _, p in _selected("member", single)))


def _signed_sum(terms):
    terms = sorted(terms, key=lambda t: -t[0])
    total = terms[0][1] if terms[0][0] > 0 else -terms[0][1]
    for sign, value in terms[1:]:
        total = total + value if sign > 0 else total - value
    return total


def _accumulate(sums, key, sign, value):
    if key not in sums:
        sums[key] = (sign, value)
    elif sums[key][0] == sign:
        sums[key] = (sign, sums[key][1] + value)
    else:
        sums[key] = (1, value - sums[key][1] if sign > 0 else sums[key][1] - value)


def _words(ref):
    return ref.bitcast(jnp.uint32) if ref.dtype == jnp.bfloat16 else ref


def _unpack(words):
    return pltpu.bitcast(words, jnp.bfloat16) if words.dtype == jnp.uint32 else words


def _load(ref, i):
    return _unpack(_words(ref)[i])


def _store(ref, i, first, value):
    rows = value.shape[0]
    if value.dtype == jnp.bfloat16:
        _words(ref)[i, pl.ds(first // 2, rows // 2), :] = pltpu.bitcast(value, jnp.uint32)
    else:
        ref[i, pl.ds(first, rows), :] = value.astype(ref.dtype)


def _lane_half(rows):
    return jax.lax.broadcasted_iota(jnp.int32, (rows, _LANES), 1) // _HALF


def _blocks(x):
    return [x[:, d * _LANES:(d + 1) * _LANES] for d in range(_TAIL + 1)]


def _store_operands(ref, first, row_blocks):
    blocks = [_blocks(x) for x in row_blocks]
    for i, terms in enumerate(_operand_keys(len(row_blocks) == 1)):
        _store(ref, i, first, _signed_sum([(s, blocks[r][d]) for s, r, d in terms]))


def _dot(a, b):
    return jnp.dot(a, b, preferred_element_type=jnp.float32)


def _expand(operands_ref, w_refs, unit, out, single=False):
    operands_ref, tile = _words(operands_ref), _tiles(w_refs, *unit)
    operand = lambda terms: operands_ref[_operand_keys(single).index(terms)]
    half = _lane_half(operands_ref.shape[1])
    freed = {}
    if unit[0] == "member":
        blocks = [unit[2] // 2] if isinstance(unit[2], int) else range(_MEMBERS // 2)
        freed = {d: half == unit[2] - 2 * d for d in blocks}
    sums, common = {key: (1, value) for key, value in out.items()}, []
    for i, p in _selected(unit[0], single):
        lhs = operand(p.low)
        if p.high != p.low:
            lhs = jnp.where(half == 0, lhs, operand(p.high))
        for d, lanes in freed.items():
            if _tail_for(p.low, d) != p.low:
                lhs = jnp.where(lanes, operand(_tail_for(p.low, d)), lhs)
        product = _dot(_unpack(lhs), _load(*tile(i)))
        if p.common:
            common = [product, product]
        else:
            if common:
                product = product + common.pop()
            for s, r, c in p.wide:
                _accumulate(sums, (r, c), s, product)
        yield
    assert all(sign > 0 for sign, _ in sums.values())
    out.update({key: value for key, (_, value) in sums.items()})


def _contract(load, w_refs, unit, sums, single=False):
    tile = _tiles(w_refs, *unit)
    freed = unit[2] // 2 if unit[0] == "member" else None
    held, mixed = [], {}
    for i, p in _selected(unit[0], single):
        product = _dot(_signed_sum([(s, load(r, c)) for s, r, c in p.wide]),
                       _load(*tile(i)))
        if p.common or held:
            held.append((p, product))
        if len(held) == 3:
            (p, common), (p1, first), (p2, second) = held
            held = []
            product = common + jnp.where(_lane_half(common.shape[0]) == 0, first, second)
            _accumulate(sums, (p1.high[0][1], _TAIL, 1), 1, first)
            _accumulate(sums, (p2.low[0][1], _TAIL, 0), 1, second)
        if not held:
            for s, r, d in p.low:
                _accumulate(mixed if d == freed else sums, (r, d), s, product)
        yield
    for (r, d), (s, both) in mixed.items():
        _accumulate(sums, (r, _TAIL, unit[2] % 2), s, both)
        _accumulate(sums, (r, d), s, jnp.where(_lane_half(both.shape[0]) == unit[2] % 2, 0.0, both))


def _residual(row_blocks):
    return {(r, d) if d < _TAIL else (r, d, 0): (1, block)
            for r, x in enumerate(row_blocks) for d, block in enumerate(_blocks(x))}


def _contracted(sums, r):
    assert all(sign > 0 for sign, _ in sums.values())
    low, high = sums[r, _TAIL, 0][1], sums[r, _TAIL, 1][1]
    tail = jnp.where(_lane_half(low.shape[0]) == 0, low, high)
    tail = tail + pltpu.roll(tail, _HALF, 1)
    return jnp.concatenate([sums[r, d][1] for d in range(_TAIL)] + [tail], axis=1)


def _weight_sum(parts):
    return _signed_sum([(s, part.astype(jnp.float32) if len(parts) > 1 else part)
                        for s, part in parts])


def _weight_sums(passes, source, starts):
    for i, p in enumerate(passes):
        for high in range(2):
            if i > high and passes[i - 1 - high].common:
                continue
            for at in starts:
                first = high * _HALF + at
                total = lambda terms: _weight_sum(
                    [(s, source(c, 2 * d + high * (d < _TAIL), at)) for s, c, d in terms])
                terms = (p.w_low, p.w_high)[high]
                value = total(terms)
                yield i, first, value, len(terms)
                if p.common:
                    other = passes[i + 1 + high]
                    other = total((other.w_low, other.w_high)[high]).astype(jnp.float32)
                    yield i + 1 + high, first, other - value.astype(jnp.float32), len(terms) + 1


def _lay_out(sums, tile):
    for i, first, value, terms in sums:
        _store(*tile(i), pl.multiple_of(first, 16), value)
        yield from range(int(4 * terms + 1) * value.shape[0] // 16)


def _lay_out_transposed(sums, tile):
    halves, pending = {}, []
    for i, first, value, terms in sums:
        halves[i, first] = value
        if (i, _HALF - first) in halves:
            pair = [halves[i, 0], halves[i, _HALF]]
            if pair[0].dtype != pair[1].dtype:
                pair = [half.astype(jnp.float32) for half in pair]
            pending.append((i, jnp.concatenate(pair, axis=0).astype(jnp.bfloat16).T))
        if len(pending) > 2:
            _store(*tile(pending[0][0]), 0, pending.pop(0)[1])
        yield from range(int(8 * terms + 22))
    for i, value in pending:
        _store(*tile(i), 0, value)


def _layernorm(x):
    low_lanes = _lane_half(x.shape[0]) == 0

    def mean(v):
        *full, tail = _blocks(v)
        total = functools.reduce(jnp.add, full) + jnp.where(low_lanes, tail, 0.0)
        return jnp.sum(total, axis=-1, keepdims=True) / (_TAIL * _LANES + _HALF)

    d = x - mean(x)
    return d * jax.lax.rsqrt(mean(d * d) + _EPS)


def _silu(x):
    half = 0.5 * x
    return half + half * jnp.tanh(half)


def _reciprocal(x):
    r = pl.reciprocal(x, approx=True)
    return r * (2.0 - x * r)


def _attention_masks(n_layers, rows, n_mem):
    i = jax.lax.broadcasted_iota(jnp.int32, (n_layers * rows, n_layers * rows), 0)
    j = jax.lax.broadcasted_iota(jnp.int32, (n_layers * rows, n_layers * rows), 1)
    if n_layers == 1:
        return (i < n_mem) | (i >= j), _MASKED * _LOG2E
    same = (i >= rows) == (j >= rows)
    visible = (i < n_mem) | ((i >= rows) & (i < rows + n_mem)) | (i >= j)
    fill = jnp.where(same, _MASKED * _LOG2E, -jnp.inf).astype(jnp.float32)
    return same & visible, fill


def _expand_member(operands_ref, w_refs, family, member, shared_ref, out, single=False):
    rows = operands_ref.shape[1]
    if member == 0:
        yield from _expand(operands_ref, w_refs, ("shared", family), out, single)
        for (r, c), value in out.items():
            shared_ref[c, r * rows:(r + 1) * rows, :] = value
    out.update({(r, c): shared_ref[c, r * rows:(r + 1) * rows, :]
                for r in range(1 if single else 2) for c in range(_COLUMNS)})
    yield from _expand(operands_ref, w_refs, ("member", family, member), out, single)


def _store_wide(ref, member, c, rows, value):
    ref[member, c, rows, :] = value
    if member == _MEMBERS - 1:
        ref[_MEMBERS, c, rows, :] = functools.reduce(
            jnp.add, [ref[m, c, rows, :] for m in range(member)] + [value])


def _contract_member(ref, w_refs, family, member, sums, single=False):
    rows = ref.shape[2] // 2
    load = lambda m: lambda r, c: ref[m, c, r * rows:(r + 1) * rows, :]
    yield from _contract(load(member), w_refs, ("member", family, member), sums, single)
    if member == _MEMBERS - 1:
        yield from _contract(load(_MEMBERS), w_refs, ("shared", family), sums, single)


def _attention_tasks(xs, operands_ref, w_refs, qkv_ref, wide_ref, outs, known=None):
    n_layers, rows = len(xs), wide_ref.shape[2] // 2
    single, n_mem = n_layers == 1, rows - xs[0].shape[0]
    visible, fill = _attention_masks(n_layers, rows, n_mem)
    scale = _LANES ** -0.5 * _LOG2E
    qkv, probs = {}, {}
    sums = _residual([jnp.concatenate([jnp.zeros_like(x[:n_mem]), x], axis=0) for x in xs])

    def project(family, g):
        out = {}
        yield from _expand_member(operands_ref, w_refs, family, g,
                                  wide_ref.at[_MEMBERS + 1 + family], out, single)
        for h in range(_COLUMNS):
            if single:
                qkv[family, g, h] = out[0, h] if family == _WQ else out[0, h].astype(jnp.bfloat16)
                continue
            parts = x, y = out[0, h], out[1, h]
            if known:
                moved = (rows + n_mem) // 2
                parts = [x[:n_mem], known(family, g, h), x[n_mem:moved], y, x[moved:]]
            qkv_ref[family, g, h] = jnp.concatenate(parts, axis=0).astype(qkv_ref.dtype)

    def stacked(*at):
        return qkv[at] if single else _load(qkv_ref, at)

    def scores(g):
        for h in range(_COLUMNS):
            s = jax.lax.dot_general(stacked(_WQ, g, h), stacked(_WK, g, h),
                                    (((1,), (1,)), ((), ())), preferred_element_type=jnp.float32)
            s = jnp.where(visible, s * scale, fill)
            p = jnp.exp2(s - jnp.max(s, axis=-1, keepdims=True))
            p = p * _reciprocal(jnp.sum(p, axis=-1, keepdims=True))
            probs[g, h] = p if single else p.astype(jnp.bfloat16)
            yield

    def values(g):
        for h in range(_COLUMNS):
            _store_wide(wide_ref, g, h, slice(0, n_layers * rows),
                        _dot(probs[g, h], stacked(_WV, g, h)))
            yield

    def output(g):
        yield from _contract_member(wide_ref, w_refs, _WO, g, sums, single)
        if g == _MEMBERS - 1:
            outs.extend(_contracted(sums, r) for r in range(n_layers))

    tasks = {}
    for g in range(_MEMBERS):
        tasks.update({f"Q{g}": project(_WQ, g), f"K{g}": project(_WK, g), f"V{g}": project(_WV, g),
                      f"S{g}": scores(g), f"A{g}": values(g), f"O{g}": output(g)})
    return tasks


def _ffn_tasks(xs, operands_ref, w_refs, wide_ref, result):
    rows = operands_ref.shape[1]
    sums = _residual(xs)

    def hidden(family, m):
        out, slot = {}, m + m // _MEMBERS
        if m < _MEMBERS:
            yield from _expand_member(operands_ref, w_refs, family, m,
                                      wide_ref.at[_MEMBERS + 2 + family - _W1], out)
        else:
            yield from _expand(operands_ref, w_refs, ("narrow", family), out)
        for (r, c), value in out.items():
            at = slice(r * rows, (r + 1) * rows)
            if family == _W1:
                wide_ref[slot, c, at, :] = _silu(value)
            else:
                _store_wide(wide_ref, slot, c, at, wide_ref[slot, c, at, :] * value)

    def finish():
        result([_contracted(sums, r) for r in range(2)])
        yield

    tasks = {"F": finish(), "D4": _contract(
        lambda r, c: wide_ref[_MEMBERS + 1, c, r * rows:(r + 1) * rows, :], w_refs,
        ("narrow", _W2), sums)}
    for m in range(_MEMBERS + 1):
        tasks.update({f"G{m}": hidden(_W1, m), f"U{m}": hidden(_W3, m)})
    for m in range(_MEMBERS):
        tasks[f"D{m}"] = _contract_member(wide_ref, w_refs, _W2, m, sums)
    return tasks


def _passes(order, tasks):
    done = object()
    for item in order.split():
        names, _, turns = item.partition(":")
        running = [(tasks[name], int(count or 1))
                   for name, _, count in (part.partition("*") for part in names.split("+"))]
        turn = 0
        while running and (not turns or turn < int(turns)):
            for task, count in tuple(running):
                for _ in range(count):
                    if next(task, done) is done:
                        running.remove((task, count))
                        break
                    yield
            turn += 1


def _chain(*tasks):
    for task in tasks:
        yield from task


def _run(*tasks):
    for _ in _chain(*tasks):
        pass


def _kernel(xt_hbm, mem0_hbm, wq_hbm, wk_hbm, wv_hbm, wot_hbm, w1_hbm, w3_hbm, w2t_hbm,
            outt_hbm, out_ref, h_ref, full_ref, short_ref, chunks_ref, qkv_ref, heads_ref,
            hidden_ref, early_ref, w_refs, x_stage, qkv_stage, qkv_shared, wo_stage, wo_shared,
            ffn_stage, ffn_shared, res_ref, mem0_ref, x_sem, attention_sem, ffn_sem, shared_sem,
            out_sem, *, seg):
    d_model, n_tok = xt_hbm.shape
    n_mem = mem0_hbm.shape[0]
    n_seg = n_tok // seg
    n_out = n_tok // _LANES

    def window(r, n):
        return res_ref.at[pl.ds(pl.multiple_of((r + _LAG) * seg, seg), n * seg)]

    def block(r, n=1):
        return pl.ds(r * seg, n * seg)

    def lanes(i, n=1):
        return pl.ds(pl.multiple_of(i * _LANES, _LANES), n * _LANES)

    def transpose_out(i, x):
        out_ref[i] = x.T[:d_model].astype(out_ref.dtype)

    def prepare(ref, blocks):
        for i, r in enumerate(blocks):
            h_ref[i, n_mem:] = _layernorm(ref[block(r), :])
        yield

    def attention(order, ref, blocks, others, early=None):
        xs, outs = [ref[block(r), :] for r in blocks], []
        hs = [h_ref[i] for i in range(len(blocks))]
        operands_ref, known = full_ref, None
        if early is not None:
            operands_ref, known = short_ref, lambda *at: early_ref[(early, *at)]
            hs = [jnp.concatenate([hs[0][:n_mem], hs[0][n_mem + seg // 2:], hs[1][seg:]], axis=0),
                  hs[1][:seg]]
        _store_operands(operands_ref, 0, hs)
        tasks = _attention_tasks(xs, operands_ref, w_refs, qkv_ref, heads_ref, outs, known)
        yield from _passes(order, {**others, **tasks})
        for i, r in enumerate(blocks):
            h_ref[i, :n_mem] = outs[i][:n_mem]
            ref[block(r), :] = outs[i][n_mem:]

    def ffn_tasks(ref, blocks, result=None):
        def update(ys):
            for r, y in zip(blocks, ys):
                ref[block(r, 2), :] = y

        def operands():
            for i in range(0, 2 * seg, 16):
                _store_operands(chunks_ref.at[0], i,
                                [_layernorm(ref[pl.ds(r * seg + i, 16), :]) for r in blocks])
            yield

        return {"N": operands(), **_ffn_tasks(
            [ref[block(r, 2), :] for r in blocks], chunks_ref.at[0], w_refs, hidden_ref,
            result or update)}

    def double_step(b):
        ref = window(b, _LAG + 2)
        _run(attention(_ORDER_DOUBLE, ref, [_LAG, 0],
                       {"X": prepare(ref, [_LAG + 1, 1])}, 1 + b))

    def two_steps(j):
        b = 6
        ref = window(2 * j - b, b + _LAG + 3)
        transpose_out(jnp.where((j % 2 == 1) & (j > 1), (j - 3) // 2, n_out - 1),
                      ref[block(0, 4), :])
        ffn = ffn_tasks(ref, [b + 2, b - 2])
        _run(attention(_ORDER_EVEN, ref, [b + _LAG, b],
                       {**ffn, "X": prepare(ref, [b + _LAG + 1, b + 1])}),
             attention(_ORDER_ODD, ref, [b + _LAG + 1, b + 1],
                       {**ffn, "X": prepare(ref, [b + _LAG + 2, b + 2])}, j + _LAG // 2))

    qkv_words = [_words(w) for w in (wq_hbm, wk_hbm, wv_hbm)]
    ffn_words = [_words(w) for w in (w1_hbm, w3_hbm, w2t_hbm)]
    pairs = _COLUMNS // 2

    def attention_copies(family, g):
        sem = attention_sem.at[family]
        if family == _WO:
            heads = _words(wot_hbm).at[pl.ds(_COLUMNS * g, _COLUMNS)]
            return [pltpu.make_async_copy(heads, wo_stage, sem)]
        return [pltpu.make_async_copy(qkv_words[family].at[:, pairs * g + p, :],
                                      qkv_stage.at[family, p], sem) for p in range(pairs)]

    def ffn_copies(m, columns=_COLUMNS):
        return [pltpu.make_async_copy(w.at[:, lanes(_COLUMNS * m, columns)],
                                      ffn_stage.at[m % 3, i, :, lanes(0, columns)],
                                      ffn_sem.at[3 * (m % 3) + i])
                for i, w in enumerate(ffn_words)]

    def shared_copies(which):
        ends = []
        for m in range(_MEMBERS):
            rows, words = pl.ds(m * _HALF, _HALF), pl.ds(m * _HALF // 2, _HALF // 2)
            if which == 0:
                ends += [(w.at[rows, pairs * m + p, :], qkv_shared.at[i, p, rows])
                         for i, w in enumerate(qkv_words) for p in range(pairs)]
            elif which == 1:
                ends += [(_words(wot_hbm).at[pl.ds(_COLUMNS * m, _COLUMNS), words],
                          wo_shared.at[:, words])]
            else:
                ends += [(w.at[words, lanes(_COLUMNS * m, _COLUMNS)], ffn_shared.at[i, words])
                         for i, w in enumerate(ffn_words)]
        return [pltpu.make_async_copy(*pair, shared_sem.at[which]) for pair in ends]

    def x_copy(chunk):
        columns = lanes(n_out // _CHUNKS * chunk, n_out // _CHUNKS)
        return pltpu.make_async_copy(xt_hbm.at[:, columns], x_stage.at[chunk], x_sem.at[chunk])

    def out_copy(i):
        return pltpu.make_async_copy(out_ref.at[i], outt_hbm.at[:, lanes(i)], out_sem.at[i])

    def start(copies):
        for c in copies:
            c.start()

    def wait(copies):
        for c in copies:
            c.wait()

    def head_pairs(ref):
        def source(c, half, first):
            rows = ref.at[c // 2, pl.ds(pl.multiple_of(half * _HALF, _HALF), _HALF)]
            words = rows[pl.ds(pl.multiple_of(first, 16), 16), :]
            words = words & jnp.uint32(0xFFFF0000) if c % 2 else words << 16
            return pltpu.bitcast(words, jnp.float32)
        return source

    def row_pairs(column, rows):
        def source(c, half, first):
            ref, at = column(c)
            words = ref.at[pl.ds(pl.multiple_of(half * (_HALF // 2), _HALF // 2), _HALF // 2)]
            return _unpack(words[pl.ds(first // 2, rows // 2), at])
        return source

    def member_sums(own, shared, m, rows, starts=None):
        places = [(jnp.where(m == h, 2 * _TAIL, h), jnp.where(m == h, _MEMBERS, h))
                  for h in range(_MEMBERS)]

        def source(c, d, high, first):
            if 2 * d >= _MEMBERS:
                return own(c, 2 * d + high, first)
            mine, theirs = places[2 * d + high]
            return (own(c, mine, first).astype(jnp.float32)
                    - shared(c, theirs, first).astype(jnp.float32))

        sets = {}
        for i, p in enumerate(_scheme("member")):
            owners = {c if c < 4 else d for _, c, d in p.w_low}
            key = -1 - min(owners) if len(owners) == 1 and rows < _HALF else i
            sets.setdefault(key, []).append((len(p.w_low), i, p))
        for tiles in sets.values():
            for high in range(2):
                for first in starts or range(0, _HALF, rows):
                    loaded = {}
                    for *_, i, p in sorted(tiles):
                        new = [(c, d) for _, c, d in p.w_low if (c, d) not in loaded]
                        loaded.update({at: source(*at, high, first) for at in new})
                        value = _weight_sum([(s, loaded[c, d]) for s, c, d in p.w_low])
                        work = len(p.w_low) + sum(1 + 2 * (d < 2) for _, d in new)
                        yield i, high * _HALF + first, value, work / 2

    def lay_out_heads(family, g, starts=None):
        sums = member_sums(head_pairs(qkv_stage.at[family]), head_pairs(qkv_shared.at[family]),
                           g, 16, starts)
        return _lay_out(sums, _tiles(w_refs, "member", family, g))

    def lay_out_shared_half(lay_out, words, rows, family, i):
        n = len(_scheme("shared")) // 2
        sums = _weight_sums(_scheme("shared")[:n], row_pairs(words, rows), range(0, _HALF, rows))
        return lay_out(sums, _tiles(w_refs, "shared", family, half=i))

    def ffn_columns(ref, family, first=0):
        return lambda c: (ref.at[family - _W1], lanes(first + c))

    def project_early(chunk, unit):
        at = lambda r, g, c: (pl.ds(8 * chunk + 4 * r, 4), unit[1], g, c)
        out = {}
        if unit[0] == "member":
            out = {(r, c): early_ref[at(r, _MEMBERS - 1, c)].reshape(2 * seg, _LANES)
                   for r in range(2) for c in range(_COLUMNS)}
        yield from _expand(chunks_ref.at[chunk], w_refs, unit, out)
        for (r, c), value in out.items():
            early_ref[at(r, unit[2] if unit[0] == "member" else _MEMBERS - 1, c)] = (
                value.reshape(4, seg // 2, _LANES))

    def load_chunk(chunk):
        x = x_stage[chunk].astype(jnp.float32)
        x = jnp.concatenate([x, x[_TAIL * _LANES:]], axis=0).T
        window(n_seg // _CHUNKS * chunk, n_seg // _CHUNKS)[...] = x
        segments = [2 * e + 1 for e in range(8)]
        if isinstance(chunk, int) and chunk == 0:
            segments[1] = _LAG
        for e in range(4):
            _store_operands(chunks_ref.at[chunk], e * seg // 2, [
                _layernorm(x[r * seg:r * seg + seg // 2]) for r in segments[e::4]])
        yield

    def clear(i):
        rows = lambda first, n=1: pl.ds(pl.multiple_of(first + 8 * n * i, 8), 8 * n)
        for spare in (res_ref.at[rows(0, _LAG)], res_ref.at[rows((_LAG + n_seg) * seg)],
                      wo_shared.at[:, rows(_MEMBERS * _HALF // 2)],
                      ffn_shared.at[:, rows(_MEMBERS * _HALF // 2)],
                      qkv_shared.at[:, :, rows(_MEMBERS * _HALF, 2)]):
            spare[...] = jnp.zeros(spare.shape, spare.dtype)

    def lay_out_shared(i):
        for family in (_WQ, _WK, _WV):
            sums = _weight_sums(_scheme("shared"), head_pairs(qkv_shared.at[family]), [16 * i])
            _run(_lay_out(sums, _tiles(w_refs, "shared", family)))

    def project_shared(chunk):
        pl.when(chunk == 1)(lambda: start(shared_copies(1) + attention_copies(_WK, 0)))
        pl.when(chunk == 2)(lambda: start(attention_copies(_WV, 0)))
        pl.when(chunk + 1 < _CHUNKS)(lambda: wait([x_copy(chunk + 1)]))
        _run(_passes(_ORDER_SHARED, {
            "E": _chain(*(project_early(chunk, ("shared", f)) for f in (_WQ, _WK, _WV))),
            "L": lay_out_heads(_WQ, 0, [16 * chunk]),
            "X": load_chunk(jnp.minimum(chunk + 1, _CHUNKS - 1))}))

    def load_group(g):
        more = g + 1 < _MEMBERS

        def arrive(family):
            if family == _WK:
                start(attention_copies(_WO, g))
                pl.when(more)(lambda: start(attention_copies(_WQ, g + 1)))
                pl.when(~more)(lambda: start(shared_copies(2)))
                wait(attention_copies(_WK, g))
            elif family == _WV:
                wait(attention_copies(_WV, g) + attention_copies(_WO, g))
                pl.when(more)(lambda: start(attention_copies(_WK, g + 1)))
                for i, copy in enumerate(ffn_copies(0)):
                    pl.when(g == i)(copy.start)
                pl.when(~more)(lambda: start(ffn_copies(1)))
            else:
                pl.when(more)(lambda: wait(attention_copies(_WQ, g + 1)))
                pl.when(more)(lambda: start(attention_copies(_WV, g + 1)))
            yield

        same = jnp.minimum(g, _MEMBERS - 1)
        wo_sums = member_sums(row_pairs(lambda c: (wo_stage.at[c], slice(None)), _HALF),
                              row_pairs(lambda c: (wo_shared.at[c], slice(None)), _HALF), g, _HALF)
        _run(_passes(_ORDER_LOAD, {
            **{f"E{f}": _chain(*(project_early(chunk, ("member", f, g)) for chunk in range(_CHUNKS)))
               for f in (_WQ, _WK, _WV)},
            **{f"W{f}": arrive(f) for f in (_WQ, _WK, _WV)},
            "L0": lay_out_heads(_WQ, jnp.minimum(g + 1, _MEMBERS - 1)),
            "L1": lay_out_heads(_WK, same), "L2": lay_out_heads(_WV, same),
            "L3": _lay_out_transposed(wo_sums, _tiles(w_refs, "member", _WO, same)),
            "L4": lay_out_shared_half(
                _lay_out_transposed, lambda c: (wo_shared.at[c + 2 * (g % 2)], slice(None)), _HALF,
                _WO, g % 2)}))

    def first_step(m):
        pl.when(m + 2 < _MEMBERS)(lambda: start(ffn_copies(m + 2)))
        pl.when(m + 2 == _MEMBERS)(lambda: start(ffn_copies(_MEMBERS, 4)))
        wait(ffn_copies(m))
        ref, stage = window(m, 2), ffn_stage.at[m % 3]
        sums = lambda family, rows: member_sums(
            row_pairs(ffn_columns(stage, family), rows),
            row_pairs(ffn_columns(ffn_shared, family), rows), m, rows)
        up = [_lay_out(sums(f, 16), _tiles(w_refs, "member", f, m)) for f in (_W1, _W3)]
        down = _lay_out_transposed(sums(_W2, _HALF), _tiles(w_refs, "member", _W2, m))
        shared = lay_out_shared_half(_lay_out, ffn_columns(ffn_shared, _W1 + m // 2, 2 * (m % 2)),
                                     16, _W1 + m // 2, m % 2)
        _run(_passes(_ORDER_FIRST, {
            "P": attention(_ORDER_SINGLE, ref, [0], {"X": prepare(ref, [1])}),
            "L": _passes("U*9+D*5", {"U": _chain(shared, *up), "D": down})}))

    def first_ffn():
        stage = ffn_stage.at[_MEMBERS % 3]
        sums = lambda kind, ref, family: _weight_sums(
            _scheme(kind), row_pairs(ffn_columns(ref, family), _HALF), [0])
        _run(*(_lay_out(sums("narrow", stage, f), _tiles(w_refs, "narrow", f)) for f in (_W1, _W3)),
             *(_lay_out_transposed(sums(kind, ref, _W2), _tiles(w_refs, kind, _W2))
               for kind, ref in (("narrow", stage), ("shared", ffn_shared))),
             _passes(_ORDER_FIRST_FFN, ffn_tasks(window(0, _LAG), [0, 2])))

    def last_steps():
        ref = window(n_seg - _LAG - 2, _LAG + 2)
        ffn = ffn_tasks(ref, [_LAG, 0])
        _run(attention(_ORDER_EVEN_SINGLE, ref, [2], {**ffn, "X": prepare(ref, [3])}),
             attention(_ORDER_ODD_SINGLE, ref, [3], {**ffn, "X": prepare(ref, [4])}))

    def last_step(i):
        tile = n_out - 3 + i
        transpose_out(tile, window(_LANES // seg * tile, _LANES // seg)[...])
        ref = window(n_seg - 2 + i, 2)
        _run(attention(_ORDER_SINGLE, ref, [0], {"X": prepare(ref, [1])}))
        out_copy(tile).start()

    def last_ffn():
        _run(_passes(_ORDER_FFN, ffn_tasks(
            window(n_seg - _LAG, _LAG), [0, 2],
            lambda ys: transpose_out(n_out - 1, jnp.concatenate(ys, axis=0)))))

    mem_copy = pltpu.make_async_copy(mem0_hbm, mem0_ref.at[0], shared_sem.at[3])
    x_copy(0).start()
    pl.loop(0, 4)(clear)
    start([mem_copy] + shared_copies(0))
    wait([x_copy(0), mem_copy])
    start([x_copy(1)] + attention_copies(_WQ, 0))
    mem0 = mem0_ref[0].astype(jnp.float32)
    h_ref[0, :n_mem] = h_ref[1, :n_mem] = jnp.concatenate(
        [mem0, mem0[:, _TAIL * _LANES:]], axis=1)
    _run(load_chunk(0), prepare(window(0, 1), [0]))
    wait(shared_copies(0))
    pl.loop(0, _HALF // 16)(lay_out_shared)
    x_copy(2).start()
    wait(attention_copies(_WQ, 0))
    x_copy(3).start()
    pl.loop(0, _CHUNKS)(project_shared)
    wait(shared_copies(1))
    pl.loop(0, _MEMBERS)(load_group)
    wait(shared_copies(2))
    pl.loop(0, _LAG)(first_step)
    wait(ffn_copies(_MEMBERS, 4))
    first_ffn()
    _run(prepare(window(0, _LAG + 1), [_LAG, 0]))
    pl.loop(0, 2)(double_step)
    pl.loop(1, (n_seg - _LAG) // 2)(two_steps)
    start([out_copy(i) for i in range(n_out - 3)])
    h_ref[0] = h_ref[1]
    last_steps()
    pl.loop(0, 2)(last_step)
    last_ffn()
    out_copy(n_out - 1).start()
    wait([out_copy(i) for i in range(n_out)])


@functools.partial(jax.jit, static_argnames=("A_seg_len",))
def pallas_interleave_layers__memory_aug_recurrent_mem_tr__glu_gated_swiglu__prompt_kernel(
    A_x: jax.Array,
    A_mem0: jax.Array,
    A_Wq: jax.Array,
    A_Wk: jax.Array,
    A_Wv: jax.Array,
    A_Wo: jax.Array,
    A_seg_len: int,
    B_x: jax.Array,
    B_w1: jax.Array,
    B_w3: jax.Array,
    B_w2: jax.Array,
):
    del B_x
    _, n_tok, d_model = A_x.shape
    n_mem = A_mem0.shape[1]
    _, n_heads, d_head = A_Wq.shape
    seg = A_seg_len
    assert A_x.shape[0] == 1 and _LAG * seg == _LANES and n_mem == 8
    assert n_tok == 16 * _CHUNKS * seg and d_model == _TAIL * _LANES + _HALF and d_head == _LANES
    assert n_heads == _MEMBERS * _COLUMNS and B_w1.shape[1] == (n_heads + 4) * _LANES
    n_operands = pl.cdiv(len(_operand_keys(False)), 8) * 8
    n_tiles = (_FAMILIES * (_MEMBERS * len(_scheme("member")) + len(_scheme("shared")))
               + 3 * len(_scheme("narrow")))
    shared_rows = (_MEMBERS + 1) * _HALF
    hbm = pl.BlockSpec(memory_space=pltpu.HBM)
    out_t = pl.pallas_call(
        functools.partial(_kernel, seg=seg),
        out_shape=jax.ShapeDtypeStruct((d_model, n_tok), A_x.dtype),
        in_specs=[hbm] * 9,
        out_specs=hbm,
        scratch_shapes=[
            pltpu.VMEM((n_tok // _LANES, d_model, _LANES), A_x.dtype),
            pltpu.VMEM((8, n_mem + seg, d_model + _HALF), jnp.float32),
            pltpu.VMEM((n_operands, n_mem + seg, _LANES), jnp.float32),
            pltpu.VMEM((n_operands, seg, _LANES), jnp.bfloat16),
            pltpu.VMEM((_CHUNKS, n_operands, 2 * seg, _LANES), jnp.bfloat16),
            pltpu.VMEM((3, _MEMBERS, _COLUMNS, 2 * (n_mem + seg), _LANES), jnp.bfloat16),
            pltpu.VMEM((_MEMBERS + 4, _COLUMNS, 2 * (n_mem + seg), _LANES), jnp.float32),
            pltpu.VMEM((_MEMBERS + 4, _COLUMNS, 4 * seg, _LANES), jnp.float32),
            pltpu.VMEM((8 * _CHUNKS, 3, _MEMBERS, _COLUMNS, seg // 2, _LANES), jnp.float32),
            [pltpu.VMEM((n_tiles // 2, _LANES, _LANES), jnp.bfloat16)] * 2,
            pltpu.VMEM((_CHUNKS, d_model, n_tok // _CHUNKS), A_x.dtype),
            pltpu.VMEM((3, _COLUMNS // 2, d_model, _LANES), jnp.uint32),
            pltpu.VMEM((3, _COLUMNS // 2, shared_rows, _LANES), jnp.uint32),
            pltpu.VMEM((_COLUMNS, d_model // 2, _LANES), jnp.uint32),
            pltpu.VMEM((_COLUMNS, shared_rows // 2, _LANES), jnp.uint32),
            pltpu.VMEM((3, 3, d_model // 2, _COLUMNS * _LANES), jnp.uint32),
            pltpu.VMEM((3, shared_rows // 2, _COLUMNS * _LANES), jnp.uint32),
            pltpu.VMEM((n_tok + 2 * _LAG * seg, d_model + _HALF), jnp.float32),
            pltpu.VMEM((16, n_mem, d_model), A_mem0.dtype),
            pltpu.SemaphoreType.DMA((_CHUNKS,)),
            pltpu.SemaphoreType.DMA((4,)),
            pltpu.SemaphoreType.DMA((9,)),
            pltpu.SemaphoreType.DMA((4,)),
            pltpu.SemaphoreType.DMA((n_tok // _LANES,)),
        ],
        compiler_params=pltpu.CompilerParams(
            vmem_limit_bytes=126 * 1024 * 1024,
            flags={"XLA_TPU_FORCE_LP_LLO_SCHEDULER": True}),
    )(A_x.reshape(n_tok, d_model).T, A_mem0.reshape(n_mem, d_model), A_Wq, A_Wk, A_Wv,
      A_Wo.transpose(0, 2, 1), B_w1, B_w3, B_w2.T)
    return out_t.T.reshape(A_x.shape)
```
